```python
import jax
import jax.numpy as jnp

def _softmax(x, axis=-1):
    return jax.nn.softmax(x, axis=axis)
def _gelu(x):
    return jax.nn.gelu(x, approximate=True)
def _silu(x):
    return jax.nn.silu(x)
def _sigmoid(x):
    return jax.nn.sigmoid(x)
def _layernorm(x, axis=-1, eps=1e-5):
    m = jnp.mean(x, axis=axis, keepdims=True)
    v = jnp.var(x, axis=axis, keepdims=True)
    return (x - m) / jnp.sqrt(v + eps)
def _scatter_add(tgt, idx, src, axis=0):
    return tgt.at[idx].add(src)
def _segment_sum(src, seg, n):
    return jax.ops.segment_sum(src, seg, n)
class _Rng:
    def __init__(self, key):
        self._k = key
    def _next(self):
        self._k, sub = jax.random.split(self._k)
        return sub
    def normal(self, shape):
        return jax.random.normal(self._next(), shape, dtype=jnp.bfloat16)
    def randint(self, lo, hi, shape):
        return jax.random.randint(self._next(), shape, lo, hi, dtype=jnp.int32)
    def uniform(self, shape, lo=0.0, hi=1.0):
        return jax.random.uniform(self._next(), shape, jnp.bfloat16, lo, hi)
    def permutation(self, n):
        return jax.random.permutation(self._next(), n)


kernel_name = 'concat_heads__ssm_conv_h3__compressed_kv_cla__prompt'

def setup_inputs():
    _rng = _Rng(jax.random.key(int.from_bytes(__import__("os").urandom(4), "little")))
    _w = (lambda a: (lambda t: t.astype(jnp.bfloat16) if jnp.issubdtype(t.dtype, jnp.floating) else t)(jnp.asarray(a)))
    def _A_setup():
        B, S, D = 1, 2048, 448
        ks = 4
        return {
            "q": _w((lambda *s: _rng.normal(s) * 0.05)(B, S, D)),
            "k": _w((lambda *s: _rng.normal(s) * 0.05)(B, S, D)),
            "v": _w((lambda *s: _rng.normal(s) * 0.05)(B, S, D)),
            "shift_k": _w((lambda *s: _rng.normal(s) * 0.05)(D, ks) * 0.5),
            "ssm_k": _w((lambda *s: _rng.normal(s) * 0.05)(D, S) * (1.0 / S ** 0.5)),
            "ssm_D": _w((lambda *s: _rng.normal(s) * 0.05)(D)),
        }
    _A_in = _A_setup()

    def _B_setup():
        B, H, Sq, Sk, D, M = 1, 16, 2048, 2048, 256, 448
        Dc = 4 * D
        return {
            "x": _w((lambda *s: _rng.normal(s) * 0.05)(B, Sq, M)),
            "c_kv": _w((lambda *s: _rng.normal(s) * 0.05)(B, Sk, Dc)),
            "w_q": _w((lambda *s: _rng.normal(s) * 0.05)(M, H, D) * (M ** -0.5)),
            "w_uk": _w((lambda *s: _rng.normal(s) * 0.05)(Dc, H, D) * (Dc ** -0.5)),
            "w_uv": _w((lambda *s: _rng.normal(s) * 0.05)(Dc, H, D) * (Dc ** -0.5)),
            "w_o": _w((lambda *s: _rng.normal(s) * 0.05)(H, D, M) * ((H * D) ** -0.5)),
        }
    _B_in = _B_setup()

    return {
        "A_q": _A_in["q"],
        "A_k": _A_in["k"],
        "A_v": _A_in["v"],
        "A_shift_k": _A_in["shift_k"],
        "A_ssm_k": _A_in["ssm_k"],
        "A_ssm_D": _A_in["ssm_D"],
        "B_x": _B_in["x"],
        "B_c_kv": _B_in["c_kv"],
        "B_w_q": _B_in["w_q"],
        "B_w_uk": _B_in["w_uk"],
        "B_w_uv": _B_in["w_uv"],
        "B_w_o": _B_in["w_o"],
    }

def reference(A_q, A_k, A_v, A_shift_k, A_ssm_k, A_ssm_D, B_x, B_c_kv, B_w_q, B_w_uk, B_w_uv, B_w_o):
    def _A_ref(q, k, v, shift_k, ssm_k, ssm_D):
        B, S, D = q.shape
        ks = shift_k.shape[-1]
        k_pad = jnp.pad(k, ((0, 0), (ks - 1, 0), (0, 0)))
        k_shift = jnp.zeros_like(k)
        for t in range(ks):
            k_shift = k_shift + k_pad[:, t:t + S, :] * shift_k[:, ks - 1 - t][None, None, :]
        kv = k_shift * v
        L = 2 * S
        kv_pad = jnp.pad(kv, ((0, 0), (0, S), (0, 0)))
        kf_pad = jnp.pad(ssm_k, ((0, 0), (0, S)))
        kv_f = (lambda x, axes=(-2,-1): jnp.fft.rfft2(x.astype(jnp.float32), axes=axes))(kv_pad[:, None, :, :], axes=(1, 2))
        kf_f = (lambda x, axes=(-2,-1): jnp.fft.rfft2(x.astype(jnp.float32), axes=axes))(kf_pad[:, None, :], axes=(1, 2))
        kf_f = (lambda x, *d: x.transpose(*d))(kf_f, 1, 2, 0)
        y_f = kv_f * kf_f[None, :, :, :]
        y = (lambda x, s, axes=(-2,-1): jnp.fft.irfft2(x, s=s, axes=axes).astype(jnp.bfloat16))(y_f, (1, L), axes=(1, 2))[:, 0, :S, :]
        y = y + kv * ssm_D[None, None, :]
        return q * y

    def _B_ref(x, c_kv, w_q, w_uk, w_uv, w_o):
        B, Sq, M = x.shape[0], x.shape[1], x.shape[2]
        Sk = c_kv.shape[1]
        H, D = w_q.shape[1], w_q.shape[2]
        q = jnp.einsum("bqm,mhd->bhqd", x, w_q)
        k = jnp.einsum("bkc,chd->bhkd", c_kv, w_uk)
        v = jnp.einsum("bkc,chd->bhkd", c_kv, w_uv)
        scores = jnp.einsum("bhqd,bhkd->bhqk", q, k) * (D ** -0.5)
        off = Sk - Sq
        qi = jnp.arange(Sq)[:, None]
        kj = jnp.arange(Sk)[None, :]
        cmask = kj <= (qi + off)
        scores = jnp.where(cmask[None, None], scores, -1e9)
        p = _softmax(scores, axis=-1)
        ctx = jnp.einsum("bhqk,bhkd->bhqd", p, v)
        return jnp.einsum("bhqd,hdm->bqm", ctx, w_o)

    a = _A_ref(A_q, A_k, A_v, A_shift_k, A_ssm_k, A_ssm_D)
    b = _B_ref(B_x, B_c_kv, B_w_q, B_w_uk, B_w_uv, B_w_o)
    return jnp.concatenate([a, b], axis=-1)
```

```python
import math

import jax
import jax.numpy as jnp
import jax.experimental.pallas as pl
import jax.experimental.pallas.tpu as pltpu

bf16 = jnp.bfloat16
f32 = jnp.float32
u32 = jnp.uint32

S = 2048
M = 448
DC = 1024
H = 16
D = 256
KS = 4
P = 128
NB = S // P
CH = 32
NCH = M // CH
T = 256
NT = S // T
NEG = -1e30
LAG_M = 0
LAG_S = 0
ORDER = 'a'


def _nn(a, b):
    return jnp.dot(a, b, preferred_element_type=f32)


def _nt(a, b):
    return jax.lax.dot_general(a, b, (((1,), (1,)), ((), ())), preferred_element_type=f32)


def _b(u):
    return pltpu.bitcast(u, bf16)


def _u(x):
    return pltpu.bitcast(x, u32)


def _split_pair(u):
    lo = pltpu.bitcast(u << 16, f32).astype(bf16)
    hi = pltpu.bitcast(u & jnp.uint32(0xFFFF0000), f32).astype(bf16)
    return lo, hi


def _fold(c, op):
    return op(c.reshape(-1, 8, c.shape[1]), axis=0)


def _gate(x, vals):
    if not vals:
        return x
    w = max(v.shape[1] for v in vals)
    top = x[:8, :w]
    for v in vals:
        if v.shape[1] < w:
            v = jnp.concatenate([v] * (w // v.shape[1]), axis=1)
        top = jnp.where(v == jnp.inf, jnp.zeros_like(top), top)
    if w < x.shape[1]:
        top = jnp.concatenate([top, x[:8, w:]], axis=1)
    return jnp.concatenate([top, x[8:]], axis=0)


def _schedule():
    ops = []
    if ORDER == 'a':
        ops += [('KP', 0), ('DFT',), ('VP', 0), ('KP', 1), ('QK', 0, 0), ('SSM', 0), ('VP', 1)]
        for i in range(NT - 1):
            u = []
            for j in range(i + 1):
                u += [('QK', i + 1, j), ('PV', i, j)]
            u.insert(len(u) - 1, ('QK', i + 1, i + 1))
            ops += u
            if i + 2 < NT:
                ops += [('KP', i + 2), ('SSM', i + 1), ('VP', i + 2)]
                if i == NT - 3:
                    ops += [('SSM', 7)]
            else:
                ops += [('OP', 0), ('OP', 1)]
        for j in range(NT):
            ops += [('PV', NT - 1, j)]
            if j + 2 < NT - 1:
                ops += [('OP', j + 2)]
        ops += [('OP', NT - 1)]
    return ops


def _kernel(qT_hbm, kT_hbm, vT_hbm, sk_ref, ssmk_hbm, dd_ref, xT_hbm, ckv_hbm,
            wq_hbm, wk_hbm, wv_hbm, woT_hbm, out_hbm,
            qT, kT, vT, ssmk, xT, ckv, wq_raw, wk_raw, wv_raw, woT,
            wqT_s, wk_s, wvT_s, QT_s, ckv_u, acc, fullT, out_s, taps, ff_s, fi_s,
            sem, sem_k, sem_v, sem_o):
    def cp(src, dst, s):
        return pltpu.make_async_copy(src, dst, s)

    c_x = cp(xT_hbm, xT, sem.at[0])
    c_wq = [cp(wq_hbm.at[:, pl.ds(128 * g, 128)], wq_raw.at[g], sem.at[1 + g]) for g in range(2)]

    def c_wk(i, g):
        r = pl.ds(pl.multiple_of(i * 2048, 2048), 2048)
        return cp(wk_hbm.at[r, pl.ds(128 * g, 128)], wk_raw.at[g, r], sem_k.at[2 * i + g])

    def c_wv(i, g):
        r = pl.ds(pl.multiple_of(i * 2048, 2048), 2048)
        return cp(wv_hbm.at[r, pl.ds(128 * g, 128)], wv_raw.at[g, r], sem_v.at[2 * i + g])

    def c_ckv(i):
        r = pl.ds(pl.multiple_of(i * T, T), T)
        return cp(ckv_hbm.at[r], ckv.at[r], sem.at[9 + i])

    c_rest = [cp(woT_hbm, woT, sem.at[4]), cp(kT_hbm, kT, sem.at[5]), cp(vT_hbm, vT, sem.at[6]),
              cp(ssmk_hbm, ssmk, sem.at[7]), cp(qT_hbm, qT, sem.at[8])]
    for c in c_wq:
        c.start()
    c_x.start()

    n_i = jax.lax.broadcasted_iota(jnp.int32, (P, P), 0)
    k_i = jax.lax.broadcasted_iota(jnp.int32, (P, P), 1)
    ang = (((2 * k_i + 1) * n_i) & 511).astype(f32) * (math.pi / 256.0)
    cs, sn = jnp.cos(ang), jnp.sin(ang)
    ff_s[:, 0:P] = cs.astype(bf16)
    ff_s[:, P:2 * P] = (-sn).astype(bf16)
    fi_s[0:P, :] = (cs.T * (1.0 / P)).astype(bf16)
    fi_s[P:2 * P, :] = (sn.T * (-1.0 / P)).astype(bf16)
    sk = sk_ref[...].astype(f32)
    for t in range(KS):
        taps[t] = jnp.broadcast_to(sk[t:t + 1, :], (128, M)).T
    taps[KS] = jnp.broadcast_to(dd_ref[...].astype(f32).reshape(1, M), (128, M)).T
    acc[...] = jnp.zeros(acc.shape, f32)

    for c in c_wq:
        c.wait()

    def start_chunk(i):
        for g in range(2):
            c_wk(i, g).start()
            c_wv(i, g).start()
        c_ckv(i).start()

    start_chunk(0)
    vq = wq_raw.bitcast(u32)
    for hp in range(H // 2):
        for g in range(2):
            e, o = _split_pair(vq[g, pl.ds(hp, M, stride=8), :])
            wqT_s[2 * hp * 128 + 64 * g:2 * hp * 128 + 64 * g + 64, :] = _u(e.T)
            wqT_s[(2 * hp + 1) * 128 + 64 * g:(2 * hp + 1) * 128 + 64 * g + 64, :] = _u(o.T)
    c_x.wait()
    start_chunk(1)

    qscale = (D ** -0.5) * math.log2(math.e)

    def q_body(i, carry):
        for g in range(2):
            c_wk(i, g).wait()
            c_wv(i, g).wait()
        c_ckv(i).wait()

        @pl.when(i + 2 < 8)
        def _():
            start_chunk(i + 2)

        @pl.when(i == 6)
        def _():
            for c in c_rest:
                c.start()

        rows = pl.ds(pl.multiple_of(i * D, D), D)
        QT_s[rows, :] = _u((_nn(_b(wqT_s[rows, :]), xT[...]) * qscale).astype(bf16))
        r0 = pl.ds(pl.multiple_of(i * 128, 128), 128)
        r0h = pl.ds(pl.multiple_of(i * 64, 64), 64)
        ru = pl.ds(pl.multiple_of(i * 1024, 1024), 1024)
        for g in range(2):
            vk = wk_raw.bitcast(u32).at[g, ru]
            vv = wv_raw.bitcast(u32).at[g, ru]
            for hp in range(H // 2):
                e, o = _split_pair(vk[pl.ds(hp, 128, stride=8), :])
                wk_s[2 * hp, r0h, 128 * g:128 * g + 128] = _u(e)
                wk_s[2 * hp + 1, r0h, 128 * g:128 * g + 128] = _u(o)
                e, o = _split_pair(vv[pl.ds(hp, 128, stride=8), :])
                wvT_s[2 * hp, 64 * g:64 * g + 64, r0] = _u(e.T)
                wvT_s[2 * hp + 1, 64 * g:64 * g + 64, r0] = _u(o.T)
        ckv_u[r0, :] = _u(ckv[pl.ds(pl.multiple_of(i * T, T), T), :])
        return carry

    jax.lax.fori_loop(0, 8, q_body, 0)
    for c in c_rest:
        c.wait()

    tri = n_i <= k_i
    lane = jax.lax.broadcasted_iota(jnp.int32, (CH, 128), 1)
    sgn = jnp.where((jax.lax.broadcasted_iota(jnp.int32, (1, P), 1) & 1) == 0, 1.0, -1.0).astype(f32)

    def head_body(h, carry):
        st = dict(K={}, V={}, S={}, m={}, mfin={}, l={}, o={})
        gates = []
        qrows = pl.ds(pl.multiple_of(h * 128, 128), 128)
        rows = pl.ds(pl.multiple_of(jnp.minimum(h, NCH - 1) * CH, CH), CH)

        def rep(t, n):
            return jnp.concatenate([taps[t, rows, :]] * n, axis=1)

        def due(pos):
            g = [v for (p, v) in gates if p <= pos]
            gates[:] = [(p, v) for (p, v) in gates if p > pos]
            return g

        for pos, op in enumerate(_schedule()):
            kind = op[0]
            if kind == 'KP':
                c = op[1]
                a = _gate(ckv_u[c * 128:(c + 1) * 128, :], due(pos))
                st['K'][c] = _nn(_b(a), _b(wk_s[h])).astype(bf16)
            elif kind == 'VP':
                c = op[1]
                w = _gate(wvT_s[h], due(pos))
                st['V'][c] = _nt(_b(w), _b(ckv_u[c * 128:(c + 1) * 128, :])).astype(bf16)
            elif kind == 'QK':
                _, i, j = op
                q = _b(_gate(QT_s[qrows, i * T:(i + 1) * T], due(pos)))
                kc = st['K'][j]
                if j < i:
                    s = _nn(kc, q)
                    st['S'][i, j] = s
                    f = _fold(s, jnp.max)
                else:
                    sa = _nn(kc[:128], q)
                    sa = jnp.concatenate([jnp.where(tri, sa[:, :128], NEG), sa[:, 128:]], axis=1)
                    sb = jnp.where(tri, _nn(kc[128:], q[:, 128:]), NEG)
                    st['S'][i, j] = (sa, sb)
                    fa = _fold(sa, jnp.max)
                    f = jnp.concatenate([fa[:, :128], jnp.maximum(fa[:, 128:], _fold(sb, jnp.max))], axis=1)
                st['m'][i] = f if j == 0 else jnp.maximum(st['m'][i], f)
                if j == i:
                    st['mfin'][i] = jnp.max(st['m'][i], axis=0, keepdims=True)
                elif LAG_M:
                    gates.append((pos + LAG_M, st['m'][i]))
            elif kind == 'PV':
                _, i, j = op
                m = st['mfin'][i]
                vc = st['V'][j]
                s = st['S'].pop((i, j))
                if j < i:
                    p = jnp.exp2(s - m)
                    lj = _fold(p, jnp.sum)
                    o = _nn(vc, p.astype(bf16))
                else:
                    pa = jnp.exp2(s[0] - m)
                    pb = jnp.exp2(s[1] - m[:, 128:])
                    la = _fold(pa, jnp.sum)
                    lj = jnp.concatenate([la[:, :128], la[:, 128:] + _fold(pb, jnp.sum)], axis=1)
                    oa = _nn(vc[:, :128], pa.astype(bf16))
                    ob = _nn(vc[:, 128:], pb.astype(bf16))
                    o = jnp.concatenate([oa[:, :128], oa[:, 128:] + ob], axis=1)
                st['l'][i] = lj if j == 0 else st['l'][i] + lj
                st['o'][i] = o if j == 0 else st['o'][i] + o
                if j < i and LAG_S:
                    gates.append((pos + LAG_S, st['l'][i]))
                if j == i:
                    r = 1.0 / jnp.sum(st['l'][i], axis=0, keepdims=True)
                    st['o'][i] = st['o'][i] * r
                    if LAG_S and i < NT - 1:
                        gates.append((pos + LAG_S, st['o'][i][D - 8:, :]))
            elif kind == 'OP':
                i = op[1]
                ot = _gate(st['o'].pop(i), due(pos)).astype(bf16)
                acc[:, T * i:T * (i + 1)] += _nn(woT[h], ot)
            elif kind == 'DFT':
                k = kT[rows, :].astype(f32)
                ks = k * rep(0, NB)
                for j in range(1, KS):
                    kr = pltpu.roll(k, j, 1)
                    kr = jnp.concatenate([jnp.where(lane >= j, kr[:, :128], 0.0), kr[:, 128:]], axis=1)
                    ks = ks + kr * rep(j, NB)
                kv = ks * vT[rows, :].astype(f32)
                kvs = jnp.concatenate([kv[:, c * P:(c + 1) * P] for c in range(NB)], axis=0).astype(bf16)
                hk = ssmk[rows, :]
                hs = jnp.concatenate([hk[:, c * P:(c + 1) * P] for c in range(NB)], axis=0)
                hf = _nn(hs, ff_s[...])
                xf = _nn(kvs, ff_s[...])
                xr = [xf[c * CH:(c + 1) * CH, :P] for c in range(NB)]
                xi = [xf[c * CH:(c + 1) * CH, P:] for c in range(NB)]
                st['hr'] = [hf[c * CH:(c + 1) * CH, :P] for c in range(NB)]
                st['hi'] = [hf[c * CH:(c + 1) * CH, P:] for c in range(NB)]
                st['pr'] = [xr[0]] + [xr[c] - sgn * xi[c - 1] for c in range(1, NB)]
                st['pi'] = [xi[0]] + [xi[c] + sgn * xr[c - 1] for c in range(1, NB)]
                st['kv'] = kv
            elif kind == 'SSM':
                hr, hi, pr, pi = st['hr'], st['hi'], st['pr'], st['pi']
                blocks = (op[1], NB - 1 - op[1])
                ws = []
                for a in blocks:
                    wr = hr[0] * pr[a] - hi[0] * pi[a]
                    wi = hr[0] * pi[a] + hi[0] * pr[a]
                    for j in range(1, a + 1):
                        wr = wr + (hr[j] * pr[a - j] - hi[j] * pi[a - j])
                        wi = wi + (hr[j] * pi[a - j] + hi[j] * pr[a - j])
                    ws.append(jnp.concatenate([wr, wi], axis=1))
                y = _nn(jnp.concatenate(ws, axis=0).astype(bf16), fi_s[...])
                for n, a in enumerate(blocks):
                    cols = slice(a * P, (a + 1) * P)
                    ya = y[n * CH:(n + 1) * CH, :] + st['kv'][:, cols] * taps[KS, rows, :]
                    fullT[rows, cols] = (qT[rows, cols].astype(f32) * ya).astype(bf16)
        return carry

    jax.lax.fori_loop(0, H, head_body, 0)

    fullT[M:2 * M, :] = acc[...].astype(bf16)
    outs = []
    for i in range(8):
        out_s[256 * i:256 * (i + 1), :] = fullT[:, 256 * i:256 * (i + 1)].T
        c = cp(out_s.at[pl.ds(256 * i, 256)], out_hbm.at[pl.ds(256 * i, 256)], sem_o.at[i])
        c.start()
        outs.append(c)
    for c in outs:
        c.wait()


@jax.jit
def pallas_concat_heads__ssm_conv_h3__compressed_kv_cla__prompt_kernel(
    A_q: jax.Array,
    A_k: jax.Array,
    A_v: jax.Array,
    A_shift_k: jax.Array,
    A_ssm_k: jax.Array,
    A_ssm_D: jax.Array,
    B_x: jax.Array,
    B_c_kv: jax.Array,
    B_w_q: jax.Array,
    B_w_uk: jax.Array,
    B_w_uv: jax.Array,
    B_w_o: jax.Array,
):
    hbm = pl.BlockSpec(memory_space=pl.ANY)
    vmem = pl.BlockSpec(memory_space=pltpu.VMEM)
    V = pltpu.VMEM
    out = pl.pallas_call(
        _kernel,
        out_shape=jax.ShapeDtypeStruct((S, 2 * M), bf16),
        in_specs=[hbm, hbm, hbm, vmem, hbm, vmem, hbm, hbm, hbm, hbm, hbm, hbm],
        out_specs=hbm,
        scratch_shapes=[
            V((M, S), bf16), V((M, S), bf16), V((M, S), bf16), V((M, S), bf16),
            V((M, S), bf16), V((S, DC), bf16),
            V((2, M * H, 128), bf16), V((2, DC * H, 128), bf16), V((2, DC * H, 128), bf16),
            V((H, M, D), bf16),
            V((H * D // 2, M), u32), V((H, DC // 2, D), u32), V((H, D // 2, DC), u32),
            V((H * D // 2, S), u32), V((S // 2, DC), u32),
            V((M, S), f32), V((2 * M, S), bf16), V((S, 2 * M), bf16),
            V((KS + 1, M, 128), f32), V((P, 2 * P), bf16), V((2 * P, P), bf16),
            pltpu.SemaphoreType.DMA((17,)), pltpu.SemaphoreType.DMA((16,)),
            pltpu.SemaphoreType.DMA((16,)), pltpu.SemaphoreType.DMA((8,)),
        ],
        compiler_params=pltpu.CompilerParams(vmem_limit_bytes=120 * 1024 * 1024,
                                             shape_invariant_numerics=False),
    )(
        A_q[0].T, A_k[0].T, A_v[0].T, A_shift_k.T, A_ssm_k, A_ssm_D,
        B_x[0].T, B_c_kv[0],
        B_w_q.reshape(M * H, D), B_w_uk.reshape(DC * H, D), B_w_uv.reshape(DC * H, D),
        jnp.transpose(B_w_o, (0, 2, 1)),
    )
    return out[None]
```

```python
import functools
import math

import jax
import jax.numpy as jnp
import jax.experimental.pallas as pl
import jax.experimental.pallas.tpu as pltpu

bf16 = jnp.bfloat16
f32 = jnp.float32
u32 = jnp.uint32

S = 2048
M = 448
DC = 1024
H = 16
D = 256
KS = 4
P = 128
NB = S // P
CH = 32
NCH = M // CH
T = 256
NT = S // T
NEG = -1e30
LAG_M = 0
LAG_S = 0
SORD = (6, 4, 3, 0, 1, 2, 5)
QW1 = 12
QW2 = 34
QW3 = 50
QLAG = 2
ORDER = 'a'


def _nn(a, b):
    return jnp.dot(a, b, preferred_element_type=f32)


def _nt(a, b):
    return jax.lax.dot_general(a, b, (((1,), (1,)), ((), ())), preferred_element_type=f32)


def _b(u):
    return pltpu.bitcast(u, bf16)


def _u(x):
    return pltpu.bitcast(x, u32)


def _split_pair(u):
    lo = pltpu.bitcast(u << 16, f32).astype(bf16)
    hi = pltpu.bitcast(u & jnp.uint32(0xFFFF0000), f32).astype(bf16)
    return lo, hi


def _fold(c, op):
    return op(c.reshape(-1, 8, c.shape[1]), axis=0)


def _gate(x, vals):
    if not vals:
        return x
    w = max(v.shape[1] for v in vals)
    top = x[:8, :w]
    for v in vals:
        if v.shape[1] < w:
            v = jnp.concatenate([v] * (w // v.shape[1]), axis=1)
        top = jnp.where(v == jnp.inf, jnp.zeros_like(top), top)
    if w < x.shape[1]:
        top = jnp.concatenate([top, x[:8, w:]], axis=1)
    return jnp.concatenate([top, x[8:]], axis=0)


def _tok(vals):
    parts = []
    for v in vals:
        for r in range(0, v.shape[0], 8):
            for c in range(0, v.shape[1], 128):
                parts.append(v[r:r + 8, c:c + 128])
    while len(parts) > 1:
        parts = [parts[i] | parts[i + 1] if i + 1 < len(parts) else parts[i] for i in range(0, len(parts), 2)]
    return (parts[0] >> 31) >> 1


def _gate_u(x, tok):
    if tok is None:
        return x
    top = jnp.concatenate([x[:8, :128] | tok, x[:8, 128:]], axis=1)
    return jnp.concatenate([top, x[8:]], axis=0)


def _schedule():
    ops = []
    if ORDER == 'a':
        ops += [('KP', 0), ('DFT',), ('VP', 0), ('KP', 1), ('QK', 0, 0), ('SSM', 0), ('VP', 1)]
        for i in range(NT - 1):
            u = []
            for j in range(i + 1):
                u += [('QK', i + 1, j), ('PV', i, j)]
            u.insert(len(u) - 1, ('QK', i + 1, i + 1))
            ops += u
            if i + 2 < NT:
                ops += [('KP', i + 2), ('SSM', i + 1), ('VP', i + 2)]
                if i == NT - 3:
                    ops += [('SSM', 7)]
            else:
                ops += [('OP', 0), ('OP', 1)]
        for j in range(NT):
            ops += [('PV', NT - 1, j)]
            if j + 2 < NT - 1:
                ops += [('OP', j + 2)]
        ops += [('OP', NT - 1)]
    return ops


def _kernel(qT_hbm, kT_hbm, vT_hbm, sk_ref, ssmk_hbm, dd_ref, xT_hbm, ckv_hbm,
            wq_hbm, wk_hbm, wv_hbm, woT_hbm, out_hbm,
            qT, kT, vT, ssmk, xT, ckv, wq_raw, wk_raw, wv_raw, woT,
            wqT_s, bk_s, bvT_s, QT_s, a_s, acc, fullT, out_s, taps, ff_s, fi_s,
            sem, sem_k, sem_v, sem_o):
    def cp(src, dst, s):
        return pltpu.make_async_copy(src, dst, s)

    c_x = cp(xT_hbm, xT, sem.at[0])
    c_wq = [cp(wq_hbm.at[:, pl.ds(128 * g, 128)], wq_raw.at[g], sem.at[1 + g]) for g in range(2)]

    def c_w(w_hbm, raw, sm, j, half, g):
        r = pl.ds(pl.multiple_of((half * 4 + j) * 2048, 2048), 2048)
        q = 2 * half + g
        return cp(w_hbm.at[r, pl.ds(128 * g, 128)], raw.at[j % 2, q], sm.at[(j % 2) * 4 + q])

    def c_wk(j):
        return [c_w(wk_hbm, wk_raw, sem_k, j, half, g) for half in range(2) for g in range(2)]

    def c_wv(j):
        return [c_w(wv_hbm, wv_raw, sem_v, j, half, g) for half in range(2) for g in range(2)]

    def c_ckv(j):
        r = pl.ds(pl.multiple_of(j * 2 * T, 2 * T), 2 * T)
        return cp(ckv_hbm.at[r], ckv.at[r], sem.at[9 + j])

    a_pairs = ((kT_hbm, kT), (vT_hbm, vT), (ssmk_hbm, ssmk), (qT_hbm, qT))
    c_early = [cp(woT_hbm.at[pl.ds(0, 1)], woT.at[pl.ds(0, 1)], sem.at[4])]
    c_early += [cp(src.at[pl.ds(0, CH)], dst.at[pl.ds(0, CH)], sem.at[5 + n]) for n, (src, dst) in enumerate(a_pairs)]
    c_late = [cp(woT_hbm.at[pl.ds(1, H - 1)], woT.at[pl.ds(1, H - 1)], sem.at[13])]
    c_late += [cp(src.at[pl.ds(CH, M - CH)], dst.at[pl.ds(CH, M - CH)], sem.at[14 + n])
               for n, (src, dst) in enumerate(a_pairs)]
    for c in c_wq:
        c.start()
    c_x.start()

    n_i = jax.lax.broadcasted_iota(jnp.int32, (P, P), 0)
    k_i = jax.lax.broadcasted_iota(jnp.int32, (P, P), 1)
    ang = (((2 * k_i + 1) * n_i) & 511).astype(f32) * (math.pi / 256.0)
    cs, sn = jnp.cos(ang), jnp.sin(ang)
    ff_s[:, 0:P] = cs.astype(bf16)
    ff_s[:, P:2 * P] = (-sn).astype(bf16)
    fi_s[0:P, :] = (cs.T * (1.0 / P)).astype(bf16)
    fi_s[P:2 * P, :] = (sn.T * (-1.0 / P)).astype(bf16)
    sk = sk_ref[...].astype(f32)
    for t in range(KS):
        taps[t] = jnp.broadcast_to(sk[t:t + 1, :], (128, M)).T
    taps[KS] = jnp.broadcast_to(dd_ref[...].astype(f32).reshape(1, M), (128, M)).T
    acc[...] = jnp.zeros(acc.shape, f32)

    for c in c_wq:
        c.wait()

    for c in c_wk(0):
        c.start()
    vq = wq_raw.bitcast(u32)
    for hp in range(H // 2):
        for g in range(2):
            e, o = _split_pair(vq[g, pl.ds(hp, M, stride=8), :])
            wqT_s[2 * hp * 128 + 64 * g:2 * hp * 128 + 64 * g + 64, :] = _u(e.T)
            wqT_s[(2 * hp + 1) * 128 + 64 * g:(2 * hp + 1) * 128 + 64 * g + 64, :] = _u(o.T)
    c_x.wait()
    for c in c_wv(0) + [c_ckv(0)]:
        c.start()

    qscale = (D ** -0.5) * math.log2(math.e)

    def lo(u):
        return pltpu.bitcast(u << 16, f32)

    def hi(u):
        return pltpu.bitcast(u & jnp.uint32(0xFFFF0000), f32)

    def b_combos(b11, b12, b21, b22):
        return [b11 + b22, b11, b12 - b22, b21 - b11, b22, b11 + b12, b21 + b22]

    def q_body(j, carry):
        def qproj(n, c, tok):
            rows = pl.ds(pl.multiple_of((4 * j + n) * 128, 128), 128)
            cols = slice(c * 128, (c + 1) * 128)
            w = _b(_gate_u(wqT_s[rows, :], tok))
            QT_s[rows, cols] = _u((_nn(w, xT[:, cols]) * qscale).astype(bf16))

        def prep_k(hp, part):
            v = wk_raw.bitcast(u32).at[j % 2]
            r0 = part * 128
            ue = [v[q, pl.ds(r0 + hp, 8, stride=16), :] for q in range(4)]
            uo = [v[q, pl.ds(r0 + hp + 8, 8, stride=16), :] for q in range(4)]
            res = []
            for par, f in enumerate((lo, hi)):
                ce = b_combos(*[f(u) for u in ue])
                co = b_combos(*[f(u) for u in uo])
                for n in range(7):
                    r = pltpu.pack_elementwise([ce[n], co[n]], packed_dtype=bf16)
                    bk_s[2 * hp + par, n, pl.ds(pl.multiple_of(j * 64 + part * 8, 8), 8), :] = r
                    res.append(r)
            return res

        def prep_v(hp, par):
            v = wv_raw.bitcast(u32).at[j % 2]
            f = (lo, hi)[par]
            parts = []
            for part in range(8):
                u = [v[q, pl.ds(part * 128 + hp, 16, stride=8), :] for q in range(4)]
                parts.append(b_combos(*[f(x) for x in u]))
            res = []
            for n in range(7):
                c = jnp.concatenate([p[n] for p in parts], axis=0)
                r = _u(c.astype(bf16).T)
                bvT_s[2 * hp + par, n, :, pl.ds(pl.multiple_of(j * 128, 128), 128)] = r
                res.append(r[56:])
            return res

        def prep_a(cl_, part):
            c = 2 * j + cl_
            r0 = 8 * part
            rt = pl.ds(pl.multiple_of(c * T + 2 * r0, 16), 16)
            rb = pl.ds(pl.multiple_of(c * T + 128 + 2 * r0, 16), 16)
            res = []
            for cb in range(4):
                cl, ch_ = slice(cb * 128, cb * 128 + 128), slice(512 + cb * 128, 512 + cb * 128 + 128)
                blk = [_u(ckv[rt, cl]), _u(ckv[rt, ch_]), _u(ckv[rb, cl]), _u(ckv[rb, ch_])]
                cc = []
                for f in (lo, hi):
                    a11, a12, a21, a22 = [f(x) for x in blk]
                    cc.append([a11 + a22, a21 + a22, None, None, a11 + a12, a21 - a11, a12 - a22])
                for n in range(7):
                    if n == 2:
                        r = blk[0]
                    elif n == 3:
                        r = blk[3]
                    else:
                        r = pltpu.pack_elementwise([cc[0][n], cc[1][n]], packed_dtype=bf16)
                    a_s[c, n, r0:r0 + 8, cl] = r
                    res.append(r)
            return res

        fill = {}

        def spread(pieces, u0, u1):
            for n, p in enumerate(pieces):
                fill.setdefault(u0 + n * (u1 - u0) // len(pieces), []).append(p)

        spread([functools.partial(prep_k, hp, part) for hp in range(8) for part in range(8)], QW1, QW2)
        spread([functools.partial(prep_v, hp, par) for hp in range(8) for par in range(2)], QW2, QW3)
        spread([functools.partial(prep_a, c, part) for c in range(2) for part in range(8)], QW3, 64 - QLAG)
        toks = {}
        for u in range(64):
            if u == QW1:
                @pl.when(j < 3)
                def _():
                    for c in c_wk(j + 1):
                        c.start()

                @pl.when(j == 3)
                def _():
                    for c in c_early:
                        c.start()

                for c in c_wk(j):
                    c.wait()
            if u == QW2:
                @pl.when(j < 3)
                def _():
                    for c in c_wv(j + 1) + [c_ckv(j + 1)]:
                        c.start()

                @pl.when(j == 3)
                def _():
                    for c in c_late:
                        c.start()

                for c in c_wv(j) + [c_ckv(j)]:
                    c.wait()
            qproj(u // 16, u % 16, toks.pop(u, None))
            res = [r for p in fill.get(u, []) for r in p()]
            if res:
                toks[u + QLAG] = _tok(res)
        return carry

    jax.lax.fori_loop(0, 4, q_body, 0)
    for c in c_early:
        c.wait()

    tri = n_i <= k_i
    lane = jax.lax.broadcasted_iota(jnp.int32, (CH, 128), 1)
    sgn = jnp.where((jax.lax.broadcasted_iota(jnp.int32, (1, P), 1) & 1) == 0, 1.0, -1.0).astype(f32)

    def head_body(h, carry):
        @pl.when(h == 1)
        def _():
            for c in c_late:
                c.wait()

        st = dict(K={}, V={}, S={}, m={}, mfin={}, l={}, o={})
        gates = []
        qrows = pl.ds(pl.multiple_of(h * 128, 128), 128)
        rows = pl.ds(pl.multiple_of(jnp.minimum(h, NCH - 1) * CH, CH), CH)

        def rep(t, n):
            return jnp.concatenate([taps[t, rows, :]] * n, axis=1)

        def due(pos):
            g = [v for (p, v) in gates if p <= pos]
            gates[:] = [(p, v) for (p, v) in gates if p > pos]
            return g

        for pos, op in enumerate(_schedule()):
            kind = op[0]
            if kind == 'KP':
                c = op[1]
                m = [_nn(_b(a_s[c, n]), _b(bk_s[h, n])) for n in SORD]
                m = dict(zip(SORD, m))
                top = jnp.concatenate([m[0] + m[3] - m[4] + m[6], m[2] + m[4]], axis=1)
                bot = jnp.concatenate([m[1] + m[3], m[0] - m[1] + m[2] + m[5]], axis=1)
                st['K'][c] = jnp.concatenate([top, bot], axis=0).astype(bf16)
            elif kind == 'VP':
                c = op[1]
                m = [_nt(_b(bvT_s[h, n]), _b(a_s[c, n])) for n in SORD]
                m = dict(zip(SORD, m))
                top = jnp.concatenate([m[0] + m[3] - m[4] + m[6], m[1] + m[3]], axis=1)
                bot = jnp.concatenate([m[2] + m[4], m[0] - m[1] + m[2] + m[5]], axis=1)
                st['V'][c] = jnp.concatenate([top, bot], axis=0).astype(bf16)
            elif kind == 'QK':
                _, i, j = op
                q = _b(_gate(QT_s[qrows, i * T:(i + 1) * T], due(pos)))
                kc = st['K'][j]
                if j < i:
                    s = _nn(kc, q)
                    st['S'][i, j] = s
                    f = _fold(s, jnp.max)
                else:
                    sa = _nn(kc[:128], q)
                    sa = jnp.concatenate([jnp.where(tri, sa[:, :128], NEG), sa[:, 128:]], axis=1)
                    sb = jnp.where(tri, _nn(kc[128:], q[:, 128:]), NEG)
                    st['S'][i, j] = (sa, sb)
                    fa = _fold(sa, jnp.max)
                    f = jnp.concatenate([fa[:, :128], jnp.maximum(fa[:, 128:], _fold(sb, jnp.max))], axis=1)
                st['m'][i] = f if j == 0 else jnp.maximum(st['m'][i], f)
                if j == i:
                    st['mfin'][i] = jnp.max(st['m'][i], axis=0, keepdims=True)
                elif LAG_M:
                    gates.append((pos + LAG_M, st['m'][i]))
            elif kind == 'PV':
                _, i, j = op
                m = st['mfin'][i]
                vc = st['V'][j]
                s = st['S'].pop((i, j))
                if j < i:
                    p = jnp.exp2(s - m)
                    lj = _fold(p, jnp.sum)
                    o = _nn(vc, p.astype(bf16))
                else:
                    pa = jnp.exp2(s[0] - m)
                    pb = jnp.exp2(s[1] - m[:, 128:])
                    la = _fold(pa, jnp.sum)
                    lj = jnp.concatenate([la[:, :128], la[:, 128:] + _fold(pb, jnp.sum)], axis=1)
                    oa = _nn(vc[:, :128], pa.astype(bf16))
                    ob = _nn(vc[:, 128:], pb.astype(bf16))
                    o = jnp.concatenate([oa[:, :128], oa[:, 128:] + ob], axis=1)
                st['l'][i] = lj if j == 0 else st['l'][i] + lj
                st['o'][i] = o if j == 0 else st['o'][i] + o
                if j < i and LAG_S:
                    gates.append((pos + LAG_S, st['l'][i]))
                if j == i:
                    r = 1.0 / jnp.sum(st['l'][i], axis=0, keepdims=True)
                    st['o'][i] = st['o'][i] * r
                    if LAG_S and i < NT - 1:
                        gates.append((pos + LAG_S, st['o'][i][D - 8:, :]))
            elif kind == 'OP':
                i = op[1]
                ot = _gate(st['o'].pop(i), due(pos)).astype(bf16)
                acc[:, T * i:T * (i + 1)] += _nn(woT[h], ot)
            elif kind == 'DFT':
                k = kT[rows, :].astype(f32)
                ks = k * rep(0, NB)
                for j in range(1, KS):
                    kr = pltpu.roll(k, j, 1)
                    kr = jnp.concatenate([jnp.where(lane >= j, kr[:, :128], 0.0), kr[:, 128:]], axis=1)
                    ks = ks + kr * rep(j, NB)
                kv = ks * vT[rows, :].astype(f32)
                kvs = jnp.concatenate([kv[:, c * P:(c + 1) * P] for c in range(NB)], axis=0).astype(bf16)
                hk = ssmk[rows, :]
                hs = jnp.concatenate([hk[:, c * P:(c + 1) * P] for c in range(NB)], axis=0)
                hf = _nn(hs, ff_s[...])
                xf = _nn(kvs, ff_s[...])
                xr = [xf[c * CH:(c + 1) * CH, :P] for c in range(NB)]
                xi = [xf[c * CH:(c + 1) * CH, P:] for c in range(NB)]
                st['hr'] = [hf[c * CH:(c + 1) * CH, :P] for c in range(NB)]
                st['hi'] = [hf[c * CH:(c + 1) * CH, P:] for c in range(NB)]
                st['pr'] = [xr[0]] + [xr[c] - sgn * xi[c - 1] for c in range(1, NB)]
                st['pi'] = [xi[0]] + [xi[c] + sgn * xr[c - 1] for c in range(1, NB)]
                st['kv'] = kv
            elif kind == 'SSM':
                hr, hi, pr, pi = st['hr'], st['hi'], st['pr'], st['pi']
                blocks = (op[1], NB - 1 - op[1])
                ws = []
                for a in blocks:
                    wr = hr[0] * pr[a] - hi[0] * pi[a]
                    wi = hr[0] * pi[a] + hi[0] * pr[a]
                    for j in range(1, a + 1):
                        wr = wr + (hr[j] * pr[a - j] - hi[j] * pi[a - j])
                        wi = wi + (hr[j] * pi[a - j] + hi[j] * pr[a - j])
                    ws.append(jnp.concatenate([wr, wi], axis=1))
                y = _nn(jnp.concatenate(ws, axis=0).astype(bf16), fi_s[...])
                for n, a in enumerate(blocks):
                    cols = slice(a * P, (a + 1) * P)
                    ya = y[n * CH:(n + 1) * CH, :] + st['kv'][:, cols] * taps[KS, rows, :]
                    fullT[rows, cols] = (qT[rows, cols].astype(f32) * ya).astype(bf16)
        return carry

    jax.lax.fori_loop(0, H, head_body, 0)

    fullT[M:2 * M, :] = acc[...].astype(bf16)
    outs = []
    for i in range(8):
        out_s[256 * i:256 * (i + 1), :] = fullT[:, 256 * i:256 * (i + 1)].T
        c = cp(out_s.at[pl.ds(256 * i, 256)], out_hbm.at[pl.ds(256 * i, 256)], sem_o.at[i])
        c.start()
        outs.append(c)
    for c in outs:
        c.wait()


@jax.jit
def pallas_concat_heads__ssm_conv_h3__compressed_kv_cla__prompt_kernel(
    A_q: jax.Array,
    A_k: jax.Array,
    A_v: jax.Array,
    A_shift_k: jax.Array,
    A_ssm_k: jax.Array,
    A_ssm_D: jax.Array,
    B_x: jax.Array,
    B_c_kv: jax.Array,
    B_w_q: jax.Array,
    B_w_uk: jax.Array,
    B_w_uv: jax.Array,
    B_w_o: jax.Array,
):
    hbm = pl.BlockSpec(memory_space=pl.ANY)
    vmem = pl.BlockSpec(memory_space=pltpu.VMEM)
    V = pltpu.VMEM
    out = pl.pallas_call(
        _kernel,
        out_shape=jax.ShapeDtypeStruct((S, 2 * M), bf16),
        in_specs=[hbm, hbm, hbm, vmem, hbm, vmem, hbm, hbm, hbm, hbm, hbm, hbm],
        out_specs=hbm,
        scratch_shapes=[
            V((M, S), bf16), V((M, S), bf16), V((M, S), bf16), V((M, S), bf16),
            V((M, S), bf16), V((S, DC), bf16),
            V((2, M * H, 128), bf16), V((2, 4, 128 * H, 128), bf16), V((2, 4, 128 * H, 128), bf16),
            V((H, M, D), bf16),
            V((H * D // 2, M), u32), V((H, 7, 256, 128), u32), V((H, 7, 64, 512), u32),
            V((H * D // 2, S), u32), V((NT, 7, 64, 512), u32),
            V((M, S), f32), V((2 * M, S), bf16), V((S, 2 * M), bf16),
            V((KS + 1, M, 128), f32), V((P, 2 * P), bf16), V((2 * P, P), bf16),
            pltpu.SemaphoreType.DMA((18,)), pltpu.SemaphoreType.DMA((8,)),
            pltpu.SemaphoreType.DMA((8,)), pltpu.SemaphoreType.DMA((8,)),
        ],
        compiler_params=pltpu.CompilerParams(vmem_limit_bytes=120 * 1024 * 1024,
                                             shape_invariant_numerics=False),
    )(
        A_q[0].T, A_k[0].T, A_v[0].T, A_shift_k.T, A_ssm_k, A_ssm_D,
        B_x[0].T, B_c_kv[0],
        B_w_q.reshape(M * H, D), B_w_uk.reshape(DC * H, D), B_w_uv.reshape(DC * H, D),
        jnp.transpose(B_w_o, (0, 2, 1)),
    )
    return out[None]
```

```python
import functools
import math

import jax
import jax.numpy as jnp
import jax.experimental.pallas as pl
import jax.experimental.pallas.tpu as pltpu

bf16 = jnp.bfloat16
f32 = jnp.float32
u32 = jnp.uint32

S = 2048
M = 448
DC = 1024
H = 16
D = 256
KS = 4
P = 128
NB = S // P
CH = 32
NCH = M // CH
T = 256
NT = S // T
NEG = -1e30
LAG_M = 0
LAG_S = 0
SORD = (6, 4, 3, 0, 1, 2, 5)
QW1 = 12
QW2 = 34
QW3 = 50
QLAG = 2
OS = 1
QKS = 1
CVMAX = 16
SIDE0 = 2
SIDEP = 3
LA = 2
SLAG = 2
ORDER = 'a'


def _nn(a, b):
    return jnp.dot(a, b, preferred_element_type=f32)


def _nt(a, b):
    return jax.lax.dot_general(a, b, (((1,), (1,)), ((), ())), preferred_element_type=f32)


def _b(u):
    return pltpu.bitcast(u, bf16)


def _u(x):
    return pltpu.bitcast(x, u32)


def _split_pair(u):
    lo = pltpu.bitcast(u << 16, f32).astype(bf16)
    hi = pltpu.bitcast(u & jnp.uint32(0xFFFF0000), f32).astype(bf16)
    return lo, hi


def _lo(u):
    return pltpu.bitcast(u << 16, f32)


def _hi(u):
    return pltpu.bitcast(u & jnp.uint32(0xFFFF0000), f32)


def _pk(e, o):
    return pltpu.pack_elementwise([e, o], packed_dtype=bf16)


def _a7(a11, a12, a21, a22):
    return [a11 + a22, a21 + a22, a11, a22, a11 + a12, a21 - a11, a12 - a22]


def _b7(b11, b12, b21, b22):
    return [b11 + b22, b11, b12 - b22, b21 - b11, b22, b11 + b12, b21 + b22]


def _c4(m):
    return m[0] + m[3] - m[4] + m[6], m[2] + m[4], m[1] + m[3], m[0] - m[1] + m[2] + m[5]


def _combos_u(f7, blk):
    e = f7(*[_lo(x) for x in blk])
    o = f7(*[_hi(x) for x in blk])
    plain = {2: 0, 3: 3} if f7 is _a7 else {1: 0, 4: 3}
    return [blk[plain[n]] if n in plain else _pk(e[n], o[n]) for n in range(7)]


def _quad(c11, c12, c21, c22):
    return jnp.concatenate([jnp.concatenate([c11, c12], axis=1), jnp.concatenate([c21, c22], axis=1)], axis=0)


def _fold(c, op):
    return op(c.reshape(-1, 8, c.shape[1]), axis=0)


def _rsum(p):
    cols = []
    for c in range(0, p.shape[1], 128):
        tot = None
        for k in range(0, p.shape[0], 128):
            acc = None
            for r in range(k + 112, k - 16, -16):
                t = p[r:r + 8, c:c + 128] + p[r + 8:r + 16, c:c + 128]
                acc = t if acc is None else acc + t
            tot = acc if tot is None else tot + acc
        cols.append(tot)
    return jnp.concatenate(cols, axis=1) if len(cols) > 1 else cols[0]


def _gate(x, vals):
    if not vals:
        return x
    w = max(v.shape[1] for v in vals)
    top = x[:8, :w]
    for v in vals:
        if v.shape[1] < w:
            v = jnp.concatenate([v] * (w // v.shape[1]), axis=1)
        top = jnp.where(v == jnp.inf, jnp.zeros_like(top), top)
    if w < x.shape[1]:
        top = jnp.concatenate([top, x[:8, w:]], axis=1)
    return jnp.concatenate([top, x[8:]], axis=0)


def _tok(vals):
    parts = []
    for v in vals:
        for r in range(0, v.shape[0], 8):
            for c in range(0, v.shape[1], 128):
                parts.append(v[r:r + 8, c:c + 128])
    while len(parts) > 1:
        parts = [parts[i] | parts[i + 1] if i + 1 < len(parts) else parts[i] for i in range(0, len(parts), 2)]
    return (parts[0] >> 31) >> 1


def _gate_u(x, tok):
    if tok is None:
        return x
    top = jnp.concatenate([x[:8, :128] | tok, x[:8, 128:]], axis=1)
    return jnp.concatenate([top, x[8:]], axis=0)


def _ssm_pieces():
    ps = [('HD', 0), ('SC', 0), ('HD', 1), ('SC', 1), ('W7', 0), ('HD', 2), ('SC', 2), ('W7', 1), ('HD', 3), ('SC', 3)]
    if not OS:
        ps = [p for p in ps if p[0] != 'W7']
    cur, cost = [], 0
    for a in range(NB):
        for half in range(2):
            if cost + a + 1 > CVMAX:
                ps.append(('CV', tuple(cur)))
                cur, cost = [], 0
            cur.append((a, half))
            cost += a + 1
        if a % 4 == 3:
            ps.append(('CV', tuple(cur)))
            cur, cost = [], 0
            ps.append(('ID', a // 4))
    return ps


def _schedule():
    ops = [('KP', 0), ('OP', NT - 1), ('AT',), ('VP', 0), ('KP', 1), ('QK', 0, 0), ('VP', 1), ('EX', 0, 0)]
    for i in range(NT - 1):
        for j in range(i + 1):
            ops += [('QK', i + 1, j)]
            if j + LA <= i:
                ops += [('EX', i, j + LA)]
            if j == i:
                ops += [('QK', i + 1, i + 1)]
            ops += [('PV', i, j)]
        e1 = [('PACE',), ('EX', i + 1, 1)] if LA == 2 else []
        if i + 2 < NT:
            ops += [('KP', i + 2), ('EX', i + 1, 0), ('VP', i + 2)] + e1
        else:
            ops += [('OP', 0), ('PACE',), ('EX', i + 1, 0), ('OP', 1)] + e1 + [('PACE',)]
    for j in range(NT):
        if j + LA < NT:
            ops += [('EX', NT - 1, j + LA)]
        ops += [('PV', NT - 1, j)]
        if j + 2 < NT - 3:
            ops += [('OP', j + 2)]
        ops += [('PACE',)]
    ops += [('OP', NT - 3), ('OP', NT - 2)]
    side = _ssm_pieces()
    out = []
    nsub = 0
    for op in ops:
        if op[0] in ('KP', 'VP'):
            for t in range(7):
                out.append(op + (t,))
                nsub += 1
                if side and nsub >= SIDE0 and (nsub - SIDE0) % SIDEP == 0:
                    out += [side.pop(0)]
        else:
            out.append(op)
    assert not side
    return out


def _kernel(qT_hbm, kT_hbm, vT_hbm, sk_ref, ssmk_hbm, dd_ref, xT_hbm, ckv_hbm,
            wq_hbm, wk_hbm, wv_hbm, woT_hbm, out_hbm,
            qT, kT, vT, ssmk, xT, ckv, wq_raw, wk_raw, wv_raw, woT,
            wqT_s, bk_s, bvT_s, QT_s, a_s, acc, fullT, out_s, taps, ff_s, fi_s,
            S0_s, S1_s, X_s, W7_s, pace_s, m0_s, m1_s, l0_s, l1_s,
            sem, sem_k, sem_v, sem_o, *kvo):
    K_s, V_s, O_s = kvo[:NT], kvo[NT:2 * NT], kvo[2 * NT:]
    def cp(src, dst, s):
        return pltpu.make_async_copy(src, dst, s)

    c_x = cp(xT_hbm, xT, sem.at[0])
    c_wq = [cp(wq_hbm.at[:, pl.ds(128 * g, 128)], wq_raw.at[g], sem.at[1 + g]) for g in range(2)]

    def c_w(w_hbm, raw, sm, j, half, g):
        r = pl.ds(pl.multiple_of((half * 4 + j) * 2048, 2048), 2048)
        q = 2 * half + g
        return cp(w_hbm.at[r, pl.ds(128 * g, 128)], raw.at[j % 2, q], sm.at[(j % 2) * 4 + q])

    def c_wk(j):
        return [c_w(wk_hbm, wk_raw, sem_k, j, half, g) for half in range(2) for g in range(2)]

    def c_wv(j):
        return [c_w(wv_hbm, wv_raw, sem_v, j, half, g) for half in range(2) for g in range(2)]

    def c_ckv(j):
        r = pl.ds(pl.multiple_of(j * 2 * T, 2 * T), 2 * T)
        return cp(ckv_hbm.at[r], ckv.at[r], sem.at[9 + j])

    a_pairs = ((kT_hbm, kT), (vT_hbm, vT), (ssmk_hbm, ssmk), (qT_hbm, qT))
    c_early = [cp(woT_hbm.at[pl.ds(0, 1)], woT.at[pl.ds(0, 1)], sem.at[4])]
    c_early += [cp(src.at[pl.ds(0, CH)], dst.at[pl.ds(0, CH)], sem.at[5 + n]) for n, (src, dst) in enumerate(a_pairs)]
    c_late = [cp(woT_hbm.at[pl.ds(1, H - 1)], woT.at[pl.ds(1, H - 1)], sem.at[13])]
    c_late += [cp(src.at[pl.ds(CH, M - CH)], dst.at[pl.ds(CH, M - CH)], sem.at[14 + n])
               for n, (src, dst) in enumerate(a_pairs)]
    for c in c_wq:
        c.start()
    c_x.start()

    n_i = jax.lax.broadcasted_iota(jnp.int32, (P, P), 0)
    k_i = jax.lax.broadcasted_iota(jnp.int32, (P, P), 1)
    ang = (((2 * k_i + 1) * n_i) & 511).astype(f32) * (math.pi / 256.0)
    cs, sn = jnp.cos(ang), jnp.sin(ang)
    ff_s[:, 0:P] = cs.astype(bf16)
    ff_s[:, P:2 * P] = (-sn).astype(bf16)
    fi_s[0:P, :] = (cs.T * (1.0 / P)).astype(bf16)
    fi_s[P:2 * P, :] = (sn.T * (-1.0 / P)).astype(bf16)
    sk = sk_ref[...].astype(f32)
    for t in range(KS):
        taps[t] = jnp.broadcast_to(sk[t:t + 1, :], (128, M)).T
    taps[KS] = jnp.broadcast_to(dd_ref[...].astype(f32).reshape(1, M), (128, M)).T
    acc[...] = jnp.zeros(acc.shape, f32)
    fullT[...] = jnp.zeros(fullT.shape, bf16)
    O_s[NT - 1][...] = jnp.zeros(O_s[0].shape, bf16)
    W7_s[...] = jnp.zeros(W7_s.shape, u32)

    for c in c_wq:
        c.wait()

    for c in c_wk(0):
        c.start()
    vq = wq_raw.bitcast(u32)
    for hp in range(H // 2):
        for g in range(2):
            e, o = _split_pair(vq[g, pl.ds(hp, M, stride=8), :])
            wqT_s[2 * hp * 128 + 64 * g:2 * hp * 128 + 64 * g + 64, :] = _u(e.T)
            wqT_s[(2 * hp + 1) * 128 + 64 * g:(2 * hp + 1) * 128 + 64 * g + 64, :] = _u(o.T)
    c_x.wait()
    for c in c_wv(0) + [c_ckv(0)]:
        c.start()

    qscale = (D ** -0.5) * math.log2(math.e)

    def lo(u):
        return pltpu.bitcast(u << 16, f32)

    def hi(u):
        return pltpu.bitcast(u & jnp.uint32(0xFFFF0000), f32)

    def b_combos(b11, b12, b21, b22):
        return [b11 + b22, b11, b12 - b22, b21 - b11, b22, b11 + b12, b21 + b22]

    def q_body(j, carry):
        def qproj(n, c, tok):
            rows = pl.ds(pl.multiple_of((4 * j + n) * 128, 128), 128)
            cols = slice(c * 128, (c + 1) * 128)
            w = _b(_gate_u(wqT_s[rows, :], tok))
            QT_s[rows, cols] = _u((_nn(w, xT[:, cols]) * qscale).astype(bf16))

        def prep_k(hp, part):
            v = wk_raw.bitcast(u32).at[j % 2]
            r0 = part * 128
            ue = [v[q, pl.ds(r0 + hp, 8, stride=16), :] for q in range(4)]
            uo = [v[q, pl.ds(r0 + hp + 8, 8, stride=16), :] for q in range(4)]
            res = []
            for par, f in enumerate((lo, hi)):
                ce = b_combos(*[f(u) for u in ue])
                co = b_combos(*[f(u) for u in uo])
                for n in range(7):
                    r = pltpu.pack_elementwise([ce[n], co[n]], packed_dtype=bf16)
                    bk_s[2 * hp + par, n, pl.ds(pl.multiple_of(j * 64 + part * 8, 8), 8), :] = r
                    res.append(r)
            return res

        def prep_v(hp, par):
            v = wv_raw.bitcast(u32).at[j % 2]
            f = (lo, hi)[par]
            parts = []
            for part in range(8):
                u = [v[q, pl.ds(part * 128 + hp, 16, stride=8), :] for q in range(4)]
                parts.append(b_combos(*[f(x) for x in u]))
            res = []
            for n in range(7):
                c = jnp.concatenate([p[n] for p in parts], axis=0)
                r = _u(c.astype(bf16).T)
                bvT_s[2 * hp + par, n, :, pl.ds(pl.multiple_of(j * 128, 128), 128)] = r
                res.append(r[56:])
            return res

        def prep_a(cl_, part):
            c = 2 * j + cl_
            r0 = 8 * part
            rt = pl.ds(pl.multiple_of(c * T + 2 * r0, 16), 16)
            rb = pl.ds(pl.multiple_of(c * T + 128 + 2 * r0, 16), 16)
            res = []
            for cb in range(4):
                cl, ch_ = slice(cb * 128, cb * 128 + 128), slice(512 + cb * 128, 512 + cb * 128 + 128)
                blk = [_u(ckv[rt, cl]), _u(ckv[rt, ch_]), _u(ckv[rb, cl]), _u(ckv[rb, ch_])]
                cc = []
                for f in (lo, hi):
                    a11, a12, a21, a22 = [f(x) for x in blk]
                    cc.append([a11 + a22, a21 + a22, None, None, a11 + a12, a21 - a11, a12 - a22])
                for n in range(7):
                    if n == 2:
                        r = blk[0]
                    elif n == 3:
                        r = blk[3]
                    else:
                        r = pltpu.pack_elementwise([cc[0][n], cc[1][n]], packed_dtype=bf16)
                    a_s[c, n, r0:r0 + 8, cl] = r
                    res.append(r)
            return res

        fill = {}

        def spread(pieces, u0, u1):
            for n, p in enumerate(pieces):
                fill.setdefault(u0 + n * (u1 - u0) // len(pieces), []).append(p)

        spread([functools.partial(prep_k, hp, part) for hp in range(8) for part in range(8)], QW1, QW2)
        spread([functools.partial(prep_v, hp, par) for hp in range(8) for par in range(2)], QW2, QW3)
        spread([functools.partial(prep_a, c, part) for c in range(2) for part in range(8)], QW3, 64 - QLAG)
        toks = {}
        for u in range(64):
            if u == QW1:
                @pl.when(j < 3)
                def _():
                    for c in c_wk(j + 1):
                        c.start()

                @pl.when(j == 3)
                def _():
                    for c in c_early:
                        c.start()

                for c in c_wk(j):
                    c.wait()
            if u == QW2:
                @pl.when(j < 3)
                def _():
                    for c in c_wv(j + 1) + [c_ckv(j + 1)]:
                        c.start()

                @pl.when(j == 3)
                def _():
                    for c in c_late:
                        c.start()

                for c in c_wv(j) + [c_ckv(j)]:
                    c.wait()
            qproj(u // 16, u % 16, toks.pop(u, None))
            res = [r for p in fill.get(u, []) for r in p()]
            if res:
                toks[u + QLAG] = _tok(res)
        return carry

    jax.lax.fori_loop(0, 4, q_body, 0)
    for c in c_early:
        c.wait()

    tri = n_i <= k_i
    sgn = jnp.where((jax.lax.broadcasted_iota(jnp.int32, (1, P), 1) & 1) == 0, 1.0, -1.0).astype(f32)

    c_outa = cp(out_s.at[:, pl.ds(0, 384)], out_hbm.at[:, pl.ds(0, 384)], sem_o.at[8])

    XP, HR, HI, PR, PI, KV, WR, WI = range(8)

    def krow(z, n):
        return pl.ds(n * 64, 64) if isinstance(z, int) else pl.ds(pl.multiple_of(z * 64 + n * 64, 64), 64)

    def vrow(z):
        return pl.ds(0, 128) if isinstance(z, int) else pl.ds(pl.multiple_of(z * 128, 128), 128)

    def blk_at(c, half=None):
        r0 = (c % 8) * CH
        rs = slice(r0, r0 + CH) if half is None else slice(r0 + 16 * half, r0 + 16 * half + 16)
        return rs, slice((c // 8) * P, (c // 8 + 1) * P)

    def out_proj(i, hw, par, zl):
        if OS:
            m = {n: _nn(_b(W7_s[par, n]), O_s[i][zl, n]) for n in SORD}
            o = _quad(*_c4(m))
        else:
            o = _nn(woT[hw], _quad(*[O_s[i][zl, n] for n in range(4)]))
        acc[:, T * i:T * (i + 1)] += o
        return o

    def head_body(h, carry):
        @pl.when(h == 1)
        def _():
            for c in c_late:
                c.wait()

        @pl.when(h == H - 1)
        def _():
            c_outa.start()

        st = dict(M={}, P={}, Q7={}, mfin={}, o={})
        zs, zl = h >> 10, 0
        m_s, l_s = (m0_s, m1_s), (l0_s, l1_s)
        qrows = pl.ds(pl.multiple_of(h * 128, 128), 128)
        rows = pl.ds(pl.multiple_of(jnp.minimum(h, NCH - 1) * CH, CH), CH)

        def rep(t, n):
            return jnp.concatenate([taps[t, rows, :]] * n, axis=1)

        toks = []

        def due():
            for t in toks:
                t[0] -= 1
            ready = [t[1] for t in toks if t[0] <= 0]
            toks[:] = [t for t in toks if t[0] > 0]
            return functools.reduce(lambda x, y: x | y, ready) if ready else None

        def gate_later(vals):
            toks.append([SLAG, _tok([v if v.dtype == u32 else pltpu.bitcast(v, u32) for v in vals])])

        for op in _schedule():
            kind = op[0]
            if kind == 'KP':
                _, c, t = op
                n = SORD[t]
                st['M'][n] = st['last'] = _nn(_b(_gate_u(a_s[c, n], due())), _b(bk_s[h, n]))
                if t == 6:
                    c4 = _c4(st['M'])
                    blks = dict(zip((2, 7, 8, 3), c4))
                    if QKS and c < NT - 1:
                        blks.update({n: x for n, x in enumerate(_a7(*c4)) if n not in (2, 3)})
                    for n, x in blks.items():
                        K_s[c][krow(zs, n), :] = _u(x.astype(bf16))
            elif kind == 'VP':
                _, c, t = op
                n = SORD[t]
                st['M'][n] = st['last'] = _nt(_b(_gate_u(bvT_s[h, n], due())), _b(a_s[c, n]))
                if t == 6:
                    c11, c12, c21, c22 = _c4(st['M'])
                    V_s[c][vrow(zs), :] = _u(_quad(c11, c21, c12, c22).astype(bf16))
            elif kind == 'QK':
                _, i, j = op
                S_s = (S0_s, S1_s)[i % 2]
                qu = QT_s[qrows, i * T:(i + 1) * T]
                if j < i:
                    if QKS:
                        if i not in st['Q7']:
                            st['Q7'][i] = _combos_u(_b7, [qu[:64, :128], qu[:64, 128:], qu[64:, :128], qu[64:, 128:]])
                        m = {n: _nn(_b(K_s[j][krow(zl, n), :]), _b(st['Q7'][i][n])) for n in SORD}
                        s = _quad(*_c4(m))
                    else:
                        s = _nn(_b(_quad(*[K_s[j][krow(zl, n), :] for n in (2, 7, 8, 3)])), _b(qu))
                    S_s[zs, j] = s
                    f = _fold(s, jnp.max)
                else:
                    q = _b(qu)
                    sa = _nn(_b(jnp.concatenate([K_s[j][krow(zl, 2), :], K_s[j][krow(zl, 7), :]], axis=1)), q)
                    sa = jnp.concatenate([jnp.where(tri, sa[:, :128], NEG), sa[:, 128:]], axis=1)
                    sb = _nn(_b(jnp.concatenate([K_s[j][krow(zl, 8), :], K_s[j][krow(zl, 3), :]], axis=1)), q[:, 128:])
                    sb = jnp.where(tri, sb, NEG)
                    S_s[zs, j, 0:128, :] = sa
                    S_s[zs, j, 128:T, 128:T] = sb
                    fa = _fold(sa, jnp.max)
                    f = jnp.concatenate([fa[:, :128], jnp.maximum(fa[:, 128:], _fold(sb, jnp.max))], axis=1)
                m_s[i % 2][zs, j] = f
                pace_s[zs] = f
            elif kind == 'EX':
                _, i, j = op
                S_s = (S0_s, S1_s)[i % 2]
                if j == 0:
                    m = m_s[i % 2][zl, 0]
                    for t in range(1, i + 1):
                        m = jnp.maximum(m, m_s[i % 2][zl, t])
                    st['mfin'][i] = jnp.max(m, axis=0, keepdims=True)
                m = st['mfin'][i]
                if j > 0:
                    m = jnp.where(pace_s[zl, 0:1, :] == jnp.inf, jnp.inf, m)
                if j < i:
                    p = jnp.exp2(S_s[zl, j] - m)
                    lj = _rsum(p)
                    st['P'][i, j] = p.astype(bf16)
                else:
                    pa = jnp.exp2(S_s[zl, j, 0:128, :] - m)
                    pb = jnp.exp2(S_s[zl, j, 128:T, 128:T] - m[:, 128:])
                    la = _rsum(pa)
                    lj = jnp.concatenate([la[:, :128], la[:, 128:] + _rsum(pb)], axis=1)
                    st['P'][i, j] = (pa.astype(bf16), pb.astype(bf16))
                l_s[i % 2][zs, j] = lj
            elif kind == 'PV':
                _, i, j = op
                vu = V_s[j][vrow(zl), :]
                p = st['P'].pop((i, j))
                if j < i:
                    o = _nn(_b(vu), p)
                else:
                    oa = _nn(_b(vu[:, :128]), p[0])
                    ob = _nn(_b(vu[:, 128:]), p[1])
                    o = jnp.concatenate([oa[:, :128], oa[:, 128:] + ob], axis=1)
                st['last'] = o
                o = o if j == 0 else st['o'][i] + o
                st['o'][i] = o
                if j == i:
                    l = l_s[i % 2][zl, 0]
                    for t in range(1, i + 1):
                        l = l + l_s[i % 2][zl, t]
                    o = o * (1.0 / jnp.sum(l, axis=0, keepdims=True))
                    blks = (o[:128, :128], o[:128, 128:], o[128:, :128], o[128:, 128:])
                    for n, x in enumerate(_b7(*blks) if OS else blks):
                        O_s[i][zs, n] = x.astype(bf16)
            elif kind == 'PACE':
                pace_s[zs] = jnp.concatenate([st['last'][-8:, -128:]] * 2, axis=1)
            elif kind == 'OP':
                i = op[1]
                st['last'] = out_proj(i, jnp.maximum(h - 1, 0) if i == NT - 1 else h,
                                      (h + 1) % 2 if i == NT - 1 else h % 2, zl)
            elif kind == 'W7':
                r = slice(56 * op[1], 56 * op[1] + 56)
                wu = _u(woT[h])
                blk = [wu[:112, :128][r], wu[:112, 128:][r], wu[112:, :128][r], wu[112:, 128:][r]]
                w7 = _combos_u(_a7, blk)
                for n, x in enumerate(w7):
                    W7_s[h % 2, n, r] = x
                gate_later(w7)
            elif kind == 'AT':
                g = jnp.clip((h - 4) // 4, 0, 2)
                t0 = jnp.minimum(((h + 12) % 4) * 6, NB - 6)
                grow = pl.ds(pl.multiple_of(g * 128, 128), 128)
                gcol = pl.ds(pl.multiple_of(jnp.where(h == H - 1, 3, g) * 128, 128), 128)
                res = []
                for n in range(6):
                    tok = pl.ds(pl.multiple_of((t0 + n) * 128, 128), 128)
                    x = fullT[grow, tok].T
                    out_s[tok, gcol] = x
                    res.append(_u(x)[56:])
                gate_later(res)
            elif kind == 'HD':
                g = op[1]
                hs = jnp.concatenate([ssmk[rows, c * P:(c + 1) * P] for c in range(4 * g, 4 * g + 4)], axis=0)
                hf = _nn(hs, ff_s[...])
                for n in range(4):
                    X_s[(zs, HR) + blk_at(4 * g + n)] = hf[n * CH:(n + 1) * CH, :P]
                    X_s[(zs, HI) + blk_at(4 * g + n)] = hf[n * CH:(n + 1) * CH, P:]
            elif kind == 'SC':
                g = op[1]
                if g == 0:
                    k = jnp.concatenate([jnp.zeros((CH, P), f32), kT[rows, 0:4 * P].astype(f32)], axis=1)
                else:
                    k = kT[rows, (4 * g - 1) * P:(4 * g + 4) * P].astype(f32)
                ks = k[:, P:] * rep(0, 4)
                for j in range(1, KS):
                    ks = ks + pltpu.roll(k, j, 1)[:, P:] * rep(j, 4)
                kv = ks * vT[rows, 4 * g * P:(4 * g + 4) * P].astype(f32)
                kvs = jnp.concatenate([kv[:, n * P:(n + 1) * P] for n in range(4)], axis=0)
                xf = _nn(kvs.astype(bf16), ff_s[...])
                for n in range(4):
                    c = 4 * g + n
                    xr, xi = xf[n * CH:(n + 1) * CH, :P], xf[n * CH:(n + 1) * CH, P:]
                    X_s[(zs, KV) + blk_at(c)] = kvs[n * CH:(n + 1) * CH]
                    X_s[(zs, PR) + blk_at(c)] = xr if c == 0 else xr - sgn * st['x'][1]
                    X_s[(zs, PI) + blk_at(c)] = xi if c == 0 else xi + sgn * st['x'][0]
                    st['x'] = (xr, xi)
            elif kind == 'CV':
                res = []
                for a, half in op[1]:
                    wr = wi = None
                    for j in range(a + 1):
                        hr, hi_ = X_s[(zl, HR) + blk_at(j, half)], X_s[(zl, HI) + blk_at(j, half)]
                        pr, pi = X_s[(zl, PR) + blk_at(a - j, half)], X_s[(zl, PI) + blk_at(a - j, half)]
                        tr, ti = hr * pr - hi_ * pi, hr * pi + hi_ * pr
                        wr, wi = (tr, ti) if wr is None else (wr + tr, wi + ti)
                    X_s[(zs, WR) + blk_at(a, half)] = wr
                    X_s[(zs, WI) + blk_at(a, half)] = wi
                    res += [wr, wi]
                gate_later(res)
            elif kind == 'ID':
                g = op[1]
                w = jnp.concatenate(
                    [jnp.concatenate([X_s[(zl, WR) + blk_at(c)], X_s[(zl, WI) + blk_at(c)]], axis=1)
                     for c in range(4 * g, 4 * g + 4)], axis=0)
                y = _nn(w.astype(bf16), fi_s[...])
                for n in range(4):
                    c = 4 * g + n
                    cols = slice(c * P, (c + 1) * P)
                    ya = y[n * CH:(n + 1) * CH, :] + X_s[(zl, KV) + blk_at(c)] * taps[KS, rows, :]
                    fullT[rows, cols] = (qT[rows, cols].astype(f32) * ya).astype(bf16)
        return carry

    jax.lax.fori_loop(0, H, head_body, 0)

    out_proj(NT - 1, H - 1, (H - 1) % 2, 0)
    outs = [c_outa]
    for i in range(NT):
        cols = slice(T * i, T * (i + 1))
        blk = jnp.concatenate([fullT[384:M, cols], acc[:, cols].astype(bf16)], axis=0)
        out_s[cols, 384:2 * M] = blk.T
        c = cp(out_s.at[pl.ds(T * i, T), pl.ds(384, 512)], out_hbm.at[pl.ds(T * i, T), pl.ds(384, 512)], sem_o.at[i])
        c.start()
        outs.append(c)
    for c in outs:
        c.wait()


@jax.jit
def pallas_concat_heads__ssm_conv_h3__compressed_kv_cla__prompt_kernel(
    A_q: jax.Array,
    A_k: jax.Array,
    A_v: jax.Array,
    A_shift_k: jax.Array,
    A_ssm_k: jax.Array,
    A_ssm_D: jax.Array,
    B_x: jax.Array,
    B_c_kv: jax.Array,
    B_w_q: jax.Array,
    B_w_uk: jax.Array,
    B_w_uv: jax.Array,
    B_w_o: jax.Array,
):
    hbm = pl.BlockSpec(memory_space=pl.ANY)
    vmem = pl.BlockSpec(memory_space=pltpu.VMEM)
    V = pltpu.VMEM
    out = pl.pallas_call(
        _kernel,
        out_shape=jax.ShapeDtypeStruct((S, 2 * M), bf16),
        in_specs=[hbm, hbm, hbm, vmem, hbm, vmem, hbm, hbm, hbm, hbm, hbm, hbm],
        out_specs=hbm,
        scratch_shapes=[
            V((M, S), bf16), V((M, S), bf16), V((M, S), bf16), V((M, S), bf16),
            V((M, S), bf16), V((S, DC), bf16),
            V((2, M * H, 128), bf16), V((2, 4, 128 * H, 128), bf16), V((2, 4, 128 * H, 128), bf16),
            V((H, M, D), bf16),
            V((H * D // 2, M), u32), V((H, 7, 256, 128), u32), V((H, 7, 64, 512), u32),
            V((H * D // 2, S), u32), V((NT, 7, 64, 512), u32),
            V((M, S), f32), V((M, S), bf16), V((S, 2 * M), bf16),
            V((KS + 1, M, 128), f32), V((P, 2 * P), bf16), V((2 * P, P), bf16),
            V((1, NT, T, T), f32), V((1, NT, T, T), f32), V((1, 8, T, T), f32),
            V((2, 7, 112, 128), u32), V((1, 8, T), f32),
            V((1, NT, 8, T), f32), V((1, NT, 8, T), f32), V((1, NT, 8, T), f32), V((1, NT, 8, T), f32),
            pltpu.SemaphoreType.DMA((18,)), pltpu.SemaphoreType.DMA((8,)),
            pltpu.SemaphoreType.DMA((8,)), pltpu.SemaphoreType.DMA((9,)),
        ] + [V((9 * 64, 128), u32)] * NT + [V((128, T), u32)] * NT + [V((1, 7, 128, 128), bf16)] * NT,
        compiler_params=pltpu.CompilerParams(vmem_limit_bytes=120 * 1024 * 1024,
                                             shape_invariant_numerics=False),
    )(
        A_q[0].T, A_k[0].T, A_v[0].T, A_shift_k.T, A_ssm_k, A_ssm_D,
        B_x[0].T, B_c_kv[0],
        B_w_q.reshape(M * H, D), B_w_uk.reshape(DC * H, D), B_w_uv.reshape(DC * H, D),
        jnp.transpose(B_w_o, (0, 2, 1)),
    )
    return out[None]
```

```python
import functools
import math

import jax
import jax.numpy as jnp
import jax.experimental.pallas as pl
import jax.experimental.pallas.tpu as pltpu

bf16 = jnp.bfloat16
f32 = jnp.float32
u32 = jnp.uint32

S = 2048
M = 448
DC = 1024
H = 16
D = 256
KS = 4
P = 128
NB = S // P
CH = 32
NCH = M // CH
T = 256
NT = S // T
NEG = -1e30
LAG_M = 0
LAG_S = 0
SORD = (6, 4, 3, 0, 1, 2, 5)
QW1 = 42
QW2 = 105
QW3 = 168
QLAG = 6
OS = 1
QKS = 1
CVMAX = 16
SIDE0 = 1
SIDEP = 3
LA = 2
SLAG = 2
APACE = 1
PROW = 0
ORDER = 'a'


def _nn(a, b):
    return jnp.dot(a, b, preferred_element_type=f32)


def _nt(a, b):
    return jax.lax.dot_general(a, b, (((1,), (1,)), ((), ())), preferred_element_type=f32)


def _b(u):
    return pltpu.bitcast(u, bf16)


def _u(x):
    return pltpu.bitcast(x, u32)


def _split_pair(u):
    lo = pltpu.bitcast(u << 16, f32).astype(bf16)
    hi = pltpu.bitcast(u & jnp.uint32(0xFFFF0000), f32).astype(bf16)
    return lo, hi


def _lo(u):
    return pltpu.bitcast(u << 16, f32)


def _hi(u):
    return pltpu.bitcast(u & jnp.uint32(0xFFFF0000), f32)


def _pk(e, o):
    return pltpu.pack_elementwise([e, o], packed_dtype=bf16)


def _a7(a11, a12, a21, a22):
    return [a11 + a22, a21 + a22, a11, a22, a11 + a12, a21 - a11, a12 - a22]


def _b7(b11, b12, b21, b22):
    return [b11 + b22, b11, b12 - b22, b21 - b11, b22, b11 + b12, b21 + b22]


def _c4(m):
    return m[0] + m[3] - m[4] + m[6], m[2] + m[4], m[1] + m[3], m[0] - m[1] + m[2] + m[5]


def _combos_u(f7, blk):
    e = f7(*[_lo(x) for x in blk])
    o = f7(*[_hi(x) for x in blk])
    plain = {2: 0, 3: 3} if f7 is _a7 else {1: 0, 4: 3}
    return [blk[plain[n]] if n in plain else _pk(e[n], o[n]) for n in range(7)]


def _quad(c11, c12, c21, c22):
    return jnp.concatenate([jnp.concatenate([c11, c12], axis=1), jnp.concatenate([c21, c22], axis=1)], axis=0)


def _fold(c, op):
    return op(c.reshape(-1, 8, c.shape[1]), axis=0)


def _rsum(p):
    cols = []
    for c in range(0, p.shape[1], 128):
        tot = None
        for k in range(0, p.shape[0], 128):
            acc = None
            for r in range(k + 112, k - 16, -16):
                t = p[r:r + 8, c:c + 128] + p[r + 8:r + 16, c:c + 128]
                acc = t if acc is None else acc + t
            tot = acc if tot is None else tot + acc
        cols.append(tot)
    return jnp.concatenate(cols, axis=1) if len(cols) > 1 else cols[0]


def _gate(x, vals):
    if not vals:
        return x
    w = max(v.shape[1] for v in vals)
    top = x[:8, :w]
    for v in vals:
        if v.shape[1] < w:
            v = jnp.concatenate([v] * (w // v.shape[1]), axis=1)
        top = jnp.where(v == jnp.inf, jnp.zeros_like(top), top)
    if w < x.shape[1]:
        top = jnp.concatenate([top, x[:8, w:]], axis=1)
    return jnp.concatenate([top, x[8:]], axis=0)


def _tok(vals):
    parts = []
    for v in vals:
        for r in range(0, v.shape[0], 8):
            for c in range(0, v.shape[1], 128):
                parts.append(v[r:r + 8, c:c + 128])
    while len(parts) > 1:
        parts = [parts[i] | parts[i + 1] if i + 1 < len(parts) else parts[i] for i in range(0, len(parts), 2)]
    return (parts[0] >> 31) >> 1


def _gate_u(x, tok):
    if tok is None:
        return x
    top = jnp.concatenate([x[:8, :128] | tok, x[:8, 128:]], axis=1)
    return jnp.concatenate([top, x[8:]], axis=0)


def _ssm_pieces():
    ps = [('HD', 0), ('SC', 0), ('HD', 1), ('SC', 1), ('W7', 0), ('HD', 2), ('SC', 2), ('W7', 1), ('HD', 3), ('SC', 3), ('WC',)]
    if not OS:
        ps = [p for p in ps if p[0] not in ('W7', 'WC')]
    cur, cost = [], 0
    for a in range(NB):
        for half in range(2):
            if cur and cost + a + 1 > CVMAX:
                ps.append(('CV', tuple(cur)))
                cur, cost = [], 0
            cur.append((a, half))
            cost += a + 1
        if a % 4 == 3:
            if cur:
                ps.append(('CV', tuple(cur)))
            cur, cost = [], 0
            ps.append(('ID', a // 4))
    return ps


def _schedule():
    ops = [('KP', 0), ('OP', NT - 1), ('AT',), ('VP', 0), ('KP', 1), ('QK', 0, 0), ('VP', 1), ('EX', 0, 0)]
    for i in range(NT - 1):
        for j in range(i + 1):
            ops += [('QK', i + 1, j)]
            if j + LA <= i:
                ops += [('EX', i, j + LA)]
            if j == i:
                ops += [('QK', i + 1, i + 1)]
            ops += [('PV', i, j)]
        e1 = [('PACE',), ('EX', i + 1, 1)] if LA == 2 else []
        if i + 2 < NT:
            ops += [('KP', i + 2), ('EX', i + 1, 0), ('VP', i + 2)] + e1
        else:
            ops += [('OP', 0), ('PACE',), ('EX', i + 1, 0), ('OP', 1)] + e1 + [('PACE',)]
    for j in range(NT):
        if j + LA < NT:
            ops += [('EX', NT - 1, j + LA)]
        ops += [('PV', NT - 1, j)]
        if j + 2 < NT - 3:
            ops += [('OP', j + 2)]
        ops += [('PACE',)]
    ops += [('OP', NT - 3), ('OP', NT - 2)]
    side = _ssm_pieces()
    out = []
    nsub = 0
    for op in ops:
        if op[0] in ('KP', 'VP'):
            for t in range(7):
                out.append(op + (t,))
                nsub += 1
                if side and nsub >= SIDE0 and (nsub - SIDE0) % SIDEP == 0:
                    out += [side.pop(0)]
        else:
            out.append(op)
    assert not side
    return out


def _kernel(qT_hbm, kT_hbm, vT_hbm, sk_ref, ssmk_hbm, dd_ref, xT_hbm, ckv_hbm,
            wq_hbm, wk_hbm, wv_hbm, woT_hbm, out_hbm,
            qT, kT, vT, ssmk, xT, ckv, wq_raw, wk_raw, wv_raw, woT,
            aq_s, bx_s, bk_s, bvT_s, QT_s, a_s, acc, fullT, out_s, taps, ff_s, fi_s,
            S0_s, S1_s, X_s, W7_s, W7p_s, pace_s, m0_s, m1_s, l0_s, l1_s,
            sem, sem_k, sem_v, sem_o, *kvo):
    K_s, V_s, O_s, Y_s = kvo[:NT], kvo[NT:2 * NT], kvo[2 * NT:3 * NT], kvo[3 * NT:]
    def cp(src, dst, s):
        return pltpu.make_async_copy(src, dst, s)

    c_x = cp(xT_hbm, xT, sem.at[0])
    QP = ((0, 128), (128, 96))

    def c_wq(p):
        cs_ = []
        for half in range(2):
            r = pl.ds((half * 224 + QP[p][0]) * H, QP[p][1] * H)
            for g in range(2):
                cs_.append(cp(wq_hbm.at[r, pl.ds(128 * g, 128)], wq_raw.at[g, r], sem.at[18 + 4 * p + 2 * half + g]))
        return cs_


    def c_w(w_hbm, raw, sm, j, half, g):
        r = pl.ds(pl.multiple_of((half * 4 + j) * 2048, 2048), 2048)
        q = 2 * half + g
        return cp(w_hbm.at[r, pl.ds(128 * g, 128)], raw.at[j % 2, q, pl.ds(0, 2048)], sm.at[(j % 2) * 4 + q])

    def c_wk(j):
        return [c_w(wk_hbm, wk_raw, sem_k, j, half, g) for half in range(2) for g in range(2)]

    def c_wv(j):
        return [c_w(wv_hbm, wv_raw, sem_v, j, half, g) for half in range(2) for g in range(2)]

    def c_ckv(j):
        r = pl.ds(pl.multiple_of(j * 2 * T, 2 * T), 2 * T)
        return cp(ckv_hbm.at[r], ckv.at[r], sem.at[9 + j])

    a_pairs = ((kT_hbm, kT), (vT_hbm, vT), (ssmk_hbm, ssmk), (qT_hbm, qT))
    c_early = [cp(woT_hbm.at[pl.ds(0, 1)], woT.at[pl.ds(0, 1)], sem.at[4])]
    c_early += [cp(src.at[pl.ds(0, CH)], dst.at[pl.ds(0, CH)], sem.at[5 + n]) for n, (src, dst) in enumerate(a_pairs)]
    c_late = [cp(woT_hbm.at[pl.ds(1, H - 1)], woT.at[pl.ds(1, H - 1)], sem.at[13])]
    c_late += [cp(src.at[pl.ds(CH, M - CH)], dst.at[pl.ds(CH, M - CH)], sem.at[14 + n])
               for n, (src, dst) in enumerate(a_pairs)]
    c_x.start()
    for c in c_wq(0):
        c.start()

    n_i = jax.lax.broadcasted_iota(jnp.int32, (P, P), 0)
    k_i = jax.lax.broadcasted_iota(jnp.int32, (P, P), 1)
    ang = (((2 * k_i + 1) * n_i) & 511).astype(f32) * (math.pi / 256.0)
    cs, sn = jnp.cos(ang), jnp.sin(ang)
    ff_s[:, 0:P] = cs.astype(bf16)
    ff_s[:, P:2 * P] = (-sn).astype(bf16)
    fi_s[0:P, :] = (cs.T * (1.0 / P)).astype(bf16)
    fi_s[P:2 * P, :] = (sn.T * (-1.0 / P)).astype(bf16)
    sk = sk_ref[...].astype(f32)
    for t in range(KS):
        taps[t] = jnp.broadcast_to(sk[t:t + 1, :], (128, M)).T
    taps[KS] = jnp.broadcast_to(dd_ref[...].astype(f32).reshape(1, M), (128, M)).T
    acc[...] = jnp.zeros(acc.shape, f32)
    fullT[...] = jnp.zeros(fullT.shape, bf16)
    O_s[NT - 1][...] = jnp.zeros(O_s[0].shape, bf16)
    W7p_s[...] = jnp.zeros(W7p_s.shape, u32)

    c_x.wait()
    for c in c_wq(1):
        c.start()
    for t in range(NT):
        for r0 in range(0, 224, 32):
            blk = [_u(xT[r:r + 32, c:c + 128]) for r in (r0, 224 + r0) for c in (t * T, t * T + 128)]
            for n, x in enumerate(_combos_u(_b7, blk)):
                bx_s[t * 112 + r0 // 2:t * 112 + r0 // 2 + 16, n * 128:(n + 1) * 128] = x
    vq = wq_raw.bitcast(u32)
    for p, (c0, nc) in enumerate(QP):
        for c in c_wq(p):
            c.wait()
        if p == 1:
            for c in c_wk(0):
                c.start()
        for hp in range(H // 2):
            u = [vq[g, pl.ds((half * 224 + c0) * 8 + hp, nc, stride=8), :] for g in range(2) for half in range(2)]
            for par, f in enumerate((_lo, _hi)):
                r0 = (2 * hp + par) * 64
                for n, x in enumerate(_a7(*[f(x) for x in u])):
                    aq_s[r0:r0 + 64, n * 256 + c0:n * 256 + c0 + nc] = _u(x.astype(bf16).T)
    for c in c_wv(0) + [c_ckv(0)]:
        c.start()

    qscale = (D ** -0.5) * math.log2(math.e)

    def lo(u):
        return pltpu.bitcast(u << 16, f32)

    def hi(u):
        return pltpu.bitcast(u & jnp.uint32(0xFFFF0000), f32)

    def b_combos(b11, b12, b21, b22):
        return [b11 + b22, b11, b12 - b22, b21 - b11, b22, b11 + b12, b21 + b22]

    def q_body(j, carry):
        mq = {}

        def qproj(u, tok):
            hh, t, n = u // 14, (u // 7) % 2, SORD[u % 7]
            w = _b(_gate_u(aq_s[hh * 64:hh * 64 + 64, n * 256:n * 256 + 224], tok))
            xr = pl.ds(pl.multiple_of((2 * j + t) * 112, 16), 112)
            mq[n] = _nn(w, _b(bx_s[xr, n * 128:(n + 1) * 128]))
            if u % 7 == 6:
                for k, x in enumerate(_c4(mq)):
                    cols = pl.ds(pl.multiple_of((2 * j + t) * T + (k % 2) * 128, 128), 128)
                    r0 = hh * 128 + (k // 2) * 64
                    QT_s[r0:r0 + 64, cols] = _u((x * qscale).astype(bf16))
            return mq[n]

        def prep_k(hp, part):
            v = wk_raw.bitcast(u32).at[j % 2]
            u = [v[q, pl.ds(part * 128 + hp, 16, stride=8), :] for q in range(4)]
            for par, f in enumerate((_lo, _hi)):
                for n, c in enumerate(_b7(*[f(x) for x in u])):
                    r = _u(c.astype(bf16))
                    r0 = (2 * hp + par) * 256 + part * 8
                    bk_s[pl.ds(pl.multiple_of(j * 64 + r0, 8), 8), n * 128:(n + 1) * 128] = r
            return []

        def prep_v(hp, par):
            v = wv_raw.bitcast(u32).at[j % 2]
            f = (lo, hi)[par]
            parts = []
            for part in range(8):
                u = [v[q, pl.ds(part * 128 + hp, 16, stride=8), :] for q in range(4)]
                parts.append(b_combos(*[f(x) for x in u]))
            res = []
            for n in range(7):
                c = jnp.concatenate([p[n] for p in parts], axis=0)
                r = _u(c.astype(bf16).T)
                bvT_s[2 * hp + par, n, :, pl.ds(pl.multiple_of(j * 128, 128), 128)] = r
                res.append(r[56:])
            return res

        def prep_a(cl_, part, cbs):
            c = 2 * j + cl_
            r0 = 8 * part
            rt = pl.ds(pl.multiple_of(c * T + 2 * r0, 16), 16)
            rb = pl.ds(pl.multiple_of(c * T + 128 + 2 * r0, 16), 16)
            res = []
            for cb in cbs:
                cl, ch_ = slice(cb * 128, cb * 128 + 128), slice(512 + cb * 128, 512 + cb * 128 + 128)
                blk = [_u(ckv[rt, cl]), _u(ckv[rt, ch_]), _u(ckv[rb, cl]), _u(ckv[rb, ch_])]
                cc = []
                for f in (lo, hi):
                    a11, a12, a21, a22 = [f(x) for x in blk]
                    cc.append([a11 + a22, a21 + a22, None, None, a11 + a12, a21 - a11, a12 - a22])
                for n in range(7):
                    if n == 2:
                        r = blk[0]
                    elif n == 3:
                        r = blk[3]
                    else:
                        r = pltpu.pack_elementwise([cc[0][n], cc[1][n]], packed_dtype=bf16)
                    a_s[c, n, r0:r0 + 8, cl] = r
                    res.append(r)
            return [] if APACE else res

        fill = {}

        def spread(pieces, u0, u1):
            for n, p in enumerate(pieces):
                fill.setdefault(u0 + n * (u1 - u0) // len(pieces), []).append(p)

        spread([functools.partial(prep_k, hp, part) for hp in range(8) for part in range(8)], QW1, QW2)
        spread([functools.partial(prep_v, hp, par) for hp in range(8) for par in range(2)], QW2, QW3)
        spread([functools.partial(prep_a, c, part, cbs) for c in range(2) for part in range(8)
                for cbs in ((0, 1), (2, 3))], QW3, 220)
        toks = {}
        for u in range(224):
            if u == QW1:
                @pl.when(j < 3)
                def _():
                    for c in c_wk(j + 1):
                        c.start()

                @pl.when(j == 3)
                def _():
                    for c in c_early:
                        c.start()

                for c in c_wk(j):
                    c.wait()
            if u == QW2:
                @pl.when(j < 3)
                def _():
                    for c in c_wv(j + 1) + [c_ckv(j + 1)]:
                        c.start()

                @pl.when(j == 3)
                def _():
                    for c in c_late:
                        c.start()

                for c in c_wv(j) + [c_ckv(j)]:
                    c.wait()
            q = qproj(u, toks.pop(u, None))
            res = []
            ps = fill.get(u, [])
            for n, p in enumerate(ps):
                row = (n * 128 // len(ps)) // 16 * 16
                if p.func is prep_k:
                    wk_raw.bitcast(u32)[j >> 4, 0, 1024:1032, :] = pltpu.bitcast(q[row:row + 8], u32)
                elif p.func is prep_a:
                    ckv[pl.ds(pl.multiple_of(S + (j >> 4) * 16, 16), 16), 0:128] = q[row:row + 16].astype(bf16)
                res += p()
            if res:
                toks[u + QLAG] = _tok(res)
        return carry

    jax.lax.fori_loop(0, 4, q_body, 0)
    for c in c_early:
        c.wait()

    tri = n_i <= k_i
    sgn = jnp.where((jax.lax.broadcasted_iota(jnp.int32, (1, P), 1) & 1) == 0, 1.0, -1.0).astype(f32)

    c_outa = cp(out_s.at[:, pl.ds(0, 384)], out_hbm.at[:, pl.ds(0, 384)], sem_o.at[8])

    HR, HI, PR, PI, KV = range(5)

    def zrow(z, n):
        return pl.ds(0, n) if isinstance(z, int) else pl.ds(pl.multiple_of(z * n, n), n)

    def blk_at(c, half=None):
        r0 = (c % 8) * CH
        rs = slice(r0, r0 + CH) if half is None else slice(r0 + 16 * half, r0 + 16 * half + 16)
        return rs, slice((c // 8) * P, (c // 8 + 1) * P)

    def out_proj(i, hw, w7, zl):
        if OS:
            m = {n: _nn(_b(w7[0, n]), O_s[i][zl, n]) for n in SORD}
            o = _quad(*_c4(m))
        else:
            o = _nn(woT[hw], _quad(*[O_s[i][zl, n] for n in range(4)]))
        acc[:, T * i:T * (i + 1)] += o
        return o

    def head_body(h, carry):
        @pl.when(h == 1)
        def _():
            for c in c_late:
                c.wait()

        @pl.when(h == H - 1)
        def _():
            c_outa.start()

        st = dict(M={}, P={}, Q7={}, mfin={}, o={})
        zs, zl = h >> 10, 0
        m_s, l_s = (m0_s, m1_s), (l0_s, l1_s)
        qrows = pl.ds(pl.multiple_of(h * 128, 128), 128)
        rows = pl.ds(pl.multiple_of(jnp.minimum(h, NCH - 1) * CH, CH), CH)

        def rep(t, n):
            return jnp.concatenate([taps[t, rows, :]] * n, axis=1)

        toks = []

        def due():
            for t in toks:
                t[0] -= 1
            ready = [t[1] for t in toks if t[0] <= 0]
            toks[:] = [t for t in toks if t[0] > 0]
            return functools.reduce(lambda x, y: x | y, ready) if ready else None

        def gate_later(vals):
            toks.append([SLAG, _tok([v if v.dtype == u32 else pltpu.bitcast(v, u32) for v in vals])])

        for op in _schedule():
            kind = op[0]
            if kind == 'KP':
                _, c, t = op
                n = SORD[t]
                st['M'][n] = st['last'] = _nn(_b(_gate_u(a_s[c, n], due())), _b(bk_s[pl.ds(pl.multiple_of(h * 256, 256), 256), n * 128:(n + 1) * 128]))
                if t == 6:
                    c4 = _c4(st['M'])
                    blks = dict(zip((2, 7, 8, 3), c4))
                    if QKS and c < NT - 1:
                        blks.update({n: x for n, x in enumerate(_a7(*c4)) if n not in (2, 3)})
                    for n, x in blks.items():
                        K_s[c][zrow(zs, 64), n * 128:(n + 1) * 128] = _u(x.astype(bf16))
            elif kind == 'VP':
                _, c, t = op
                n = SORD[t]
                st['M'][n] = st['last'] = _nt(_b(_gate_u(bvT_s[h, n], due())), _b(a_s[c, n]))
                if t == 6:
                    c11, c12, c21, c22 = _c4(st['M'])
                    V_s[c][zrow(zs, 128), :T] = _u(_quad(c11, c21, c12, c22).astype(bf16))
            elif kind == 'QK':
                _, i, j = op
                S_s = (S0_s, S1_s)[i % 2]
                qu = QT_s[qrows, i * T:(i + 1) * T]
                if j < i:
                    if QKS:
                        if i not in st['Q7']:
                            st['Q7'][i] = _combos_u(_b7, [qu[:64, :128], qu[:64, 128:], qu[64:, :128], qu[64:, 128:]])
                        m = {n: _nn(_b(K_s[j][zrow(zl, 64), n * 128:(n + 1) * 128]), _b(st['Q7'][i][n])) for n in SORD}
                        s = _quad(*_c4(m))
                    else:
                        s = _nn(_b(_quad(*[K_s[j][zrow(zl, 64), n * 128:(n + 1) * 128] for n in (2, 7, 8, 3)])), _b(qu))
                    S_s[zs, j] = s
                    f = _fold(s, jnp.max)
                else:
                    q = _b(qu)
                    sa = _nn(_b(jnp.concatenate([K_s[j][zrow(zl, 64), 2 * 128:(2 + 1) * 128], K_s[j][zrow(zl, 64), 7 * 128:(7 + 1) * 128]], axis=1)), q)
                    sa = jnp.concatenate([jnp.where(tri, sa[:, :128], NEG), sa[:, 128:]], axis=1)
                    sb = _nn(_b(jnp.concatenate([K_s[j][zrow(zl, 64), 8 * 128:(8 + 1) * 128], K_s[j][zrow(zl, 64), 3 * 128:(3 + 1) * 128]], axis=1)), q[:, 128:])
                    sb = jnp.where(tri, sb, NEG)
                    S_s[zs, j, 0:128, :] = sa
                    S_s[zs, j, 128:T, 128:T] = sb
                    fa = _fold(sa, jnp.max)
                    f = jnp.concatenate([fa[:, :128], jnp.maximum(fa[:, 128:], _fold(sb, jnp.max))], axis=1)
                m_s[i % 2][zs, j] = f
                pace_s[zs] = f
            elif kind == 'EX':
                _, i, j = op
                S_s = (S0_s, S1_s)[i % 2]
                if j == 0:
                    m = m_s[i % 2][zl, 0]
                    for t in range(1, i + 1):
                        m = jnp.maximum(m, m_s[i % 2][zl, t])
                    st['mfin'][i] = jnp.max(m, axis=0, keepdims=True)
                m = st['mfin'][i]
                if j > 0:
                    m = jnp.where(pace_s[zl, 0:1, :] == jnp.inf, jnp.inf, m)
                if j < i:
                    p = jnp.exp2(S_s[zl, j] - m)
                    lj = _rsum(p)
                    st['P'][i, j] = p.astype(bf16)
                else:
                    pa = jnp.exp2(S_s[zl, j, 0:128, :] - m)
                    pb = jnp.exp2(S_s[zl, j, 128:T, 128:T] - m[:, 128:])
                    la = _rsum(pa)
                    lj = jnp.concatenate([la[:, :128], la[:, 128:] + _rsum(pb)], axis=1)
                    st['P'][i, j] = (pa.astype(bf16), pb.astype(bf16))
                l_s[i % 2][zs, j] = lj
            elif kind == 'PV':
                _, i, j = op
                vu = V_s[j][zrow(zl, 128), :T]
                p = st['P'].pop((i, j))
                if j < i:
                    o = _nn(_b(vu), p)
                else:
                    oa = _nn(_b(vu[:, :128]), p[0])
                    ob = _nn(_b(vu[:, 128:]), p[1])
                    o = jnp.concatenate([oa[:, :128], oa[:, 128:] + ob], axis=1)
                st['last'] = o
                o = o if j == 0 else st['o'][i] + o
                st['o'][i] = o
                if j == i:
                    l = l_s[i % 2][zl, 0]
                    for t in range(1, i + 1):
                        l = l + l_s[i % 2][zl, t]
                    o = o * (1.0 / jnp.sum(l, axis=0, keepdims=True))
                    blks = (o[:128, :128], o[:128, 128:], o[128:, :128], o[128:, 128:])
                    for n, x in enumerate(_b7(*blks) if OS else blks):
                        O_s[i][zs, n] = x.astype(bf16)
            elif kind == 'PACE':
                pace_s[zs] = jnp.concatenate([st['last'][-8:, -128:]] * 2, axis=1)
            elif kind == 'OP':
                i = op[1]
                st['last'] = out_proj(i, jnp.maximum(h - 1, 0) if i == NT - 1 else h,
                                      W7p_s if i == NT - 1 else W7_s, zl)
            elif kind == 'W7':
                res = []
                for r0 in range(112 * op[1], 112 * op[1] + 112, 16):
                    blk = [_u(woT[h, r:r + 16, c:c + 128]) for r in (r0, 224 + r0) for c in (0, 128)]
                    w7 = _combos_u(_a7, blk)
                    for n, x in enumerate(w7):
                        W7_s[zs, n, r0 // 2:r0 // 2 + 8] = x
                    res += [w7[0], w7[4], w7[5], w7[6], w7[1]]
                gate_later(res)
            elif kind == 'WC':
                x = W7_s[0]
                W7p_s[zs] = x
                gate_later([x[n] for n in range(7)])
            elif kind == 'AT':
                g = jnp.clip((h - 4) // 4, 0, 2)
                t0 = jnp.minimum(((h + 12) % 4) * 6, NB - 6)
                grow = pl.ds(pl.multiple_of(g * 128, 128), 128)
                gcol = pl.ds(pl.multiple_of(jnp.where(h == H - 1, 3, g) * 128, 128), 128)
                res = []
                for n in range(6):
                    tok = pl.ds(pl.multiple_of((t0 + n) * 128, 128), 128)
                    x = fullT[grow, tok].T
                    out_s[tok, gcol] = x
                    res.append(_u(x)[56:])
                gate_later(res)
            elif kind == 'HD':
                g = op[1]
                hs = jnp.concatenate([ssmk[rows, c * P:(c + 1) * P] for c in range(4 * g, 4 * g + 4)], axis=0)
                hf = _nn(hs, ff_s[...])
                for n in range(4):
                    X_s[(zs, HR) + blk_at(4 * g + n)] = hf[n * CH:(n + 1) * CH, :P]
                    X_s[(zs, HI) + blk_at(4 * g + n)] = hf[n * CH:(n + 1) * CH, P:]
            elif kind == 'SC':
                g = op[1]
                if g == 0:
                    k = jnp.concatenate([jnp.zeros((CH, P), f32), kT[rows, 0:4 * P].astype(f32)], axis=1)
                else:
                    k = kT[rows, (4 * g - 1) * P:(4 * g + 4) * P].astype(f32)
                ks = k[:, P:] * rep(0, 4)
                for j in range(1, KS):
                    ks = ks + pltpu.roll(k, j, 1)[:, P:] * rep(j, 4)
                kv = ks * vT[rows, 4 * g * P:(4 * g + 4) * P].astype(f32)
                kvs = jnp.concatenate([kv[:, n * P:(n + 1) * P] for n in range(4)], axis=0)
                xf = _nn(kvs.astype(bf16), ff_s[...])
                for n in range(4):
                    c = 4 * g + n
                    xr, xi = xf[n * CH:(n + 1) * CH, :P], xf[n * CH:(n + 1) * CH, P:]
                    X_s[(zs, KV) + blk_at(c)] = kvs[n * CH:(n + 1) * CH]
                    X_s[(zs, PR) + blk_at(c)] = xr if c == 0 else xr - sgn * st['x'][1]
                    X_s[(zs, PI) + blk_at(c)] = xi if c == 0 else xi + sgn * st['x'][0]
                    st['x'] = (xr, xi)
            elif kind == 'CV':
                res = []
                for a, half in op[1]:
                    wr = wi = None
                    for j in range(a + 1):
                        hr, hi_ = X_s[(zl, HR) + blk_at(j, half)], X_s[(zl, HI) + blk_at(j, half)]
                        pr, pi = X_s[(zl, PR) + blk_at(a - j, half)], X_s[(zl, PI) + blk_at(a - j, half)]
                        tr, ti = hr * pr - hi_ * pi, hr * pi + hi_ * pr
                        wr, wi = (tr, ti) if wr is None else (wr + tr, wi + ti)
                    r0 = (a % 4) * CH + 16 * half
                    Y_s[a // 4][zs, r0:r0 + 16, :P] = wr
                    Y_s[a // 4][zs, r0:r0 + 16, P:] = wi
                    res += [wr, wi]
                gate_later(res)
            elif kind == 'ID':
                g = op[1]
                w = Y_s[g][0]
                y = _nn(w.astype(bf16), fi_s[...])
                for n in range(4):
                    c = 4 * g + n
                    cols = slice(c * P, (c + 1) * P)
                    ya = y[n * CH:(n + 1) * CH, :] + X_s[(zl, KV) + blk_at(c)] * taps[KS, rows, :]
                    fullT[rows, cols] = (qT[rows, cols].astype(f32) * ya).astype(bf16)
        return carry

    jax.lax.fori_loop(0, H, head_body, 0)

    out_proj(NT - 1, H - 1, W7_s, 0)
    outs = [c_outa]
    for i in range(NT):
        cols = slice(T * i, T * (i + 1))
        blk = jnp.concatenate([fullT[384:M, cols], acc[:, cols].astype(bf16)], axis=0)
        out_s[cols, 384:2 * M] = blk.T
        c = cp(out_s.at[pl.ds(T * i, T), pl.ds(384, 512)], out_hbm.at[pl.ds(T * i, T), pl.ds(384, 512)], sem_o.at[i])
        c.start()
        outs.append(c)
    for c in outs:
        c.wait()


@jax.jit
def pallas_concat_heads__ssm_conv_h3__compressed_kv_cla__prompt_kernel(
    A_q: jax.Array,
    A_k: jax.Array,
    A_v: jax.Array,
    A_shift_k: jax.Array,
    A_ssm_k: jax.Array,
    A_ssm_D: jax.Array,
    B_x: jax.Array,
    B_c_kv: jax.Array,
    B_w_q: jax.Array,
    B_w_uk: jax.Array,
    B_w_uv: jax.Array,
    B_w_o: jax.Array,
):
    hbm = pl.BlockSpec(memory_space=pl.ANY)
    vmem = pl.BlockSpec(memory_space=pltpu.VMEM)
    V = pltpu.VMEM
    out = pl.pallas_call(
        _kernel,
        out_shape=jax.ShapeDtypeStruct((S, 2 * M), bf16),
        in_specs=[hbm, hbm, hbm, vmem, hbm, vmem, hbm, hbm, hbm, hbm, hbm, hbm],
        out_specs=hbm,
        scratch_shapes=[
            V((M, S), bf16), V((M, S), bf16), V((M, S), bf16), V((M, S), bf16),
            V((M, S), bf16), V((S + 16, DC), bf16),
            V((2, M * H, 128), bf16), V((2, 4, 128 * H + 16, 128), bf16), V((2, 4, 128 * H + 16, 128), bf16),
            V((H, M, D), bf16),
            V((H * 64, 7 * 256), u32), V((NT * 112, 7 * 128), u32), V((H * 256, 7 * 128), u32), V((H, 7, 64, 512), u32),
            V((H * D // 2, S), u32), V((NT, 7, 64, 512), u32),
            V((M, S), f32), V((M, S), bf16), V((S, 2 * M), bf16),
            V((KS + 1, M, 128), f32), V((P, 2 * P), bf16), V((2 * P, P), bf16),
            V((1, NT, T, T), f32), V((1, NT, T, T), f32), V((1, 5, T, T), f32),
            V((1, 7, 112, 128), u32), V((1, 7, 112, 128), u32), V((1, 8, T), f32),
            V((1, NT, 8, T), f32), V((1, NT, 8, T), f32), V((1, NT, 8, T), f32), V((1, NT, 8, T), f32),
            pltpu.SemaphoreType.DMA((26,)), pltpu.SemaphoreType.DMA((8,)),
            pltpu.SemaphoreType.DMA((8,)), pltpu.SemaphoreType.DMA((9,)),
        ] + [V((64, 9 * 128), u32)] * NT + [V((128, T + 128), u32)] * NT + [V((1, 7, 128, 128), bf16)] * NT
        + [V((1, 4 * CH, 2 * P), f32)] * 4,
        compiler_params=pltpu.CompilerParams(vmem_limit_bytes=120 * 1024 * 1024,
                                             shape_invariant_numerics=False),
    )(
        A_q[0].T, A_k[0].T, A_v[0].T, A_shift_k.T, A_ssm_k, A_ssm_D,
        B_x[0].T, B_c_kv[0],
        B_w_q.reshape(M * H, D), B_w_uk.reshape(DC * H, D), B_w_uv.reshape(DC * H, D),
        jnp.transpose(B_w_o, (0, 2, 1)),
    )
    return out[None]
```

```python
import functools
import math

import jax
import jax.numpy as jnp
import jax.experimental.pallas as pl
import jax.experimental.pallas.tpu as pltpu

bf16 = jnp.bfloat16
f32 = jnp.float32
u32 = jnp.uint32

S = 2048
M = 448
DC = 1024
H = 16
D = 256
KS = 4
P = 128
NB = S // P
CH = 32
NCH = M // CH
T = 256
NT = S // T
NEG = -1e30
LAG_M = 0
LAG_S = 0
SORD = (6, 4, 3, 0, 1, 2, 5)
QW1 = 63
QW2 = 119
QW3 = 175
QLAG = 6
OS = 1
QKS = 1
CVMAX = 12
SIDE0 = 1
SIDEP = 3
LA = 2
SLAG = 2
APACE = 1
PROW = 0
PVS = 1
NOP = 3
L0 = 1
LEND = 4
LLAG = 2
ORDER = 'a'


def _nn(a, b):
    return jnp.dot(a, b, preferred_element_type=f32)


def _nt(a, b):
    return jax.lax.dot_general(a, b, (((1,), (1,)), ((), ())), preferred_element_type=f32)


def _b(u):
    return pltpu.bitcast(u, bf16)


def _u(x):
    return pltpu.bitcast(x, u32)


def _split_pair(u):
    lo = pltpu.bitcast(u << 16, f32).astype(bf16)
    hi = pltpu.bitcast(u & jnp.uint32(0xFFFF0000), f32).astype(bf16)
    return lo, hi


def _lo(u):
    return pltpu.bitcast(u << 16, f32)


def _hi(u):
    return pltpu.bitcast(u & jnp.uint32(0xFFFF0000), f32)


def _pk(e, o):
    return pltpu.pack_elementwise([e, o], packed_dtype=bf16)


def _a7(a11, a12, a21, a22):
    return [a11 + a22, a21 + a22, a11, a22, a11 + a12, a21 - a11, a12 - a22]


def _b7(b11, b12, b21, b22):
    return [b11 + b22, b11, b12 - b22, b21 - b11, b22, b11 + b12, b21 + b22]


def _c4(m):
    return m[0] + m[3] - m[4] + m[6], m[2] + m[4], m[1] + m[3], m[0] - m[1] + m[2] + m[5]


def _combos_u(f7, blk):
    e = f7(*[_lo(x) for x in blk])
    o = f7(*[_hi(x) for x in blk])
    plain = {2: 0, 3: 3} if f7 is _a7 else {1: 0, 4: 3}
    return [blk[plain[n]] if n in plain else _pk(e[n], o[n]) for n in range(7)]


def _quad(c11, c12, c21, c22):
    return jnp.concatenate([jnp.concatenate([c11, c12], axis=1), jnp.concatenate([c21, c22], axis=1)], axis=0)


def _fold(c, op):
    return op(c.reshape(-1, 8, c.shape[1]), axis=0)


def _rsum(p):
    cols = []
    for c in range(0, p.shape[1], 128):
        tot = None
        for k in range(0, p.shape[0], 128):
            acc = None
            for r in range(k + 112, k - 16, -16):
                t = p[r:r + 8, c:c + 128] + p[r + 8:r + 16, c:c + 128]
                acc = t if acc is None else acc + t
            tot = acc if tot is None else tot + acc
        cols.append(tot)
    return jnp.concatenate(cols, axis=1) if len(cols) > 1 else cols[0]


def _gate(x, vals):
    if not vals:
        return x
    w = max(v.shape[1] for v in vals)
    top = x[:8, :w]
    for v in vals:
        if v.shape[1] < w:
            v = jnp.concatenate([v] * (w // v.shape[1]), axis=1)
        top = jnp.where(v == jnp.inf, jnp.zeros_like(top), top)
    if w < x.shape[1]:
        top = jnp.concatenate([top, x[:8, w:]], axis=1)
    return jnp.concatenate([top, x[8:]], axis=0)


def _tok(vals):
    parts = []
    for v in vals:
        for r in range(0, v.shape[0], 8):
            for c in range(0, v.shape[1], 128):
                parts.append(v[r:r + 8, c:c + 128])
    while len(parts) > 1:
        parts = [parts[i] | parts[i + 1] if i + 1 < len(parts) else parts[i] for i in range(0, len(parts), 2)]
    return (parts[0] >> 31) >> 1


def _gate_u(x, tok):
    if tok is None:
        return x
    top = x[:8, :128] | tok
    if x.shape[1] > 128:
        top = jnp.concatenate([top, x[:8, 128:]], axis=1)
    return jnp.concatenate([top, x[8:]], axis=0)


def _ssm_pieces():
    ps = [('HD', 0), ('SC', 0), ('HD', 1), ('SC', 1), ('W7', 0), ('HD', 2), ('SC', 2), ('W7', 1), ('HD', 3), ('SC', 3)]
    if not OS:
        ps = [p for p in ps if p[0] != 'W7']
    cur, cost = [], 0
    for a in range(NB):
        for half in range(2):
            if cur and cost + a + 1 > CVMAX:
                ps.append(('CV', tuple(cur)))
                cur, cost = [], 0
            cur.append((a, half))
            cost += a + 1
        if a % 4 == 3:
            if cur:
                ps.append(('CV', tuple(cur)))
            cur, cost = [], 0
            ps.append(('ID', a // 4))
    return ps


def _schedule():
    side = _ssm_pieces()
    out = []
    cnt = [0]

    def block(units, att, ssm=True):
        k = 0
        for u in units:
            for t in range(7):
                out.append(u + (t,))
                out.extend(att.get(k, []))
                k += 1
                if ssm:
                    cnt[0] += 1
                    if side and cnt[0] >= SIDE0 and (cnt[0] - SIDE0) % SIDEP == 0:
                        out.append(side.pop(0))

    def softmax_head(i, n):
        att = {}
        if PVS:
            for j in range(2 * i + 2):
                att.setdefault(L0 + j * (n - LEND - L0) // (2 * i + 2), []).append(('L', i, j // 2, j % 2))
            att.setdefault(n - LEND + 1, []).append(('EX', i, 0))
        else:
            att.setdefault(n // 2 - 1, []).append(('EX', i, 0))
        if i > 0:
            att.setdefault(n - 1, []).extend([('PACE',), ('EX', i, 1)])
        return att

    block([('KP', 0)], {})
    block([('OP', NT - 1)], {6: [('AT',)]}, False)
    block([('VP', 0), ('KP', 1)], {13: [('QK', 0, 0)]})
    block([('VP', 1)], softmax_head(0, 7))
    for i in range(NT - 1):
        for j in range(i + 1):
            out.append(('QK', i + 1, j))
            if j + 2 <= i:
                out.append(('EX', i, j + 2))
            if j == i:
                out.append(('QK', i + 1, i + 1))
            out.append(('PV', i, j))
        if i + 2 < NT:
            block([('KP', i + 2), ('VP', i + 2)], softmax_head(i + 1, 14))
        else:
            block([('OP', n) for n in range(NOP)], softmax_head(i + 1, 7 * NOP), False)
            out.append(('PACE',))
    for j in range(NT):
        if j + 2 < NT:
            out.append(('EX', NT - 1, j + 2))
        out.append(('PV', NT - 1, j))
        if j + NOP < NT - 3:
            block([('OP', j + NOP)], {}, False)
        out.append(('PACE',))
    block([('OP', NT - 3), ('OP', NT - 2)], {}, False)
    assert not side
    return out


def _kernel(qT_hbm, kT_hbm, vT_hbm, sk_ref, ssmk_hbm, dd_ref, xT_hbm, ckv_hbm,
            wq_hbm, wk_hbm, wv_hbm, woT_hbm, out_hbm,
            qT, kT, vT, ssmk, xT, ckv, wq_raw, wk_raw, wv_raw, woT,
            aq_s, bx_s, bk_s, bvT_s, QT_s, a_s, acc, fullT, out_s, taps, ff_s, fi_s,
            S0_s, S1_s, X_s, W7_s, pace_s, m0_s, m1_s, l0_s, l1_s,
            sem, sem_k, sem_v, sem_o, *kvo):
    K_s, V_s, O_s, Y_s = kvo[:NT], kvo[NT:2 * NT], kvo[2 * NT:3 * NT], kvo[3 * NT:]
    def cp(src, dst, s):
        return pltpu.make_async_copy(src, dst, s)

    c_x = cp(xT_hbm, xT, sem.at[0])
    QP = ((0, 128), (128, 96))

    def c_wq(p):
        cs_ = []
        for half in range(2):
            r = pl.ds((half * 224 + QP[p][0]) * H, QP[p][1] * H)
            for g in range(2):
                cs_.append(cp(wq_hbm.at[r, pl.ds(128 * g, 128)], wq_raw.at[g, r], sem.at[18 + 4 * p + 2 * half + g]))
        return cs_


    def c_w(w_hbm, raw, sm, j, half, g):
        r = pl.ds(pl.multiple_of((half * 4 + j) * 2048, 2048), 2048)
        q = 2 * half + g
        return cp(w_hbm.at[r, pl.ds(128 * g, 128)], raw.at[j % 2, q, pl.ds(0, 2048)], sm.at[(j % 2) * 4 + q])

    def c_wk(j):
        return [c_w(wk_hbm, wk_raw, sem_k, j, half, g) for half in range(2) for g in range(2)]

    def c_wv(j):
        return [c_w(wv_hbm, wv_raw, sem_v, j, half, g) for half in range(2) for g in range(2)]

    def c_ckv(j):
        r = pl.ds(pl.multiple_of(j * 2 * T, 2 * T), 2 * T)
        return cp(ckv_hbm.at[r], ckv.at[r], sem.at[9 + j])

    a_pairs = ((kT_hbm, kT), (vT_hbm, vT), (ssmk_hbm, ssmk), (qT_hbm, qT))
    c_early = [cp(woT_hbm.at[pl.ds(0, 1)], woT.at[pl.ds(0, 1)], sem.at[4])]
    c_early += [cp(src.at[pl.ds(0, CH)], dst.at[pl.ds(0, CH)], sem.at[5 + n]) for n, (src, dst) in enumerate(a_pairs)]
    c_late = [cp(woT_hbm.at[pl.ds(1, H - 1)], woT.at[pl.ds(1, H - 1)], sem.at[13])]
    c_late += [cp(src.at[pl.ds(CH, M - CH)], dst.at[pl.ds(CH, M - CH)], sem.at[14 + n])
               for n, (src, dst) in enumerate(a_pairs)]
    c_x.start()
    for c in c_wq(0):
        c.start()

    n_i = jax.lax.broadcasted_iota(jnp.int32, (P, P), 0)
    k_i = jax.lax.broadcasted_iota(jnp.int32, (P, P), 1)
    ang = (((2 * k_i + 1) * n_i) & 511).astype(f32) * (math.pi / 256.0)
    cs, sn = jnp.cos(ang), jnp.sin(ang)
    ff_s[:, 0:P] = cs.astype(bf16)
    ff_s[:, P:2 * P] = (-sn).astype(bf16)
    fi_s[0:P, :] = (cs.T * (1.0 / P)).astype(bf16)
    fi_s[P:2 * P, :] = (sn.T * (-1.0 / P)).astype(bf16)
    sk = sk_ref[...].astype(f32)
    for t in range(KS):
        taps[t] = jnp.broadcast_to(sk[t:t + 1, :], (128, M)).T
    taps[KS] = jnp.broadcast_to(dd_ref[...].astype(f32).reshape(1, M), (128, M)).T
    acc[...] = jnp.zeros(acc.shape, f32)
    fullT[...] = jnp.zeros(fullT.shape, bf16)
    O_s[NT - 1][...] = jnp.zeros(O_s[0].shape, bf16)
    W7_s[...] = jnp.zeros(W7_s.shape, u32)

    c_x.wait()
    for c in c_wq(1):
        c.start()
    for t in range(0 if 0 else NT):
        for r0 in range(0, 224, 32):
            blk = [_u(xT[r:r + 32, c:c + 128]) for r in (r0, 224 + r0) for c in (t * T, t * T + 128)]
            for n, x in enumerate(_combos_u(_b7, blk)):
                bx_s[t * 112 + r0 // 2:t * 112 + r0 // 2 + 16, n * 128:(n + 1) * 128] = x
    vq = wq_raw.bitcast(u32)
    for p, (c0, nc) in enumerate(QP):
        for c in c_wq(p):
            c.wait()
        if p == 1:
            for c in c_wk(0):
                c.start()
        for hp in range(0 if 0 else H // 2):
            u = [vq[g, pl.ds((half * 224 + c0) * 8 + hp, nc, stride=8), :] for g in range(2) for half in range(2)]
            for par, f in enumerate((_lo, _hi)):
                r0 = (2 * hp + par) * 64
                for n, x in enumerate(_a7(*[f(x) for x in u])):
                    aq_s[r0:r0 + 64, n * 256 + c0:n * 256 + c0 + nc] = _u(x.astype(bf16).T)
    for c in c_wv(0) + [c_ckv(0)]:
        c.start()

    qscale = (D ** -0.5) * math.log2(math.e)

    def lo(u):
        return pltpu.bitcast(u << 16, f32)

    def hi(u):
        return pltpu.bitcast(u & jnp.uint32(0xFFFF0000), f32)

    def b_combos(b11, b12, b21, b22):
        return [b11 + b22, b11, b12 - b22, b21 - b11, b22, b11 + b12, b21 + b22]

    def q_body(j, carry):
        mq = {}

        def qproj(u, tok):
            hh, t, n = u // 14, (u // 7) % 2, SORD[u % 7]
            w = _b(_gate_u(aq_s[hh * 64:hh * 64 + 64, n * 256:n * 256 + 224], tok))
            xr = pl.ds(pl.multiple_of((2 * j + t) * 112, 16), 112)
            mq[n] = _nn(w, _b(bx_s[xr, n * 128:(n + 1) * 128]))
            if u % 7 == 6:
                for k, x in enumerate(_c4(mq)):
                    cols = pl.ds(pl.multiple_of((2 * j + t) * T + (k % 2) * 128, 128), 128)
                    r0 = hh * 128 + (k // 2) * 64
                    QT_s[r0:r0 + 64, cols] = _u((x * qscale).astype(bf16))
            return mq[n]

        def prep_k(hp, part):
            v = wk_raw.bitcast(u32).at[j % 2]
            u = [v[q, pl.ds(part * 128 + hp, 16, stride=8), :] for q in range(4)]
            for par, f in enumerate((_lo, _hi)):
                for n, c in enumerate(_b7(*[f(x) for x in u])):
                    r = _u(c.astype(bf16))
                    r0 = (2 * hp + par) * 256 + part * 8
                    bk_s[pl.ds(pl.multiple_of(j * 64 + r0, 8), 8), n * 128:(n + 1) * 128] = r
            return []

        def prep_v(hp, par):
            v = wv_raw.bitcast(u32).at[j % 2]
            f = (lo, hi)[par]
            parts = []
            for part in range(8):
                u = [v[q, pl.ds(part * 128 + hp, 16, stride=8), :] for q in range(4)]
                parts.append(b_combos(*[f(x) for x in u]))
            res = []
            for n in range(7):
                c = jnp.concatenate([p[n] for p in parts], axis=0)
                r = _u(c.astype(bf16).T)
                bvT_s[2 * hp + par, n, :, pl.ds(pl.multiple_of(j * 128, 128), 128)] = r
                res.append(r[56:])
            return res

        def prep_a(cl_, part, cbs):
            c = 2 * j + cl_
            r0 = 8 * part
            rt = pl.ds(pl.multiple_of(c * T + 2 * r0, 16), 16)
            rb = pl.ds(pl.multiple_of(c * T + 128 + 2 * r0, 16), 16)
            res = []
            for cb in cbs:
                cl, ch_ = slice(cb * 128, cb * 128 + 128), slice(512 + cb * 128, 512 + cb * 128 + 128)
                blk = [_u(ckv[rt, cl]), _u(ckv[rt, ch_]), _u(ckv[rb, cl]), _u(ckv[rb, ch_])]
                cc = []
                for f in (lo, hi):
                    a11, a12, a21, a22 = [f(x) for x in blk]
                    cc.append([a11 + a22, a21 + a22, None, None, a11 + a12, a21 - a11, a12 - a22])
                for n in range(7):
                    if n == 2:
                        r = blk[0]
                    elif n == 3:
                        r = blk[3]
                    else:
                        r = pltpu.pack_elementwise([cc[0][n], cc[1][n]], packed_dtype=bf16)
                    a_s[c, n, r0:r0 + 8, cl] = r
                    res.append(r)
            return [] if APACE else res

        fill = {}

        def spread(pieces, u0, u1):
            for n, p in enumerate(pieces):
                fill.setdefault(u0 + n * (u1 - u0) // len(pieces), []).append(p)

        spread([functools.partial(prep_k, hp, part) for hp in range(8) for part in range(8)], QW1, QW2)
        spread([functools.partial(prep_v, hp, par) for hp in range(8) for par in range(2)], QW2, QW3)
        spread([functools.partial(prep_a, c, part, cbs) for c in range(2) for part in range(8)
                for cbs in ((0, 1), (2, 3))], QW3, 220)
        toks = {}
        for u in range(224):
            if u == QW1:
                @pl.when(j < 3)
                def _():
                    for c in c_wk(j + 1):
                        c.start()

                @pl.when(j == 3)
                def _():
                    for c in c_early:
                        c.start()

                for c in c_wk(j):
                    c.wait()
            if u == QW2:
                @pl.when(j < 3)
                def _():
                    for c in c_wv(j + 1) + [c_ckv(j + 1)]:
                        c.start()

                @pl.when(j == 3)
                def _():
                    for c in c_late:
                        c.start()

                for c in c_wv(j) + [c_ckv(j)]:
                    c.wait()
            q = qproj(u, toks.pop(u, None))
            res = []
            ps = fill.get(u, [])
            for n, p in enumerate(ps):
                row = (n * 128 // len(ps)) // 16 * 16
                if p.func is prep_k:
                    wk_raw.bitcast(u32)[j >> 4, 0, 1024:1032, :] = pltpu.bitcast(q[row:row + 8], u32)
                elif p.func is prep_a:
                    ckv[pl.ds(pl.multiple_of(S + (j >> 4) * 16, 16), 16), 0:128] = q[row:row + 16].astype(bf16)
                res += p()
            if res:
                toks[u + QLAG] = _tok(res)
        return carry

    if not 0:
        jax.lax.fori_loop(0, 4, q_body, 0)
    for c in c_early:
        c.wait()

    tri = n_i <= k_i
    sgn = jnp.where((jax.lax.broadcasted_iota(jnp.int32, (1, P), 1) & 1) == 0, 1.0, -1.0).astype(f32)

    c_outa = cp(out_s.at[:, pl.ds(0, 384)], out_hbm.at[:, pl.ds(0, 384)], sem_o.at[8])

    HR, HI, PR, PI, KV = range(5)

    def zrow(z, n):
        return pl.ds(0, n) if isinstance(z, int) else pl.ds(pl.multiple_of(z * n, n), n)

    def blk_at(c, half=None):
        r0 = (c % 8) * CH
        rs = slice(r0, r0 + CH) if half is None else slice(r0 + 16 * half, r0 + 16 * half + 16)
        return rs, slice((c // 8) * P, (c // 8 + 1) * P)

    def head_body(h, carry):
        @pl.when(h == 1)
        def _():
            for c in c_late:
                c.wait()

        @pl.when(h == H - 1)
        def _():
            c_outa.start()

        st = dict(l={}, M={}, P={}, Q7={}, mfin={}, o={})
        zs, zl = h >> 10, 0
        m_s, l_s = (m0_s, m1_s), (l0_s, l1_s)
        qrows = pl.ds(pl.multiple_of(h * 128, 128), 128)
        rows = pl.ds(pl.multiple_of(jnp.minimum(h, NCH - 1) * CH, CH), CH)

        def rep(t, n):
            return jnp.concatenate([taps[t, rows, :]] * n, axis=1)

        toks = []

        def due():
            for t in toks:
                t[0] -= 1
            ready = [t[1] for t in toks if t[0] <= 0]
            toks[:] = [t for t in toks if t[0] > 0]
            return functools.reduce(lambda x, y: x | y, ready) if ready else None

        def gate_later(vals, lag=SLAG):
            toks.append([lag, _tok([v if v.dtype == u32 else pltpu.bitcast(v, u32) for v in vals])])

        def row_max(i):
            if i not in st['mfin']:
                m = m_s[i % 2][zl, 0]
                for t in range(1, i + 1):
                    m = jnp.maximum(m, m_s[i % 2][zl, t])
                st['mfin'][i] = jnp.max(m, axis=0, keepdims=True)
            return st['mfin'][i]

        for op in _schedule():
            kind = op[0]
            if kind == 'KP':
                _, c, t = op
                n = SORD[t]
                st['M'][n] = st['last'] = _nn(_b(_gate_u(a_s[c, n], due())), _b(bk_s[pl.ds(pl.multiple_of(h * 256, 256), 256), n * 128:(n + 1) * 128]))
                if t == 6:
                    c4 = _c4(st['M'])
                    blks = dict(zip((2, 7, 8, 3), c4))
                    if QKS and c < NT - 1:
                        blks.update({n: x for n, x in enumerate(_a7(*c4)) if n not in (2, 3)})
                    for n, x in blks.items():
                        K_s[c][zrow(zs, 64), n * 128:(n + 1) * 128] = _u(x.astype(bf16))
            elif kind == 'VP':
                _, c, t = op
                n = SORD[t]
                st['M'][n] = st['last'] = _nt(_b(_gate_u(bvT_s[h, n], due())), _b(a_s[c, n]))
                if t == 6:
                    c11, c12, c21, c22 = _c4(st['M'])
                    c4 = (c11, c21, c12, c22)
                    blks = dict(zip((2, 7, 8, 3), c4))
                    if PVS and c < NT - 1:
                        blks.update({n: x for n, x in enumerate(_a7(*c4)) if n not in (2, 3)})
                    for n, x in blks.items():
                        V_s[c][zrow(zs, 64), n * 128:(n + 1) * 128] = _u(x.astype(bf16))
            elif kind == 'QK':
                _, i, j = op
                S_s = (S0_s, S1_s)[i % 2]
                qu = QT_s[qrows, i * T:(i + 1) * T]
                if j < i:
                    if QKS:
                        if i not in st['Q7']:
                            st['Q7'][i] = _combos_u(_b7, [qu[:64, :128], qu[:64, 128:], qu[64:, :128], qu[64:, 128:]])
                        m = {n: _nn(_b(K_s[j][zrow(zl, 64), n * 128:(n + 1) * 128]), _b(st['Q7'][i][n])) for n in SORD}
                        s = _quad(*_c4(m))
                    else:
                        s = _nn(_b(_quad(*[K_s[j][zrow(zl, 64), n * 128:(n + 1) * 128] for n in (2, 7, 8, 3)])), _b(qu))
                    S_s[zs, j] = s
                    f = _fold(s, jnp.max)
                else:
                    q = _b(qu)
                    sa = _nn(_b(jnp.concatenate([K_s[j][zrow(zl, 64), 2 * 128:(2 + 1) * 128], K_s[j][zrow(zl, 64), 7 * 128:(7 + 1) * 128]], axis=1)), q)
                    sa = jnp.concatenate([jnp.where(tri, sa[:, :128], NEG), sa[:, 128:]], axis=1)
                    sb = _nn(_b(jnp.concatenate([K_s[j][zrow(zl, 64), 8 * 128:(8 + 1) * 128], K_s[j][zrow(zl, 64), 3 * 128:(3 + 1) * 128]], axis=1)), q[:, 128:])
                    sb = jnp.where(tri, sb, NEG)
                    S_s[zs, j, 0:128, :] = sa
                    S_s[zs, j, 128:T, 128:T] = sb
                    fa = _fold(sa, jnp.max)
                    f = jnp.concatenate([fa[:, :128], jnp.maximum(fa[:, 128:], _fold(sb, jnp.max))], axis=1)
                m_s[i % 2][zs, j] = f
                pace_s[zs] = f
            elif kind == 'L':
                _, i, j, hf = op
                S_s = (S0_s, S1_s)[i % 2]
                m = row_max(i)
                l = st['l'].get(i)
                if j < i or hf == 0:
                    for r in range(128 * hf, 128 * hf + 128, 16):
                        p = jnp.exp2(S_s[zl, j, r:r + 16, :] - m)
                        p = p[:8] + p[8:]
                        l = p if l is None else l + p
                    gate_later([l], LLAG)
                else:
                    lb = l[:, 128:]
                    for r in range(128, T, 16):
                        p = jnp.exp2(S_s[zl, j, r:r + 16, 128:T] - m[:, 128:])
                        lb = lb + (p[:8] + p[8:])
                    l = jnp.concatenate([l[:, :128], lb], axis=1)
                    st['mfin'][i] = m + jnp.log2(jnp.sum(l, axis=0, keepdims=True))
                st['l'][i] = l
            elif kind == 'EX':
                _, i, j = op
                S_s = (S0_s, S1_s)[i % 2]
                m = row_max(i)
                if j > 0:
                    m = jnp.where(pace_s[zl, 0:1, :] == jnp.inf, jnp.inf, m)
                if j < i:
                    p = jnp.exp2(S_s[zl, j] - m)
                    if PVS:
                        p7 = _b7(p[:128, :128], p[:128, 128:], p[128:, :128], p[128:, 128:])
                        st['P'][i, j] = [x.astype(bf16) for x in p7]
                    else:
                        lj = _rsum(p)
                        st['P'][i, j] = p.astype(bf16)
                else:
                    pa = jnp.exp2(S_s[zl, j, 0:128, :] - m)
                    pb = jnp.exp2(S_s[zl, j, 128:T, 128:T] - m[:, 128:])
                    if not PVS:
                        la = _rsum(pa)
                        lj = jnp.concatenate([la[:, :128], la[:, 128:] + _rsum(pb)], axis=1)
                    st['P'][i, j] = (pa.astype(bf16), pb.astype(bf16))
                if not PVS:
                    l_s[i % 2][zs, j] = lj
            elif kind == 'PV':
                _, i, j = op
                vb = [V_s[j][zrow(zl, 64), n * 128:(n + 1) * 128] for n in range(9)]
                p = st['P'].pop((i, j))
                if j < i and PVS:
                    for n in SORD:
                        st['last'] = _nn(_b(vb[n]), p[n])
                        st['o'][i, n] = st['last'] if j == 0 else st['o'][i, n] + st['last']
                    continue
                if j < i:
                    o = _nn(_b(_quad(vb[2], vb[7], vb[8], vb[3])), p)
                else:
                    oa = _nn(_b(jnp.concatenate([vb[2], vb[8]], axis=0)), p[0])
                    ob = _nn(_b(jnp.concatenate([vb[7], vb[3]], axis=0)), p[1])
                    o = jnp.concatenate([oa[:, :128], oa[:, 128:] + ob], axis=1)
                st['last'] = o
                if PVS:
                    if i > 0:
                        o = o + _quad(*_c4({n: st['o'].pop((i, n)) for n in range(7)}))
                else:
                    o = o if j == 0 else st['o'][i] + o
                    st['o'][i] = o
                if j == i:
                    if not PVS:
                        l = l_s[i % 2][zl, 0]
                        for t in range(1, i + 1):
                            l = l + l_s[i % 2][zl, t]
                        o = o * (1.0 / jnp.sum(l, axis=0, keepdims=True))
                    blks = (o[:128, :128], o[:128, 128:], o[128:, :128], o[128:, 128:])
                    for n, x in enumerate(_b7(*blks)):
                        O_s[i][zs, n] = x.astype(bf16)
            elif kind == 'PACE':
                pace_s[zs] = jnp.concatenate([st['last'][-8:, -128:]] * 2, axis=1)
            elif kind == 'OP':
                _, i, t = op
                n = SORD[t]
                st['M'][n] = st['last'] = _nn(_b(_gate_u(W7_s[0, n], due())), O_s[i][0, n])
                if t == 6:
                    acc[:, T * i:T * (i + 1)] += _quad(*_c4(st['M']))
            elif kind == 'W7':
                res = []
                for r0 in range(112 * op[1], 112 * op[1] + 112, 16):
                    blk = [_u(woT[h, r:r + 16, c:c + 128]) for r in (r0, 224 + r0) for c in (0, 128)]
                    w7 = _combos_u(_a7, blk)
                    for n, x in enumerate(w7):
                        W7_s[zs, n, r0 // 2:r0 // 2 + 8] = x
                    res += w7
                gate_later(res)
            elif kind == 'AT':
                g = jnp.clip((h - 4) // 4, 0, 2)
                t0 = jnp.minimum(((h + 12) % 4) * 6, NB - 6)
                grow = pl.ds(pl.multiple_of(g * 128, 128), 128)
                gcol = pl.ds(pl.multiple_of(jnp.where(h == H - 1, 3, g) * 128, 128), 128)
                res = []
                for n in range(6):
                    tok = pl.ds(pl.multiple_of((t0 + n) * 128, 128), 128)
                    x = fullT[grow, tok].T
                    out_s[tok, gcol] = x
                    res.append(_u(x)[56:])
                gate_later(res)
            elif kind == 'HD':
                g = op[1]
                hs = jnp.concatenate([ssmk[rows, c * P:(c + 1) * P] for c in range(4 * g, 4 * g + 4)], axis=0)
                hf = _nn(hs, ff_s[...])
                for n in range(4):
                    X_s[(zs, HR) + blk_at(4 * g + n)] = hf[n * CH:(n + 1) * CH, :P]
                    X_s[(zs, HI) + blk_at(4 * g + n)] = hf[n * CH:(n + 1) * CH, P:]
            elif kind == 'SC':
                g = op[1]
                if g == 0:
                    k = jnp.concatenate([jnp.zeros((CH, P), f32), kT[rows, 0:4 * P].astype(f32)], axis=1)
                else:
                    k = kT[rows, (4 * g - 1) * P:(4 * g + 4) * P].astype(f32)
                ks = k[:, P:] * rep(0, 4)
                for j in range(1, KS):
                    ks = ks + pltpu.roll(k, j, 1)[:, P:] * rep(j, 4)
                kv = ks * vT[rows, 4 * g * P:(4 * g + 4) * P].astype(f32)
                kvs = jnp.concatenate([kv[:, n * P:(n + 1) * P] for n in range(4)], axis=0)
                xf = _nn(kvs.astype(bf16), ff_s[...])
                for n in range(4):
                    c = 4 * g + n
                    xr, xi = xf[n * CH:(n + 1) * CH, :P], xf[n * CH:(n + 1) * CH, P:]
                    X_s[(zs, KV) + blk_at(c)] = kvs[n * CH:(n + 1) * CH]
                    X_s[(zs, PR) + blk_at(c)] = xr if c == 0 else xr - sgn * st['x'][1]
                    X_s[(zs, PI) + blk_at(c)] = xi if c == 0 else xi + sgn * st['x'][0]
                    st['x'] = (xr, xi)
            elif kind == 'CV':
                res = []
                for a, half in op[1]:
                    wr = wi = None
                    for j in range(a + 1):
                        hr, hi_ = X_s[(zl, HR) + blk_at(j, half)], X_s[(zl, HI) + blk_at(j, half)]
                        pr, pi = X_s[(zl, PR) + blk_at(a - j, half)], X_s[(zl, PI) + blk_at(a - j, half)]
                        tr, ti = hr * pr - hi_ * pi, hr * pi + hi_ * pr
                        wr, wi = (tr, ti) if wr is None else (wr + tr, wi + ti)
                    r0 = (a % 4) * CH + 16 * half
                    Y_s[a // 4][zs, r0:r0 + 16, :P] = wr
                    Y_s[a // 4][zs, r0:r0 + 16, P:] = wi
                    res += [wr, wi]
                gate_later(res)
            elif kind == 'ID':
                g = op[1]
                w = Y_s[g][0]
                y = _nn(w.astype(bf16), fi_s[...])
                for n in range(4):
                    c = 4 * g + n
                    cols = slice(c * P, (c + 1) * P)
                    ya = y[n * CH:(n + 1) * CH, :] + X_s[(zl, KV) + blk_at(c)] * taps[KS, rows, :]
                    fullT[rows, cols] = (qT[rows, cols].astype(f32) * ya).astype(bf16)
        return carry

    if not 0:
        jax.lax.fori_loop(0, H, head_body, 0)

    acc[:, T * (NT - 1):] += _quad(*_c4({n: _nn(_b(W7_s[0, n]), O_s[NT - 1][0, n]) for n in SORD}))
    outs = [c_outa]
    for i in range(NT):
        cols = slice(T * i, T * (i + 1))
        blk = jnp.concatenate([fullT[384:M, cols], acc[:, cols].astype(bf16)], axis=0)
        out_s[cols, 384:2 * M] = blk.T
        c = cp(out_s.at[pl.ds(T * i, T), pl.ds(384, 512)], out_hbm.at[pl.ds(T * i, T), pl.ds(384, 512)], sem_o.at[i])
        c.start()
        outs.append(c)
    for c in outs:
        c.wait()


@jax.jit
def pallas_concat_heads__ssm_conv_h3__compressed_kv_cla__prompt_kernel(
    A_q: jax.Array,
    A_k: jax.Array,
    A_v: jax.Array,
    A_shift_k: jax.Array,
    A_ssm_k: jax.Array,
    A_ssm_D: jax.Array,
    B_x: jax.Array,
    B_c_kv: jax.Array,
    B_w_q: jax.Array,
    B_w_uk: jax.Array,
    B_w_uv: jax.Array,
    B_w_o: jax.Array,
):
    hbm = pl.BlockSpec(memory_space=pl.ANY)
    vmem = pl.BlockSpec(memory_space=pltpu.VMEM)
    V = pltpu.VMEM
    out = pl.pallas_call(
        _kernel,
        out_shape=jax.ShapeDtypeStruct((S, 2 * M), bf16),
        in_specs=[hbm, hbm, hbm, vmem, hbm, vmem, hbm, hbm, hbm, hbm, hbm, hbm],
        out_specs=hbm,
        scratch_shapes=[
            V((M, S), bf16), V((M, S), bf16), V((M, S), bf16), V((M, S), bf16),
            V((M, S), bf16), V((S + 16, DC), bf16),
            V((2, M * H, 128), bf16), V((2, 4, 128 * H + 16, 128), bf16), V((2, 4, 128 * H + 16, 128), bf16),
            V((H, M, D), bf16),
            V((H * 64, 7 * 256), u32), V((NT * 112, 7 * 128), u32), V((H * 256, 7 * 128), u32), V((H, 7, 64, 512), u32),
            V((H * D // 2, S), u32), V((NT, 7, 64, 512), u32),
            V((M, S), f32), V((M, S), bf16), V((S, 2 * M), bf16),
            V((KS + 1, M, 128), f32), V((P, 2 * P), bf16), V((2 * P, P), bf16),
            V((1, NT, T, T), f32), V((1, NT, T, T), f32), V((1, 5, T, T), f32),
            V((1, 7, 112, 128), u32), V((1, 8, T), f32),
            V((1, NT, 8, T), f32), V((1, NT, 8, T), f32), V((1, NT, 8, T), f32), V((1, NT, 8, T), f32),
            pltpu.SemaphoreType.DMA((26,)), pltpu.SemaphoreType.DMA((8,)),
            pltpu.SemaphoreType.DMA((8,)), pltpu.SemaphoreType.DMA((9,)),
        ] + [V((64, 9 * 128), u32)] * NT + [V((64, 9 * 128), u32)] * NT + [V((1, 7, 128, 128), bf16)] * NT
        + [V((1, 4 * CH, 2 * P), f32)] * 4,
        compiler_params=pltpu.CompilerParams(vmem_limit_bytes=120 * 1024 * 1024,
                                             shape_invariant_numerics=False),
    )(
        A_q[0].T, A_k[0].T, A_v[0].T, A_shift_k.T, A_ssm_k, A_ssm_D,
        B_x[0].T, B_c_kv[0],
        B_w_q.reshape(M * H, D), B_w_uk.reshape(DC * H, D), B_w_uv.reshape(DC * H, D),
        jnp.transpose(B_w_o, (0, 2, 1)),
    )
    return out[None]
```

```python
import functools
import math

import jax
import jax.numpy as jnp
import jax.experimental.pallas as pl
import jax.experimental.pallas.tpu as pltpu

bf16 = jnp.bfloat16
f32 = jnp.float32
u32 = jnp.uint32

S = 2048
M = 448
DC = 1024
H = 16
D = 256
KS = 4
P = 128
NB = S // P
CH = 32
NCH = M // CH
T = 256
NT = S // T
NEG = -1e30
LAG_M = 0
LAG_S = 0
SORD = (6, 4, 3, 0, 1, 2, 5)
QW1 = 63
QW2 = 119
QW3 = 175
QLAG = 6
OS = 1
QKS = 1
CVMAX = 12
SIDE0 = 1
SIDEP = 3
LA = 2
SLAG = 2
APACE = 1
PROW = 0
PVS = 1
NOP = 3
L0 = 1
LEND = 4
LLAG = 2
EXR = 16
EX0 = 11
P0 = 1
ORDER = 'a'


def _nn(a, b):
    return jnp.dot(a, b, preferred_element_type=f32)


def _nt(a, b):
    return jax.lax.dot_general(a, b, (((1,), (1,)), ((), ())), preferred_element_type=f32)


def _b(u):
    return pltpu.bitcast(u, bf16)


def _u(x):
    return pltpu.bitcast(x, u32)


def _split_pair(u):
    lo = pltpu.bitcast(u << 16, f32).astype(bf16)
    hi = pltpu.bitcast(u & jnp.uint32(0xFFFF0000), f32).astype(bf16)
    return lo, hi


def _lo(u):
    return pltpu.bitcast(u << 16, f32)


def _hi(u):
    return pltpu.bitcast(u & jnp.uint32(0xFFFF0000), f32)


def _pk(e, o):
    return pltpu.pack_elementwise([e, o], packed_dtype=bf16)


def _a7(a11, a12, a21, a22):
    return [a11 + a22, a21 + a22, a11, a22, a11 + a12, a21 - a11, a12 - a22]


def _b7(b11, b12, b21, b22):
    return [b11 + b22, b11, b12 - b22, b21 - b11, b22, b11 + b12, b21 + b22]


def _c4(m):
    return m[0] + m[3] - m[4] + m[6], m[2] + m[4], m[1] + m[3], m[0] - m[1] + m[2] + m[5]


def _combos_u(f7, blk):
    e = f7(*[_lo(x) for x in blk])
    o = f7(*[_hi(x) for x in blk])
    plain = {2: 0, 3: 3} if f7 is _a7 else {1: 0, 4: 3}
    return [blk[plain[n]] if n in plain else _pk(e[n], o[n]) for n in range(7)]


def _quad(c11, c12, c21, c22):
    return jnp.concatenate([jnp.concatenate([c11, c12], axis=1), jnp.concatenate([c21, c22], axis=1)], axis=0)


def _fold(c, op):
    return op(c.reshape(-1, 8, c.shape[1]), axis=0)


def _rsum(p):
    cols = []
    for c in range(0, p.shape[1], 128):
        tot = None
        for k in range(0, p.shape[0], 128):
            acc = None
            for r in range(k + 112, k - 16, -16):
                t = p[r:r + 8, c:c + 128] + p[r + 8:r + 16, c:c + 128]
                acc = t if acc is None else acc + t
            tot = acc if tot is None else tot + acc
        cols.append(tot)
    return jnp.concatenate(cols, axis=1) if len(cols) > 1 else cols[0]


def _gate(x, vals):
    if not vals:
        return x
    w = max(v.shape[1] for v in vals)
    top = x[:8, :w]
    for v in vals:
        if v.shape[1] < w:
            v = jnp.concatenate([v] * (w // v.shape[1]), axis=1)
        top = jnp.where(v == jnp.inf, jnp.zeros_like(top), top)
    if w < x.shape[1]:
        top = jnp.concatenate([top, x[:8, w:]], axis=1)
    return jnp.concatenate([top, x[8:]], axis=0)


def _tok(vals):
    parts = []
    for v in vals:
        for r in range(0, v.shape[0], 8):
            for c in range(0, v.shape[1], 128):
                parts.append(v[r:r + 8, c:c + 128])
    while len(parts) > 1:
        parts = [parts[i] | parts[i + 1] if i + 1 < len(parts) else parts[i] for i in range(0, len(parts), 2)]
    return (parts[0] >> 31) >> 1


def _gate_u(x, tok):
    if tok is None:
        return x
    top = x[:8, :128] | tok
    if x.shape[1] > 128:
        top = jnp.concatenate([top, x[:8, 128:]], axis=1)
    return jnp.concatenate([top, x[8:]], axis=0)


def _ssm_pieces():
    ps = [('HD', 0), ('SC', 0), ('HD', 1), ('SC', 1), ('W7', 0), ('HD', 2), ('SC', 2), ('W7', 1), ('HD', 3), ('SC', 3)]
    if not OS:
        ps = [p for p in ps if p[0] != 'W7']
    cur, cost = [], 0
    for a in range(NB):
        for half in range(2):
            if cur and cost + a + 1 > CVMAX:
                ps.append(('CV', tuple(cur)))
                cur, cost = [], 0
            cur.append((a, half))
            cost += a + 1
        if a % 4 == 3:
            if cur:
                ps.append(('CV', tuple(cur)))
            cur, cost = [], 0
            ps.append(('ID', a // 4))
    return ps


def _schedule():
    side = _ssm_pieces()
    out = []
    cnt = [0]

    def block(units, att, ssm=True):
        k = 0
        for u in units:
            for t in range(7):
                out.append(u + (t,))
                out.extend(att.get(k, []))
                k += 1
                if ssm:
                    cnt[0] += 1
                    if side and cnt[0] >= SIDE0 and (cnt[0] - SIDE0) % SIDEP == 0:
                        out.append(side.pop(0))

    def softmax_head(i, n):
        att = {}
        att.setdefault(min(EX0, n - 2), []).extend(([('PACE',)] if P0 else []) + [('EX', i, 0)])
        if i > 0:
            att.setdefault(n - 1, []).extend([('PACE',), ('EX', i, 1)])
        return att

    block([('KP', 0)], {})
    block([('OP', NT - 1)], {6: [('AT',)]}, False)
    block([('VP', 0), ('KP', 1)], {13: [('QK', 0, 0)]})
    block([('VP', 1)], softmax_head(0, 7))
    for i in range(NT - 1):
        for j in range(i + 1):
            out.append(('QK', i + 1, j))
            if j + 2 <= i:
                out.append(('EX', i, j + 2))
            if j == i:
                out.append(('QK', i + 1, i + 1))
            out.append(('PV', i, j))
        if i + 2 < NT:
            block([('KP', i + 2), ('VP', i + 2)], softmax_head(i + 1, 14))
        else:
            block([('OP', n) for n in range(NOP)], softmax_head(i + 1, 7 * NOP), False)
            out.append(('PACE',))
    for j in range(NT):
        if j + 2 < NT:
            out.append(('EX', NT - 1, j + 2))
        out.append(('PV', NT - 1, j))
        if j + NOP < NT - 3:
            block([('OP', j + NOP)], {}, False)
        out.append(('PACE',))
    block([('OP', NT - 3), ('OP', NT - 2)], {}, False)
    assert not side
    return out


def _kernel(qT_hbm, kT_hbm, vT_hbm, sk_ref, ssmk_hbm, dd_ref, xT_hbm, ckv_hbm,
            wq_hbm, wk_hbm, wv_hbm, woT_hbm, out_hbm,
            qT, kT, vT, ssmk, xT, ckv, wq_raw, wk_raw, wv_raw, woT,
            aq_s, bx_s, bk_s, bvT_s, QT_s, a_s, acc, fullT, out_s, taps, ff_s, fi_s,
            S0_s, S1_s, X_s, W7_s, pace_s, m0_s, m1_s, l0_s, l1_s,
            sem, sem_k, sem_v, sem_o, *kvo):
    K_s, V_s, O_s, Y_s = kvo[:NT], kvo[NT:2 * NT], kvo[2 * NT:3 * NT], kvo[3 * NT:]
    def cp(src, dst, s):
        return pltpu.make_async_copy(src, dst, s)

    c_x = cp(xT_hbm, xT, sem.at[0])
    QP = ((0, 128), (128, 96))

    def c_wq(p):
        cs_ = []
        for half in range(2):
            r = pl.ds((half * 224 + QP[p][0]) * H, QP[p][1] * H)
            for g in range(2):
                cs_.append(cp(wq_hbm.at[r, pl.ds(128 * g, 128)], wq_raw.at[g, r], sem.at[18 + 4 * p + 2 * half + g]))
        return cs_


    def c_w(w_hbm, raw, sm, j, half, g):
        r = pl.ds(pl.multiple_of((half * 4 + j) * 2048, 2048), 2048)
        q = 2 * half + g
        return cp(w_hbm.at[r, pl.ds(128 * g, 128)], raw.at[j % 2, q, pl.ds(0, 2048)], sm.at[(j % 2) * 4 + q])

    def c_wk(j):
        return [c_w(wk_hbm, wk_raw, sem_k, j, half, g) for half in range(2) for g in range(2)]

    def c_wv(j):
        return [c_w(wv_hbm, wv_raw, sem_v, j, half, g) for half in range(2) for g in range(2)]

    def c_ckv(j):
        r = pl.ds(pl.multiple_of(j * 2 * T, 2 * T), 2 * T)
        return cp(ckv_hbm.at[r], ckv.at[r], sem.at[9 + j])

    a_pairs = ((kT_hbm, kT), (vT_hbm, vT), (ssmk_hbm, ssmk), (qT_hbm, qT))
    c_early = [cp(woT_hbm.at[pl.ds(0, 1)], woT.at[pl.ds(0, 1)], sem.at[4])]
    c_early += [cp(src.at[pl.ds(0, CH)], dst.at[pl.ds(0, CH)], sem.at[5 + n]) for n, (src, dst) in enumerate(a_pairs)]
    c_late = [cp(woT_hbm.at[pl.ds(1, H - 1)], woT.at[pl.ds(1, H - 1)], sem.at[13])]
    c_late += [cp(src.at[pl.ds(CH, M - CH)], dst.at[pl.ds(CH, M - CH)], sem.at[14 + n])
               for n, (src, dst) in enumerate(a_pairs)]
    c_x.start()
    for c in c_wq(0):
        c.start()

    n_i = jax.lax.broadcasted_iota(jnp.int32, (P, P), 0)
    k_i = jax.lax.broadcasted_iota(jnp.int32, (P, P), 1)
    ang = (((2 * k_i + 1) * n_i) & 511).astype(f32) * (math.pi / 256.0)
    cs, sn = jnp.cos(ang), jnp.sin(ang)
    ff_s[:, 0:P] = cs.astype(bf16)
    ff_s[:, P:2 * P] = (-sn).astype(bf16)
    fi_s[0:P, :] = (cs.T * (1.0 / P)).astype(bf16)
    fi_s[P:2 * P, :] = (sn.T * (-1.0 / P)).astype(bf16)
    sk = sk_ref[...].astype(f32)
    for t in range(KS):
        taps[t] = jnp.broadcast_to(sk[t:t + 1, :], (128, M)).T
    taps[KS] = jnp.broadcast_to(dd_ref[...].astype(f32).reshape(1, M), (128, M)).T
    acc[...] = jnp.zeros(acc.shape, f32)
    fullT[...] = jnp.zeros(fullT.shape, bf16)
    O_s[NT - 1][...] = jnp.zeros(O_s[0].shape, bf16)
    W7_s[...] = jnp.zeros(W7_s.shape, u32)

    c_x.wait()
    for c in c_wq(1):
        c.start()
    for t in range(0 if 0 else NT):
        for r0 in range(0, 224, 32):
            blk = [_u(xT[r:r + 32, c:c + 128]) for r in (r0, 224 + r0) for c in (t * T, t * T + 128)]
            for n, x in enumerate(_combos_u(_b7, blk)):
                bx_s[t * 112 + r0 // 2:t * 112 + r0 // 2 + 16, n * 128:(n + 1) * 128] = x
    vq = wq_raw.bitcast(u32)
    for p, (c0, nc) in enumerate(QP):
        for c in c_wq(p):
            c.wait()
        if p == 1:
            for c in c_wk(0):
                c.start()
        for hp in range(0 if 0 else H // 2):
            u = [vq[g, pl.ds((half * 224 + c0) * 8 + hp, nc, stride=8), :] for g in range(2) for half in range(2)]
            for par, f in enumerate((_lo, _hi)):
                r0 = (2 * hp + par) * 64
                for n, x in enumerate(_a7(*[f(x) for x in u])):
                    aq_s[r0:r0 + 64, n * 256 + c0:n * 256 + c0 + nc] = _u(x.astype(bf16).T)
    for c in c_wv(0) + [c_ckv(0)]:
        c.start()

    qscale = (D ** -0.5) * math.log2(math.e)

    def lo(u):
        return pltpu.bitcast(u << 16, f32)

    def hi(u):
        return pltpu.bitcast(u & jnp.uint32(0xFFFF0000), f32)

    def b_combos(b11, b12, b21, b22):
        return [b11 + b22, b11, b12 - b22, b21 - b11, b22, b11 + b12, b21 + b22]

    def q_body(j, carry):
        mq = {}

        def qproj(u, tok):
            hh, t, n = u // 14, (u // 7) % 2, SORD[u % 7]
            w = _b(_gate_u(aq_s[hh * 64:hh * 64 + 64, n * 256:n * 256 + 224], tok))
            xr = pl.ds(pl.multiple_of((2 * j + t) * 112, 16), 112)
            mq[n] = _nn(w, _b(bx_s[xr, n * 128:(n + 1) * 128]))
            if u % 7 == 6:
                for k, x in enumerate(_c4(mq)):
                    cols = pl.ds(pl.multiple_of((2 * j + t) * T + (k % 2) * 128, 128), 128)
                    r0 = hh * 128 + (k // 2) * 64
                    QT_s[r0:r0 + 64, cols] = _u((x * qscale).astype(bf16))
            return mq[n]

        def prep_k(hp, part):
            v = wk_raw.bitcast(u32).at[j % 2]
            u = [v[q, pl.ds(part * 128 + hp, 16, stride=8), :] for q in range(4)]
            for par, f in enumerate((_lo, _hi)):
                for n, c in enumerate(_b7(*[f(x) for x in u])):
                    r = _u(c.astype(bf16))
                    r0 = (2 * hp + par) * 256 + part * 8
                    bk_s[pl.ds(pl.multiple_of(j * 64 + r0, 8), 8), n * 128:(n + 1) * 128] = r
            return []

        def prep_v(hp, par):
            v = wv_raw.bitcast(u32).at[j % 2]
            f = (lo, hi)[par]
            parts = []
            for part in range(8):
                u = [v[q, pl.ds(part * 128 + hp, 16, stride=8), :] for q in range(4)]
                parts.append(b_combos(*[f(x) for x in u]))
            res = []
            for n in range(7):
                c = jnp.concatenate([p[n] for p in parts], axis=0)
                r = _u(c.astype(bf16).T)
                bvT_s[2 * hp + par, n, :, pl.ds(pl.multiple_of(j * 128, 128), 128)] = r
                res.append(r[56:])
            return res

        def prep_a(cl_, part, cbs):
            c = 2 * j + cl_
            r0 = 8 * part
            rt = pl.ds(pl.multiple_of(c * T + 2 * r0, 16), 16)
            rb = pl.ds(pl.multiple_of(c * T + 128 + 2 * r0, 16), 16)
            res = []
            for cb in cbs:
                cl, ch_ = slice(cb * 128, cb * 128 + 128), slice(512 + cb * 128, 512 + cb * 128 + 128)
                blk = [_u(ckv[rt, cl]), _u(ckv[rt, ch_]), _u(ckv[rb, cl]), _u(ckv[rb, ch_])]
                cc = []
                for f in (lo, hi):
                    a11, a12, a21, a22 = [f(x) for x in blk]
                    cc.append([a11 + a22, a21 + a22, None, None, a11 + a12, a21 - a11, a12 - a22])
                for n in range(7):
                    if n == 2:
                        r = blk[0]
                    elif n == 3:
                        r = blk[3]
                    else:
                        r = pltpu.pack_elementwise([cc[0][n], cc[1][n]], packed_dtype=bf16)
                    a_s[c, n, r0:r0 + 8, cl] = r
                    res.append(r)
            return [] if APACE else res

        fill = {}

        def spread(pieces, u0, u1):
            for n, p in enumerate(pieces):
                fill.setdefault(u0 + n * (u1 - u0) // len(pieces), []).append(p)

        spread([functools.partial(prep_k, hp, part) for hp in range(8) for part in range(8)], QW1, QW2)
        spread([functools.partial(prep_v, hp, par) for hp in range(8) for par in range(2)], QW2, QW3)
        spread([functools.partial(prep_a, c, part, cbs) for c in range(2) for part in range(8)
                for cbs in ((0, 1), (2, 3))], QW3, 220)
        toks = {}
        for u in range(224):
            if u == QW1:
                @pl.when(j < 3)
                def _():
                    for c in c_wk(j + 1):
                        c.start()

                @pl.when(j == 3)
                def _():
                    for c in c_early:
                        c.start()

                for c in c_wk(j):
                    c.wait()
            if u == QW2:
                @pl.when(j < 3)
                def _():
                    for c in c_wv(j + 1) + [c_ckv(j + 1)]:
                        c.start()

                @pl.when(j == 3)
                def _():
                    for c in c_late:
                        c.start()

                for c in c_wv(j) + [c_ckv(j)]:
                    c.wait()
            q = qproj(u, toks.pop(u, None))
            res = []
            ps = fill.get(u, [])
            for n, p in enumerate(ps):
                row = (n * 128 // len(ps)) // 16 * 16
                if p.func is prep_k:
                    wk_raw.bitcast(u32)[j >> 4, 0, 1024:1032, :] = pltpu.bitcast(q[row:row + 8], u32)
                elif p.func is prep_a:
                    ckv[pl.ds(pl.multiple_of(S + (j >> 4) * 16, 16), 16), 0:128] = q[row:row + 16].astype(bf16)
                res += p()
            if res:
                toks[u + QLAG] = _tok(res)
        return carry

    if not 0:
        jax.lax.fori_loop(0, 4, q_body, 0)
    for c in c_early:
        c.wait()

    tri = n_i <= k_i
    sgn = jnp.where((jax.lax.broadcasted_iota(jnp.int32, (1, P), 1) & 1) == 0, 1.0, -1.0).astype(f32)

    c_outa = cp(out_s.at[:, pl.ds(0, 384)], out_hbm.at[:, pl.ds(0, 384)], sem_o.at[8])

    HR, HI, PR, PI, KV = range(5)

    def zrow(z, n):
        return pl.ds(0, n) if isinstance(z, int) else pl.ds(pl.multiple_of(z * n, n), n)

    def blk_at(c, half=None):
        r0 = (c % 8) * CH
        rs = slice(r0, r0 + CH) if half is None else slice(r0 + 16 * half, r0 + 16 * half + 16)
        return rs, slice((c // 8) * P, (c // 8 + 1) * P)

    def head_body(h, carry):
        @pl.when(h == 1)
        def _():
            for c in c_late:
                c.wait()

        @pl.when(h == H - 1)
        def _():
            c_outa.start()

        st = dict(l={}, M={}, P={}, Q7={}, mfin={}, o={})
        zs, zl = h >> 10, 0
        m_s, l_s = (m0_s, m1_s), (l0_s, l1_s)
        qrows = pl.ds(pl.multiple_of(h * 128, 128), 128)
        rows = pl.ds(pl.multiple_of(jnp.minimum(h, NCH - 1) * CH, CH), CH)

        def rep(t, n):
            return jnp.concatenate([taps[t, rows, :]] * n, axis=1)

        toks = []

        def due():
            for t in toks:
                t[0] -= 1
            ready = [t[1] for t in toks if t[0] <= 0]
            toks[:] = [t for t in toks if t[0] > 0]
            return functools.reduce(lambda x, y: x | y, ready) if ready else None

        def gate_later(vals, lag=SLAG):
            toks.append([lag, _tok([v if v.dtype == u32 else pltpu.bitcast(v, u32) for v in vals])])

        def row_max(i):
            if i not in st['mfin']:
                m = m_s[i % 2][zl, 0]
                for t in range(1, i + 1):
                    m = jnp.maximum(m, m_s[i % 2][zl, t])
                m = jnp.max(m, axis=0, keepdims=True)
                if PVS and i > 0:
                    lo_ = jnp.exp2(m_s[i % 2][zl, 0] - m)
                    for t in range(1, i + 1):
                        lo_ = lo_ + jnp.exp2(m_s[i % 2][zl, t] - m)
                    m = m + jnp.log2(jnp.sum(lo_, axis=0, keepdims=True))
                st['mfin'][i] = m
            return st['mfin'][i]

        for op in _schedule():
            kind = op[0]
            if kind == 'KP':
                _, c, t = op
                n = SORD[t]
                st['M'][n] = st['last'] = _nn(_b(_gate_u(a_s[c, n], due())), _b(bk_s[pl.ds(pl.multiple_of(h * 256, 256), 256), n * 128:(n + 1) * 128]))
                if t == 6:
                    c4 = _c4(st['M'])
                    blks = dict(zip((2, 7, 8, 3), c4))
                    if QKS and c < NT - 1:
                        blks.update({n: x for n, x in enumerate(_a7(*c4)) if n not in (2, 3)})
                    for n, x in blks.items():
                        K_s[c][zrow(zs, 64), n * 128:(n + 1) * 128] = _u(x.astype(bf16))
            elif kind == 'VP':
                _, c, t = op
                n = SORD[t]
                st['M'][n] = st['last'] = _nt(_b(_gate_u(bvT_s[h, n], due())), _b(a_s[c, n]))
                if t == 6:
                    c11, c12, c21, c22 = _c4(st['M'])
                    c4 = (c11, c21, c12, c22)
                    blks = dict(zip((2, 7, 8, 3), c4))
                    if PVS and c < NT - 1:
                        blks.update({n: x for n, x in enumerate(_a7(*c4)) if n not in (2, 3)})
                    for n, x in blks.items():
                        V_s[c][zrow(zs, 64), n * 128:(n + 1) * 128] = _u(x.astype(bf16))
            elif kind == 'QK':
                _, i, j = op
                S_s = (S0_s, S1_s)[i % 2]
                qu = QT_s[qrows, i * T:(i + 1) * T]
                if j < i:
                    if QKS:
                        if i not in st['Q7']:
                            st['Q7'][i] = _combos_u(_b7, [qu[:64, :128], qu[:64, 128:], qu[64:, :128], qu[64:, 128:]])
                        m = {n: _nn(_b(K_s[j][zrow(zl, 64), n * 128:(n + 1) * 128]), _b(st['Q7'][i][n])) for n in SORD}
                        s = _quad(*_c4(m))
                    else:
                        s = _nn(_b(_quad(*[K_s[j][zrow(zl, 64), n * 128:(n + 1) * 128] for n in (2, 7, 8, 3)])), _b(qu))
                    S_s[zs, j] = s
                    f = _fold(s, jnp.max)
                else:
                    q = _b(qu)
                    sa = _nn(_b(jnp.concatenate([K_s[j][zrow(zl, 64), 2 * 128:(2 + 1) * 128], K_s[j][zrow(zl, 64), 7 * 128:(7 + 1) * 128]], axis=1)), q)
                    sa = jnp.concatenate([jnp.where(tri, sa[:, :128], NEG), sa[:, 128:]], axis=1)
                    sb = _nn(_b(jnp.concatenate([K_s[j][zrow(zl, 64), 8 * 128:(8 + 1) * 128], K_s[j][zrow(zl, 64), 3 * 128:(3 + 1) * 128]], axis=1)), q[:, 128:])
                    sb = jnp.where(tri, sb, NEG)
                    S_s[zs, j, 0:128, :] = sa
                    S_s[zs, j, 128:T, 128:T] = sb
                    fa = _fold(sa, jnp.max)
                    f = jnp.concatenate([fa[:, :128], jnp.maximum(fa[:, 128:], _fold(sb, jnp.max))], axis=1)
                m_s[i % 2][zs, j] = f
                pace_s[zs] = f
            elif kind == 'EX':
                _, i, j = op
                S_s = (S0_s, S1_s)[i % 2]
                m = row_max(i)
                if j > 0 or P0:
                    m = jnp.where(pace_s[zl, 0:1, :] == jnp.inf, jnp.inf, m)
                if j < i:
                    if PVS:
                        parts, lj = [], None
                        for r in range(112, -16, -16):
                            pt = jnp.exp2(S_s[zl, j, r:r + 16, :] - m)
                            pb = jnp.exp2(S_s[zl, j, 128 + r:128 + r + 16, :] - m)
                            parts.insert(0, _b7(pt[:, :128], pt[:, 128:], pb[:, :128], pb[:, 128:]))
                            x = (pt[:8] + pt[8:]) + (pb[:8] + pb[8:])
                            lj = x if lj is None else lj + x
                        st['P'][i, j] = [jnp.concatenate([x[n] for x in parts], axis=0).astype(bf16) for n in range(7)]
                    else:
                        p = jnp.exp2(S_s[zl, j] - m)
                        lj = _rsum(p)
                        st['P'][i, j] = p.astype(bf16)
                else:
                    pa = jnp.exp2(S_s[zl, j, 0:128, :] - m)
                    pb = jnp.exp2(S_s[zl, j, 128:T, 128:T] - m[:, 128:])
                    la = _rsum(pa)
                    lj = jnp.concatenate([la[:, :128], la[:, 128:] + _rsum(pb)], axis=1)
                    st['P'][i, j] = (pa.astype(bf16), pb.astype(bf16))
                l_s[i % 2][zs, j] = lj
            elif kind == 'PV':
                _, i, j = op
                vb = [V_s[j][zrow(zl, 64), n * 128:(n + 1) * 128] for n in range(9)]
                p = st['P'].pop((i, j))
                if j < i and PVS:
                    for n in SORD:
                        st['last'] = _nn(_b(vb[n]), p[n])
                        st['o'][i, n] = st['last'] if j == 0 else st['o'][i, n] + st['last']
                    continue
                if j < i:
                    o = _nn(_b(_quad(vb[2], vb[7], vb[8], vb[3])), p)
                else:
                    oa = _nn(_b(jnp.concatenate([vb[2], vb[8]], axis=0)), p[0])
                    ob = _nn(_b(jnp.concatenate([vb[7], vb[3]], axis=0)), p[1])
                    o = jnp.concatenate([oa[:, :128], oa[:, 128:] + ob], axis=1)
                st['last'] = o
                if PVS:
                    if i > 0:
                        o = o + _quad(*_c4({n: st['o'].pop((i, n)) for n in range(7)}))
                else:
                    o = o if j == 0 else st['o'][i] + o
                    st['o'][i] = o
                if j == i:
                    l = l_s[i % 2][zl, 0]
                    for t in range(1, i + 1):
                        l = l + l_s[i % 2][zl, t]
                    o = o * (1.0 / jnp.sum(l, axis=0, keepdims=True))
                    blks = (o[:128, :128], o[:128, 128:], o[128:, :128], o[128:, 128:])
                    for n, x in enumerate(_b7(*blks)):
                        O_s[i][zs, n] = x.astype(bf16)
            elif kind == 'PACE':
                pace_s[zs] = jnp.concatenate([st['last'][-8:, -128:]] * 2, axis=1)
            elif kind == 'OP':
                _, i, t = op
                n = SORD[t]
                st['M'][n] = st['last'] = _nn(_b(_gate_u(W7_s[0, n], due())), O_s[i][0, n])
                if t == 6:
                    acc[:, T * i:T * (i + 1)] += _quad(*_c4(st['M']))
            elif kind == 'W7':
                res = []
                for r0 in range(112 * op[1], 112 * op[1] + 112, 16):
                    blk = [_u(woT[h, r:r + 16, c:c + 128]) for r in (r0, 224 + r0) for c in (0, 128)]
                    w7 = _combos_u(_a7, blk)
                    for n, x in enumerate(w7):
                        W7_s[zs, n, r0 // 2:r0 // 2 + 8] = x
                    res += w7
                gate_later(res)
            elif kind == 'AT':
                g = jnp.clip((h - 4) // 4, 0, 2)
                t0 = jnp.minimum(((h + 12) % 4) * 6, NB - 6)
                grow = pl.ds(pl.multiple_of(g * 128, 128), 128)
                gcol = pl.ds(pl.multiple_of(jnp.where(h == H - 1, 3, g) * 128, 128), 128)
                res = []
                for n in range(6):
                    tok = pl.ds(pl.multiple_of((t0 + n) * 128, 128), 128)
                    x = fullT[grow, tok].T
                    out_s[tok, gcol] = x
                    res.append(_u(x)[56:])
                gate_later(res)
            elif kind == 'HD':
                g = op[1]
                hs = jnp.concatenate([ssmk[rows, c * P:(c + 1) * P] for c in range(4 * g, 4 * g + 4)], axis=0)
                hf = _nn(hs, ff_s[...])
                for n in range(4):
                    X_s[(zs, HR) + blk_at(4 * g + n)] = hf[n * CH:(n + 1) * CH, :P]
                    X_s[(zs, HI) + blk_at(4 * g + n)] = hf[n * CH:(n + 1) * CH, P:]
            elif kind == 'SC':
                g = op[1]
                if g == 0:
                    k = jnp.concatenate([jnp.zeros((CH, P), f32), kT[rows, 0:4 * P].astype(f32)], axis=1)
                else:
                    k = kT[rows, (4 * g - 1) * P:(4 * g + 4) * P].astype(f32)
                ks = k[:, P:] * rep(0, 4)
                for j in range(1, KS):
                    ks = ks + pltpu.roll(k, j, 1)[:, P:] * rep(j, 4)
                kv = ks * vT[rows, 4 * g * P:(4 * g + 4) * P].astype(f32)
                kvs = jnp.concatenate([kv[:, n * P:(n + 1) * P] for n in range(4)], axis=0)
                xf = _nn(kvs.astype(bf16), ff_s[...])
                for n in range(4):
                    c = 4 * g + n
                    xr, xi = xf[n * CH:(n + 1) * CH, :P], xf[n * CH:(n + 1) * CH, P:]
                    X_s[(zs, KV) + blk_at(c)] = kvs[n * CH:(n + 1) * CH]
                    X_s[(zs, PR) + blk_at(c)] = xr if c == 0 else xr - sgn * st['x'][1]
                    X_s[(zs, PI) + blk_at(c)] = xi if c == 0 else xi + sgn * st['x'][0]
                    st['x'] = (xr, xi)
            elif kind == 'CV':
                res = []
                for a, half in op[1]:
                    wr = wi = None
                    for j in range(a + 1):
                        hr, hi_ = X_s[(zl, HR) + blk_at(j, half)], X_s[(zl, HI) + blk_at(j, half)]
                        pr, pi = X_s[(zl, PR) + blk_at(a - j, half)], X_s[(zl, PI) + blk_at(a - j, half)]
                        tr, ti = hr * pr - hi_ * pi, hr * pi + hi_ * pr
                        wr, wi = (tr, ti) if wr is None else (wr + tr, wi + ti)
                    r0 = (a % 4) * CH + 16 * half
                    Y_s[a // 4][zs, r0:r0 + 16, :P] = wr
                    Y_s[a // 4][zs, r0:r0 + 16, P:] = wi
                    res += [wr, wi]
                gate_later(res)
            elif kind == 'ID':
                g = op[1]
                w = Y_s[g][0]
                y = _nn(w.astype(bf16), fi_s[...])
                for n in range(4):
                    c = 4 * g + n
                    cols = slice(c * P, (c + 1) * P)
                    ya = y[n * CH:(n + 1) * CH, :] + X_s[(zl, KV) + blk_at(c)] * taps[KS, rows, :]
                    fullT[rows, cols] = (qT[rows, cols].astype(f32) * ya).astype(bf16)
        return carry

    if not 0:
        jax.lax.fori_loop(0, H, head_body, 0)

    acc[:, T * (NT - 1):] += _quad(*_c4({n: _nn(_b(W7_s[0, n]), O_s[NT - 1][0, n]) for n in SORD}))
    outs = [c_outa]
    for i in range(NT):
        cols = slice(T * i, T * (i + 1))
        blk = jnp.concatenate([fullT[384:M, cols], acc[:, cols].astype(bf16)], axis=0)
        out_s[cols, 384:2 * M] = blk.T
        c = cp(out_s.at[pl.ds(T * i, T), pl.ds(384, 512)], out_hbm.at[pl.ds(T * i, T), pl.ds(384, 512)], sem_o.at[i])
        c.start()
        outs.append(c)
    for c in outs:
        c.wait()


@jax.jit
def pallas_concat_heads__ssm_conv_h3__compressed_kv_cla__prompt_kernel(
    A_q: jax.Array,
    A_k: jax.Array,
    A_v: jax.Array,
    A_shift_k: jax.Array,
    A_ssm_k: jax.Array,
    A_ssm_D: jax.Array,
    B_x: jax.Array,
    B_c_kv: jax.Array,
    B_w_q: jax.Array,
    B_w_uk: jax.Array,
    B_w_uv: jax.Array,
    B_w_o: jax.Array,
):
    hbm = pl.BlockSpec(memory_space=pl.ANY)
    vmem = pl.BlockSpec(memory_space=pltpu.VMEM)
    V = pltpu.VMEM
    out = pl.pallas_call(
        _kernel,
        out_shape=jax.ShapeDtypeStruct((S, 2 * M), bf16),
        in_specs=[hbm, hbm, hbm, vmem, hbm, vmem, hbm, hbm, hbm, hbm, hbm, hbm],
        out_specs=hbm,
        scratch_shapes=[
            V((M, S), bf16), V((M, S), bf16), V((M, S), bf16), V((M, S), bf16),
            V((M, S), bf16), V((S + 16, DC), bf16),
            V((2, M * H, 128), bf16), V((2, 4, 128 * H + 16, 128), bf16), V((2, 4, 128 * H + 16, 128), bf16),
            V((H, M, D), bf16),
            V((H * 64, 7 * 256), u32), V((NT * 112, 7 * 128), u32), V((H * 256, 7 * 128), u32), V((H, 7, 64, 512), u32),
            V((H * D // 2, S), u32), V((NT, 7, 64, 512), u32),
            V((M, S), f32), V((M, S), bf16), V((S, 2 * M), bf16),
            V((KS + 1, M, 128), f32), V((P, 2 * P), bf16), V((2 * P, P), bf16),
            V((1, NT, T, T), f32), V((1, NT, T, T), f32), V((1, 5, T, T), f32),
            V((1, 7, 112, 128), u32), V((1, 8, T), f32),
            V((1, NT, 8, T), f32), V((1, NT, 8, T), f32), V((1, NT, 8, T), f32), V((1, NT, 8, T), f32),
            pltpu.SemaphoreType.DMA((26,)), pltpu.SemaphoreType.DMA((8,)),
            pltpu.SemaphoreType.DMA((8,)), pltpu.SemaphoreType.DMA((9,)),
        ] + [V((64, 9 * 128), u32)] * NT + [V((64, 9 * 128), u32)] * NT + [V((1, 7, 128, 128), bf16)] * NT
        + [V((1, 4 * CH, 2 * P), f32)] * 4,
        compiler_params=pltpu.CompilerParams(vmem_limit_bytes=120 * 1024 * 1024,
                                             shape_invariant_numerics=False),
    )(
        A_q[0].T, A_k[0].T, A_v[0].T, A_shift_k.T, A_ssm_k, A_ssm_D,
        B_x[0].T, B_c_kv[0],
        B_w_q.reshape(M * H, D), B_w_uk.reshape(DC * H, D), B_w_uv.reshape(DC * H, D),
        jnp.transpose(B_w_o, (0, 2, 1)),
    )
    return out[None]
```

```python
import functools
import math

import jax
import jax.numpy as jnp
import jax.experimental.pallas as pl
import jax.experimental.pallas.tpu as pltpu

bf16 = jnp.bfloat16
f32 = jnp.float32
u32 = jnp.uint32

S = 2048
M = 448
DC = 1024
H = 16
D = 256
KS = 4
P = 128
NB = S // P
CH = 32
NCH = M // CH
T = 256
NT = S // T
NEG = -1e30
LAG_M = 0
LAG_S = 0
SORD = (6, 4, 3, 0, 1, 2, 5)
QW1 = 63
QW2 = 119
QW3 = 175
QLAG = 6
OS = 1
QKS = 1
CVMAX = 12
SIDE0 = 1
SIDEP = 3
LA = 2
SLAG = 2
APACE = 1
PROW = 0
PVS = 1
NOP = 3
L0 = 1
LEND = 4
LLAG = 2
EXR = 16
EX0 = 11
P0 = 1
VG = 0
QW4 = 203
ORDER = 'a'


def _nn(a, b):
    return jnp.dot(a, b, preferred_element_type=f32)


def _nt(a, b):
    return jax.lax.dot_general(a, b, (((1,), (1,)), ((), ())), preferred_element_type=f32)


def _b(u):
    return pltpu.bitcast(u, bf16)


def _u(x):
    return pltpu.bitcast(x, u32)


def _split_pair(u):
    lo = pltpu.bitcast(u << 16, f32).astype(bf16)
    hi = pltpu.bitcast(u & jnp.uint32(0xFFFF0000), f32).astype(bf16)
    return lo, hi


def _lo(u):
    return pltpu.bitcast(u << 16, f32)


def _hi(u):
    return pltpu.bitcast(u & jnp.uint32(0xFFFF0000), f32)


def _pk(e, o):
    return pltpu.pack_elementwise([e, o], packed_dtype=bf16)


def _a7(a11, a12, a21, a22):
    return [a11 + a22, a21 + a22, a11, a22, a11 + a12, a21 - a11, a12 - a22]


def _b7(b11, b12, b21, b22):
    return [b11 + b22, b11, b12 - b22, b21 - b11, b22, b11 + b12, b21 + b22]


def _c4(m):
    return m[0] + m[3] - m[4] + m[6], m[2] + m[4], m[1] + m[3], m[0] - m[1] + m[2] + m[5]


def _combos_u(f7, blk):
    e = f7(*[_lo(x) for x in blk])
    o = f7(*[_hi(x) for x in blk])
    plain = {2: 0, 3: 3} if f7 is _a7 else {1: 0, 4: 3}
    return [blk[plain[n]] if n in plain else _pk(e[n], o[n]) for n in range(7)]


def _quad(c11, c12, c21, c22):
    return jnp.concatenate([jnp.concatenate([c11, c12], axis=1), jnp.concatenate([c21, c22], axis=1)], axis=0)


def _fold(c, op):
    return op(c.reshape(-1, 8, c.shape[1]), axis=0)


def _rsum(p):
    cols = []
    for c in range(0, p.shape[1], 128):
        tot = None
        for k in range(0, p.shape[0], 128):
            acc = None
            for r in range(k + 112, k - 16, -16):
                t = p[r:r + 8, c:c + 128] + p[r + 8:r + 16, c:c + 128]
                acc = t if acc is None else acc + t
            tot = acc if tot is None else tot + acc
        cols.append(tot)
    return jnp.concatenate(cols, axis=1) if len(cols) > 1 else cols[0]


def _gate(x, vals):
    if not vals:
        return x
    w = max(v.shape[1] for v in vals)
    top = x[:8, :w]
    for v in vals:
        if v.shape[1] < w:
            v = jnp.concatenate([v] * (w // v.shape[1]), axis=1)
        top = jnp.where(v == jnp.inf, jnp.zeros_like(top), top)
    if w < x.shape[1]:
        top = jnp.concatenate([top, x[:8, w:]], axis=1)
    return jnp.concatenate([top, x[8:]], axis=0)


def _tok(vals):
    parts = []
    for v in vals:
        for r in range(0, v.shape[0], 8):
            for c in range(0, v.shape[1], 128):
                parts.append(v[r:r + 8, c:c + 128])
    while len(parts) > 1:
        parts = [parts[i] | parts[i + 1] if i + 1 < len(parts) else parts[i] for i in range(0, len(parts), 2)]
    return (parts[0] >> 31) >> 1


def _gate_u(x, tok):
    if tok is None:
        return x
    top = x[:8, :128] | tok
    if x.shape[1] > 128:
        top = jnp.concatenate([top, x[:8, 128:]], axis=1)
    return jnp.concatenate([top, x[8:]], axis=0)


def _ssm_pieces():
    ps = [('HD', 0), ('SC', 0), ('HD', 1), ('SC', 1), ('W7', 0), ('HD', 2), ('SC', 2), ('W7', 1), ('HD', 3), ('SC', 3)]
    if not OS:
        ps = [p for p in ps if p[0] != 'W7']
    cur, cost = [], 0
    for a in range(NB):
        for half in range(2):
            if cur and cost + a + 1 > CVMAX:
                ps.append(('CV', tuple(cur)))
                cur, cost = [], 0
            cur.append((a, half))
            cost += a + 1
        if a % 4 == 3:
            if cur:
                ps.append(('CV', tuple(cur)))
            cur, cost = [], 0
            ps.append(('ID', a // 4))
    return ps


def _schedule():
    side = _ssm_pieces()
    out = []
    cnt = [0]

    def block(units, att, ssm=True):
        k = 0
        for u in units:
            for t in range(7):
                out.append(u + (t,))
                out.extend(att.get(k, []))
                k += 1
                if ssm:
                    cnt[0] += 1
                    if side and cnt[0] >= SIDE0 and (cnt[0] - SIDE0) % SIDEP == 0:
                        out.append(side.pop(0))

    def softmax_head(i, n):
        att = {}
        att.setdefault(min(EX0, n - 2), []).extend(([('PACE',)] if P0 else []) + [('EX', i, 0)])
        if i > 0:
            att.setdefault(n - 1, []).extend([('PACE',), ('EX', i, 1)])
        return att

    block([('KP', 0)], {})
    block([('OP', NT - 1)], {6: [('AT',)]}, False)
    block([('VP', 0), ('KP', 1)], {13: [('QK', 0, 0)]})
    block([('VP', 1)], softmax_head(0, 7))
    for i in range(NT - 1):
        for j in range(i + 1):
            out.append(('QK', i + 1, j))
            if j + 2 <= i:
                out.append(('EX', i, j + 2))
            if j == i:
                out.append(('QK', i + 1, i + 1))
            out.append(('PV', i, j))
        if i + 2 < NT:
            block([('KP', i + 2), ('VP', i + 2)], softmax_head(i + 1, 14))
        else:
            block([('OP', n) for n in range(NOP)], softmax_head(i + 1, 7 * NOP), False)
            out.append(('PACE',))
    for j in range(NT):
        if j + 2 < NT:
            out.append(('EX', NT - 1, j + 2))
        out.append(('PV', NT - 1, j))
        if j + NOP < NT - 3:
            block([('OP', j + NOP)], {}, False)
        out.append(('PACE',))
    block([('OP', NT - 3), ('OP', NT - 2)], {}, False)
    assert not side
    return out


def _kernel(qT_hbm, kT_hbm, vT_hbm, sk_ref, ssmk_hbm, dd_ref, xT_hbm, ckv_hbm,
            wq_hbm, wk_hbm, wv_hbm, woT_hbm, out_hbm,
            qT, kT, vT, ssmk, xT, ckv, wq_raw, wk_raw, wv_raw, woT,
            aq_s, bx_s, bk_s, bvT_s, QT_s, a_s, acc, fullT, out_s, taps, ff_s, fi_s,
            S0_s, S1_s, X_s, W7_s, pace_s, m0_s, m1_s, l0_s, l1_s,
            sem, sem_k, sem_v, sem_o, *kvo):
    K_s, V_s, O_s, Y_s = kvo[:NT], kvo[NT:2 * NT], kvo[2 * NT:3 * NT], kvo[3 * NT:]
    def cp(src, dst, s):
        return pltpu.make_async_copy(src, dst, s)

    def c_x(j):
        cols = pl.ds(pl.multiple_of(j * 2 * T, 2 * T), 2 * T)
        return cp(xT_hbm.at[:, cols], xT.at[pl.ds(0, M), cols], sem.at[j])

    QP = ((0, 128), (128, 96))

    def c_wq(p):
        cs_ = []
        for half in range(2):
            r = pl.ds((half * 224 + QP[p][0]) * H, QP[p][1] * H)
            for g in range(2):
                cs_.append(cp(wq_hbm.at[r, pl.ds(128 * g, 128)], wq_raw.at[g, r], sem.at[18 + 4 * p + 2 * half + g]))
        return cs_


    def c_w(w_hbm, raw, sm, j, half, g):
        r = pl.ds(pl.multiple_of((half * 4 + j) * 2048, 2048), 2048)
        q = 2 * half + g
        return cp(w_hbm.at[r, pl.ds(128 * g, 128)], raw.at[j % 2, q, pl.ds(0, 2048)], sm.at[(j % 2) * 4 + q])

    def c_wk(j):
        return [c_w(wk_hbm, wk_raw, sem_k, j, half, g) for half in range(2) for g in range(2)]

    def c_wv(j):
        return [c_w(wv_hbm, wv_raw, sem_v, j, half, g) for half in range(2) for g in range(2)]

    def c_ckv(j):
        r = pl.ds(pl.multiple_of(j * 2 * T, 2 * T), 2 * T)
        return cp(ckv_hbm.at[r], ckv.at[r], sem.at[9 + j])

    a_pairs = ((kT_hbm, kT), (vT_hbm, vT), (ssmk_hbm, ssmk), (qT_hbm, qT))
    c_early = [cp(woT_hbm.at[pl.ds(0, 1)], woT.at[pl.ds(0, 1)], sem.at[4])]
    c_early += [cp(src.at[pl.ds(0, CH)], dst.at[pl.ds(0, CH)], sem.at[5 + n]) for n, (src, dst) in enumerate(a_pairs)]
    c_late = [cp(woT_hbm.at[pl.ds(1, H - 1)], woT.at[pl.ds(1, H - 1)], sem.at[13])]
    c_late += [cp(src.at[pl.ds(CH, M - CH)], dst.at[pl.ds(CH, M - CH)], sem.at[14 + n])
               for n, (src, dst) in enumerate(a_pairs)]
    for c in [c_x(0)] + c_wq(0) + c_wq(1):
        c.start()
    for c in c_wk(0):
        c.start(priority=1)

    n_i = jax.lax.broadcasted_iota(jnp.int32, (P, P), 0)
    k_i = jax.lax.broadcasted_iota(jnp.int32, (P, P), 1)
    ang = (((2 * k_i + 1) * n_i) & 511).astype(f32) * (math.pi / 256.0)
    cs, sn = jnp.cos(ang), jnp.sin(ang)
    ff_s[:, 0:P] = cs.astype(bf16)
    ff_s[:, P:2 * P] = (-sn).astype(bf16)
    fi_s[0:P, :] = (cs.T * (1.0 / P)).astype(bf16)
    fi_s[P:2 * P, :] = (sn.T * (-1.0 / P)).astype(bf16)
    sk = sk_ref[...].astype(f32)
    for t in range(KS):
        taps[t] = jnp.broadcast_to(sk[t:t + 1, :], (128, M)).T
    taps[KS] = jnp.broadcast_to(dd_ref[...].astype(f32).reshape(1, M), (128, M)).T
    acc[...] = jnp.zeros(acc.shape, f32)
    fullT[...] = jnp.zeros(fullT.shape, bf16)
    O_s[NT - 1][...] = jnp.zeros(O_s[0].shape, bf16)
    W7_s[...] = jnp.zeros(W7_s.shape, u32)

    def prep_x(jj, t, r0):
        c0 = (2 * jj + t) * T
        cs_ = [c0, c0 + 128] if isinstance(jj, int) else [pl.multiple_of(c0, 128), pl.multiple_of(c0 + 128, 128)]
        blk = [_u(xT[r:r + 32, pl.ds(c, 128)]) for r in (r0, 224 + r0) for c in cs_]
        row = (2 * jj + t) * 112 + r0 // 2
        row = pl.ds(row if isinstance(jj, int) else pl.multiple_of(row, 16), 16)
        for n, x in enumerate(_combos_u(_b7, blk)):
            bx_s[row, n * 128:(n + 1) * 128] = x
        return []

    c_x(0).wait()
    for t in range(2):
        for r0 in range(0, 224, 32):
            prep_x(0, t, r0)
    vq = wq_raw.bitcast(u32)
    for p, (c0, nc) in enumerate(QP):
        for c in c_wq(p):
            c.wait()
        for hp in range(0 if 0 else H // 2):
            ut = [vq[g, pl.ds((half * 224 + c0) * 8 + hp, nc, stride=8), :].T for g in range(2) for half in range(2)]
            for r in range(0, 128, 16):
                u = [x[r:r + 16] for x in ut]
                for par, f in enumerate((_lo, _hi)):
                    r0 = (2 * hp + par) * 64 + r // 2
                    for n, x in enumerate(_a7(*[f(x) for x in u])):
                        aq_s[r0:r0 + 8, n * 256 + c0:n * 256 + c0 + nc] = _u(x.astype(bf16))
    for c in c_wv(0) + [c_ckv(0), c_x(1)]:
        c.start(priority=1)

    qscale = (D ** -0.5) * math.log2(math.e)

    def lo(u):
        return pltpu.bitcast(u << 16, f32)

    def hi(u):
        return pltpu.bitcast(u & jnp.uint32(0xFFFF0000), f32)

    def b_combos(b11, b12, b21, b22):
        return [b11 + b22, b11, b12 - b22, b21 - b11, b22, b11 + b12, b21 + b22]

    def q_body(j, carry):
        mq = {}

        bx = [[bx_s[pl.ds(pl.multiple_of((2 * j + t) * 112, 16), 112), n * 128:(n + 1) * 128] for n in range(7)]
              for t in range(2)]

        def qproj(u, tok):
            hh, t, n = u // 14, (u // 7) % 2, SORD[u % 7]
            w = _b(_gate_u(aq_s[hh * 64:hh * 64 + 64, n * 256:n * 256 + 224], tok))
            mq[n] = _nn(w, _b(bx[t][n]))
            if u % 7 == 6:
                for k, x in enumerate(_c4(mq)):
                    cols = pl.ds(pl.multiple_of((2 * j + t) * T + (k % 2) * 128, 128), 128)
                    r0 = hh * 128 + (k // 2) * 64
                    QT_s[r0:r0 + 64, cols] = _u((x * qscale).astype(bf16))
            return mq[n]

        def prep_k(hp, part):
            v = wk_raw.bitcast(u32).at[j % 2]
            u = [v[q, pl.ds(part * 128 + hp, 16, stride=8), :] for q in range(4)]
            for par, f in enumerate((_lo, _hi)):
                for n, c in enumerate(_b7(*[f(x) for x in u])):
                    r = _u(c.astype(bf16))
                    r0 = (2 * hp + par) * 256 + part * 8
                    bk_s[pl.ds(pl.multiple_of(j * 64 + r0, 8), 8), n * 128:(n + 1) * 128] = r
            return []

        vt = {}

        def prep_v(hp, part):
            if part == 0:
                v = wv_raw.bitcast(u32).at[j % 2]
                vt[hp] = [v[q, pl.ds(hp, 128, stride=8), :].T for q in range(4)]
                return [x[120:] for x in vt[hp]] if VG else []
            for r in range(32 * (part - 1), 32 * part, 16):
                u = [x[r:r + 16] for x in vt[hp]]
                for par, f in enumerate((_lo, _hi)):
                    r0 = (2 * hp + par) * 64 + r // 2
                    for n, c in enumerate(_b7(*[f(x) for x in u])):
                        cols = pl.ds(pl.multiple_of(n * 512 + j * 128, 128), 128)
                        bvT_s[r0:r0 + 8, cols] = _u(c.astype(bf16))
            return []

        def prep_a(cl_, part, cbs):
            c = 2 * j + cl_
            r0 = 8 * part
            rt = pl.ds(pl.multiple_of(c * T + 2 * r0, 16), 16)
            rb = pl.ds(pl.multiple_of(c * T + 128 + 2 * r0, 16), 16)
            res = []
            for cb in cbs:
                cl, ch_ = slice(cb * 128, cb * 128 + 128), slice(512 + cb * 128, 512 + cb * 128 + 128)
                blk = [_u(ckv[rt, cl]), _u(ckv[rt, ch_]), _u(ckv[rb, cl]), _u(ckv[rb, ch_])]
                cc = []
                for f in (lo, hi):
                    a11, a12, a21, a22 = [f(x) for x in blk]
                    cc.append([a11 + a22, a21 + a22, None, None, a11 + a12, a21 - a11, a12 - a22])
                for n in range(7):
                    if n == 2:
                        r = blk[0]
                    elif n == 3:
                        r = blk[3]
                    else:
                        r = pltpu.pack_elementwise([cc[0][n], cc[1][n]], packed_dtype=bf16)
                    a_s[c, n, r0:r0 + 8, cl] = r
                    res.append(r)
            return [] if APACE else res

        fill = {}

        def spread(pieces, u0, u1):
            for n, p in enumerate(pieces):
                fill.setdefault(u0 + n * (u1 - u0) // len(pieces), []).append(p)

        spread([functools.partial(prep_k, hp, part) for hp in range(8) for part in range(8)], QW1, QW2)
        spread([functools.partial(prep_v, hp, part) for hp in range(8) for part in range(5)], QW2, QW3)
        spread([functools.partial(prep_a, c, part, cbs) for c in range(2) for part in range(8)
                for cbs in ((0, 1), (2, 3))], QW3, QW4)
        spread([functools.partial(prep_x, jnp.minimum(j + 1, 3), t, r0) for t in range(2) for r0 in range(0, 224, 32)], QW4, 221)
        toks = {}
        for u in range(224):
            if u == QW1:
                @pl.when(j < 3)
                def _():
                    for c in c_wk(j + 1):
                        c.start(priority=1)

                @pl.when(j == 3)
                def _():
                    for c in c_early + c_late:
                        c.start(priority=1)

                for c in c_wk(j):
                    c.wait()
            if u == QW2:
                @pl.when(j < 3)
                def _():
                    for c in c_wv(j + 1) + [c_ckv(j + 1)]:
                        c.start(priority=1)

                @pl.when(j < 2)
                def _():
                    c_x(j + 2).start(priority=1)

                @pl.when(j < 3)
                def _():
                    c_x(j + 1).wait()

                for c in c_wv(j) + [c_ckv(j)]:
                    c.wait()
            q = qproj(u, toks.pop(u, None))
            res = []
            ps = fill.get(u, [])
            for n, p in enumerate(ps):
                row = (n * 128 // len(ps)) // 16 * 16
                if p.func is prep_k:
                    wk_raw.bitcast(u32)[j >> 4, 0, 1024:1032, :] = pltpu.bitcast(q[row:row + 8], u32)
                elif p.func is prep_v and p.args[1] == 0:
                    wv_raw.bitcast(u32)[j >> 4, 0, 1024:1032, :] = pltpu.bitcast(q[row:row + 8], u32)
                elif p.func is prep_x:
                    xT[pl.ds(pl.multiple_of(M + (j >> 4) * 16, 16), 16), 0:128] = q[row:row + 16].astype(bf16)
                elif p.func is prep_a:
                    ckv[pl.ds(pl.multiple_of(S + (j >> 4) * 16, 16), 16), 0:128] = q[row:row + 16].astype(bf16)
                res += p()
            if res:
                toks[u + QLAG] = _tok(res)
        return carry

    if not 0:
        jax.lax.fori_loop(0, 4, q_body, 0)
    for c in c_early:
        c.wait()

    tri = n_i <= k_i
    sgn = jnp.where((jax.lax.broadcasted_iota(jnp.int32, (1, P), 1) & 1) == 0, 1.0, -1.0).astype(f32)

    c_outa = cp(out_s.at[:, pl.ds(0, 384)], out_hbm.at[:, pl.ds(0, 384)], sem_o.at[8])

    HR, HI, PR, PI, KV = range(5)

    def zrow(z, n):
        return pl.ds(0, n) if isinstance(z, int) else pl.ds(pl.multiple_of(z * n, n), n)

    def blk_at(c, half=None):
        r0 = (c % 8) * CH
        rs = slice(r0, r0 + CH) if half is None else slice(r0 + 16 * half, r0 + 16 * half + 16)
        return rs, slice((c // 8) * P, (c // 8 + 1) * P)

    def head_body(h, carry):
        @pl.when(h == 1)
        def _():
            for c in c_late:
                c.wait()

        @pl.when(h == H - 1)
        def _():
            c_outa.start()

        st = dict(l={}, M={}, P={}, Q7={}, mfin={}, o={})
        zs, zl = h >> 10, 0
        m_s, l_s = (m0_s, m1_s), (l0_s, l1_s)
        qrows = pl.ds(pl.multiple_of(h * 128, 128), 128)
        rows = pl.ds(pl.multiple_of(jnp.minimum(h, NCH - 1) * CH, CH), CH)

        def rep(t, n):
            return jnp.concatenate([taps[t, rows, :]] * n, axis=1)

        toks = []

        def due():
            for t in toks:
                t[0] -= 1
            ready = [t[1] for t in toks if t[0] <= 0]
            toks[:] = [t for t in toks if t[0] > 0]
            return functools.reduce(lambda x, y: x | y, ready) if ready else None

        def gate_later(vals, lag=SLAG):
            toks.append([lag, _tok([v if v.dtype == u32 else pltpu.bitcast(v, u32) for v in vals])])

        def row_max(i):
            if i not in st['mfin']:
                m = m_s[i % 2][zl, 0]
                for t in range(1, i + 1):
                    m = jnp.maximum(m, m_s[i % 2][zl, t])
                m = jnp.max(m, axis=0, keepdims=True)
                if PVS and i > 0:
                    lo_ = jnp.exp2(m_s[i % 2][zl, 0] - m)
                    for t in range(1, i + 1):
                        lo_ = lo_ + jnp.exp2(m_s[i % 2][zl, t] - m)
                    m = m + jnp.log2(jnp.sum(lo_, axis=0, keepdims=True))
                st['mfin'][i] = m
            return st['mfin'][i]

        for op in _schedule():
            kind = op[0]
            if kind == 'KP':
                _, c, t = op
                n = SORD[t]
                st['M'][n] = st['last'] = _nn(_b(_gate_u(a_s[c, n], due())), _b(bk_s[pl.ds(pl.multiple_of(h * 256, 256), 256), n * 128:(n + 1) * 128]))
                if t == 6:
                    c4 = _c4(st['M'])
                    blks = dict(zip((2, 7, 8, 3), c4))
                    if QKS and c < NT - 1:
                        blks.update({n: x for n, x in enumerate(_a7(*c4)) if n not in (2, 3)})
                    for n, x in blks.items():
                        K_s[c][zrow(zs, 64), n * 128:(n + 1) * 128] = _u(x.astype(bf16))
            elif kind == 'VP':
                _, c, t = op
                n = SORD[t]
                st['M'][n] = st['last'] = _nt(_b(_gate_u(bvT_s[pl.ds(pl.multiple_of(h * 64, 64), 64), n * 512:(n + 1) * 512], due())), _b(a_s[c, n]))
                if t == 6:
                    c11, c12, c21, c22 = _c4(st['M'])
                    c4 = (c11, c21, c12, c22)
                    blks = dict(zip((2, 7, 8, 3), c4))
                    if PVS and c < NT - 1:
                        blks.update({n: x for n, x in enumerate(_a7(*c4)) if n not in (2, 3)})
                    for n, x in blks.items():
                        V_s[c][zrow(zs, 64), n * 128:(n + 1) * 128] = _u(x.astype(bf16))
            elif kind == 'QK':
                _, i, j = op
                S_s = (S0_s, S1_s)[i % 2]
                qu = QT_s[qrows, i * T:(i + 1) * T]
                if j < i:
                    if QKS:
                        if i not in st['Q7']:
                            st['Q7'][i] = _combos_u(_b7, [qu[:64, :128], qu[:64, 128:], qu[64:, :128], qu[64:, 128:]])
                        m = {n: _nn(_b(K_s[j][zrow(zl, 64), n * 128:(n + 1) * 128]), _b(st['Q7'][i][n])) for n in SORD}
                        s = _quad(*_c4(m))
                    else:
                        s = _nn(_b(_quad(*[K_s[j][zrow(zl, 64), n * 128:(n + 1) * 128] for n in (2, 7, 8, 3)])), _b(qu))
                    S_s[zs, j] = s
                    f = _fold(s, jnp.max)
                else:
                    q = _b(qu)
                    sa = _nn(_b(jnp.concatenate([K_s[j][zrow(zl, 64), 2 * 128:(2 + 1) * 128], K_s[j][zrow(zl, 64), 7 * 128:(7 + 1) * 128]], axis=1)), q)
                    sa = jnp.concatenate([jnp.where(tri, sa[:, :128], NEG), sa[:, 128:]], axis=1)
                    sb = _nn(_b(jnp.concatenate([K_s[j][zrow(zl, 64), 8 * 128:(8 + 1) * 128], K_s[j][zrow(zl, 64), 3 * 128:(3 + 1) * 128]], axis=1)), q[:, 128:])
                    sb = jnp.where(tri, sb, NEG)
                    S_s[zs, j, 0:128, :] = sa
                    S_s[zs, j, 128:T, 128:T] = sb
                    fa = _fold(sa, jnp.max)
                    f = jnp.concatenate([fa[:, :128], jnp.maximum(fa[:, 128:], _fold(sb, jnp.max))], axis=1)
                m_s[i % 2][zs, j] = f
                pace_s[zs] = f
            elif kind == 'EX':
                _, i, j = op
                S_s = (S0_s, S1_s)[i % 2]
                m = row_max(i)
                if j > 0 or P0:
                    m = jnp.where(pace_s[zl, 0:1, :] == jnp.inf, jnp.inf, m)
                if j < i:
                    if PVS:
                        parts, lj = [], None
                        for r in range(112, -16, -16):
                            pt = jnp.exp2(S_s[zl, j, r:r + 16, :] - m)
                            pb = jnp.exp2(S_s[zl, j, 128 + r:128 + r + 16, :] - m)
                            parts.insert(0, _b7(pt[:, :128], pt[:, 128:], pb[:, :128], pb[:, 128:]))
                            x = (pt[:8] + pt[8:]) + (pb[:8] + pb[8:])
                            lj = x if lj is None else lj + x
                        st['P'][i, j] = [jnp.concatenate([x[n] for x in parts], axis=0).astype(bf16) for n in range(7)]
                    else:
                        p = jnp.exp2(S_s[zl, j] - m)
                        lj = _rsum(p)
                        st['P'][i, j] = p.astype(bf16)
                else:
                    pa = jnp.exp2(S_s[zl, j, 0:128, :] - m)
                    pb = jnp.exp2(S_s[zl, j, 128:T, 128:T] - m[:, 128:])
                    la = _rsum(pa)
                    lj = jnp.concatenate([la[:, :128], la[:, 128:] + _rsum(pb)], axis=1)
                    st['P'][i, j] = (pa.astype(bf16), pb.astype(bf16))
                l_s[i % 2][zs, j] = lj
            elif kind == 'PV':
                _, i, j = op
                vb = [V_s[j][zrow(zl, 64), n * 128:(n + 1) * 128] for n in range(9)]
                p = st['P'].pop((i, j))
                if j < i and PVS:
                    for n in SORD:
                        st['last'] = _nn(_b(vb[n]), p[n])
                        st['o'][i, n] = st['last'] if j == 0 else st['o'][i, n] + st['last']
                    continue
                if j < i:
                    o = _nn(_b(_quad(vb[2], vb[7], vb[8], vb[3])), p)
                else:
                    oa = _nn(_b(jnp.concatenate([vb[2], vb[8]], axis=0)), p[0])
                    ob = _nn(_b(jnp.concatenate([vb[7], vb[3]], axis=0)), p[1])
                    o = jnp.concatenate([oa[:, :128], oa[:, 128:] + ob], axis=1)
                st['last'] = o
                if PVS:
                    if i > 0:
                        o = o + _quad(*_c4({n: st['o'].pop((i, n)) for n in range(7)}))
                else:
                    o = o if j == 0 else st['o'][i] + o
                    st['o'][i] = o
                if j == i:
                    l = l_s[i % 2][zl, 0]
                    for t in range(1, i + 1):
                        l = l + l_s[i % 2][zl, t]
                    o = o * (1.0 / jnp.sum(l, axis=0, keepdims=True))
                    blks = (o[:128, :128], o[:128, 128:], o[128:, :128], o[128:, 128:])
                    for n, x in enumerate(_b7(*blks)):
                        O_s[i][zs, n] = x.astype(bf16)
            elif kind == 'PACE':
                pace_s[zs] = jnp.concatenate([st['last'][-8:, -128:]] * 2, axis=1)
            elif kind == 'OP':
                _, i, t = op
                n = SORD[t]
                st['M'][n] = st['last'] = _nn(_b(_gate_u(W7_s[0, n], due())), O_s[i][0, n])
                if t == 6:
                    acc[:, T * i:T * (i + 1)] += _quad(*_c4(st['M']))
            elif kind == 'W7':
                res = []
                for r0 in range(112 * op[1], 112 * op[1] + 112, 16):
                    blk = [_u(woT[h, r:r + 16, c:c + 128]) for r in (r0, 224 + r0) for c in (0, 128)]
                    w7 = _combos_u(_a7, blk)
                    for n, x in enumerate(w7):
                        W7_s[zs, n, r0 // 2:r0 // 2 + 8] = x
                    res += w7
                gate_later(res)
            elif kind == 'AT':
                g = jnp.clip((h - 4) // 4, 0, 2)
                t0 = jnp.minimum(((h + 12) % 4) * 6, NB - 6)
                grow = pl.ds(pl.multiple_of(g * 128, 128), 128)
                gcol = pl.ds(pl.multiple_of(jnp.where(h == H - 1, 3, g) * 128, 128), 128)
                res = []
                for n in range(6):
                    tok = pl.ds(pl.multiple_of((t0 + n) * 128, 128), 128)
                    x = fullT[grow, tok].T
                    out_s[tok, gcol] = x
                    res.append(_u(x)[56:])
                gate_later(res)
            elif kind == 'HD':
                g = op[1]
                hs = jnp.concatenate([ssmk[rows, c * P:(c + 1) * P] for c in range(4 * g, 4 * g + 4)], axis=0)
                hf = _nn(hs, ff_s[...])
                for n in range(4):
                    X_s[(zs, HR) + blk_at(4 * g + n)] = hf[n * CH:(n + 1) * CH, :P]
                    X_s[(zs, HI) + blk_at(4 * g + n)] = hf[n * CH:(n + 1) * CH, P:]
            elif kind == 'SC':
                g = op[1]
                if g == 0:
                    k = jnp.concatenate([jnp.zeros((CH, P), f32), kT[rows, 0:4 * P].astype(f32)], axis=1)
                else:
                    k = kT[rows, (4 * g - 1) * P:(4 * g + 4) * P].astype(f32)
                ks = k[:, P:] * rep(0, 4)
                for j in range(1, KS):
                    ks = ks + pltpu.roll(k, j, 1)[:, P:] * rep(j, 4)
                kv = ks * vT[rows, 4 * g * P:(4 * g + 4) * P].astype(f32)
                kvs = jnp.concatenate([kv[:, n * P:(n + 1) * P] for n in range(4)], axis=0)
                xf = _nn(kvs.astype(bf16), ff_s[...])
                for n in range(4):
                    c = 4 * g + n
                    xr, xi = xf[n * CH:(n + 1) * CH, :P], xf[n * CH:(n + 1) * CH, P:]
                    X_s[(zs, KV) + blk_at(c)] = kvs[n * CH:(n + 1) * CH]
                    X_s[(zs, PR) + blk_at(c)] = xr if c == 0 else xr - sgn * st['x'][1]
                    X_s[(zs, PI) + blk_at(c)] = xi if c == 0 else xi + sgn * st['x'][0]
                    st['x'] = (xr, xi)
            elif kind == 'CV':
                res = []
                for a, half in op[1]:
                    wr = wi = None
                    for j in range(a + 1):
                        hr, hi_ = X_s[(zl, HR) + blk_at(j, half)], X_s[(zl, HI) + blk_at(j, half)]
                        pr, pi = X_s[(zl, PR) + blk_at(a - j, half)], X_s[(zl, PI) + blk_at(a - j, half)]
                        tr, ti = hr * pr - hi_ * pi, hr * pi + hi_ * pr
                        wr, wi = (tr, ti) if wr is None else (wr + tr, wi + ti)
                    r0 = (a % 4) * CH + 16 * half
                    Y_s[a // 4][zs, r0:r0 + 16, :P] = wr
                    Y_s[a // 4][zs, r0:r0 + 16, P:] = wi
                    res += [wr, wi]
                gate_later(res)
            elif kind == 'ID':
                g = op[1]
                w = Y_s[g][0]
                y = _nn(w.astype(bf16), fi_s[...])
                for n in range(4):
                    c = 4 * g + n
                    cols = slice(c * P, (c + 1) * P)
                    ya = y[n * CH:(n + 1) * CH, :] + X_s[(zl, KV) + blk_at(c)] * taps[KS, rows, :]
                    fullT[rows, cols] = (qT[rows, cols].astype(f32) * ya).astype(bf16)
        return carry

    if not 0:
        jax.lax.fori_loop(0, H, head_body, 0)

    acc[:, T * (NT - 1):] += _quad(*_c4({n: _nn(_b(W7_s[0, n]), O_s[NT - 1][0, n]) for n in SORD}))
    outs = [c_outa]
    for i in range(NT):
        cols = slice(T * i, T * (i + 1))
        blk = jnp.concatenate([fullT[384:M, cols], acc[:, cols].astype(bf16)], axis=0)
        out_s[cols, 384:2 * M] = blk.T
        c = cp(out_s.at[pl.ds(T * i, T), pl.ds(384, 512)], out_hbm.at[pl.ds(T * i, T), pl.ds(384, 512)], sem_o.at[i])
        c.start()
        outs.append(c)
    for c in outs:
        c.wait()


@jax.jit
def pallas_concat_heads__ssm_conv_h3__compressed_kv_cla__prompt_kernel(
    A_q: jax.Array,
    A_k: jax.Array,
    A_v: jax.Array,
    A_shift_k: jax.Array,
    A_ssm_k: jax.Array,
    A_ssm_D: jax.Array,
    B_x: jax.Array,
    B_c_kv: jax.Array,
    B_w_q: jax.Array,
    B_w_uk: jax.Array,
    B_w_uv: jax.Array,
    B_w_o: jax.Array,
):
    hbm = pl.BlockSpec(memory_space=pl.ANY)
    vmem = pl.BlockSpec(memory_space=pltpu.VMEM)
    V = pltpu.VMEM
    out = pl.pallas_call(
        _kernel,
        out_shape=jax.ShapeDtypeStruct((S, 2 * M), bf16),
        in_specs=[hbm, hbm, hbm, vmem, hbm, vmem, hbm, hbm, hbm, hbm, hbm, hbm],
        out_specs=hbm,
        scratch_shapes=[
            V((M, S), bf16), V((M, S), bf16), V((M, S), bf16), V((M, S), bf16),
            V((M + 16, S), bf16), V((S + 16, DC), bf16),
            V((2, M * H, 128), bf16), V((2, 4, 128 * H + 16, 128), bf16), V((2, 4, 128 * H + 16, 128), bf16),
            V((H, M, D), bf16),
            V((H * 64, 7 * 256), u32), V((NT * 112, 7 * 128), u32), V((H * 256, 7 * 128), u32), V((H * 64, 7 * 512), u32),
            V((H * D // 2, S), u32), V((NT, 7, 64, 512), u32),
            V((M, S), f32), V((M, S), bf16), V((S, 2 * M), bf16),
            V((KS + 1, M, 128), f32), V((P, 2 * P), bf16), V((2 * P, P), bf16),
            V((1, NT, T, T), f32), V((1, NT, T, T), f32), V((1, 5, T, T), f32),
            V((1, 7, 112, 128), u32), V((1, 8, T), f32),
            V((1, NT, 8, T), f32), V((1, NT, 8, T), f32), V((1, NT, 8, T), f32), V((1, NT, 8, T), f32),
            pltpu.SemaphoreType.DMA((26,)), pltpu.SemaphoreType.DMA((8,)),
            pltpu.SemaphoreType.DMA((8,)), pltpu.SemaphoreType.DMA((9,)),
        ] + [V((64, 9 * 128), u32)] * NT + [V((64, 9 * 128), u32)] * NT + [V((1, 7, 128, 128), bf16)] * NT
        + [V((1, 4 * CH, 2 * P), f32)] * 4,
        compiler_params=pltpu.CompilerParams(vmem_limit_bytes=120 * 1024 * 1024,
                                             shape_invariant_numerics=False),
    )(
        A_q[0].T, A_k[0].T, A_v[0].T, A_shift_k.T, A_ssm_k, A_ssm_D,
        B_x[0].T, B_c_kv[0],
        B_w_q.reshape(M * H, D), B_w_uk.reshape(DC * H, D), B_w_uv.reshape(DC * H, D),
        jnp.transpose(B_w_o, (0, 2, 1)),
    )
    return out[None]
```

```python
import functools
import math

import jax
import jax.numpy as jnp
import jax.experimental.pallas as pl
import jax.experimental.pallas.tpu as pltpu

bf16 = jnp.bfloat16
f32 = jnp.float32
u32 = jnp.uint32

S = 2048
M = 448
DC = 1024
H = 16
D = 256
KS = 4
P = 128
NB = S // P
CH = 32
NCH = M // CH
T = 256
NT = S // T
NEG = -1e30
LAG_M = 0
LAG_S = 0
SORD = tuple(int(c) for c in '6430125')
SK = tuple(int(c) for c in '0364521')
SV = tuple(int(c) for c in '0364125')
SQ = tuple(int(c) for c in '3064125')
SP = tuple(int(c) for c in '0364125')
SO = tuple(int(c) for c in '0364125')
QW1 = 63
QW2 = 119
QW3 = 175
QLAG = 6
OS = 1
QKS = 1
CVMAX = 12
SIDE0 = 1
SIDEP = 3
LA = 2
SLAG = 2
APACE = 1
PROW = 0
PVS = 1
NOP = 3
L0 = 1
LEND = 4
LLAG = 2
EXR = 16
EX0 = 11
P0 = 1
VG = 0
QW4 = 203
VST = 0
ORD = 3
M3 = 0
ORDER = 'a'


def _nn(a, b):
    return jnp.dot(a, b, preferred_element_type=f32)


def _nt(a, b):
    return jax.lax.dot_general(a, b, (((1,), (1,)), ((), ())), preferred_element_type=f32)


def _b(u):
    return pltpu.bitcast(u, bf16)


def _u(x):
    return pltpu.bitcast(x, u32)


def _split_pair(u):
    lo = pltpu.bitcast(u << 16, f32).astype(bf16)
    hi = pltpu.bitcast(u & jnp.uint32(0xFFFF0000), f32).astype(bf16)
    return lo, hi


def _lo(u):
    return pltpu.bitcast(u << 16, f32)


def _hi(u):
    return pltpu.bitcast(u & jnp.uint32(0xFFFF0000), f32)


def _pk(e, o):
    return pltpu.pack_elementwise([e, o], packed_dtype=bf16)


def _a7(a11, a12, a21, a22):
    return [a11 + a22, a21 + a22, a11, a22, a11 + a12, a21 - a11, a12 - a22]


def _b7(b11, b12, b21, b22):
    return [b11 + b22, b11, b12 - b22, b21 - b11, b22, b11 + b12, b21 + b22]


def _c4(m):
    return m[0] + m[3] - m[4] + m[6], m[2] + m[4], m[1] + m[3], m[0] - m[1] + m[2] + m[5]


def _combos_u(f7, blk):
    e = f7(*[_lo(x) for x in blk])
    o = f7(*[_hi(x) for x in blk])
    plain = {2: 0, 3: 3} if f7 is _a7 else {1: 0, 4: 3}
    return [blk[plain[n]] if n in plain else _pk(e[n], o[n]) for n in range(7)]


def _quad(c11, c12, c21, c22):
    return jnp.concatenate([jnp.concatenate([c11, c12], axis=1), jnp.concatenate([c21, c22], axis=1)], axis=0)


def _fold(c, op):
    return op(c.reshape(-1, 8, c.shape[1]), axis=0)


def _rsum(p):
    cols = []
    for c in range(0, p.shape[1], 128):
        tot = None
        for k in range(0, p.shape[0], 128):
            acc = None
            for r in range(k + 112, k - 16, -16):
                t = p[r:r + 8, c:c + 128] + p[r + 8:r + 16, c:c + 128]
                acc = t if acc is None else acc + t
            tot = acc if tot is None else tot + acc
        cols.append(tot)
    return jnp.concatenate(cols, axis=1) if len(cols) > 1 else cols[0]


def _gate(x, vals):
    if not vals:
        return x
    w = max(v.shape[1] for v in vals)
    top = x[:8, :w]
    for v in vals:
        if v.shape[1] < w:
            v = jnp.concatenate([v] * (w // v.shape[1]), axis=1)
        top = jnp.where(v == jnp.inf, jnp.zeros_like(top), top)
    if w < x.shape[1]:
        top = jnp.concatenate([top, x[:8, w:]], axis=1)
    return jnp.concatenate([top, x[8:]], axis=0)


def _tok(vals):
    parts = []
    for v in vals:
        for r in range(0, v.shape[0], 8):
            for c in range(0, v.shape[1], 128):
                parts.append(v[r:r + 8, c:c + 128])
    while len(parts) > 1:
        parts = [parts[i] | parts[i + 1] if i + 1 < len(parts) else parts[i] for i in range(0, len(parts), 2)]
    return (parts[0] >> 31) >> 1


def _gate_u(x, tok):
    if tok is None:
        return x
    top = x[:8, :128] | tok
    if x.shape[1] > 128:
        top = jnp.concatenate([top, x[:8, 128:]], axis=1)
    return jnp.concatenate([top, x[8:]], axis=0)


def _ssm_pieces():
    ps = [('HD', 0), ('SC', 0), ('HD', 1), ('SC', 1), ('W7', 0), ('HD', 2), ('SC', 2), ('W7', 1), ('HD', 3), ('SC', 3)]
    if not OS:
        ps = [p for p in ps if p[0] != 'W7']
    cur, cost = [], 0
    for a in range(NB):
        for half in range(2):
            if cur and cost + a + 1 > CVMAX:
                ps.append(('CV', tuple(cur)))
                cur, cost = [], 0
            cur.append((a, half))
            cost += a + 1
        if a % 4 == 3:
            if cur:
                ps.append(('CV', tuple(cur)))
            cur, cost = [], 0
            ps.append(('ID', a // 4))
    return ps


def _schedule():
    side = _ssm_pieces()
    out = []
    cnt = [0]

    def block(units, att, ssm=True):
        k = 0
        for u in units:
            for t in range(7):
                out.append(u + (t,))
                out.extend(att.get(k, []))
                k += 1
                if ssm:
                    cnt[0] += 1
                    if side and cnt[0] >= SIDE0 and (cnt[0] - SIDE0) % SIDEP == 0:
                        out.append(side.pop(0))

    def softmax_head(i, n):
        att = {}
        att.setdefault(min(EX0, n - 2), []).extend(([('PACE',)] if P0 else []) + [('EX', i, 0)])
        if i > 0:
            att.setdefault(n - 1, []).extend([('PACE',), ('EX', i, 1)])
        return att

    block([('KP', 0)], {})
    block([('OP', NT - 1)], {6: [('AT',)]}, False)
    block([('VP', 0), ('KP', 1)], {13: [('QK', 0, 0)]})
    block([('VP', 1)], softmax_head(0, 7))
    for i in range(NT - 1):
        for j in range(i + 1):
            out.append(('QK', i + 1, j))
            if j + 2 <= i:
                out.append(('EX', i, j + 2))
            if j == i and not ORD & 1:
                out.append(('QK', i + 1, i + 1))
            out.append(('PV', i, j))
            if j == i and ORD & 1:
                out.append(('QK', i + 1, i + 1))
        if i + 2 < NT:
            block([('KP', i + 2), ('VP', i + 2)][::-1 if ORD & 2 else 1], softmax_head(i + 1, 14))
        else:
            block([('OP', n) for n in range(NOP)], softmax_head(i + 1, 7 * NOP), False)
            out.append(('PACE',))
    for j in range(NT):
        if j + 2 < NT:
            out.append(('EX', NT - 1, j + 2))
        out.append(('PV', NT - 1, j))
        if j + NOP < NT - 3:
            block([('OP', j + NOP)], {}, False)
        out.append(('PACE',))
    block([('OP', NT - 3), ('OP', NT - 2)], {}, False)
    assert not side
    return out


def _kernel(qT_hbm, kT_hbm, vT_hbm, sk_ref, ssmk_hbm, dd_ref, xT_hbm, ckv_hbm,
            wq_hbm, wk_hbm, wv_hbm, woT_hbm, out_hbm,
            qT, kT, vT, ssmk, xT, ckv, wq_raw, wk_raw, wv_raw, woT,
            aq_s, bx_s, bk_s, bvT_s, QT_s, a_s, acc, fullT, out_s, taps, ff_s, fi_s,
            S0_s, S1_s, X_s, W7_s, pace_s, m0_s, m1_s, l0_s, l1_s,
            sem, sem_k, sem_v, sem_o, *kvo):
    K_s, V_s, O_s, Y_s = kvo[:NT], kvo[NT:2 * NT], kvo[2 * NT:3 * NT], kvo[3 * NT:]
    def cp(src, dst, s):
        return pltpu.make_async_copy(src, dst, s)

    def c_x(j):
        cols = pl.ds(pl.multiple_of(j * 2 * T, 2 * T), 2 * T)
        return cp(xT_hbm.at[:, cols], xT.at[pl.ds(0, M), cols], sem.at[j])

    QP = ((0, 128), (128, 96))

    def c_wq(p):
        cs_ = []
        for half in range(2):
            r = pl.ds((half * 224 + QP[p][0]) * H, QP[p][1] * H)
            for g in range(2):
                cs_.append(cp(wq_hbm.at[r, pl.ds(128 * g, 128)], wq_raw.at[g, r], sem.at[18 + 4 * p + 2 * half + g]))
        return cs_


    def c_w(w_hbm, raw, sm, j, half, g):
        r = pl.ds(pl.multiple_of((half * 4 + j) * 2048, 2048), 2048)
        q = 2 * half + g
        return cp(w_hbm.at[r, pl.ds(128 * g, 128)], raw.at[j % 2, q, pl.ds(0, 2048)], sm.at[(j % 2) * 4 + q])

    def c_wk(j):
        return [c_w(wk_hbm, wk_raw, sem_k, j, half, g) for half in range(2) for g in range(2)]

    def c_wv(j):
        return [c_w(wv_hbm, wv_raw, sem_v, j, half, g) for half in range(2) for g in range(2)]

    def c_ckv(j):
        r = pl.ds(pl.multiple_of(j * 2 * T, 2 * T), 2 * T)
        return cp(ckv_hbm.at[r], ckv.at[r], sem.at[9 + j])

    a_pairs = ((kT_hbm, kT), (vT_hbm, vT), (ssmk_hbm, ssmk), (qT_hbm, qT))
    c_early = [cp(woT_hbm.at[pl.ds(0, 1)], woT.at[pl.ds(0, 1)], sem.at[4])]
    c_early += [cp(src.at[pl.ds(0, CH)], dst.at[pl.ds(0, CH)], sem.at[5 + n]) for n, (src, dst) in enumerate(a_pairs)]
    c_late = [cp(woT_hbm.at[pl.ds(1, H - 1)], woT.at[pl.ds(1, H - 1)], sem.at[13])]
    c_late += [cp(src.at[pl.ds(CH, M - CH)], dst.at[pl.ds(CH, M - CH)], sem.at[14 + n])
               for n, (src, dst) in enumerate(a_pairs)]
    for c in [c_x(0)] + c_wq(0) + c_wq(1):
        c.start()
    for c in c_wk(0) + [c_x(1)]:
        c.start(priority=1)

    n_i = jax.lax.broadcasted_iota(jnp.int32, (P, P), 0)
    k_i = jax.lax.broadcasted_iota(jnp.int32, (P, P), 1)
    ang = (((2 * k_i + 1) * n_i) & 511).astype(f32) * (math.pi / 256.0)
    cs, sn = jnp.cos(ang), jnp.sin(ang)
    ff_s[:, 0:P] = cs.astype(bf16)
    ff_s[:, P:2 * P] = (-sn).astype(bf16)
    fi_s[0:P, :] = (cs.T * (1.0 / P)).astype(bf16)
    fi_s[P:2 * P, :] = (sn.T * (-1.0 / P)).astype(bf16)
    sk = sk_ref[...].astype(f32)
    for t in range(KS):
        taps[t] = jnp.broadcast_to(sk[t:t + 1, :], (128, M)).T
    taps[KS] = jnp.broadcast_to(dd_ref[...].astype(f32).reshape(1, M), (128, M)).T
    acc[...] = jnp.zeros(acc.shape, f32)
    fullT[...] = jnp.zeros(fullT.shape, bf16)
    O_s[NT - 1][...] = jnp.zeros(O_s[0].shape, bf16)
    W7_s[...] = jnp.zeros(W7_s.shape, u32)

    def prep_x(jj, t, r0):
        c0 = (2 * jj + t) * T
        cs_ = [c0, c0 + 128] if isinstance(jj, int) else [pl.multiple_of(c0, 128), pl.multiple_of(c0 + 128, 128)]
        blk = [_u(xT[r:r + 32, pl.ds(c, 128)]) for r in (r0, 224 + r0) for c in cs_]
        row = (2 * jj + t) * 112 + r0 // 2
        row = pl.ds(row if isinstance(jj, int) else pl.multiple_of(row, 16), 16)
        for n, x in enumerate(_combos_u(_b7, blk)):
            bx_s[row, n * 128:(n + 1) * 128] = x
        return []

    c_x(0).wait()
    for t in range(2):
        for r0 in range(0, 224, 32):
            prep_x(0, t, r0)
    vq = wq_raw.bitcast(u32)
    for p, (c0, nc) in enumerate(QP):
        for c in c_wq(p):
            c.wait()
        if p == 1 and VST:
            for c in c_wv(0) + [c_ckv(0)]:
                c.start(priority=1)
        for hp in range(0 if 0 else H // 2):
            ut = [vq[g, pl.ds((half * 224 + c0) * 8 + hp, nc, stride=8), :].T for g in range(2) for half in range(2)]
            for r in range(0, 128, 16):
                u = [x[r:r + 16] for x in ut]
                for par, f in enumerate((_lo, _hi)):
                    r0 = (2 * hp + par) * 64 + r // 2
                    for n, x in enumerate(_a7(*[f(x) for x in u])):
                        aq_s[r0:r0 + 8, n * 256 + c0:n * 256 + c0 + nc] = _u(x.astype(bf16))
    if not VST:
        for c in c_wv(0) + [c_ckv(0)]:
            c.start(priority=1)

    qscale = (D ** -0.5) * math.log2(math.e)

    def lo(u):
        return pltpu.bitcast(u << 16, f32)

    def hi(u):
        return pltpu.bitcast(u & jnp.uint32(0xFFFF0000), f32)

    def b_combos(b11, b12, b21, b22):
        return [b11 + b22, b11, b12 - b22, b21 - b11, b22, b11 + b12, b21 + b22]

    def q_body(j, carry):
        mq = {}

        bx = [[bx_s[pl.ds(pl.multiple_of((2 * j + t) * 112, 16), 112), n * 128:(n + 1) * 128] for n in range(7)]
              for t in range(2)]

        def qproj(u, tok):
            hh, t, n = u // 14, (u // 7) % 2, SORD[u % 7]
            w = _b(_gate_u(aq_s[hh * 64:hh * 64 + 64, n * 256:n * 256 + 224], tok))
            mq[n] = _nn(w, _b(bx[t][n]))
            if u % 7 == 6:
                for k, x in enumerate(_c4(mq)):
                    cols = pl.ds(pl.multiple_of((2 * j + t) * T + (k % 2) * 128, 128), 128)
                    r0 = hh * 128 + (k // 2) * 64
                    QT_s[r0:r0 + 64, cols] = _u((x * qscale).astype(bf16))
            return mq[n]

        def prep_k(hp, part):
            v = wk_raw.bitcast(u32).at[j % 2]
            u = [v[q, pl.ds(part * 128 + hp, 16, stride=8), :] for q in range(4)]
            for par, f in enumerate((_lo, _hi)):
                for n, c in enumerate(_b7(*[f(x) for x in u])):
                    r = _u(c.astype(bf16))
                    r0 = (2 * hp + par) * 256 + part * 8
                    bk_s[pl.ds(pl.multiple_of(j * 64 + r0, 8), 8), n * 128:(n + 1) * 128] = r
            return []

        vt = {}

        def prep_v(hp, part):
            if part == 0:
                v = wv_raw.bitcast(u32).at[j % 2]
                vt[hp] = [v[q, pl.ds(hp, 128, stride=8), :].T for q in range(4)]
                return [x[120:] for x in vt[hp]] if VG else []
            for r in range(32 * (part - 1), 32 * part, 16):
                u = [x[r:r + 16] for x in vt[hp]]
                for par, f in enumerate((_lo, _hi)):
                    r0 = (2 * hp + par) * 64 + r // 2
                    for n, c in enumerate(_b7(*[f(x) for x in u])):
                        cols = pl.ds(pl.multiple_of(n * 512 + j * 128, 128), 128)
                        bvT_s[r0:r0 + 8, cols] = _u(c.astype(bf16))
            return []

        def prep_a(cl_, part, cbs):
            c = 2 * j + cl_
            r0 = 8 * part
            rt = pl.ds(pl.multiple_of(c * T + 2 * r0, 16), 16)
            rb = pl.ds(pl.multiple_of(c * T + 128 + 2 * r0, 16), 16)
            res = []
            for cb in cbs:
                cl, ch_ = slice(cb * 128, cb * 128 + 128), slice(512 + cb * 128, 512 + cb * 128 + 128)
                blk = [_u(ckv[rt, cl]), _u(ckv[rt, ch_]), _u(ckv[rb, cl]), _u(ckv[rb, ch_])]
                cc = []
                for f in (lo, hi):
                    a11, a12, a21, a22 = [f(x) for x in blk]
                    cc.append([a11 + a22, a21 + a22, None, None, a11 + a12, a21 - a11, a12 - a22])
                for n in range(7):
                    if n == 2:
                        r = blk[0]
                    elif n == 3:
                        r = blk[3]
                    else:
                        r = pltpu.pack_elementwise([cc[0][n], cc[1][n]], packed_dtype=bf16)
                    a_s[c, n, r0:r0 + 8, cl] = r
                    res.append(r)
            return [] if APACE else res

        fill = {}

        def spread(pieces, u0, u1):
            for n, p in enumerate(pieces):
                fill.setdefault(u0 + n * (u1 - u0) // len(pieces), []).append(p)

        spread([functools.partial(prep_k, hp, part) for hp in range(8) for part in range(8)], QW1, QW2)
        spread([functools.partial(prep_v, hp, part) for hp in range(8) for part in range(5)], QW2, QW3)
        spread([functools.partial(prep_a, c, part, cbs) for c in range(2) for part in range(8)
                for cbs in ((0, 1), (2, 3))], QW3, QW4)
        spread([functools.partial(prep_x, jnp.minimum(j + 1, 3), t, r0) for t in range(2) for r0 in range(0, 224, 32)], QW4, 221)
        toks = {}
        for u in range(224):
            if u == QW1:
                @pl.when(j < 3)
                def _():
                    for c in c_wk(j + 1):
                        c.start(priority=1)

                @pl.when(j == 3)
                def _():
                    for c in c_early + c_late:
                        c.start(priority=1)

                for c in c_wk(j):
                    c.wait()
            if u == QW2:
                @pl.when(j < 3)
                def _():
                    for c in c_wv(j + 1) + [c_ckv(j + 1)]:
                        c.start(priority=1)

                @pl.when(j < 2)
                def _():
                    c_x(j + 2).start(priority=1)

                @pl.when(j < 3)
                def _():
                    c_x(j + 1).wait()

                for c in c_wv(j) + [c_ckv(j)]:
                    c.wait()
            q = qproj(u, toks.pop(u, None))
            res = []
            ps = fill.get(u, [])
            for n, p in enumerate(ps):
                row = (n * 128 // len(ps)) // 16 * 16
                if p.func is prep_k:
                    wk_raw.bitcast(u32)[j >> 4, 0, 1024:1032, :] = pltpu.bitcast(q[row:row + 8], u32)
                elif p.func is prep_v and p.args[1] == 0:
                    wv_raw.bitcast(u32)[j >> 4, 0, 1024:1032, :] = pltpu.bitcast(q[row:row + 8], u32)
                elif p.func is prep_x:
                    xT[pl.ds(pl.multiple_of(M + (j >> 4) * 16, 16), 16), 0:128] = q[row:row + 16].astype(bf16)
                elif p.func is prep_a:
                    ckv[pl.ds(pl.multiple_of(S + (j >> 4) * 16, 16), 16), 0:128] = q[row:row + 16].astype(bf16)
                res += p()
            if res:
                toks[u + QLAG] = _tok(res)
        return carry

    if not 0:
        jax.lax.fori_loop(0, 4, q_body, 0)
    for c in c_early:
        c.wait()

    tri = n_i <= k_i
    sgn = jnp.where((jax.lax.broadcasted_iota(jnp.int32, (1, P), 1) & 1) == 0, 1.0, -1.0).astype(f32)

    c_outa = cp(out_s.at[:, pl.ds(0, 384)], out_hbm.at[:, pl.ds(0, 384)], sem_o.at[8])

    HR, HI, PR, PI, KV, HS, PS = range(7)

    def zrow(z, n):
        return pl.ds(0, n) if isinstance(z, int) else pl.ds(pl.multiple_of(z * n, n), n)

    def blk_at(c, half=None):
        r0 = (c % 8) * CH
        rs = slice(r0, r0 + CH) if half is None else slice(r0 + 16 * half, r0 + 16 * half + 16)
        return rs, slice((c // 8) * P, (c // 8 + 1) * P)

    def head_body(h, carry):
        @pl.when(h == 1)
        def _():
            for c in c_late:
                c.wait()

        @pl.when(h == H - 1)
        def _():
            c_outa.start()

        st = dict(l={}, M={}, P={}, Q7={}, mfin={}, o={})
        zs, zl = h >> 10, 0
        m_s, l_s = (m0_s, m1_s), (l0_s, l1_s)
        qrows = pl.ds(pl.multiple_of(h * 128, 128), 128)
        rows = pl.ds(pl.multiple_of(jnp.minimum(h, NCH - 1) * CH, CH), CH)

        def rep(t, n):
            return jnp.concatenate([taps[t, rows, :]] * n, axis=1)

        toks = []

        def due():
            for t in toks:
                t[0] -= 1
            ready = [t[1] for t in toks if t[0] <= 0]
            toks[:] = [t for t in toks if t[0] > 0]
            return functools.reduce(lambda x, y: x | y, ready) if ready else None

        def gate_later(vals, lag=SLAG):
            toks.append([lag, _tok([v if v.dtype == u32 else pltpu.bitcast(v, u32) for v in vals])])

        def row_max(i):
            if i not in st['mfin']:
                m = m_s[i % 2][zl, 0]
                for t in range(1, i + 1):
                    m = jnp.maximum(m, m_s[i % 2][zl, t])
                m = jnp.max(m, axis=0, keepdims=True)
                if PVS and i > 0:
                    lo_ = jnp.exp2(m_s[i % 2][zl, 0] - m)
                    for t in range(1, i + 1):
                        lo_ = lo_ + jnp.exp2(m_s[i % 2][zl, t] - m)
                    m = m + jnp.log2(jnp.sum(lo_, axis=0, keepdims=True))
                st['mfin'][i] = m
            return st['mfin'][i]

        for op in _schedule():
            kind = op[0]
            if kind == 'KP':
                _, c, t = op
                n = SK[t]
                st['M'][n] = st['last'] = _nn(_b(_gate_u(a_s[c, n], due())), _b(bk_s[pl.ds(pl.multiple_of(h * 256, 256), 256), n * 128:(n + 1) * 128]))
                if t == 6:
                    c4 = _c4(st['M'])
                    blks = dict(zip((2, 7, 8, 3), c4))
                    if QKS and c < NT - 1:
                        blks.update({n: x for n, x in enumerate(_a7(*c4)) if n not in (2, 3)})
                    for n, x in blks.items():
                        K_s[c][zrow(zs, 64), n * 128:(n + 1) * 128] = _u(x.astype(bf16))
            elif kind == 'VP':
                _, c, t = op
                n = SV[t]
                st['M'][n] = st['last'] = _nt(_b(_gate_u(bvT_s[pl.ds(pl.multiple_of(h * 64, 64), 64), n * 512:(n + 1) * 512], due())), _b(a_s[c, n]))
                if t == 6:
                    c11, c12, c21, c22 = _c4(st['M'])
                    c4 = (c11, c21, c12, c22)
                    blks = dict(zip((2, 7, 8, 3), c4))
                    if PVS and c < NT - 1:
                        blks.update({n: x for n, x in enumerate(_a7(*c4)) if n not in (2, 3)})
                    for n, x in blks.items():
                        V_s[c][zrow(zs, 64), n * 128:(n + 1) * 128] = _u(x.astype(bf16))
            elif kind == 'QK':
                _, i, j = op
                S_s = (S0_s, S1_s)[i % 2]
                qu = QT_s[qrows, i * T:(i + 1) * T]
                if j < i:
                    if QKS:
                        if i not in st['Q7']:
                            st['Q7'][i] = _combos_u(_b7, [qu[:64, :128], qu[:64, 128:], qu[64:, :128], qu[64:, 128:]])
                        m = {n: _nn(_b(K_s[j][zrow(zl, 64), n * 128:(n + 1) * 128]), _b(st['Q7'][i][n])) for n in SQ}
                        s = _quad(*_c4(m))
                    else:
                        s = _nn(_b(_quad(*[K_s[j][zrow(zl, 64), n * 128:(n + 1) * 128] for n in (2, 7, 8, 3)])), _b(qu))
                    S_s[zs, j] = s
                    f = _fold(s, jnp.max)
                else:
                    q = _b(qu)
                    sa = _nn(_b(jnp.concatenate([K_s[j][zrow(zl, 64), 2 * 128:(2 + 1) * 128], K_s[j][zrow(zl, 64), 7 * 128:(7 + 1) * 128]], axis=1)), q)
                    sa = jnp.concatenate([jnp.where(tri, sa[:, :128], NEG), sa[:, 128:]], axis=1)
                    sb = _nn(_b(jnp.concatenate([K_s[j][zrow(zl, 64), 8 * 128:(8 + 1) * 128], K_s[j][zrow(zl, 64), 3 * 128:(3 + 1) * 128]], axis=1)), q[:, 128:])
                    sb = jnp.where(tri, sb, NEG)
                    S_s[zs, j, 0:128, :] = sa
                    S_s[zs, j, 128:T, 128:T] = sb
                    fa = _fold(sa, jnp.max)
                    f = jnp.concatenate([fa[:, :128], jnp.maximum(fa[:, 128:], _fold(sb, jnp.max))], axis=1)
                m_s[i % 2][zs, j] = f
                pace_s[zs] = f
            elif kind == 'EX':
                _, i, j = op
                S_s = (S0_s, S1_s)[i % 2]
                m = row_max(i)
                if j > 0 or P0:
                    m = jnp.where(pace_s[zl, 0:1, :] == jnp.inf, jnp.inf, m)
                if j < i:
                    if PVS:
                        parts, lj = [], None
                        for r in range(112, -16, -16):
                            pt = jnp.exp2(S_s[zl, j, r:r + 16, :] - m)
                            pb = jnp.exp2(S_s[zl, j, 128 + r:128 + r + 16, :] - m)
                            parts.insert(0, _b7(pt[:, :128], pt[:, 128:], pb[:, :128], pb[:, 128:]))
                            x = (pt[:8] + pt[8:]) + (pb[:8] + pb[8:])
                            lj = x if lj is None else lj + x
                        st['P'][i, j] = [jnp.concatenate([x[n] for x in parts], axis=0).astype(bf16) for n in range(7)]
                    else:
                        p = jnp.exp2(S_s[zl, j] - m)
                        lj = _rsum(p)
                        st['P'][i, j] = p.astype(bf16)
                else:
                    pa = jnp.exp2(S_s[zl, j, 0:128, :] - m)
                    pb = jnp.exp2(S_s[zl, j, 128:T, 128:T] - m[:, 128:])
                    la = _rsum(pa)
                    lj = jnp.concatenate([la[:, :128], la[:, 128:] + _rsum(pb)], axis=1)
                    st['P'][i, j] = (pa.astype(bf16), pb.astype(bf16))
                l_s[i % 2][zs, j] = lj
            elif kind == 'PV':
                _, i, j = op
                vb = [V_s[j][zrow(zl, 64), n * 128:(n + 1) * 128] for n in range(9)]
                p = st['P'].pop((i, j))
                if j < i and PVS:
                    for n in SP:
                        st['last'] = _nn(_b(vb[n]), p[n])
                        st['o'][i, n] = st['last'] if j == 0 else st['o'][i, n] + st['last']
                    continue
                if j < i:
                    o = _nn(_b(_quad(vb[2], vb[7], vb[8], vb[3])), p)
                else:
                    oa = _nn(_b(jnp.concatenate([vb[2], vb[8]], axis=0)), p[0])
                    ob = _nn(_b(jnp.concatenate([vb[7], vb[3]], axis=0)), p[1])
                    o = jnp.concatenate([oa[:, :128], oa[:, 128:] + ob], axis=1)
                st['last'] = o
                if PVS:
                    if i > 0:
                        o = o + _quad(*_c4({n: st['o'].pop((i, n)) for n in range(7)}))
                else:
                    o = o if j == 0 else st['o'][i] + o
                    st['o'][i] = o
                if j == i:
                    l = l_s[i % 2][zl, 0]
                    for t in range(1, i + 1):
                        l = l + l_s[i % 2][zl, t]
                    o = o * (1.0 / jnp.sum(l, axis=0, keepdims=True))
                    blks = (o[:128, :128], o[:128, 128:], o[128:, :128], o[128:, 128:])
                    for n, x in enumerate(_b7(*blks)):
                        O_s[i][zs, n] = x.astype(bf16)
            elif kind == 'PACE':
                pace_s[zs] = jnp.concatenate([st['last'][-8:, -128:]] * 2, axis=1)
            elif kind == 'OP':
                _, i, t = op
                n = SO[t]
                st['M'][n] = st['last'] = _nn(_b(_gate_u(W7_s[0, n], due())), O_s[i][0, n])
                if t == 6:
                    acc[:, T * i:T * (i + 1)] += _quad(*_c4(st['M']))
            elif kind == 'W7':
                res = []
                for r0 in range(112 * op[1], 112 * op[1] + 112, 16):
                    blk = [_u(woT[h, r:r + 16, c:c + 128]) for r in (r0, 224 + r0) for c in (0, 128)]
                    w7 = _combos_u(_a7, blk)
                    for n, x in enumerate(w7):
                        W7_s[zs, n, r0 // 2:r0 // 2 + 8] = x
                    res += w7
                gate_later(res)
            elif kind == 'AT':
                g = jnp.clip((h - 4) // 4, 0, 2)
                t0 = jnp.minimum(((h + 12) % 4) * 6, NB - 6)
                grow = pl.ds(pl.multiple_of(g * 128, 128), 128)
                gcol = pl.ds(pl.multiple_of(jnp.where(h == H - 1, 3, g) * 128, 128), 128)
                res = []
                for n in range(6):
                    tok = pl.ds(pl.multiple_of((t0 + n) * 128, 128), 128)
                    x = fullT[grow, tok].T
                    out_s[tok, gcol] = x
                    res.append(_u(x)[56:])
                gate_later(res)
            elif kind == 'HD':
                g = op[1]
                hs = jnp.concatenate([ssmk[rows, c * P:(c + 1) * P] for c in range(4 * g, 4 * g + 4)], axis=0)
                hf = _nn(hs, ff_s[...])
                for n in range(4):
                    X_s[(zs, HR) + blk_at(4 * g + n)] = hf[n * CH:(n + 1) * CH, :P]
                    X_s[(zs, HI) + blk_at(4 * g + n)] = hf[n * CH:(n + 1) * CH, P:]
                    if M3:
                        X_s[(zs, HS) + blk_at(4 * g + n)] = hf[n * CH:(n + 1) * CH, :P] + hf[n * CH:(n + 1) * CH, P:]
            elif kind == 'SC':
                g = op[1]
                if g == 0:
                    k = jnp.concatenate([jnp.zeros((CH, P), f32), kT[rows, 0:4 * P].astype(f32)], axis=1)
                else:
                    k = kT[rows, (4 * g - 1) * P:(4 * g + 4) * P].astype(f32)
                ks = k[:, P:] * rep(0, 4)
                for j in range(1, KS):
                    ks = ks + pltpu.roll(k, j, 1)[:, P:] * rep(j, 4)
                kv = ks * vT[rows, 4 * g * P:(4 * g + 4) * P].astype(f32)
                kvs = jnp.concatenate([kv[:, n * P:(n + 1) * P] for n in range(4)], axis=0)
                xf = _nn(kvs.astype(bf16), ff_s[...])
                for n in range(4):
                    c = 4 * g + n
                    xr, xi = xf[n * CH:(n + 1) * CH, :P], xf[n * CH:(n + 1) * CH, P:]
                    X_s[(zs, KV) + blk_at(c)] = kvs[n * CH:(n + 1) * CH]
                    pr = xr if c == 0 else xr - sgn * st['x'][1]
                    pi = xi if c == 0 else xi + sgn * st['x'][0]
                    X_s[(zs, PR) + blk_at(c)] = pr
                    if M3:
                        X_s[(zs, PI) + blk_at(c)] = pi - pr
                        X_s[(zs, PS) + blk_at(c)] = pi + pr
                    else:
                        X_s[(zs, PI) + blk_at(c)] = pi
                    st['x'] = (xr, xi)
            elif kind == 'CV':
                res = []
                for a, half in op[1]:
                    wr = wi = None
                    k123 = None
                    for j in range(a + 1 if M3 else 0):
                        t = [X_s[(zl, u) + blk_at(j, half)] * X_s[(zl, v) + blk_at(a - j, half)]
                             for u, v in ((HS, PR), (HR, PI), (HI, PS))]
                        k123 = t if k123 is None else [x + y for x, y in zip(k123, t)]
                    if M3:
                        wr, wi = k123[0] - k123[2], k123[0] + k123[1]
                    for j in range(0 if M3 else a + 1):
                        hr, hi_ = X_s[(zl, HR) + blk_at(j, half)], X_s[(zl, HI) + blk_at(j, half)]
                        pr, pi = X_s[(zl, PR) + blk_at(a - j, half)], X_s[(zl, PI) + blk_at(a - j, half)]
                        tr, ti = hr * pr - hi_ * pi, hr * pi + hi_ * pr
                        wr, wi = (tr, ti) if wr is None else (wr + tr, wi + ti)
                    r0 = (a % 4) * CH + 16 * half
                    Y_s[a // 4][zs, r0:r0 + 16, :P] = wr
                    Y_s[a // 4][zs, r0:r0 + 16, P:] = wi
                    res += [wr, wi]
                gate_later(res)
            elif kind == 'ID':
                g = op[1]
                w = Y_s[g][0]
                y = _nn(w.astype(bf16), fi_s[...])
                for n in range(4):
                    c = 4 * g + n
                    cols = slice(c * P, (c + 1) * P)
                    ya = y[n * CH:(n + 1) * CH, :] + X_s[(zl, KV) + blk_at(c)] * taps[KS, rows, :]
                    fullT[rows, cols] = (qT[rows, cols].astype(f32) * ya).astype(bf16)
        return carry

    if not 0:
        jax.lax.fori_loop(0, H, head_body, 0)

    acc[:, T * (NT - 1):] += _quad(*_c4({n: _nn(_b(W7_s[0, n]), O_s[NT - 1][0, n]) for n in SORD}))
    outs = [c_outa]
    for i in range(NT):
        cols = slice(T * i, T * (i + 1))
        blk = jnp.concatenate([fullT[384:M, cols], acc[:, cols].astype(bf16)], axis=0)
        out_s[cols, 384:2 * M] = blk.T
        c = cp(out_s.at[pl.ds(T * i, T), pl.ds(384, 512)], out_hbm.at[pl.ds(T * i, T), pl.ds(384, 512)], sem_o.at[i])
        c.start()
        outs.append(c)
    for c in outs:
        c.wait()


@jax.jit
def pallas_concat_heads__ssm_conv_h3__compressed_kv_cla__prompt_kernel(
    A_q: jax.Array,
    A_k: jax.Array,
    A_v: jax.Array,
    A_shift_k: jax.Array,
    A_ssm_k: jax.Array,
    A_ssm_D: jax.Array,
    B_x: jax.Array,
    B_c_kv: jax.Array,
    B_w_q: jax.Array,
    B_w_uk: jax.Array,
    B_w_uv: jax.Array,
    B_w_o: jax.Array,
):
    hbm = pl.BlockSpec(memory_space=pl.ANY)
    vmem = pl.BlockSpec(memory_space=pltpu.VMEM)
    V = pltpu.VMEM
    out = pl.pallas_call(
        _kernel,
        out_shape=jax.ShapeDtypeStruct((S, 2 * M), bf16),
        in_specs=[hbm, hbm, hbm, vmem, hbm, vmem, hbm, hbm, hbm, hbm, hbm, hbm],
        out_specs=hbm,
        scratch_shapes=[
            V((M, S), bf16), V((M, S), bf16), V((M, S), bf16), V((M, S), bf16),
            V((M + 16, S), bf16), V((S + 16, DC), bf16),
            V((2, M * H, 128), bf16), V((2, 4, 128 * H + 16, 128), bf16), V((2, 4, 128 * H + 16, 128), bf16),
            V((H, M, D), bf16),
            V((H * 64, 7 * 256), u32), V((NT * 112, 7 * 128), u32), V((H * 256, 7 * 128), u32), V((H * 64, 7 * 512), u32),
            V((H * D // 2, S), u32), V((NT, 7, 64, 512), u32),
            V((M, S), f32), V((M, S), bf16), V((S, 2 * M), bf16),
            V((KS + 1, M, 128), f32), V((P, 2 * P), bf16), V((2 * P, P), bf16),
            V((1, NT, T, T), f32), V((1, NT, T, T), f32), V((1, 7, T, T), f32),
            V((1, 7, 112, 128), u32), V((1, 8, T), f32),
            V((1, NT, 8, T), f32), V((1, NT, 8, T), f32), V((1, NT, 8, T), f32), V((1, NT, 8, T), f32),
            pltpu.SemaphoreType.DMA((26,)), pltpu.SemaphoreType.DMA((8,)),
            pltpu.SemaphoreType.DMA((8,)), pltpu.SemaphoreType.DMA((9,)),
        ] + [V((64, 9 * 128), u32)] * NT + [V((64, 9 * 128), u32)] * NT + [V((1, 7, 128, 128), bf16)] * NT
        + [V((1, 4 * CH, 2 * P), f32)] * 4,
        compiler_params=pltpu.CompilerParams(vmem_limit_bytes=120 * 1024 * 1024,
                                             shape_invariant_numerics=False),
    )(
        A_q[0].T, A_k[0].T, A_v[0].T, A_shift_k.T, A_ssm_k, A_ssm_D,
        B_x[0].T, B_c_kv[0],
        B_w_q.reshape(M * H, D), B_w_uk.reshape(DC * H, D), B_w_uv.reshape(DC * H, D),
        jnp.transpose(B_w_o, (0, 2, 1)),
    )
    return out[None]
```

```python
import functools
import math

import jax
import jax.numpy as jnp
import jax.experimental.pallas as pl
import jax.experimental.pallas.tpu as pltpu

bf16 = jnp.bfloat16
f32 = jnp.float32
u32 = jnp.uint32

S = 2048
M = 448
DC = 1024
H = 16
D = 256
KS = 4
P = 128
NB = S // P
CH = 32
NCH = M // CH
T = 256
NT = S // T
NEG = -1e30
LAG_M = 0
LAG_S = 0
SORD = tuple(int(c) for c in '6430125')
SK = tuple(int(c) for c in '0364521')
SV = tuple(int(c) for c in '0364125')
SQ = tuple(int(c) for c in '3064125')
SP = tuple(int(c) for c in '0364125')
SO = tuple(int(c) for c in '0364125')
QW1 = 63
QW2 = 126
QW3 = 182
QLAG = 12
OS = 1
QKS = 1
CVMAX = 12
SIDE0 = 1
SIDEP = 3
LA = 2
SLAG = 2
APACE = 1
PROW = 0
PVS = 1
NOP = 3
L0 = 1
LEND = 4
LLAG = 2
EXR = 16
EX0 = 11
P0 = 1
VG = 1
QW4 = 207
VST = 0
ORD = 3
M3 = 0
IDL = 1
W7N = 2
W7P = 10
W7D = 3
ORDER = 'a'


def _nn(a, b):
    return jnp.dot(a, b, preferred_element_type=f32)


def _nt(a, b):
    return jax.lax.dot_general(a, b, (((1,), (1,)), ((), ())), preferred_element_type=f32)


def _b(u):
    return pltpu.bitcast(u, bf16)


def _u(x):
    return pltpu.bitcast(x, u32)


def _split_pair(u):
    lo = pltpu.bitcast(u << 16, f32).astype(bf16)
    hi = pltpu.bitcast(u & jnp.uint32(0xFFFF0000), f32).astype(bf16)
    return lo, hi


def _lo(u):
    return pltpu.bitcast(u << 16, f32)


def _hi(u):
    return pltpu.bitcast(u & jnp.uint32(0xFFFF0000), f32)


def _pk(e, o):
    return pltpu.pack_elementwise([e, o], packed_dtype=bf16)


def _a7(a11, a12, a21, a22):
    return [a11 + a22, a21 + a22, a11, a22, a11 + a12, a21 - a11, a12 - a22]


def _b7(b11, b12, b21, b22):
    return [b11 + b22, b11, b12 - b22, b21 - b11, b22, b11 + b12, b21 + b22]


def _c4(m):
    return m[0] + m[3] - m[4] + m[6], m[2] + m[4], m[1] + m[3], m[0] - m[1] + m[2] + m[5]


def _combos_u(f7, blk):
    e = f7(*[_lo(x) for x in blk])
    o = f7(*[_hi(x) for x in blk])
    plain = {2: 0, 3: 3} if f7 is _a7 else {1: 0, 4: 3}
    return [blk[plain[n]] if n in plain else _pk(e[n], o[n]) for n in range(7)]


def _quad(c11, c12, c21, c22):
    return jnp.concatenate([jnp.concatenate([c11, c12], axis=1), jnp.concatenate([c21, c22], axis=1)], axis=0)


def _fold(c, op):
    return op(c.reshape(-1, 8, c.shape[1]), axis=0)


def _rsum(p):
    cols = []
    for c in range(0, p.shape[1], 128):
        tot = None
        for k in range(0, p.shape[0], 128):
            acc = None
            for r in range(k + 112, k - 16, -16):
                t = p[r:r + 8, c:c + 128] + p[r + 8:r + 16, c:c + 128]
                acc = t if acc is None else acc + t
            tot = acc if tot is None else tot + acc
        cols.append(tot)
    return jnp.concatenate(cols, axis=1) if len(cols) > 1 else cols[0]


def _gate(x, vals):
    if not vals:
        return x
    w = max(v.shape[1] for v in vals)
    top = x[:8, :w]
    for v in vals:
        if v.shape[1] < w:
            v = jnp.concatenate([v] * (w // v.shape[1]), axis=1)
        top = jnp.where(v == jnp.inf, jnp.zeros_like(top), top)
    if w < x.shape[1]:
        top = jnp.concatenate([top, x[:8, w:]], axis=1)
    return jnp.concatenate([top, x[8:]], axis=0)


def _tok(vals):
    parts = []
    for v in vals:
        for r in range(0, v.shape[0], 8):
            for c in range(0, v.shape[1], 128):
                parts.append(v[r:r + 8, c:c + 128])
    while len(parts) > 1:
        parts = [parts[i] | parts[i + 1] if i + 1 < len(parts) else parts[i] for i in range(0, len(parts), 2)]
    return (parts[0] >> 31) >> 1


def _gate_u(x, tok):
    if tok is None:
        return x
    top = x[:8, :128] | tok
    if x.shape[1] > 128:
        top = jnp.concatenate([top, x[:8, 128:]], axis=1)
    return jnp.concatenate([top, x[8:]], axis=0)


def _ssm_pieces():
    ps = [('HD', 0), ('SC', 0), ('HD', 1), ('SC', 1), ('HD', 2), ('SC', 2), ('HD', 3), ('SC', 3)]
    cuts = [14 * k // W7N for k in range(W7N + 1)]
    for k in range(W7N):
        ps.insert(W7P + k * W7D, ('W7', cuts[k], cuts[k + 1]))
    if not OS:
        ps = [p for p in ps if p[0] != 'W7']
    cur, cost = [], 0
    for a in range(NB):
        for half in range(2):
            if cur and cost + a + 1 > CVMAX:
                ps.append(('CV', tuple(cur)))
                cur, cost = [], 0
            cur.append((a, half))
            cost += a + 1
        if a % 4 == 3:
            if cur:
                ps.append(('CV', tuple(cur)))
            cur, cost = [], 0
            ps.append(('ID', a // 4))
    return ps


def _schedule():
    side = _ssm_pieces()
    out = []
    cnt = [0]

    def block(units, att, ssm=True):
        k = 0
        for u in units:
            for t in range(7):
                out.append(u + (t,))
                out.extend(att.get(k, []))
                k += 1
                if ssm:
                    cnt[0] += 1
                    if side and cnt[0] >= SIDE0 and (cnt[0] - SIDE0) % SIDEP == 0:
                        out.append(side.pop(0))

    def softmax_head(i, n):
        att = {}
        att.setdefault(min(EX0, n - 2), []).extend(([('PACE',)] if P0 else []) + [('EX', i, 0)])
        if i > 0:
            att.setdefault(n - 1, []).extend([('PACE',), ('EX', i, 1)])
        return att

    block([('KP', 0)], {})
    block([('OP', NT - 1)], {6: [('AT',)]}, False)
    block([('VP', 0), ('KP', 1)], {13: [('QK', 0, 0)]})
    block([('VP', 1)], softmax_head(0, 7))
    for i in range(NT - 1):
        for j in range(i + 1):
            out.append(('QK', i + 1, j))
            if j + 2 <= i:
                out.append(('EX', i, j + 2))
            if j == i and not ORD & 1:
                out.append(('QK', i + 1, i + 1))
            out.append(('PV', i, j))
            if j == i and ORD & 1:
                out.append(('QK', i + 1, i + 1))
        if i + 2 < NT:
            block([('KP', i + 2), ('VP', i + 2)][::-1 if ORD & 2 else 1], softmax_head(i + 1, 14))
        else:
            block([('OP', n) for n in range(NOP)], softmax_head(i + 1, 7 * NOP), False)
            out.append(('PACE',))
    for j in range(NT):
        if j + 2 < NT:
            out.append(('EX', NT - 1, j + 2))
        out.append(('PV', NT - 1, j))
        if j + NOP < NT - 3:
            block([('OP', j + NOP)], {}, False)
        out.append(('PACE',))
    block([('OP', NT - 3), ('OP', NT - 2)], {}, False)
    assert not side
    if IDL:
        out.remove(('ID', 3))
        out.append(('ID', 3))
    return out


def _kernel(qT_hbm, kT_hbm, vT_hbm, sk_ref, ssmk_hbm, dd_ref, xT_hbm, ckv_hbm,
            wq_hbm, wk_hbm, wv_hbm, woT_hbm, out_hbm,
            qT, kT, vT, ssmk, xT, ckv, wq_raw, wk_raw, wv_raw, woT,
            aq_s, bx_s, bk_s, bvT_s, QT_s, a_s, acc, fullT, out_s, taps, ff_s, fi_s,
            S0_s, S1_s, X_s, W7_s, pace_s, m0_s, m1_s, l0_s, l1_s,
            sem, sem_k, sem_v, sem_o, *kvo):
    K_s, V_s, O_s, Y_s = kvo[:NT], kvo[NT:2 * NT], kvo[2 * NT:3 * NT], kvo[3 * NT:]
    def cp(src, dst, s):
        return pltpu.make_async_copy(src, dst, s)

    def c_x(j):
        cols = pl.ds(pl.multiple_of(j * 2 * T, 2 * T), 2 * T)
        return cp(xT_hbm.at[:, cols], xT.at[pl.ds(0, M), cols], sem.at[j])

    QP = ((0, 128), (128, 96))

    def c_wq(p):
        cs_ = []
        for half in range(2):
            r = pl.ds((half * 224 + QP[p][0]) * H, QP[p][1] * H)
            for g in range(2):
                cs_.append(cp(wq_hbm.at[r, pl.ds(128 * g, 128)], wq_raw.at[g, r], sem.at[18 + 4 * p + 2 * half + g]))
        return cs_


    def c_w(w_hbm, raw, sm, j, half, g):
        r = pl.ds(pl.multiple_of((half * 4 + j) * 2048, 2048), 2048)
        q = 2 * half + g
        return cp(w_hbm.at[r, pl.ds(128 * g, 128)], raw.at[j % 2, q, pl.ds(0, 2048)], sm.at[(j % 2) * 4 + q])

    def c_wk(j):
        return [c_w(wk_hbm, wk_raw, sem_k, j, half, g) for half in range(2) for g in range(2)]

    def c_wv(j):
        return [c_w(wv_hbm, wv_raw, sem_v, j, half, g) for half in range(2) for g in range(2)]

    def c_ckv(j):
        r = pl.ds(pl.multiple_of(j * 2 * T, 2 * T), 2 * T)
        return cp(ckv_hbm.at[r], ckv.at[r], sem.at[9 + j])

    a_pairs = ((kT_hbm, kT), (vT_hbm, vT), (ssmk_hbm, ssmk), (qT_hbm, qT))
    c_early = [cp(woT_hbm.at[pl.ds(0, 1)], woT.at[pl.ds(0, 1)], sem.at[4])]
    c_early += [cp(src.at[pl.ds(0, CH)], dst.at[pl.ds(0, CH)], sem.at[5 + n]) for n, (src, dst) in enumerate(a_pairs)]
    c_late = [cp(woT_hbm.at[pl.ds(1, H - 1)], woT.at[pl.ds(1, H - 1)], sem.at[13])]
    c_late += [cp(src.at[pl.ds(CH, M - CH)], dst.at[pl.ds(CH, M - CH)], sem.at[14 + n])
               for n, (src, dst) in enumerate(a_pairs)]
    for c in [c_x(0)] + c_wq(0) + c_wq(1):
        c.start()
    for c in c_wk(0) + [c_x(1)]:
        c.start(priority=1)

    n_i = jax.lax.broadcasted_iota(jnp.int32, (P, P), 0)
    k_i = jax.lax.broadcasted_iota(jnp.int32, (P, P), 1)
    ang = (((2 * k_i + 1) * n_i) & 511).astype(f32) * (math.pi / 256.0)
    cs, sn = jnp.cos(ang), jnp.sin(ang)
    ff_s[:, 0:P] = cs.astype(bf16)
    ff_s[:, P:2 * P] = (-sn).astype(bf16)
    fi_s[0:P, :] = (cs.T * (1.0 / P)).astype(bf16)
    fi_s[P:2 * P, :] = (sn.T * (-1.0 / P)).astype(bf16)
    sk = sk_ref[...].astype(f32)
    for t in range(KS):
        taps[t] = jnp.broadcast_to(sk[t:t + 1, :], (128, M)).T
    taps[KS] = jnp.broadcast_to(dd_ref[...].astype(f32).reshape(1, M), (128, M)).T
    acc[...] = jnp.zeros(acc.shape, f32)
    fullT[...] = jnp.zeros(fullT.shape, bf16)
    O_s[NT - 1][...] = jnp.zeros(O_s[0].shape, bf16)
    W7_s[...] = jnp.zeros(W7_s.shape, u32)

    def prep_x(jj, t, r0):
        c0 = (2 * jj + t) * T
        cs_ = [c0, c0 + 128] if isinstance(jj, int) else [pl.multiple_of(c0, 128), pl.multiple_of(c0 + 128, 128)]
        blk = [_u(xT[r:r + 32, pl.ds(c, 128)]) for r in (r0, 224 + r0) for c in cs_]
        row = (2 * jj + t) * 112 + r0 // 2
        row = pl.ds(row if isinstance(jj, int) else pl.multiple_of(row, 16), 16)
        for n, x in enumerate(_combos_u(_b7, blk)):
            bx_s[row, n * 128:(n + 1) * 128] = x
        return []

    c_x(0).wait()
    for t in range(2):
        for r0 in range(0, 224, 32):
            prep_x(0, t, r0)
    vq = wq_raw.bitcast(u32)
    for p, (c0, nc) in enumerate(QP):
        for c in c_wq(p):
            c.wait()
        if p == 1 and VST:
            for c in c_wv(0) + [c_ckv(0)]:
                c.start(priority=1)
        for hp in range(0 if 0 else H // 2):
            ut = [vq[g, pl.ds((half * 224 + c0) * 8 + hp, nc, stride=8), :].T for g in range(2) for half in range(2)]
            for r in range(0, 128, 16):
                u = [x[r:r + 16] for x in ut]
                for par, f in enumerate((_lo, _hi)):
                    r0 = (2 * hp + par) * 64 + r // 2
                    for n, x in enumerate(_a7(*[f(x) for x in u])):
                        aq_s[r0:r0 + 8, n * 256 + c0:n * 256 + c0 + nc] = _u(x.astype(bf16))
    if not VST:
        for c in c_wv(0) + [c_ckv(0)]:
            c.start(priority=1)

    qscale = (D ** -0.5) * math.log2(math.e)

    def lo(u):
        return pltpu.bitcast(u << 16, f32)

    def hi(u):
        return pltpu.bitcast(u & jnp.uint32(0xFFFF0000), f32)

    def b_combos(b11, b12, b21, b22):
        return [b11 + b22, b11, b12 - b22, b21 - b11, b22, b11 + b12, b21 + b22]

    def q_body(j, carry):
        mq = {}

        bx = [[bx_s[pl.ds(pl.multiple_of((2 * j + t) * 112, 16), 112), n * 128:(n + 1) * 128] for n in range(7)]
              for t in range(2)]

        def qproj(u, tok):
            hh, t, n = u // 14, (u // 7) % 2, SORD[u % 7]
            w = _b(_gate_u(aq_s[hh * 64:hh * 64 + 64, n * 256:n * 256 + 224], tok))
            mq[n] = _nn(w, _b(bx[t][n]))
            if u % 7 == 6:
                for k, x in enumerate(_c4(mq)):
                    cols = pl.ds(pl.multiple_of((2 * j + t) * T + (k % 2) * 128, 128), 128)
                    r0 = hh * 128 + (k // 2) * 64
                    QT_s[r0:r0 + 64, cols] = _u((x * qscale).astype(bf16))
            return mq[n]

        def prep_k(hp, part):
            v = wk_raw.bitcast(u32).at[j % 2]
            u = [v[q, pl.ds(part * 128 + hp, 16, stride=8), :] for q in range(4)]
            for par, f in enumerate((_lo, _hi)):
                for n, c in enumerate(_b7(*[f(x) for x in u])):
                    r = _u(c.astype(bf16))
                    r0 = (2 * hp + par) * 256 + part * 8
                    bk_s[pl.ds(pl.multiple_of(j * 64 + r0, 8), 8), n * 128:(n + 1) * 128] = r
            return []

        vt = {}

        def prep_v(hp, part):
            if part == 0:
                v = wv_raw.bitcast(u32).at[j % 2]
                vt[hp] = [v[q, pl.ds(hp, 128, stride=8), :].T for q in range(4)]
                return [x[120:] for x in vt[hp]] if VG else []
            for r in range(32 * (part - 1), 32 * part, 16):
                u = [x[r:r + 16] for x in vt[hp]]
                for par, f in enumerate((_lo, _hi)):
                    r0 = (2 * hp + par) * 64 + r // 2
                    for n, c in enumerate(_b7(*[f(x) for x in u])):
                        cols = pl.ds(pl.multiple_of(n * 512 + j * 128, 128), 128)
                        bvT_s[r0:r0 + 8, cols] = _u(c.astype(bf16))
            return []

        def prep_a(cl_, part, cbs):
            c = 2 * j + cl_
            r0 = 8 * part
            rt = pl.ds(pl.multiple_of(c * T + 2 * r0, 16), 16)
            rb = pl.ds(pl.multiple_of(c * T + 128 + 2 * r0, 16), 16)
            res = []
            for cb in cbs:
                cl, ch_ = slice(cb * 128, cb * 128 + 128), slice(512 + cb * 128, 512 + cb * 128 + 128)
                blk = [_u(ckv[rt, cl]), _u(ckv[rt, ch_]), _u(ckv[rb, cl]), _u(ckv[rb, ch_])]
                cc = []
                for f in (lo, hi):
                    a11, a12, a21, a22 = [f(x) for x in blk]
                    cc.append([a11 + a22, a21 + a22, None, None, a11 + a12, a21 - a11, a12 - a22])
                for n in range(7):
                    if n == 2:
                        r = blk[0]
                    elif n == 3:
                        r = blk[3]
                    else:
                        r = pltpu.pack_elementwise([cc[0][n], cc[1][n]], packed_dtype=bf16)
                    a_s[c, n, r0:r0 + 8, cl] = r
                    res.append(r)
            return [] if APACE else res

        fill = {}

        def spread(pieces, u0, u1):
            for n, p in enumerate(pieces):
                fill.setdefault(u0 + n * (u1 - u0) // len(pieces), []).append(p)

        spread([functools.partial(prep_k, hp, part) for hp in range(8) for part in range(8)], QW1, QW2)
        spread([functools.partial(prep_v, hp, part) for hp in range(8) for part in range(5)], QW2, QW3)
        spread([functools.partial(prep_a, c, part, cbs) for c in range(2) for part in range(8)
                for cbs in ((0, 1), (2, 3))], QW3, QW4)
        spread([functools.partial(prep_x, jnp.minimum(j + 1, 3), t, r0) for t in range(2) for r0 in range(0, 224, 32)], QW4, 221)
        toks = {}
        for u in range(224):
            if u == QW1:
                @pl.when(j < 3)
                def _():
                    for c in c_wk(j + 1):
                        c.start(priority=1)

                @pl.when(j == 3)
                def _():
                    for c in c_early + c_late:
                        c.start(priority=1)

                for c in c_wk(j):
                    c.wait()
            if u == QW2:
                @pl.when(j < 3)
                def _():
                    for c in c_wv(j + 1) + [c_ckv(j + 1)]:
                        c.start(priority=1)

                @pl.when(j < 2)
                def _():
                    c_x(j + 2).start(priority=1)

                @pl.when(j < 3)
                def _():
                    c_x(j + 1).wait()

                for c in c_wv(j) + [c_ckv(j)]:
                    c.wait()
            q = qproj(u, toks.pop(u, None))
            res = []
            ps = fill.get(u, [])
            for n, p in enumerate(ps):
                row = (n * 128 // len(ps)) // 16 * 16
                if p.func is prep_k:
                    wk_raw.bitcast(u32)[j >> 4, 0, 1024:1032, :] = pltpu.bitcast(q[row:row + 8], u32)
                elif p.func is prep_v and p.args[1] == 0:
                    wv_raw.bitcast(u32)[j >> 4, 0, 1024:1032, :] = pltpu.bitcast(q[row:row + 8], u32)
                elif p.func is prep_x:
                    xT[pl.ds(pl.multiple_of(M + (j >> 4) * 16, 16), 16), 0:128] = q[row:row + 16].astype(bf16)
                elif p.func is prep_a:
                    ckv[pl.ds(pl.multiple_of(S + (j >> 4) * 16, 16), 16), 0:128] = q[row:row + 16].astype(bf16)
                res += p()
            if res:
                toks[u + QLAG] = _tok(res)
        return carry

    if not 0:
        jax.lax.fori_loop(0, 4, q_body, 0)
    for c in c_early:
        c.wait()

    tri = n_i <= k_i
    sgn = jnp.where((jax.lax.broadcasted_iota(jnp.int32, (1, P), 1) & 1) == 0, 1.0, -1.0).astype(f32)

    c_outa = cp(out_s.at[:, pl.ds(0, 384)], out_hbm.at[:, pl.ds(0, 384)], sem_o.at[8])

    HR, HI, PR, PI, KV, HS, PS = range(7)

    def zrow(z, n):
        return pl.ds(0, n) if isinstance(z, int) else pl.ds(pl.multiple_of(z * n, n), n)

    def blk_at(c, half=None):
        r0 = (c % 8) * CH
        rs = slice(r0, r0 + CH) if half is None else slice(r0 + 16 * half, r0 + 16 * half + 16)
        return rs, slice((c // 8) * P, (c // 8 + 1) * P)

    def head_body(h, carry):
        @pl.when(h == 1)
        def _():
            for c in c_late:
                c.wait()

        @pl.when(h == H - 1)
        def _():
            c_outa.start()

        st = dict(l={}, M={}, P={}, Q7={}, mfin={}, o={})
        zs, zl = h >> 10, 0
        m_s, l_s = (m0_s, m1_s), (l0_s, l1_s)
        qrows = pl.ds(pl.multiple_of(h * 128, 128), 128)
        rows = pl.ds(pl.multiple_of(jnp.minimum(h, NCH - 1) * CH, CH), CH)

        def rep(t, n):
            return jnp.concatenate([taps[t, rows, :]] * n, axis=1)

        toks = []

        def due():
            for t in toks:
                t[0] -= 1
            ready = [t[1] for t in toks if t[0] <= 0]
            toks[:] = [t for t in toks if t[0] > 0]
            return functools.reduce(lambda x, y: x | y, ready) if ready else None

        def gate_later(vals, lag=SLAG):
            toks.append([lag, _tok([v if v.dtype == u32 else pltpu.bitcast(v, u32) for v in vals])])

        def row_max(i):
            if i not in st['mfin']:
                m = m_s[i % 2][zl, 0]
                for t in range(1, i + 1):
                    m = jnp.maximum(m, m_s[i % 2][zl, t])
                m = jnp.max(m, axis=0, keepdims=True)
                if PVS and i > 0:
                    lo_ = jnp.exp2(m_s[i % 2][zl, 0] - m)
                    for t in range(1, i + 1):
                        lo_ = lo_ + jnp.exp2(m_s[i % 2][zl, t] - m)
                    m = m + jnp.log2(jnp.sum(lo_, axis=0, keepdims=True))
                st['mfin'][i] = m
            return st['mfin'][i]

        for op in _schedule():
            kind = op[0]
            if kind == 'KP':
                _, c, t = op
                n = SK[t]
                st['M'][n] = st['last'] = _nn(_b(_gate_u(a_s[c, n], due())), _b(bk_s[pl.ds(pl.multiple_of(h * 256, 256), 256), n * 128:(n + 1) * 128]))
                if t == 6:
                    c4 = _c4(st['M'])
                    blks = dict(zip((2, 7, 8, 3), c4))
                    if QKS and c < NT - 1:
                        blks.update({n: x for n, x in enumerate(_a7(*c4)) if n not in (2, 3)})
                    for n, x in blks.items():
                        K_s[c][zrow(zs, 64), n * 128:(n + 1) * 128] = _u(x.astype(bf16))
            elif kind == 'VP':
                _, c, t = op
                n = SV[t]
                st['M'][n] = st['last'] = _nt(_b(_gate_u(bvT_s[pl.ds(pl.multiple_of(h * 64, 64), 64), n * 512:(n + 1) * 512], due())), _b(a_s[c, n]))
                if t == 6:
                    c11, c12, c21, c22 = _c4(st['M'])
                    c4 = (c11, c21, c12, c22)
                    blks = dict(zip((2, 7, 8, 3), c4))
                    if PVS and c < NT - 1:
                        blks.update({n: x for n, x in enumerate(_a7(*c4)) if n not in (2, 3)})
                    for n, x in blks.items():
                        V_s[c][zrow(zs, 64), n * 128:(n + 1) * 128] = _u(x.astype(bf16))
            elif kind == 'QK':
                _, i, j = op
                S_s = (S0_s, S1_s)[i % 2]
                qu = QT_s[qrows, i * T:(i + 1) * T]
                if j < i:
                    if QKS:
                        if i not in st['Q7']:
                            st['Q7'][i] = _combos_u(_b7, [qu[:64, :128], qu[:64, 128:], qu[64:, :128], qu[64:, 128:]])
                        m = {n: _nn(_b(K_s[j][zrow(zl, 64), n * 128:(n + 1) * 128]), _b(st['Q7'][i][n])) for n in SQ}
                        s = _quad(*_c4(m))
                    else:
                        s = _nn(_b(_quad(*[K_s[j][zrow(zl, 64), n * 128:(n + 1) * 128] for n in (2, 7, 8, 3)])), _b(qu))
                    S_s[zs, j] = s
                    f = _fold(s, jnp.max)
                else:
                    q = _b(qu)
                    sa = _nn(_b(jnp.concatenate([K_s[j][zrow(zl, 64), 2 * 128:(2 + 1) * 128], K_s[j][zrow(zl, 64), 7 * 128:(7 + 1) * 128]], axis=1)), q)
                    sa = jnp.concatenate([jnp.where(tri, sa[:, :128], NEG), sa[:, 128:]], axis=1)
                    sb = _nn(_b(jnp.concatenate([K_s[j][zrow(zl, 64), 8 * 128:(8 + 1) * 128], K_s[j][zrow(zl, 64), 3 * 128:(3 + 1) * 128]], axis=1)), q[:, 128:])
                    sb = jnp.where(tri, sb, NEG)
                    S_s[zs, j, 0:128, :] = sa
                    S_s[zs, j, 128:T, 128:T] = sb
                    fa = _fold(sa, jnp.max)
                    f = jnp.concatenate([fa[:, :128], jnp.maximum(fa[:, 128:], _fold(sb, jnp.max))], axis=1)
                m_s[i % 2][zs, j] = f
                pace_s[zs] = f
            elif kind == 'EX':
                _, i, j = op
                S_s = (S0_s, S1_s)[i % 2]
                m = row_max(i)
                if j > 0 or P0:
                    m = jnp.where(pace_s[zl, 0:1, :] == jnp.inf, jnp.inf, m)
                if j < i:
                    if PVS:
                        parts, lj = [], None
                        for r in range(112, -16, -16):
                            pt = jnp.exp2(S_s[zl, j, r:r + 16, :] - m)
                            pb = jnp.exp2(S_s[zl, j, 128 + r:128 + r + 16, :] - m)
                            parts.insert(0, _b7(pt[:, :128], pt[:, 128:], pb[:, :128], pb[:, 128:]))
                            x = (pt[:8] + pt[8:]) + (pb[:8] + pb[8:])
                            lj = x if lj is None else lj + x
                        st['P'][i, j] = [jnp.concatenate([x[n] for x in parts], axis=0).astype(bf16) for n in range(7)]
                    else:
                        p = jnp.exp2(S_s[zl, j] - m)
                        lj = _rsum(p)
                        st['P'][i, j] = p.astype(bf16)
                else:
                    pa = jnp.exp2(S_s[zl, j, 0:128, :] - m)
                    pb = jnp.exp2(S_s[zl, j, 128:T, 128:T] - m[:, 128:])
                    la = _rsum(pa)
                    lj = jnp.concatenate([la[:, :128], la[:, 128:] + _rsum(pb)], axis=1)
                    st['P'][i, j] = (pa.astype(bf16), pb.astype(bf16))
                l_s[i % 2][zs, j] = lj
            elif kind == 'PV':
                _, i, j = op
                vb = [V_s[j][zrow(zl, 64), n * 128:(n + 1) * 128] for n in range(9)]
                p = st['P'].pop((i, j))
                if j < i and PVS:
                    for n in SP:
                        st['last'] = _nn(_b(vb[n]), p[n])
                        st['o'][i, n] = st['last'] if j == 0 else st['o'][i, n] + st['last']
                    continue
                if j < i:
                    o = _nn(_b(_quad(vb[2], vb[7], vb[8], vb[3])), p)
                else:
                    oa = _nn(_b(jnp.concatenate([vb[2], vb[8]], axis=0)), p[0])
                    ob = _nn(_b(jnp.concatenate([vb[7], vb[3]], axis=0)), p[1])
                    o = jnp.concatenate([oa[:, :128], oa[:, 128:] + ob], axis=1)
                st['last'] = o
                if PVS:
                    if i > 0:
                        o = o + _quad(*_c4({n: st['o'].pop((i, n)) for n in range(7)}))
                else:
                    o = o if j == 0 else st['o'][i] + o
                    st['o'][i] = o
                if j == i:
                    l = l_s[i % 2][zl, 0]
                    for t in range(1, i + 1):
                        l = l + l_s[i % 2][zl, t]
                    o = o * (1.0 / jnp.sum(l, axis=0, keepdims=True))
                    blks = (o[:128, :128], o[:128, 128:], o[128:, :128], o[128:, 128:])
                    for n, x in enumerate(_b7(*blks)):
                        O_s[i][zs, n] = x.astype(bf16)
            elif kind == 'PACE':
                pace_s[zs] = jnp.concatenate([st['last'][-8:, -128:]] * 2, axis=1)
            elif kind == 'OP':
                _, i, t = op
                n = SO[t]
                st['M'][n] = st['last'] = _nn(_b(_gate_u(W7_s[0, n], due())), O_s[i][0, n])
                if t == 6:
                    acc[:, T * i:T * (i + 1)] += _quad(*_c4(st['M']))
            elif kind == 'W7':
                res = []
                for r0 in range(16 * op[1], 16 * op[2], 16):
                    blk = [_u(woT[h, r:r + 16, c:c + 128]) for r in (r0, 224 + r0) for c in (0, 128)]
                    w7 = _combos_u(_a7, blk)
                    for n, x in enumerate(w7):
                        W7_s[zs, n, r0 // 2:r0 // 2 + 8] = x
                    res += w7
                gate_later(res)
            elif kind == 'AT':
                g = jnp.clip((h - 4) // 4, 0, 2)
                t0 = jnp.minimum(((h + 12) % 4) * 6, NB - 6)
                grow = pl.ds(pl.multiple_of(g * 128, 128), 128)
                gcol = pl.ds(pl.multiple_of(jnp.where(h == H - 1, 3, g) * 128, 128), 128)
                res = []
                for n in range(6):
                    tok = pl.ds(pl.multiple_of((t0 + n) * 128, 128), 128)
                    x = fullT[grow, tok].T
                    out_s[tok, gcol] = x
                    res.append(_u(x)[56:])
                gate_later(res)
            elif kind == 'HD':
                g = op[1]
                hs = jnp.concatenate([ssmk[rows, c * P:(c + 1) * P] for c in range(4 * g, 4 * g + 4)], axis=0)
                hf = _nn(hs, ff_s[...])
                for n in range(4):
                    X_s[(zs, HR) + blk_at(4 * g + n)] = hf[n * CH:(n + 1) * CH, :P]
                    X_s[(zs, HI) + blk_at(4 * g + n)] = hf[n * CH:(n + 1) * CH, P:]
                    if M3:
                        X_s[(zs, HS) + blk_at(4 * g + n)] = hf[n * CH:(n + 1) * CH, :P] + hf[n * CH:(n + 1) * CH, P:]
            elif kind == 'SC':
                g = op[1]
                if g == 0:
                    k = jnp.concatenate([jnp.zeros((CH, P), f32), kT[rows, 0:4 * P].astype(f32)], axis=1)
                else:
                    k = kT[rows, (4 * g - 1) * P:(4 * g + 4) * P].astype(f32)
                ks = k[:, P:] * rep(0, 4)
                for j in range(1, KS):
                    ks = ks + pltpu.roll(k, j, 1)[:, P:] * rep(j, 4)
                kv = ks * vT[rows, 4 * g * P:(4 * g + 4) * P].astype(f32)
                kvs = jnp.concatenate([kv[:, n * P:(n + 1) * P] for n in range(4)], axis=0)
                xf = _nn(kvs.astype(bf16), ff_s[...])
                for n in range(4):
                    c = 4 * g + n
                    xr, xi = xf[n * CH:(n + 1) * CH, :P], xf[n * CH:(n + 1) * CH, P:]
                    X_s[(zs, KV) + blk_at(c)] = kvs[n * CH:(n + 1) * CH]
                    pr = xr if c == 0 else xr - sgn * st['x'][1]
                    pi = xi if c == 0 else xi + sgn * st['x'][0]
                    X_s[(zs, PR) + blk_at(c)] = pr
                    if M3:
                        X_s[(zs, PI) + blk_at(c)] = pi - pr
                        X_s[(zs, PS) + blk_at(c)] = pi + pr
                    else:
                        X_s[(zs, PI) + blk_at(c)] = pi
                    st['x'] = (xr, xi)
            elif kind == 'CV':
                res = []
                for a, half in op[1]:
                    wr = wi = None
                    k123 = None
                    for j in range(a + 1 if M3 else 0):
                        t = [X_s[(zl, u) + blk_at(j, half)] * X_s[(zl, v) + blk_at(a - j, half)]
                             for u, v in ((HS, PR), (HR, PI), (HI, PS))]
                        k123 = t if k123 is None else [x + y for x, y in zip(k123, t)]
                    if M3:
                        wr, wi = k123[0] - k123[2], k123[0] + k123[1]
                    for j in range(0 if M3 else a + 1):
                        hr, hi_ = X_s[(zl, HR) + blk_at(j, half)], X_s[(zl, HI) + blk_at(j, half)]
                        pr, pi = X_s[(zl, PR) + blk_at(a - j, half)], X_s[(zl, PI) + blk_at(a - j, half)]
                        tr, ti = hr * pr - hi_ * pi, hr * pi + hi_ * pr
                        wr, wi = (tr, ti) if wr is None else (wr + tr, wi + ti)
                    r0 = (a % 4) * CH + 16 * half
                    Y_s[a // 4][zs, r0:r0 + 16, :P] = wr
                    Y_s[a // 4][zs, r0:r0 + 16, P:] = wi
                    res += [wr, wi]
                gate_later(res)
            elif kind == 'ID':
                g = op[1]
                w = Y_s[g][0]
                y = _nn(w.astype(bf16), fi_s[...])
                for n in range(4):
                    c = 4 * g + n
                    cols = slice(c * P, (c + 1) * P)
                    ya = y[n * CH:(n + 1) * CH, :] + X_s[(zl, KV) + blk_at(c)] * taps[KS, rows, :]
                    fullT[rows, cols] = (qT[rows, cols].astype(f32) * ya).astype(bf16)
        return carry

    if not 0:
        jax.lax.fori_loop(0, H, head_body, 0)

    acc[:, T * (NT - 1):] += _quad(*_c4({n: _nn(_b(W7_s[0, n]), O_s[NT - 1][0, n]) for n in SORD}))
    outs = [c_outa]
    for i in range(NT):
        cols = slice(T * i, T * (i + 1))
        blk = jnp.concatenate([fullT[384:M, cols], acc[:, cols].astype(bf16)], axis=0)
        out_s[cols, 384:2 * M] = blk.T
        c = cp(out_s.at[pl.ds(T * i, T), pl.ds(384, 512)], out_hbm.at[pl.ds(T * i, T), pl.ds(384, 512)], sem_o.at[i])
        c.start()
        outs.append(c)
    for c in outs:
        c.wait()


@jax.jit
def pallas_concat_heads__ssm_conv_h3__compressed_kv_cla__prompt_kernel(
    A_q: jax.Array,
    A_k: jax.Array,
    A_v: jax.Array,
    A_shift_k: jax.Array,
    A_ssm_k: jax.Array,
    A_ssm_D: jax.Array,
    B_x: jax.Array,
    B_c_kv: jax.Array,
    B_w_q: jax.Array,
    B_w_uk: jax.Array,
    B_w_uv: jax.Array,
    B_w_o: jax.Array,
):
    hbm = pl.BlockSpec(memory_space=pl.ANY)
    vmem = pl.BlockSpec(memory_space=pltpu.VMEM)
    V = pltpu.VMEM
    out = pl.pallas_call(
        _kernel,
        out_shape=jax.ShapeDtypeStruct((S, 2 * M), bf16),
        in_specs=[hbm, hbm, hbm, vmem, hbm, vmem, hbm, hbm, hbm, hbm, hbm, hbm],
        out_specs=hbm,
        scratch_shapes=[
            V((M, S), bf16), V((M, S), bf16), V((M, S), bf16), V((M, S), bf16),
            V((M + 16, S), bf16), V((S + 16, DC), bf16),
            V((2, M * H, 128), bf16), V((2, 4, 128 * H + 16, 128), bf16), V((2, 4, 128 * H + 16, 128), bf16),
            V((H, M, D), bf16),
            V((H * 64, 7 * 256), u32), V((NT * 112, 7 * 128), u32), V((H * 256, 7 * 128), u32), V((H * 64, 7 * 512), u32),
            V((H * D // 2, S), u32), V((NT, 7, 64, 512), u32),
            V((M, S), f32), V((M, S), bf16), V((S, 2 * M), bf16),
            V((KS + 1, M, 128), f32), V((P, 2 * P), bf16), V((2 * P, P), bf16),
            V((1, NT, T, T), f32), V((1, NT, T, T), f32), V((1, 7, T, T), f32),
            V((1, 7, 112, 128), u32), V((1, 8, T), f32),
            V((1, NT, 8, T), f32), V((1, NT, 8, T), f32), V((1, NT, 8, T), f32), V((1, NT, 8, T), f32),
            pltpu.SemaphoreType.DMA((26,)), pltpu.SemaphoreType.DMA((8,)),
            pltpu.SemaphoreType.DMA((8,)), pltpu.SemaphoreType.DMA((9,)),
        ] + [V((64, 9 * 128), u32)] * NT + [V((64, 9 * 128), u32)] * NT + [V((1, 7, 128, 128), bf16)] * NT
        + [V((1, 4 * CH, 2 * P), f32)] * 4,
        compiler_params=pltpu.CompilerParams(vmem_limit_bytes=120 * 1024 * 1024,
                                             shape_invariant_numerics=False),
    )(
        A_q[0].T, A_k[0].T, A_v[0].T, A_shift_k.T, A_ssm_k, A_ssm_D,
        B_x[0].T, B_c_kv[0],
        B_w_q.reshape(M * H, D), B_w_uk.reshape(DC * H, D), B_w_uv.reshape(DC * H, D),
        jnp.transpose(B_w_o, (0, 2, 1)),
    )
    return out[None]
```

```python
import functools
import math

import jax
import jax.numpy as jnp
import jax.experimental.pallas as pl
import jax.experimental.pallas.tpu as pltpu

bf16 = jnp.bfloat16
f32 = jnp.float32
u32 = jnp.uint32

S = 2048
M = 448
DC = 1024
H = 16
D = 256
KS = 4
P = 128
NB = S // P
CH = 32
NCH = M // CH
T = 256
NT = S // T
NEG = -1e30
LAG_M = 0
LAG_S = 0
SORD = tuple(int(c) for c in '6430125')
SK = tuple(int(c) for c in '0364521')
SV = tuple(int(c) for c in '4603125')
SQ = tuple(int(c) for c in '6043125')
SP = tuple(int(c) for c in '3640125')
SO = tuple(int(c) for c in '5210346')
QW1 = 70
QW2 = 126
QW3 = 188
QLAG = 12
OS = 1
QKS = 1
CVMAX = 12
SIDE0 = 1
SIDEP = 3
LA = 2
SLAG = 1
APACE = 1
PROW = 0
PVS = 1
NOP = 3
L0 = 1
LEND = 4
LLAG = 2
EXR = 16
EX0 = 11
P0 = 1
VG = 1
QW4 = 211
VST = 0
ORD = 3
M3 = 0
IDL = 1
W7N = 2
W7P = 16
W7D = 3
ILV = 0
PV2 = 0
ORDER = 'a'


def _nn(a, b):
    return jnp.dot(a, b, preferred_element_type=f32)


def _nt(a, b):
    return jax.lax.dot_general(a, b, (((1,), (1,)), ((), ())), preferred_element_type=f32)


def _b(u):
    return pltpu.bitcast(u, bf16)


def _u(x):
    return pltpu.bitcast(x, u32)


def _split_pair(u):
    lo = pltpu.bitcast(u << 16, f32).astype(bf16)
    hi = pltpu.bitcast(u & jnp.uint32(0xFFFF0000), f32).astype(bf16)
    return lo, hi


def _lo(u):
    return pltpu.bitcast(u << 16, f32)


def _hi(u):
    return pltpu.bitcast(u & jnp.uint32(0xFFFF0000), f32)


def _pk(e, o):
    return pltpu.pack_elementwise([e, o], packed_dtype=bf16)


def _a7(a11, a12, a21, a22):
    return [a11 + a22, a21 + a22, a11, a22, a11 + a12, a21 - a11, a12 - a22]


def _b7(b11, b12, b21, b22):
    return [b11 + b22, b11, b12 - b22, b21 - b11, b22, b11 + b12, b21 + b22]


def _c4(m):
    return m[0] + m[3] - m[4] + m[6], m[2] + m[4], m[1] + m[3], m[0] - m[1] + m[2] + m[5]


def _combos_u(f7, blk):
    e = f7(*[_lo(x) for x in blk])
    o = f7(*[_hi(x) for x in blk])
    plain = {2: 0, 3: 3} if f7 is _a7 else {1: 0, 4: 3}
    return [blk[plain[n]] if n in plain else _pk(e[n], o[n]) for n in range(7)]


def _quad(c11, c12, c21, c22):
    return jnp.concatenate([jnp.concatenate([c11, c12], axis=1), jnp.concatenate([c21, c22], axis=1)], axis=0)


def _fold(c, op):
    return op(c.reshape(-1, 8, c.shape[1]), axis=0)


def _rsum(p):
    cols = []
    for c in range(0, p.shape[1], 128):
        tot = None
        for k in range(0, p.shape[0], 128):
            acc = None
            for r in range(k + 112, k - 16, -16):
                t = p[r:r + 8, c:c + 128] + p[r + 8:r + 16, c:c + 128]
                acc = t if acc is None else acc + t
            tot = acc if tot is None else tot + acc
        cols.append(tot)
    return jnp.concatenate(cols, axis=1) if len(cols) > 1 else cols[0]


def _gate(x, vals):
    if not vals:
        return x
    w = max(v.shape[1] for v in vals)
    top = x[:8, :w]
    for v in vals:
        if v.shape[1] < w:
            v = jnp.concatenate([v] * (w // v.shape[1]), axis=1)
        top = jnp.where(v == jnp.inf, jnp.zeros_like(top), top)
    if w < x.shape[1]:
        top = jnp.concatenate([top, x[:8, w:]], axis=1)
    return jnp.concatenate([top, x[8:]], axis=0)


def _tok(vals):
    parts = []
    for v in vals:
        for r in range(0, v.shape[0], 8):
            for c in range(0, v.shape[1], 128):
                parts.append(v[r:r + 8, c:c + 128])
    while len(parts) > 1:
        parts = [parts[i] | parts[i + 1] if i + 1 < len(parts) else parts[i] for i in range(0, len(parts), 2)]
    return (parts[0] >> 31) >> 1


def _gate_u(x, tok):
    if tok is None:
        return x
    top = x[:8, :128] | tok
    if x.shape[1] > 128:
        top = jnp.concatenate([top, x[:8, 128:]], axis=1)
    return jnp.concatenate([top, x[8:]], axis=0)


def _ssm_pieces():
    ps = [('HD', 0), ('SC', 0), ('HD', 1), ('SC', 1), ('HD', 2), ('SC', 2), ('HD', 3), ('SC', 3)]
    cuts = [14 * k // W7N for k in range(W7N + 1)]
    for k in range(W7N):
        ps.insert(W7P + k * W7D, ('W7', cuts[k], cuts[k + 1]))
    if not OS:
        ps = [p for p in ps if p[0] != 'W7']
    cur, cost = [], 0
    for a in range(NB):
        for half in range(2):
            if cur and cost + a + 1 > CVMAX:
                ps.append(('CV', tuple(cur)))
                cur, cost = [], 0
            cur.append((a, half))
            cost += a + 1
        if a % 4 == 3:
            if cur:
                ps.append(('CV', tuple(cur)))
            cur, cost = [], 0
            ps.append(('ID', a // 4))
    return ps


def _schedule():
    side = _ssm_pieces()
    out = []
    cnt = [0]

    def block(units, att, ssm=True):
        k = 0
        for u in units:
            for t in range(7):
                out.append(u + (t,))
                out.extend(att.get(k, []))
                k += 1
                if ssm:
                    cnt[0] += 1
                    if side and cnt[0] >= SIDE0 and (cnt[0] - SIDE0) % SIDEP == 0:
                        out.append(side.pop(0))

    def softmax_head(i, n):
        att = {}
        att.setdefault(min(EX0, n - 2), []).extend(([('PACE',)] if P0 else []) + [('EX', i, 0)])
        if i > 0:
            att.setdefault(n - 1, []).extend([('PACE',), ('EX', i, 1)])
        return att

    block([('KP', 0)], {})
    block([('OP', NT - 1)], {6: [('AT',)]}, False)
    block([('VP', 0), ('KP', 1)], {13: [('QK', 0, 0)]})
    block([('VP', 1)], softmax_head(0, 7))
    for i in range(NT - 1):
        for j in range(i + 1):
            if ILV and j < i:
                for a, b in ((0, 4), (4, 7)) if ILV == 1 else ((0, 2), (2, 4), (4, 6), (6, 7)):
                    out.append(('QK', i + 1, j, a, b))
                    if b == 7 and j + 2 <= i:
                        out.append(('EX', i, j + 2))
                    out.append(('PV', i, j, a, b))
                continue
            out.append(('QK', i + 1, j))
            if j + 2 <= i:
                out.append(('EX', i, j + 2))
            if j == i and not ORD & 1:
                out.append(('QK', i + 1, i + 1))
            out.append(('PV', i, j))
            if j == i and ORD & 1:
                out.append(('QK', i + 1, i + 1))
        if i + 2 < NT:
            block([('KP', i + 2), ('VP', i + 2)][::-1 if ORD & 2 else 1], softmax_head(i + 1, 14))
        else:
            block([('OP', n) for n in range(NOP)], softmax_head(i + 1, 7 * NOP), False)
            out.append(('PACE',))
    for j in range(NT):
        if j + 2 < NT:
            out.append(('EX', NT - 1, j + 2))
        out.append(('PV', NT - 1, j))
        if j + NOP < NT - 3:
            block([('OP', j + NOP)], {}, False)
        out.append(('PACE',))
    block([('OP', NT - 3), ('OP', NT - 2)], {}, False)
    assert not side
    if IDL:
        out.remove(('ID', 3))
        out.append(('ID', 3))
    return out


def _kernel(qT_hbm, kT_hbm, vT_hbm, sk_ref, ssmk_hbm, dd_ref, xT_hbm, ckv_hbm,
            wq_hbm, wk_hbm, wv_hbm, woT_hbm, out_hbm,
            qT, kT, vT, ssmk, xT, ckv, wq_raw, wk_raw, wv_raw, woT,
            aq_s, bx_s, bk_s, bvT_s, QT_s, a_s, acc, fullT, out_s, taps, ff_s, fi_s,
            S0_s, S1_s, X_s, W7_s, pace_s, m0_s, m1_s, l0_s, l1_s,
            sem, sem_k, sem_v, sem_o, *kvo):
    K_s, V_s, O_s, Y_s = kvo[:NT], kvo[NT:2 * NT], kvo[2 * NT:3 * NT], kvo[3 * NT:]
    def cp(src, dst, s):
        return pltpu.make_async_copy(src, dst, s)

    def c_x(j):
        cols = pl.ds(pl.multiple_of(j * 2 * T, 2 * T), 2 * T)
        return cp(xT_hbm.at[:, cols], xT.at[pl.ds(0, M), cols], sem.at[j])

    QP = ((0, 128), (128, 96))

    def c_wq(p):
        cs_ = []
        for half in range(2):
            r = pl.ds((half * 224 + QP[p][0]) * H, QP[p][1] * H)
            for g in range(2):
                cs_.append(cp(wq_hbm.at[r, pl.ds(128 * g, 128)], wq_raw.at[g, r], sem.at[18 + 4 * p + 2 * half + g]))
        return cs_


    def c_w(w_hbm, raw, sm, j, half, g):
        r = pl.ds(pl.multiple_of((half * 4 + j) * 2048, 2048), 2048)
        q = 2 * half + g
        return cp(w_hbm.at[r, pl.ds(128 * g, 128)], raw.at[j % 2, q, pl.ds(0, 2048)], sm.at[(j % 2) * 4 + q])

    def c_wk(j):
        return [c_w(wk_hbm, wk_raw, sem_k, j, half, g) for half in range(2) for g in range(2)]

    def c_wv(j):
        return [c_w(wv_hbm, wv_raw, sem_v, j, half, g) for half in range(2) for g in range(2)]

    def c_ckv(j):
        r = pl.ds(pl.multiple_of(j * 2 * T, 2 * T), 2 * T)
        return cp(ckv_hbm.at[r], ckv.at[r], sem.at[9 + j])

    a_pairs = ((kT_hbm, kT), (vT_hbm, vT), (ssmk_hbm, ssmk), (qT_hbm, qT))
    c_early = [cp(woT_hbm.at[pl.ds(0, 1)], woT.at[pl.ds(0, 1)], sem.at[4])]
    c_early += [cp(src.at[pl.ds(0, CH)], dst.at[pl.ds(0, CH)], sem.at[5 + n]) for n, (src, dst) in enumerate(a_pairs)]
    c_late = [cp(woT_hbm.at[pl.ds(1, H - 1)], woT.at[pl.ds(1, H - 1)], sem.at[13])]
    c_late += [cp(src.at[pl.ds(CH, M - CH)], dst.at[pl.ds(CH, M - CH)], sem.at[14 + n])
               for n, (src, dst) in enumerate(a_pairs)]
    for c in [c_x(0)] + c_wq(0) + c_wq(1):
        c.start()
    for c in c_wk(0) + [c_x(1)]:
        c.start(priority=1)

    n_i = jax.lax.broadcasted_iota(jnp.int32, (P, P), 0)
    k_i = jax.lax.broadcasted_iota(jnp.int32, (P, P), 1)
    ang = (((2 * k_i + 1) * n_i) & 511).astype(f32) * (math.pi / 256.0)
    cs, sn = jnp.cos(ang), jnp.sin(ang)
    ff_s[:, 0:P] = cs.astype(bf16)
    ff_s[:, P:2 * P] = (-sn).astype(bf16)
    fi_s[0:P, :] = (cs.T * (1.0 / P)).astype(bf16)
    fi_s[P:2 * P, :] = (sn.T * (-1.0 / P)).astype(bf16)
    sk = sk_ref[...].astype(f32)
    for t in range(KS):
        taps[t] = jnp.broadcast_to(sk[t:t + 1, :], (128, M)).T
    taps[KS] = jnp.broadcast_to(dd_ref[...].astype(f32).reshape(1, M), (128, M)).T
    acc[...] = jnp.zeros(acc.shape, f32)
    fullT[...] = jnp.zeros(fullT.shape, bf16)
    O_s[NT - 1][...] = jnp.zeros(O_s[0].shape, bf16)
    W7_s[...] = jnp.zeros(W7_s.shape, u32)

    def prep_x(jj, t, r0):
        c0 = (2 * jj + t) * T
        cs_ = [c0, c0 + 128] if isinstance(jj, int) else [pl.multiple_of(c0, 128), pl.multiple_of(c0 + 128, 128)]
        blk = [_u(xT[r:r + 32, pl.ds(c, 128)]) for r in (r0, 224 + r0) for c in cs_]
        row = (2 * jj + t) * 112 + r0 // 2
        row = pl.ds(row if isinstance(jj, int) else pl.multiple_of(row, 16), 16)
        for n, x in enumerate(_combos_u(_b7, blk)):
            bx_s[row, n * 128:(n + 1) * 128] = x
        return []

    c_x(0).wait()
    for t in range(2):
        for r0 in range(0, 224, 32):
            prep_x(0, t, r0)
    vq = wq_raw.bitcast(u32)
    for p, (c0, nc) in enumerate(QP):
        for c in c_wq(p):
            c.wait()
        if p == 1 and VST:
            for c in c_wv(0) + [c_ckv(0)]:
                c.start(priority=1)
        for hp in range(0 if 0 else H // 2):
            ut = [vq[g, pl.ds((half * 224 + c0) * 8 + hp, nc, stride=8), :].T for g in range(2) for half in range(2)]
            for r in range(0, 128, 16):
                u = [x[r:r + 16] for x in ut]
                for par, f in enumerate((_lo, _hi)):
                    r0 = (2 * hp + par) * 64 + r // 2
                    for n, x in enumerate(_a7(*[f(x) for x in u])):
                        aq_s[r0:r0 + 8, n * 256 + c0:n * 256 + c0 + nc] = _u(x.astype(bf16))
    if not VST:
        for c in c_wv(0) + [c_ckv(0)]:
            c.start(priority=1)

    qscale = (D ** -0.5) * math.log2(math.e)

    def lo(u):
        return pltpu.bitcast(u << 16, f32)

    def hi(u):
        return pltpu.bitcast(u & jnp.uint32(0xFFFF0000), f32)

    def b_combos(b11, b12, b21, b22):
        return [b11 + b22, b11, b12 - b22, b21 - b11, b22, b11 + b12, b21 + b22]

    def q_body(j, carry):
        mq = {}

        bx = [[bx_s[pl.ds(pl.multiple_of((2 * j + t) * 112, 16), 112), n * 128:(n + 1) * 128] for n in range(7)]
              for t in range(2)]

        def qproj(u, tok):
            hh, t, n = u // 14, (u // 7) % 2, SORD[u % 7]
            w = _b(_gate_u(aq_s[hh * 64:hh * 64 + 64, n * 256:n * 256 + 224], tok))
            mq[n] = _nn(w, _b(bx[t][n]))
            if u % 7 == 6:
                for k, x in enumerate(_c4(mq)):
                    cols = pl.ds(pl.multiple_of((2 * j + t) * T + (k % 2) * 128, 128), 128)
                    r0 = hh * 128 + (k // 2) * 64
                    QT_s[r0:r0 + 64, cols] = _u((x * qscale).astype(bf16))
            return mq[n]

        def prep_k(hp, part):
            v = wk_raw.bitcast(u32).at[j % 2]
            u = [v[q, pl.ds(part * 128 + hp, 16, stride=8), :] for q in range(4)]
            for par, f in enumerate((_lo, _hi)):
                for n, c in enumerate(_b7(*[f(x) for x in u])):
                    r = _u(c.astype(bf16))
                    r0 = (2 * hp + par) * 256 + part * 8
                    bk_s[pl.ds(pl.multiple_of(j * 64 + r0, 8), 8), n * 128:(n + 1) * 128] = r
            return []

        vt = {}

        def prep_v(hp, part):
            if part == 0:
                v = wv_raw.bitcast(u32).at[j % 2]
                vt[hp] = [v[q, pl.ds(hp, 128, stride=8), :].T for q in range(4)]
                return [x[120:] for x in vt[hp]] if VG else []
            for r in range(32 * (part - 1), 32 * part, 16):
                u = [x[r:r + 16] for x in vt[hp]]
                for par, f in enumerate((_lo, _hi)):
                    r0 = (2 * hp + par) * 64 + r // 2
                    for n, c in enumerate(_b7(*[f(x) for x in u])):
                        cols = pl.ds(pl.multiple_of(n * 512 + j * 128, 128), 128)
                        bvT_s[r0:r0 + 8, cols] = _u(c.astype(bf16))
            return []

        def prep_a(cl_, part, cbs):
            c = 2 * j + cl_
            r0 = 8 * part
            rt = pl.ds(pl.multiple_of(c * T + 2 * r0, 16), 16)
            rb = pl.ds(pl.multiple_of(c * T + 128 + 2 * r0, 16), 16)
            res = []
            for cb in cbs:
                cl, ch_ = slice(cb * 128, cb * 128 + 128), slice(512 + cb * 128, 512 + cb * 128 + 128)
                blk = [_u(ckv[rt, cl]), _u(ckv[rt, ch_]), _u(ckv[rb, cl]), _u(ckv[rb, ch_])]
                cc = []
                for f in (lo, hi):
                    a11, a12, a21, a22 = [f(x) for x in blk]
                    cc.append([a11 + a22, a21 + a22, None, None, a11 + a12, a21 - a11, a12 - a22])
                for n in range(7):
                    if n == 2:
                        r = blk[0]
                    elif n == 3:
                        r = blk[3]
                    else:
                        r = pltpu.pack_elementwise([cc[0][n], cc[1][n]], packed_dtype=bf16)
                    a_s[c, n, r0:r0 + 8, cl] = r
                    res.append(r)
            return [] if APACE else res

        fill = {}

        def spread(pieces, u0, u1):
            for n, p in enumerate(pieces):
                fill.setdefault(u0 + n * (u1 - u0) // len(pieces), []).append(p)

        spread([functools.partial(prep_k, hp, part) for hp in range(8) for part in range(8)], QW1, QW2)
        spread([functools.partial(prep_v, hp, part) for hp in range(8) for part in range(5)], QW2, QW3)
        spread([functools.partial(prep_a, c, part, cbs) for c in range(2) for part in range(8)
                for cbs in ((0, 1), (2, 3))], QW3, QW4)
        spread([functools.partial(prep_x, jnp.minimum(j + 1, 3), t, r0) for t in range(2) for r0 in range(0, 224, 32)], QW4, 221)
        toks = {}
        for u in range(224):
            if u == QW1:
                @pl.when(j < 3)
                def _():
                    for c in c_wk(j + 1):
                        c.start(priority=1)

                @pl.when(j == 3)
                def _():
                    for c in c_early + c_late:
                        c.start(priority=1)

                for c in c_wk(j):
                    c.wait()
            if u == QW2:
                @pl.when(j < 3)
                def _():
                    for c in c_wv(j + 1) + [c_ckv(j + 1)]:
                        c.start(priority=1)

                @pl.when(j < 2)
                def _():
                    c_x(j + 2).start(priority=1)

                @pl.when(j < 3)
                def _():
                    c_x(j + 1).wait()

                for c in c_wv(j) + [c_ckv(j)]:
                    c.wait()
            q = qproj(u, toks.pop(u, None))
            res = []
            ps = fill.get(u, [])
            for n, p in enumerate(ps):
                row = (n * 128 // len(ps)) // 16 * 16
                if p.func is prep_k:
                    wk_raw.bitcast(u32)[j >> 4, 0, 1024:1032, :] = pltpu.bitcast(q[row:row + 8], u32)
                elif p.func is prep_v and p.args[1] == 0:
                    wv_raw.bitcast(u32)[j >> 4, 0, 1024:1032, :] = pltpu.bitcast(q[row:row + 8], u32)
                elif p.func is prep_x:
                    xT[pl.ds(pl.multiple_of(M + (j >> 4) * 16, 16), 16), 0:128] = q[row:row + 16].astype(bf16)
                elif p.func is prep_a:
                    ckv[pl.ds(pl.multiple_of(S + (j >> 4) * 16, 16), 16), 0:128] = q[row:row + 16].astype(bf16)
                res += p()
            if res:
                toks[u + QLAG] = _tok(res)
        return carry

    if not 0:
        jax.lax.fori_loop(0, 4, q_body, 0)
    for c in c_early:
        c.wait()

    tri = n_i <= k_i
    sgn = jnp.where((jax.lax.broadcasted_iota(jnp.int32, (1, P), 1) & 1) == 0, 1.0, -1.0).astype(f32)

    c_outa = cp(out_s.at[:, pl.ds(0, 384)], out_hbm.at[:, pl.ds(0, 384)], sem_o.at[8])

    HR, HI, PR, PI, KV, HS, PS = range(7)

    def zrow(z, n):
        return pl.ds(0, n) if isinstance(z, int) else pl.ds(pl.multiple_of(z * n, n), n)

    def blk_at(c, half=None):
        r0 = (c % 8) * CH
        rs = slice(r0, r0 + CH) if half is None else slice(r0 + 16 * half, r0 + 16 * half + 16)
        return rs, slice((c // 8) * P, (c // 8 + 1) * P)

    def head_body(h, carry):
        @pl.when(h == 1)
        def _():
            for c in c_late:
                c.wait()

        @pl.when(h == H - 1)
        def _():
            c_outa.start()

        st = dict(MQ={}, l={}, M={}, P={}, Q7={}, mfin={}, o={})
        zs, zl = h >> 10, 0
        m_s, l_s = (m0_s, m1_s), (l0_s, l1_s)
        qrows = pl.ds(pl.multiple_of(h * 128, 128), 128)
        rows = pl.ds(pl.multiple_of(jnp.minimum(h, NCH - 1) * CH, CH), CH)

        def rep(t, n):
            return jnp.concatenate([taps[t, rows, :]] * n, axis=1)

        toks = []

        def due():
            for t in toks:
                t[0] -= 1
            ready = [t[1] for t in toks if t[0] <= 0]
            toks[:] = [t for t in toks if t[0] > 0]
            return functools.reduce(lambda x, y: x | y, ready) if ready else None

        def gate_later(vals, lag=SLAG):
            toks.append([lag, _tok([v if v.dtype == u32 else pltpu.bitcast(v, u32) for v in vals])])

        def row_max(i):
            if i not in st['mfin']:
                m = m_s[i % 2][zl, 0]
                for t in range(1, i + 1):
                    m = jnp.maximum(m, m_s[i % 2][zl, t])
                m = jnp.max(m, axis=0, keepdims=True)
                if PVS and i > 0:
                    lo_ = jnp.exp2(m_s[i % 2][zl, 0] - m)
                    for t in range(1, i + 1):
                        lo_ = lo_ + jnp.exp2(m_s[i % 2][zl, t] - m)
                    m = m + jnp.log2(jnp.sum(lo_, axis=0, keepdims=True))
                st['mfin'][i] = m
            return st['mfin'][i]

        for op in _schedule():
            kind = op[0]
            if kind == 'KP':
                _, c, t = op
                n = SK[t]
                st['M'][n] = st['last'] = _nn(_b(_gate_u(a_s[c, n], due())), _b(bk_s[pl.ds(pl.multiple_of(h * 256, 256), 256), n * 128:(n + 1) * 128]))
                if t == 6:
                    c4 = _c4(st['M'])
                    blks = dict(zip((2, 7, 8, 3), c4))
                    if QKS and c < NT - 1:
                        blks.update({n: x for n, x in enumerate(_a7(*c4)) if n not in (2, 3)})
                    for n, x in blks.items():
                        K_s[c][zrow(zs, 64), n * 128:(n + 1) * 128] = _u(x.astype(bf16))
            elif kind == 'VP':
                _, c, t = op
                n = SV[t]
                st['M'][n] = st['last'] = _nt(_b(_gate_u(bvT_s[pl.ds(pl.multiple_of(h * 64, 64), 64), n * 512:(n + 1) * 512], due())), _b(a_s[c, n]))
                if t == 6:
                    c11, c12, c21, c22 = _c4(st['M'])
                    c4 = (c11, c21, c12, c22)
                    blks = dict(zip((2, 7, 8, 3), c4))
                    if PVS and c < NT - 1:
                        blks.update({n: x for n, x in enumerate(_a7(*c4)) if n not in (2, 3)})
                    for n, x in blks.items():
                        V_s[c][zrow(zs, 64), n * 128:(n + 1) * 128] = _u(x.astype(bf16))
            elif kind == 'QK':
                i, j = op[1:3]
                S_s = (S0_s, S1_s)[i % 2]
                qu = QT_s[qrows, i * T:(i + 1) * T]
                if j < i:
                    if QKS:
                        if i not in st['Q7']:
                            st['Q7'][i] = _combos_u(_b7, [qu[:64, :128], qu[:64, 128:], qu[64:, :128], qu[64:, 128:]])
                        for n in (SQ if len(op) == 3 else SQ[op[3]:op[4]]):
                            st['MQ'][n] = _nn(_b(K_s[j][zrow(zl, 64), n * 128:(n + 1) * 128]), _b(st['Q7'][i][n]))
                        if len(op) > 3 and op[4] < 7:
                            continue
                        s = _quad(*_c4(st['MQ']))
                    else:
                        s = _nn(_b(_quad(*[K_s[j][zrow(zl, 64), n * 128:(n + 1) * 128] for n in (2, 7, 8, 3)])), _b(qu))
                    S_s[zs, j] = s
                    f = _fold(s, jnp.max)
                else:
                    q = _b(qu)
                    sa = _nn(_b(jnp.concatenate([K_s[j][zrow(zl, 64), 2 * 128:(2 + 1) * 128], K_s[j][zrow(zl, 64), 7 * 128:(7 + 1) * 128]], axis=1)), q)
                    sa = jnp.concatenate([jnp.where(tri, sa[:, :128], NEG), sa[:, 128:]], axis=1)
                    sb = _nn(_b(jnp.concatenate([K_s[j][zrow(zl, 64), 8 * 128:(8 + 1) * 128], K_s[j][zrow(zl, 64), 3 * 128:(3 + 1) * 128]], axis=1)), q[:, 128:])
                    sb = jnp.where(tri, sb, NEG)
                    S_s[zs, j, 0:128, :] = sa
                    S_s[zs, j, 128:T, 128:T] = sb
                    fa = _fold(sa, jnp.max)
                    f = jnp.concatenate([fa[:, :128], jnp.maximum(fa[:, 128:], _fold(sb, jnp.max))], axis=1)
                m_s[i % 2][zs, j] = f
                pace_s[zs] = f
            elif kind == 'EX':
                _, i, j = op
                S_s = (S0_s, S1_s)[i % 2]
                m = row_max(i)
                if j > 0 or P0:
                    m = jnp.where(pace_s[zl, 0:1, :] == jnp.inf, jnp.inf, m)
                if j < i:
                    if PVS:
                        parts, lj = [], None
                        for r in range(112, -16, -16):
                            pt = jnp.exp2(S_s[zl, j, r:r + 16, :] - m)
                            pb = jnp.exp2(S_s[zl, j, 128 + r:128 + r + 16, :] - m)
                            parts.insert(0, _b7(pt[:, :128], pt[:, 128:], pb[:, :128], pb[:, 128:]))
                            x = (pt[:8] + pt[8:]) + (pb[:8] + pb[8:])
                            lj = x if lj is None else lj + x
                        st['P'][i, j] = [jnp.concatenate([x[n] for x in parts], axis=0).astype(bf16) for n in range(7)]
                    else:
                        p = jnp.exp2(S_s[zl, j] - m)
                        lj = _rsum(p)
                        st['P'][i, j] = p.astype(bf16)
                else:
                    pa = jnp.exp2(S_s[zl, j, 0:128, :] - m)
                    pb = jnp.exp2(S_s[zl, j, 128:T, 128:T] - m[:, 128:])
                    la = _rsum(pa)
                    lj = jnp.concatenate([la[:, :128], la[:, 128:] + _rsum(pb)], axis=1)
                    st['P'][i, j] = (pa.astype(bf16), pb.astype(bf16))
                l_s[i % 2][zs, j] = lj
            elif kind == 'PV':
                i, j = op[1:3]
                vb = [V_s[j][zrow(zl, 64), n * 128:(n + 1) * 128] for n in range(9)]
                p = st['P'][i, j]
                if j < i and PVS:
                    if PV2 and j % 2 == 0 and j + 1 < i:
                        continue
                    for n in (SP if len(op) == 3 else SP[op[3]:op[4]]):
                        if PV2 and j % 2 == 1:
                            v2 = jnp.concatenate([V_s[j - 1][zrow(zl, 64), n * 128:(n + 1) * 128], vb[n]], axis=1)
                            st['last'] = _nn(_b(v2), jnp.concatenate([st['P'][i, j - 1][n], p[n]], axis=0))
                        else:
                            st['last'] = _nn(_b(vb[n]), p[n])
                        st['o'][i, n] = st['o'][i, n] + st['last'] if (i, n) in st['o'] else st['last']
                    continue
                if j < i:
                    o = _nn(_b(_quad(vb[2], vb[7], vb[8], vb[3])), p)
                else:
                    oa = _nn(_b(jnp.concatenate([vb[2], vb[8]], axis=0)), p[0])
                    ob = _nn(_b(jnp.concatenate([vb[7], vb[3]], axis=0)), p[1])
                    o = jnp.concatenate([oa[:, :128], oa[:, 128:] + ob], axis=1)
                st['last'] = o
                if PVS:
                    if i > 0:
                        o = o + _quad(*_c4({n: st['o'].pop((i, n)) for n in range(7)}))
                else:
                    o = o if j == 0 else st['o'][i] + o
                    st['o'][i] = o
                if j == i:
                    l = l_s[i % 2][zl, 0]
                    for t in range(1, i + 1):
                        l = l + l_s[i % 2][zl, t]
                    o = o * (1.0 / jnp.sum(l, axis=0, keepdims=True))
                    blks = (o[:128, :128], o[:128, 128:], o[128:, :128], o[128:, 128:])
                    for n, x in enumerate(_b7(*blks)):
                        O_s[i][zs, n] = x.astype(bf16)
            elif kind == 'PACE':
                pace_s[zs] = jnp.concatenate([st['last'][-8:, -128:]] * 2, axis=1)
            elif kind == 'OP':
                _, i, t = op
                n = SO[t]
                st['M'][n] = st['last'] = _nn(_b(_gate_u(W7_s[0, n], due())), O_s[i][0, n])
                if t == 6:
                    acc[:, T * i:T * (i + 1)] += _quad(*_c4(st['M']))
            elif kind == 'W7':
                res = []
                for r0 in range(16 * op[1], 16 * op[2], 16):
                    blk = [_u(woT[h, r:r + 16, c:c + 128]) for r in (r0, 224 + r0) for c in (0, 128)]
                    w7 = _combos_u(_a7, blk)
                    for n, x in enumerate(w7):
                        W7_s[zs, n, r0 // 2:r0 // 2 + 8] = x
                    res += w7
                gate_later(res)
            elif kind == 'AT':
                g = jnp.clip((h - 4) // 4, 0, 2)
                t0 = jnp.minimum(((h + 12) % 4) * 6, NB - 6)
                grow = pl.ds(pl.multiple_of(g * 128, 128), 128)
                gcol = pl.ds(pl.multiple_of(jnp.where(h == H - 1, 3, g) * 128, 128), 128)
                res = []
                for n in range(6):
                    tok = pl.ds(pl.multiple_of((t0 + n) * 128, 128), 128)
                    x = fullT[grow, tok].T
                    out_s[tok, gcol] = x
                    res.append(_u(x)[56:])
                gate_later(res)
            elif kind == 'HD':
                g = op[1]
                hs = jnp.concatenate([ssmk[rows, c * P:(c + 1) * P] for c in range(4 * g, 4 * g + 4)], axis=0)
                hf = _nn(hs, ff_s[...])
                for n in range(4):
                    X_s[(zs, HR) + blk_at(4 * g + n)] = hf[n * CH:(n + 1) * CH, :P]
                    X_s[(zs, HI) + blk_at(4 * g + n)] = hf[n * CH:(n + 1) * CH, P:]
                    if M3:
                        X_s[(zs, HS) + blk_at(4 * g + n)] = hf[n * CH:(n + 1) * CH, :P] + hf[n * CH:(n + 1) * CH, P:]
            elif kind == 'SC':
                g = op[1]
                if g == 0:
                    k = jnp.concatenate([jnp.zeros((CH, P), f32), kT[rows, 0:4 * P].astype(f32)], axis=1)
                else:
                    k = kT[rows, (4 * g - 1) * P:(4 * g + 4) * P].astype(f32)
                ks = k[:, P:] * rep(0, 4)
                for j in range(1, KS):
                    ks = ks + pltpu.roll(k, j, 1)[:, P:] * rep(j, 4)
                kv = ks * vT[rows, 4 * g * P:(4 * g + 4) * P].astype(f32)
                kvs = jnp.concatenate([kv[:, n * P:(n + 1) * P] for n in range(4)], axis=0)
                xf = _nn(kvs.astype(bf16), ff_s[...])
                for n in range(4):
                    c = 4 * g + n
                    xr, xi = xf[n * CH:(n + 1) * CH, :P], xf[n * CH:(n + 1) * CH, P:]
                    X_s[(zs, KV) + blk_at(c)] = kvs[n * CH:(n + 1) * CH]
                    pr = xr if c == 0 else xr - sgn * st['x'][1]
                    pi = xi if c == 0 else xi + sgn * st['x'][0]
                    X_s[(zs, PR) + blk_at(c)] = pr
                    if M3:
                        X_s[(zs, PI) + blk_at(c)] = pi - pr
                        X_s[(zs, PS) + blk_at(c)] = pi + pr
                    else:
                        X_s[(zs, PI) + blk_at(c)] = pi
                    st['x'] = (xr, xi)
            elif kind == 'CV':
                res = []
                for a, half in op[1]:
                    wr = wi = None
                    k123 = None
                    for j in range(a + 1 if M3 else 0):
                        t = [X_s[(zl, u) + blk_at(j, half)] * X_s[(zl, v) + blk_at(a - j, half)]
                             for u, v in ((HS, PR), (HR, PI), (HI, PS))]
                        k123 = t if k123 is None else [x + y for x, y in zip(k123, t)]
                    if M3:
                        wr, wi = k123[0] - k123[2], k123[0] + k123[1]
                    for j in range(0 if M3 else a + 1):
                        hr, hi_ = X_s[(zl, HR) + blk_at(j, half)], X_s[(zl, HI) + blk_at(j, half)]
                        pr, pi = X_s[(zl, PR) + blk_at(a - j, half)], X_s[(zl, PI) + blk_at(a - j, half)]
                        tr, ti = hr * pr - hi_ * pi, hr * pi + hi_ * pr
                        wr, wi = (tr, ti) if wr is None else (wr + tr, wi + ti)
                    r0 = (a % 4) * CH + 16 * half
                    Y_s[a // 4][zs, r0:r0 + 16, :P] = wr
                    Y_s[a // 4][zs, r0:r0 + 16, P:] = wi
                    res += [wr, wi]
                gate_later(res)
            elif kind == 'ID':
                g = op[1]
                w = Y_s[g][0]
                y = _nn(w.astype(bf16), fi_s[...])
                for n in range(4):
                    c = 4 * g + n
                    cols = slice(c * P, (c + 1) * P)
                    ya = y[n * CH:(n + 1) * CH, :] + X_s[(zl, KV) + blk_at(c)] * taps[KS, rows, :]
                    fullT[rows, cols] = (qT[rows, cols].astype(f32) * ya).astype(bf16)
        return carry

    if not 0:
        jax.lax.fori_loop(0, H, head_body, 0)

    acc[:, T * (NT - 1):] += _quad(*_c4({n: _nn(_b(W7_s[0, n]), O_s[NT - 1][0, n]) for n in SORD}))
    outs = [c_outa]
    for i in range(NT):
        cols = slice(T * i, T * (i + 1))
        blk = jnp.concatenate([fullT[384:M, cols], acc[:, cols].astype(bf16)], axis=0)
        out_s[cols, 384:2 * M] = blk.T
        c = cp(out_s.at[pl.ds(T * i, T), pl.ds(384, 512)], out_hbm.at[pl.ds(T * i, T), pl.ds(384, 512)], sem_o.at[i])
        c.start()
        outs.append(c)
    for c in outs:
        c.wait()


@jax.jit
def pallas_concat_heads__ssm_conv_h3__compressed_kv_cla__prompt_kernel(
    A_q: jax.Array,
    A_k: jax.Array,
    A_v: jax.Array,
    A_shift_k: jax.Array,
    A_ssm_k: jax.Array,
    A_ssm_D: jax.Array,
    B_x: jax.Array,
    B_c_kv: jax.Array,
    B_w_q: jax.Array,
    B_w_uk: jax.Array,
    B_w_uv: jax.Array,
    B_w_o: jax.Array,
):
    hbm = pl.BlockSpec(memory_space=pl.ANY)
    vmem = pl.BlockSpec(memory_space=pltpu.VMEM)
    V = pltpu.VMEM
    out = pl.pallas_call(
        _kernel,
        out_shape=jax.ShapeDtypeStruct((S, 2 * M), bf16),
        in_specs=[hbm, hbm, hbm, vmem, hbm, vmem, hbm, hbm, hbm, hbm, hbm, hbm],
        out_specs=hbm,
        scratch_shapes=[
            V((M, S), bf16), V((M, S), bf16), V((M, S), bf16), V((M, S), bf16),
            V((M + 16, S), bf16), V((S + 16, DC), bf16),
            V((2, M * H, 128), bf16), V((2, 4, 128 * H + 16, 128), bf16), V((2, 4, 128 * H + 16, 128), bf16),
            V((H, M, D), bf16),
            V((H * 64, 7 * 256), u32), V((NT * 112, 7 * 128), u32), V((H * 256, 7 * 128), u32), V((H * 64, 7 * 512), u32),
            V((H * D // 2, S), u32), V((NT, 7, 64, 512), u32),
            V((M, S), f32), V((M, S), bf16), V((S, 2 * M), bf16),
            V((KS + 1, M, 128), f32), V((P, 2 * P), bf16), V((2 * P, P), bf16),
            V((1, NT, T, T), f32), V((1, NT, T, T), f32), V((1, 7, T, T), f32),
            V((1, 7, 112, 128), u32), V((1, 8, T), f32),
            V((1, NT, 8, T), f32), V((1, NT, 8, T), f32), V((1, NT, 8, T), f32), V((1, NT, 8, T), f32),
            pltpu.SemaphoreType.DMA((26,)), pltpu.SemaphoreType.DMA((8,)),
            pltpu.SemaphoreType.DMA((8,)), pltpu.SemaphoreType.DMA((9,)),
        ] + [V((64, 9 * 128), u32)] * NT + [V((64, 9 * 128), u32)] * NT + [V((1, 7, 128, 128), bf16)] * NT
        + [V((1, 4 * CH, 2 * P), f32)] * 4,
        compiler_params=pltpu.CompilerParams(vmem_limit_bytes=120 * 1024 * 1024,
                                             shape_invariant_numerics=False),
    )(
        A_q[0].T, A_k[0].T, A_v[0].T, A_shift_k.T, A_ssm_k, A_ssm_D,
        B_x[0].T, B_c_kv[0],
        B_w_q.reshape(M * H, D), B_w_uk.reshape(DC * H, D), B_w_uv.reshape(DC * H, D),
        jnp.transpose(B_w_o, (0, 2, 1)),
    )
    return out[None]
```

```python
import functools
import math

import jax
import jax.numpy as jnp
import jax.experimental.pallas as pl
import jax.experimental.pallas.tpu as pltpu

bf16 = jnp.bfloat16
f32 = jnp.float32
u32 = jnp.uint32

S = 2048
M = 448
DC = 1024
H = 16
D = 256
KS = 4
P = 128
NB = S // P
CH = 32
NCH = M // CH
T = 256
NT = S // T
NEG = -1e30
LAG_M = 0
LAG_S = 0
SORD = tuple(int(c) for c in '6430125')
SK = tuple(int(c) for c in '0364125')
SV = tuple(int(c) for c in '0364125')
SQ = tuple(int(c) for c in '6043125')
SP = tuple(int(c) for c in '3640125')
SO = tuple(int(c) for c in '5210346')
QW1 = 70
QW2 = 126
QW3 = 188
QLAG = 12
OS = 1
QKS = 1
CVMAX = 12
SIDE0 = 30
SIDEP = 4
LA = 2
SLAG = 3
APACE = 1
PROW = 0
PVS = 1
NOP = 2
L0 = 1
LEND = 4
LLAG = 2
EXR = 16
EX0 = 11
P0 = 1
VG = 1
QW4 = 211
VST = 0
ORD = 3
M3 = 0
IDL = 1
W7N = 2
W7P = 20
W7D = 6
ILV = 0
PV2 = 0
QC1 = 150
KVH = 35
EXB = 6
NOP6 = 2
RMW = 0
ORDER = 'a'


def _nn(a, b):
    return jnp.dot(a, b, preferred_element_type=f32)


def _nt(a, b):
    return jax.lax.dot_general(a, b, (((1,), (1,)), ((), ())), preferred_element_type=f32)


def _b(u):
    return pltpu.bitcast(u, bf16)


def _u(x):
    return pltpu.bitcast(x, u32)


def _split_pair(u):
    lo = pltpu.bitcast(u << 16, f32).astype(bf16)
    hi = pltpu.bitcast(u & jnp.uint32(0xFFFF0000), f32).astype(bf16)
    return lo, hi


def _lo(u):
    return pltpu.bitcast(u << 16, f32)


def _hi(u):
    return pltpu.bitcast(u & jnp.uint32(0xFFFF0000), f32)


def _pk(e, o):
    return pltpu.pack_elementwise([e, o], packed_dtype=bf16)


def _a7(a11, a12, a21, a22):
    return [a11 + a22, a21 + a22, a11, a22, a11 + a12, a21 - a11, a12 - a22]


def _b7(b11, b12, b21, b22):
    return [b11 + b22, b11, b12 - b22, b21 - b11, b22, b11 + b12, b21 + b22]


def _c4(m):
    return m[0] + m[3] - m[4] + m[6], m[2] + m[4], m[1] + m[3], m[0] - m[1] + m[2] + m[5]


def _combos_u(f7, blk):
    e = f7(*[_lo(x) for x in blk])
    o = f7(*[_hi(x) for x in blk])
    plain = {2: 0, 3: 3} if f7 is _a7 else {1: 0, 4: 3}
    return [blk[plain[n]] if n in plain else _pk(e[n], o[n]) for n in range(7)]


def _quad(c11, c12, c21, c22):
    return jnp.concatenate([jnp.concatenate([c11, c12], axis=1), jnp.concatenate([c21, c22], axis=1)], axis=0)


def _fold(c, op):
    return op(c.reshape(-1, 8, c.shape[1]), axis=0)


def _rsum(p):
    cols = []
    for c in range(0, p.shape[1], 128):
        tot = None
        for k in range(0, p.shape[0], 128):
            acc = None
            for r in range(k + 112, k - 16, -16):
                t = p[r:r + 8, c:c + 128] + p[r + 8:r + 16, c:c + 128]
                acc = t if acc is None else acc + t
            tot = acc if tot is None else tot + acc
        cols.append(tot)
    return jnp.concatenate(cols, axis=1) if len(cols) > 1 else cols[0]


def _gate(x, vals):
    if not vals:
        return x
    w = max(v.shape[1] for v in vals)
    top = x[:8, :w]
    for v in vals:
        if v.shape[1] < w:
            v = jnp.concatenate([v] * (w // v.shape[1]), axis=1)
        top = jnp.where(v == jnp.inf, jnp.zeros_like(top), top)
    if w < x.shape[1]:
        top = jnp.concatenate([top, x[:8, w:]], axis=1)
    return jnp.concatenate([top, x[8:]], axis=0)


def _tok(vals):
    parts = []
    for v in vals:
        for r in range(0, v.shape[0], 8):
            for c in range(0, v.shape[1], 128):
                parts.append(v[r:r + 8, c:c + 128])
    while len(parts) > 1:
        parts = [parts[i] | parts[i + 1] if i + 1 < len(parts) else parts[i] for i in range(0, len(parts), 2)]
    return (parts[0] >> 31) >> 1


def _gate_u(x, tok):
    if tok is None:
        return x
    top = x[:8, :128] | tok
    if x.shape[1] > 128:
        top = jnp.concatenate([top, x[:8, 128:]], axis=1)
    return jnp.concatenate([top, x[8:]], axis=0)


def _ssm_pieces():
    ps = [('HD', 0), ('SC', 0), ('HD', 1), ('SC', 1), ('HD', 2), ('SC', 2), ('HD', 3), ('SC', 3)]
    if not OS:
        ps = [p for p in ps if p[0] != 'W7']
    cur, cost = [], 0
    for a in range(NB):
        for half in range(2):
            if cur and cost + a + 1 > CVMAX:
                ps.append(('CV', tuple(cur)))
                cur, cost = [], 0
            cur.append((a, half))
            cost += a + 1
        if a % 4 == 3:
            if cur:
                ps.append(('CV', tuple(cur)))
            cur, cost = [], 0
            ps.append(('ID', a // 4))
    cuts = [14 * k // W7N for k in range(W7N + 1)]
    for k in range(W7N):
        ps.insert(W7P + k * W7D, ('W7', cuts[k], cuts[k + 1]))
    return ps


def _schedule():
    side = _ssm_pieces()
    out = []
    cnt = [0]

    def block(subs, att, ssm):
        for k, u in enumerate(subs):
            out.append(u)
            out.extend(att.get(k, []))
            if ssm:
                cnt[0] += 1
                if side and cnt[0] >= SIDE0 and (cnt[0] - SIDE0) % SIDEP == 0:
                    out.append(side.pop(0))

    def kv(p, half):
        return [('KV', p, t) for t in (range(KVH) if half == 0 else range(KVH, 49))]

    def op_(*idx):
        return [('OP', i, t) for i in idx for t in range(7)]

    def softmax_head(i, n):
        att = {max(n - EXB, 0): [('PACE',), ('EX', i, 0)]}
        if i > 0:
            att.setdefault(n - 1, []).extend([('PACE',), ('EX', i, 1)])
        return att

    ops_left = list(range(NT - 1))
    block(kv(0, 0) + kv(0, 1), {}, True)
    block(op_(NT - 1), {6: [('AT',), ('QK', 0, 0)]}, False)
    block(kv(1, 0), softmax_head(0, KVH), True)
    for i in range(NT - 1):
        for j in range(i + 1):
            out.append(('QK', i + 1, j))
            if j + 2 <= i:
                out.append(('EX', i, j + 2))
            out.append(('PV', i, j))
        out.append(('QK', i + 1, i + 1))
        if i < 5:
            subs = kv((i + 3) // 2, (i + 1) % 2)
            block(subs, softmax_head(i + 1, len(subs)), True)
        else:
            n = NOP6 if i == 5 else NOP
            block(op_(*ops_left[:n]), softmax_head(i + 1, 7 * n), False)
            del ops_left[:n]
    out.append(('PACE',))
    for j in range(NT):
        if j + 2 < NT:
            out.append(('EX', NT - 1, j + 2))
        out.append(('PV', NT - 1, j))
        if len(ops_left) > 2:
            block(op_(ops_left.pop(0)), {}, False)
        out.append(('PACE',))
    block(op_(*ops_left), {}, False)
    assert not side
    assert out.index(('OP', NT - 1, 6)) < min(k for k, o in enumerate(out) if o[0] == 'W7')
    assert out.index(('OP', 0, 0)) > max(k for k, o in enumerate(out) if o[0] == 'W7')
    if IDL:
        out.remove(('ID', 3))
        out.append(('ID', 3))
    return out


def _kernel(qT_hbm, kT_hbm, vT_hbm, sk_ref, ssmk_hbm, dd_ref, xT_hbm, ckv_hbm,
            wq_hbm, wk_hbm, wv_hbm, woT_hbm, out_hbm,
            qT, kT, vT, ssmk, xT, ckv, wq_raw, wk_raw, wv_raw, woT,
            aq_s, bx_s, w1_s, w2_s, cT_s, QT_s, c2_s, acc, fullT, out_s, taps, ff_s, fi_s,
            S0_s, S1_s, X_s, W7_s, pace_s, m0_s, m1_s, l0_s, l1_s,
            sem, sem_k, sem_v, sem_o, *kvo):
    K_s, V_s, O_s, Y_s, CO_s = kvo[:NT], kvo[NT:2 * NT], kvo[2 * NT:3 * NT], kvo[3 * NT:-4], kvo[-4:]
    def cp(src, dst, s):
        return pltpu.make_async_copy(src, dst, s)

    def c_x(j):
        cols = pl.ds(pl.multiple_of(j * 2 * T, 2 * T), 2 * T)
        return cp(xT_hbm.at[:, cols], xT.at[pl.ds(0, M), cols], sem.at[j])

    QP = ((0, 128), (128, 96))

    def c_wq(p):
        cs_ = []
        for half in range(2):
            r = pl.ds((half * 224 + QP[p][0]) * H, QP[p][1] * H)
            for g in range(2):
                cs_.append(cp(wq_hbm.at[r, pl.ds(128 * g, 128)], wq_raw.at[g, r], sem.at[18 + 4 * p + 2 * half + g]))
        return cs_


    def c_w(w_hbm, raw, sm, j, half, g):
        r = pl.ds(pl.multiple_of((half * 4 + j) * 2048, 2048), 2048)
        q = 2 * half + g
        return cp(w_hbm.at[r, pl.ds(128 * g, 128)], raw.at[j % 2, q, pl.ds(0, 2048)], sm.at[(j % 2) * 4 + q])

    def c_wk(j):
        return [c_w(wk_hbm, wk_raw, sem_k, j, half, g) for half in range(2) for g in range(2)]

    def c_wv(j):
        return [c_w(wv_hbm, wv_raw, sem_v, j, half, g) for half in range(2) for g in range(2)]

    def c_ckv(j):
        r = pl.ds(pl.multiple_of(j * 2 * T, 2 * T), 2 * T)
        return cp(ckv_hbm.at[r], ckv.at[r], sem.at[9 + j])

    a_pairs = ((kT_hbm, kT), (vT_hbm, vT), (ssmk_hbm, ssmk), (qT_hbm, qT))
    c_early = [cp(woT_hbm.at[pl.ds(0, 1)], woT.at[pl.ds(0, 1)], sem.at[4])]
    c_early += [cp(src.at[pl.ds(0, CH)], dst.at[pl.ds(0, CH)], sem.at[5 + n]) for n, (src, dst) in enumerate(a_pairs)]
    c_late = [cp(woT_hbm.at[pl.ds(1, H - 1)], woT.at[pl.ds(1, H - 1)], sem.at[13])]
    c_late += [cp(src.at[pl.ds(CH, M - CH)], dst.at[pl.ds(CH, M - CH)], sem.at[14 + n])
               for n, (src, dst) in enumerate(a_pairs)]
    for c in [c_x(0)] + c_wq(0) + c_wq(1):
        c.start()
    for c in c_wk(0) + [c_x(1)]:
        c.start(priority=1)

    n_i = jax.lax.broadcasted_iota(jnp.int32, (P, P), 0)
    k_i = jax.lax.broadcasted_iota(jnp.int32, (P, P), 1)
    ang = (((2 * k_i + 1) * n_i) & 511).astype(f32) * (math.pi / 256.0)
    cs, sn = jnp.cos(ang), jnp.sin(ang)
    ff_s[:, 0:P] = cs.astype(bf16)
    ff_s[:, P:2 * P] = (-sn).astype(bf16)
    fi_s[0:P, :] = (cs.T * (1.0 / P)).astype(bf16)
    fi_s[P:2 * P, :] = (sn.T * (-1.0 / P)).astype(bf16)
    sk = sk_ref[...].astype(f32)
    for t in range(KS):
        taps[t] = jnp.broadcast_to(sk[t:t + 1, :], (128, M)).T
    taps[KS] = jnp.broadcast_to(dd_ref[...].astype(f32).reshape(1, M), (128, M)).T
    acc[...] = jnp.zeros(acc.shape, f32)
    fullT[...] = jnp.zeros(fullT.shape, bf16)
    O_s[NT - 1][...] = jnp.zeros(O_s[0].shape, bf16)
    W7_s[...] = jnp.zeros(W7_s.shape, u32)

    def prep_x(jj, t, r0):
        c0 = (2 * jj + t) * T
        cs_ = [c0, c0 + 128] if isinstance(jj, int) else [pl.multiple_of(c0, 128), pl.multiple_of(c0 + 128, 128)]
        blk = [_u(xT[r:r + 32, pl.ds(c, 128)]) for r in (r0, 224 + r0) for c in cs_]
        row = (2 * jj + t) * 112 + r0 // 2
        row = pl.ds(row if isinstance(jj, int) else pl.multiple_of(row, 16), 16)
        for n, x in enumerate(_combos_u(_b7, blk)):
            bx_s[row, n * 128:(n + 1) * 128] = x
        return []

    c_x(0).wait()
    for t in range(2):
        for r0 in range(0, 224, 32):
            prep_x(0, t, r0)
    vq = wq_raw.bitcast(u32)
    for p, (c0, nc) in enumerate(QP):
        for c in c_wq(p):
            c.wait()
        if p == 1 and VST:
            for c in c_wv(0) + [c_ckv(0)]:
                c.start(priority=1)
        for hp in range(0 if 0 else H // 2):
            ut = [vq[g, pl.ds((half * 224 + c0) * 8 + hp, nc, stride=8), :].T for g in range(2) for half in range(2)]
            for r in range(0, 128, 16):
                u = [x[r:r + 16] for x in ut]
                for par, f in enumerate((_lo, _hi)):
                    r0 = (2 * hp + par) * 64 + r // 2
                    for n, x in enumerate(_a7(*[f(x) for x in u])):
                        aq_s[r0:r0 + 8, n * 256 + c0:n * 256 + c0 + nc] = _u(x.astype(bf16))
    if not VST:
        for c in c_wv(0) + [c_ckv(0)]:
            c.start(priority=1)

    qscale = (D ** -0.5) * math.log2(math.e)

    def lo(u):
        return pltpu.bitcast(u << 16, f32)

    def hi(u):
        return pltpu.bitcast(u & jnp.uint32(0xFFFF0000), f32)

    def b_combos(b11, b12, b21, b22):
        return [b11 + b22, b11, b12 - b22, b21 - b11, b22, b11 + b12, b21 + b22]

    def q_body(j, carry):
        mq = {}

        bx = [[bx_s[pl.ds(pl.multiple_of((2 * j + t) * 112, 16), 112), n * 128:(n + 1) * 128] for n in range(7)]
              for t in range(2)]

        def qproj(u, tok):
            hh, t, n = u // 14, (u // 7) % 2, SORD[u % 7]
            w = _b(_gate_u(aq_s[hh * 64:hh * 64 + 64, n * 256:n * 256 + 224], tok))
            mq[n] = _nn(w, _b(bx[t][n]))
            if u % 7 == 6:
                for k, x in enumerate(_c4(mq)):
                    cols = pl.ds(pl.multiple_of((2 * j + t) * T + (k % 2) * 128, 128), 128)
                    r0 = hh * 128 + (k // 2) * 64
                    QT_s[r0:r0 + 64, cols] = _u((x * qscale).astype(bf16))
            return mq[n]

        wt = {}

        def prep_w(kv, hp, part):
            if part == 0:
                v = (wk_raw, wv_raw)[kv].bitcast(u32).at[j % 2]
                wt[kv, hp] = [v[q, pl.ds(hp, 128, stride=8), :].T for q in (0, 2, 1, 3)]
                return [x[120:] for x in wt[kv, hp]]
            for r in range(32 * (part - 1), 32 * part, 16):
                u = [x[r:r + 16] for x in wt[kv, hp]]
                for par, f in enumerate((_lo, _hi)):
                    r0 = (2 * hp + par) * 128 + kv * 64 + r // 2
                    for n, c in enumerate(_a7(*[f(x) for x in u])):
                        cols = pl.ds(pl.multiple_of(n * 512 + j * 128, 128), 128)
                        w1_s[r0:r0 + 8, cols] = _u(c.astype(bf16))
            return []

        def prep_ct(half, cq):
            res = []
            ct = 2 * cq + half
            for tb in range(4):
                x = _u(ckv[pl.ds(pl.multiple_of(j * 512 + tb * 128, 128), 128), ct * 128:(ct + 1) * 128].T)
                cT_s[pl.ds(pl.multiple_of((j >> 4) * 64 + ct * 64, 64), 64), tb * 128:(tb + 1) * 128] = x
                res.append(x[56:])
            return res

        def prep_c2(r):
            blk = [[cT_s[cq * 128 + r:cq * 128 + r + 8, tb * 128:(tb + 1) * 128] for tb in range(4)] for cq in range(4)]
            two = []
            for f in (_lo, _hi):
                x = [[f(v) for v in row] for row in blk]
                outer = [[_b7(x[ci][ti], x[ci][2 + ti], x[2 + ci][ti], x[2 + ci][2 + ti]) for ti in range(2)]
                         for ci in range(2)]
                two.append([_b7(outer[0][0][n], outer[0][1][n], outer[1][0][n], outer[1][1][n]) for n in range(7)])
            row = pl.ds(pl.multiple_of(j * 128 + r, 8), 8)
            for n in range(7):
                for m in range(7):
                    c2_s[row, (n * 7 + m) * 128:(n * 7 + m + 1) * 128] = _pk(two[0][n][m], two[1][n][m])
            return []

        fill = {}

        def spread(pieces, u0, u1):
            for n, p in enumerate(pieces):
                fill.setdefault(u0 + n * (u1 - u0) // len(pieces), []).append(p)

        spread([functools.partial(prep_w, 0, hp, part) for hp in range(8) for part in range(5)], QW1, QW2)
        spread([functools.partial(prep_w, 1, hp, part) for hp in range(8) for part in range(5)], QW2, QW3)
        spread([functools.partial(prep_ct, 0, cq) for cq in range(4)], QW2 + 2, QC1)
        spread([functools.partial(prep_ct, 1, cq) for cq in range(4)], QC1, QW3)
        spread([functools.partial(prep_c2, r) for r in range(0, 128, 8)], QW3, QW4)
        spread([functools.partial(prep_x, jnp.minimum(j + 1, 3), t, r0) for t in range(2) for r0 in range(0, 224, 32)], QW4, 221)
        toks = {}
        for u in range(224):
            if u == QW1:
                @pl.when(j < 3)
                def _():
                    for c in c_wk(j + 1):
                        c.start(priority=1)

                @pl.when(j == 3)
                def _():
                    for c in c_early + c_late:
                        c.start(priority=1)

                for c in c_wk(j):
                    c.wait()
            if u == QW2:
                @pl.when(j < 3)
                def _():
                    for c in c_wv(j + 1) + [c_ckv(j + 1)]:
                        c.start(priority=1)

                @pl.when(j < 2)
                def _():
                    c_x(j + 2).start(priority=1)

                @pl.when(j < 3)
                def _():
                    c_x(j + 1).wait()

                for c in c_wv(j) + [c_ckv(j)]:
                    c.wait()
            q = qproj(u, toks.pop(u, None))
            res = []
            ps = fill.get(u, [])
            for n, p in enumerate(ps):
                row = (n * 128 // len(ps)) // 16 * 16
                if p.func is prep_w and p.args[2] == 0:
                    (wk_raw, wv_raw)[p.args[0]].bitcast(u32)[j >> 4, 0, 1024:1032, :] = pltpu.bitcast(q[row:row + 8], u32)
                elif p.func is prep_c2:
                    cT_s[pl.ds(pl.multiple_of(512 + (j >> 4) * 8, 8), 8), 0:128] = pltpu.bitcast(q[row:row + 8], u32)
                elif p.func is prep_x:
                    xT[pl.ds(pl.multiple_of(M + (j >> 4) * 16, 16), 16), 0:128] = q[row:row + 16].astype(bf16)
                elif p.func is prep_ct:
                    ckv[pl.ds(pl.multiple_of(S + (j >> 4) * 16, 16), 16), 0:128] = q[row:row + 16].astype(bf16)
                res += p()
            if res:
                toks[u + QLAG] = _tok(res)
        return carry

    if not 0:
        jax.lax.fori_loop(0, 4, q_body, 0)
    for c in c_early:
        c.wait()

    tri = n_i <= k_i
    sgn = jnp.where((jax.lax.broadcasted_iota(jnp.int32, (1, P), 1) & 1) == 0, 1.0, -1.0).astype(f32)

    c_outa = cp(out_s.at[:, pl.ds(0, 384)], out_hbm.at[:, pl.ds(0, 384)], sem_o.at[8])

    HR, HI, PR, PI, KV, HS, PS = range(7)

    def zrow(z, n):
        return pl.ds(0, n) if isinstance(z, int) else pl.ds(pl.multiple_of(z * n, n), n)

    def blk_at(c, half=None):
        r0 = (c % 8) * CH
        rs = slice(r0, r0 + CH) if half is None else slice(r0 + 16 * half, r0 + 16 * half + 16)
        return rs, slice((c // 8) * P, (c // 8 + 1) * P)

    def head_body(h, carry):
        @pl.when(h == 1)
        def _():
            for c in c_late:
                c.wait()

        @pl.when(h == H - 1)
        def _():
            c_outa.start()

        st = dict(co={}, cnt={}, fin=set(), MQ={}, l={}, M={}, P={}, Q7={}, mfin={}, o={})
        zs, zl = h >> 10, 0
        m_s, l_s = (m0_s, m1_s), (l0_s, l1_s)
        qrows = pl.ds(pl.multiple_of(h * 128, 128), 128)
        rows = pl.ds(pl.multiple_of(jnp.minimum(h, NCH - 1) * CH, CH), CH)

        def rep(t, n):
            return jnp.concatenate([taps[t, rows, :]] * n, axis=1)

        toks = []

        def due():
            for t in toks:
                t[0] -= 1
            ready = [t[1] for t in toks if t[0] <= 0]
            toks[:] = [t for t in toks if t[0] > 0]
            return functools.reduce(lambda x, y: x | y, ready) if ready else None

        def gate_later(vals, lag=SLAG):
            toks.append([lag, _tok([v if v.dtype == u32 else pltpu.bitcast(v, u32) for v in vals])])

        def row_max(i):
            if i not in st['mfin']:
                m = m_s[i % 2][zl, 0]
                for t in range(1, i + 1):
                    m = jnp.maximum(m, m_s[i % 2][zl, t])
                m = jnp.max(m, axis=0, keepdims=True)
                if PVS and i > 0:
                    lo_ = jnp.exp2(m_s[i % 2][zl, 0] - m)
                    for t in range(1, i + 1):
                        lo_ = lo_ + jnp.exp2(m_s[i % 2][zl, t] - m)
                    m = m + jnp.log2(jnp.sum(lo_, axis=0, keepdims=True))
                st['mfin'][i] = m
            return st['mfin'][i]

        for op in _schedule():
            kind = op[0]
            if kind == 'KV':
                _, p, t = op
                n, m = SK[t // 7], SV[t % 7]

                def wblk(q):
                    w = w1_s[qrows, n * 512 + (q % 2) * 256:n * 512 + (q % 2) * 256 + 256]
                    r = (q // 2) * 32
                    return jnp.concatenate([w[r:r + 32], w[64 + r:64 + r + 32]], axis=0)

                cols = slice((n * 7 + m) * 256, (n * 7 + m + 1) * 256)
                if m in (2, 3):
                    w = wblk(0 if m == 2 else 3)
                elif p > 0:
                    w = w2_s[:, cols]
                else:
                    i1, i2, sg = {0: (0, 3, 1), 1: (2, 3, 1), 4: (0, 1, 1), 5: (2, 0, -1), 6: (1, 3, -1)}[m]
                    x, y = wblk(i1), wblk(i2)
                    w = _pk(*[f(x) + f(y) if sg > 0 else f(x) - f(y) for f in (_lo, _hi)])
                    w2_s[zrow(zs, 64), cols] = w
                c2 = c2_s[p * 128:(p + 1) * 128, (n * 7 + m) * 128:(n * 7 + m + 1) * 128]
                st['M'][m] = st['last'] = _nn(_b(_gate_u(w, due())), _b(c2))
                if t % 7 == 6:
                    mo = _quad(*_c4(st['M']))
                    fin = {}
                    for o, sg in ((0, 1), (3, 1), (2, 1), (3, -1), (1, 1), (3, 1), (0, 1), (2, 1), (0, -1), (1, 1),
                                  (3, 1), (0, 1))[(0, 2, 4, 6, 8, 10, 11)[n]:(2, 4, 6, 8, 10, 11, 12)[n]]:
                        k = st['cnt'][o] = st['cnt'].get(o, 0) + 1
                        if k == 1:
                            x = mo if sg > 0 else -mo
                        else:
                            prev = CO_s[o][0] if RMW else st['co'][o]
                            x = prev + mo if sg > 0 else prev - mo
                        if k == (4, 2, 2, 4)[o]:
                            st['cnt'][o] = 0
                            st['fin'].add(o)
                            fin[o] = x
                        if k < (4, 2, 2, 4)[o] or (o + 2) % 4 not in st['fin']:
                            st['co'][o] = x
                            if RMW:
                                CO_s[o][zs] = x
                    for tok in range(2):
                        if not {tok, 2 + tok} <= st['fin']:
                            continue
                        st['fin'] -= {tok, 2 + tok}
                        c = 2 * p + tok
                        co = [fin[o] if o in fin else CO_s[o][0] if RMW else st['co'][o] for o in (tok, 2 + tok)]

                        def full(dh, kb, off):
                            x = co[dh][:, kb * 128:(kb + 1) * 128]
                            return jnp.concatenate([x[off:off + 64], x[128 + off:128 + off + 64]], axis=0)

                        kb4 = (full(0, 0, 0).T, full(1, 0, 0).T, full(0, 1, 0).T, full(1, 1, 0).T)
                        vb4 = (full(0, 0, 64), full(0, 1, 64), full(1, 0, 64), full(1, 1, 64))
                        for ref, c4 in ((K_s[c], kb4), (V_s[c], vb4)):
                            blks = dict(zip((2, 7, 8, 3), c4))
                            if c < NT - 1:
                                blks.update({n: x for n, x in enumerate(_a7(*c4)) if n not in (2, 3)})
                            for n, x in blks.items():
                                ref[zrow(zs, 64), n * 128:(n + 1) * 128] = _u(x.astype(bf16))
            elif kind == 'QK':
                i, j = op[1:3]
                S_s = (S0_s, S1_s)[i % 2]
                qu = QT_s[qrows, i * T:(i + 1) * T]
                if j < i:
                    if QKS:
                        if i not in st['Q7']:
                            st['Q7'][i] = _combos_u(_b7, [qu[:64, :128], qu[:64, 128:], qu[64:, :128], qu[64:, 128:]])
                        for n in (SQ if len(op) == 3 else SQ[op[3]:op[4]]):
                            st['MQ'][n] = _nn(_b(K_s[j][zrow(zl, 64), n * 128:(n + 1) * 128]), _b(st['Q7'][i][n]))
                        if len(op) > 3 and op[4] < 7:
                            continue
                        s = _quad(*_c4(st['MQ']))
                    else:
                        s = _nn(_b(_quad(*[K_s[j][zrow(zl, 64), n * 128:(n + 1) * 128] for n in (2, 7, 8, 3)])), _b(qu))
                    S_s[zs, j] = s
                    f = _fold(s, jnp.max)
                else:
                    q = _b(qu)
                    sa = _nn(_b(jnp.concatenate([K_s[j][zrow(zl, 64), 2 * 128:(2 + 1) * 128], K_s[j][zrow(zl, 64), 7 * 128:(7 + 1) * 128]], axis=1)), q)
                    sa = jnp.concatenate([jnp.where(tri, sa[:, :128], NEG), sa[:, 128:]], axis=1)
                    sb = _nn(_b(jnp.concatenate([K_s[j][zrow(zl, 64), 8 * 128:(8 + 1) * 128], K_s[j][zrow(zl, 64), 3 * 128:(3 + 1) * 128]], axis=1)), q[:, 128:])
                    sb = jnp.where(tri, sb, NEG)
                    S_s[zs, j, 0:128, :] = sa
                    S_s[zs, j, 128:T, 128:T] = sb
                    fa = _fold(sa, jnp.max)
                    f = jnp.concatenate([fa[:, :128], jnp.maximum(fa[:, 128:], _fold(sb, jnp.max))], axis=1)
                m_s[i % 2][zs, j] = f
                pace_s[zs] = f
            elif kind == 'EX':
                _, i, j = op
                S_s = (S0_s, S1_s)[i % 2]
                m = row_max(i)
                if j > 0 or P0:
                    m = jnp.where(pace_s[zl, 0:1, :] == jnp.inf, jnp.inf, m)
                if j < i:
                    if PVS:
                        parts, lj = [], None
                        for r in range(112, -16, -16):
                            pt = jnp.exp2(S_s[zl, j, r:r + 16, :] - m)
                            pb = jnp.exp2(S_s[zl, j, 128 + r:128 + r + 16, :] - m)
                            parts.insert(0, _b7(pt[:, :128], pt[:, 128:], pb[:, :128], pb[:, 128:]))
                            x = (pt[:8] + pt[8:]) + (pb[:8] + pb[8:])
                            lj = x if lj is None else lj + x
                        st['P'][i, j] = [jnp.concatenate([x[n] for x in parts], axis=0).astype(bf16) for n in range(7)]
                    else:
                        p = jnp.exp2(S_s[zl, j] - m)
                        lj = _rsum(p)
                        st['P'][i, j] = p.astype(bf16)
                else:
                    pa = jnp.exp2(S_s[zl, j, 0:128, :] - m)
                    pb = jnp.exp2(S_s[zl, j, 128:T, 128:T] - m[:, 128:])
                    la = _rsum(pa)
                    lj = jnp.concatenate([la[:, :128], la[:, 128:] + _rsum(pb)], axis=1)
                    st['P'][i, j] = (pa.astype(bf16), pb.astype(bf16))
                l_s[i % 2][zs, j] = lj
            elif kind == 'PV':
                i, j = op[1:3]
                vb = [V_s[j][zrow(zl, 64), n * 128:(n + 1) * 128] for n in range(9)]
                p = st['P'][i, j]
                if j < i and PVS:
                    if PV2 and j % 2 == 0 and j + 1 < i:
                        continue
                    for n in (SP if len(op) == 3 else SP[op[3]:op[4]]):
                        if PV2 and j % 2 == 1:
                            v2 = jnp.concatenate([V_s[j - 1][zrow(zl, 64), n * 128:(n + 1) * 128], vb[n]], axis=1)
                            st['last'] = _nn(_b(v2), jnp.concatenate([st['P'][i, j - 1][n], p[n]], axis=0))
                        else:
                            st['last'] = _nn(_b(vb[n]), p[n])
                        st['o'][i, n] = st['o'][i, n] + st['last'] if (i, n) in st['o'] else st['last']
                    continue
                if j < i:
                    o = _nn(_b(_quad(vb[2], vb[7], vb[8], vb[3])), p)
                else:
                    oa = _nn(_b(jnp.concatenate([vb[2], vb[8]], axis=0)), p[0])
                    ob = _nn(_b(jnp.concatenate([vb[7], vb[3]], axis=0)), p[1])
                    o = jnp.concatenate([oa[:, :128], oa[:, 128:] + ob], axis=1)
                st['last'] = o
                if PVS:
                    if i > 0:
                        o = o + _quad(*_c4({n: st['o'].pop((i, n)) for n in range(7)}))
                else:
                    o = o if j == 0 else st['o'][i] + o
                    st['o'][i] = o
                if j == i:
                    l = l_s[i % 2][zl, 0]
                    for t in range(1, i + 1):
                        l = l + l_s[i % 2][zl, t]
                    o = o * (1.0 / jnp.sum(l, axis=0, keepdims=True))
                    blks = (o[:128, :128], o[:128, 128:], o[128:, :128], o[128:, 128:])
                    for n, x in enumerate(_b7(*blks)):
                        O_s[i][zs, n] = x.astype(bf16)
            elif kind == 'PACE':
                pace_s[zs] = jnp.concatenate([st['last'][-8:, -128:]] * 2, axis=1)
            elif kind == 'OP':
                _, i, t = op
                n = SO[t]
                st['M'][n] = st['last'] = _nn(_b(_gate_u(W7_s[0, n], due())), O_s[i][0, n])
                if t == 6:
                    acc[:, T * i:T * (i + 1)] += _quad(*_c4(st['M']))
            elif kind == 'W7':
                res = []
                for r0 in range(16 * op[1], 16 * op[2], 16):
                    blk = [_u(woT[h, r:r + 16, c:c + 128]) for r in (r0, 224 + r0) for c in (0, 128)]
                    w7 = _combos_u(_a7, blk)
                    for n, x in enumerate(w7):
                        W7_s[zs, n, r0 // 2:r0 // 2 + 8] = x
                    res += w7
                gate_later(res)
            elif kind == 'AT':
                g = jnp.clip((h - 4) // 4, 0, 2)
                t0 = jnp.minimum(((h + 12) % 4) * 6, NB - 6)
                grow = pl.ds(pl.multiple_of(g * 128, 128), 128)
                gcol = pl.ds(pl.multiple_of(jnp.where(h == H - 1, 3, g) * 128, 128), 128)
                res = []
                for n in range(6):
                    tok = pl.ds(pl.multiple_of((t0 + n) * 128, 128), 128)
                    x = fullT[grow, tok].T
                    out_s[tok, gcol] = x
                    res.append(_u(x)[56:])
                gate_later(res)
            elif kind == 'HD':
                g = op[1]
                hs = jnp.concatenate([ssmk[rows, c * P:(c + 1) * P] for c in range(4 * g, 4 * g + 4)], axis=0)
                hf = _nn(hs, ff_s[...])
                for n in range(4):
                    X_s[(zs, HR) + blk_at(4 * g + n)] = hf[n * CH:(n + 1) * CH, :P]
                    X_s[(zs, HI) + blk_at(4 * g + n)] = hf[n * CH:(n + 1) * CH, P:]
                    if M3:
                        X_s[(zs, HS) + blk_at(4 * g + n)] = hf[n * CH:(n + 1) * CH, :P] + hf[n * CH:(n + 1) * CH, P:]
            elif kind == 'SC':
                g = op[1]
                if g == 0:
                    k = jnp.concatenate([jnp.zeros((CH, P), f32), kT[rows, 0:4 * P].astype(f32)], axis=1)
                else:
                    k = kT[rows, (4 * g - 1) * P:(4 * g + 4) * P].astype(f32)
                ks = k[:, P:] * rep(0, 4)
                for j in range(1, KS):
                    ks = ks + pltpu.roll(k, j, 1)[:, P:] * rep(j, 4)
                kv = ks * vT[rows, 4 * g * P:(4 * g + 4) * P].astype(f32)
                kvs = jnp.concatenate([kv[:, n * P:(n + 1) * P] for n in range(4)], axis=0)
                xf = _nn(kvs.astype(bf16), ff_s[...])
                for n in range(4):
                    c = 4 * g + n
                    xr, xi = xf[n * CH:(n + 1) * CH, :P], xf[n * CH:(n + 1) * CH, P:]
                    X_s[(zs, KV) + blk_at(c)] = kvs[n * CH:(n + 1) * CH]
                    pr = xr if c == 0 else xr - sgn * st['x'][1]
                    pi = xi if c == 0 else xi + sgn * st['x'][0]
                    X_s[(zs, PR) + blk_at(c)] = pr
                    if M3:
                        X_s[(zs, PI) + blk_at(c)] = pi - pr
                        X_s[(zs, PS) + blk_at(c)] = pi + pr
                    else:
                        X_s[(zs, PI) + blk_at(c)] = pi
                    st['x'] = (xr, xi)
            elif kind == 'CV':
                res = []
                for a, half in op[1]:
                    wr = wi = None
                    k123 = None
                    for j in range(a + 1 if M3 else 0):
                        t = [X_s[(zl, u) + blk_at(j, half)] * X_s[(zl, v) + blk_at(a - j, half)]
                             for u, v in ((HS, PR), (HR, PI), (HI, PS))]
                        k123 = t if k123 is None else [x + y for x, y in zip(k123, t)]
                    if M3:
                        wr, wi = k123[0] - k123[2], k123[0] + k123[1]
                    for j in range(0 if M3 else a + 1):
                        hr, hi_ = X_s[(zl, HR) + blk_at(j, half)], X_s[(zl, HI) + blk_at(j, half)]
                        pr, pi = X_s[(zl, PR) + blk_at(a - j, half)], X_s[(zl, PI) + blk_at(a - j, half)]
                        tr, ti = hr * pr - hi_ * pi, hr * pi + hi_ * pr
                        wr, wi = (tr, ti) if wr is None else (wr + tr, wi + ti)
                    r0 = (a % 4) * CH + 16 * half
                    Y_s[a // 4][zs, r0:r0 + 16, :P] = wr
                    Y_s[a // 4][zs, r0:r0 + 16, P:] = wi
                    res += [wr, wi]
                gate_later(res)
            elif kind == 'ID':
                g = op[1]
                w = Y_s[g][0]
                y = _nn(w.astype(bf16), fi_s[...])
                for n in range(4):
                    c = 4 * g + n
                    cols = slice(c * P, (c + 1) * P)
                    ya = y[n * CH:(n + 1) * CH, :] + X_s[(zl, KV) + blk_at(c)] * taps[KS, rows, :]
                    fullT[rows, cols] = (qT[rows, cols].astype(f32) * ya).astype(bf16)
        return carry

    if not 0:
        jax.lax.fori_loop(0, H, head_body, 0)

    acc[:, T * (NT - 1):] += _quad(*_c4({n: _nn(_b(W7_s[0, n]), O_s[NT - 1][0, n]) for n in SORD}))
    outs = [c_outa]
    for i in range(NT):
        cols = slice(T * i, T * (i + 1))
        blk = jnp.concatenate([fullT[384:M, cols], acc[:, cols].astype(bf16)], axis=0)
        out_s[cols, 384:2 * M] = blk.T
        c = cp(out_s.at[pl.ds(T * i, T), pl.ds(384, 512)], out_hbm.at[pl.ds(T * i, T), pl.ds(384, 512)], sem_o.at[i])
        c.start()
        outs.append(c)
    for c in outs:
        c.wait()


@jax.jit
def pallas_concat_heads__ssm_conv_h3__compressed_kv_cla__prompt_kernel(
    A_q: jax.Array,
    A_k: jax.Array,
    A_v: jax.Array,
    A_shift_k: jax.Array,
    A_ssm_k: jax.Array,
    A_ssm_D: jax.Array,
    B_x: jax.Array,
    B_c_kv: jax.Array,
    B_w_q: jax.Array,
    B_w_uk: jax.Array,
    B_w_uv: jax.Array,
    B_w_o: jax.Array,
):
    hbm = pl.BlockSpec(memory_space=pl.ANY)
    vmem = pl.BlockSpec(memory_space=pltpu.VMEM)
    V = pltpu.VMEM
    out = pl.pallas_call(
        _kernel,
        out_shape=jax.ShapeDtypeStruct((S, 2 * M), bf16),
        in_specs=[hbm, hbm, hbm, vmem, hbm, vmem, hbm, hbm, hbm, hbm, hbm, hbm],
        out_specs=hbm,
        scratch_shapes=[
            V((M, S), bf16), V((M, S), bf16), V((M, S), bf16), V((M, S), bf16),
            V((M + 16, S), bf16), V((S + 16, DC), bf16),
            V((2, M * H, 128), bf16), V((2, 4, 128 * H + 16, 128), bf16), V((2, 4, 128 * H + 16, 128), bf16),
            V((H, M, D), bf16),
            V((H * 64, 7 * 256), u32), V((NT * 112, 7 * 128), u32), V((H * 128, 7 * 512), u32),
            V((64, 49 * 256), u32), V((512 + 8, 512), u32),
            V((H * D // 2, S), u32), V((4 * 128, 49 * 128), u32),
            V((M, S), f32), V((M, S), bf16), V((S, 2 * M), bf16),
            V((KS + 1, M, 128), f32), V((P, 2 * P), bf16), V((2 * P, P), bf16),
            V((1, NT, T, T), f32), V((1, NT, T, T), f32), V((1, 5 + 2 * M3, T, T), f32),
            V((1, 7, 112, 128), u32), V((1, 8, T), f32),
            V((1, NT, 8, T), f32), V((1, NT, 8, T), f32), V((1, NT, 8, T), f32), V((1, NT, 8, T), f32),
            pltpu.SemaphoreType.DMA((26,)), pltpu.SemaphoreType.DMA((8,)),
            pltpu.SemaphoreType.DMA((8,)), pltpu.SemaphoreType.DMA((9,)),
        ] + [V((64, 9 * 128), u32)] * NT + [V((64, 9 * 128), u32)] * NT + [V((1, 7, 128, 128), bf16)] * NT
        + [V((1, 4 * CH, 2 * P), f32)] * 4 + [V((1, T if RMW else 8, T), f32)] * 4,
        compiler_params=pltpu.CompilerParams(vmem_limit_bytes=126 * 1024 * 1024,
                                             shape_invariant_numerics=False),
    )(
        A_q[0].T, A_k[0].T, A_v[0].T, A_shift_k.T, A_ssm_k, A_ssm_D,
        B_x[0].T, B_c_kv[0],
        B_w_q.reshape(M * H, D), B_w_uk.reshape(DC * H, D), B_w_uv.reshape(DC * H, D),
        jnp.transpose(B_w_o, (0, 2, 1)),
    )
    return out[None]
```

```python
import functools
import math

import jax
import jax.numpy as jnp
import jax.experimental.pallas as pl
import jax.experimental.pallas.tpu as pltpu

bf16 = jnp.bfloat16
f32 = jnp.float32
u32 = jnp.uint32

S = 2048
M = 448
DC = 1024
H = 16
D = 256
KS = 4
P = 128
NB = S // P
CH = 32
NCH = M // CH
T = 256
NT = S // T
NEG = -1e30

SORD = tuple(int(c) for c in '6430125')
SK = tuple(int(c) for c in '0364125')
SV = tuple(int(c) for c in '0634125')
SQ = tuple(int(c) for c in '6043125')
SP = tuple(int(c) for c in '3640125')
SO = tuple(int(c) for c in '5210346')
QW1 = 70
QW2 = 126
QW3 = 188
QW4 = 211
QC1 = 150
QLAG = 12
CVMAX = 12
SIDE0 = 30
SIDEP = 4
SLAG = 5
PRE = 0
W7P = 20
W7D = 1
KVH = 35
EXB = 6
NOP6 = 2
NOP = 2


def _nn(a, b):
    return jnp.dot(a, b, preferred_element_type=f32)


def _b(u):
    return pltpu.bitcast(u, bf16)


def _u(x):
    return pltpu.bitcast(x, u32)


def _lo(u):
    return pltpu.bitcast(u << 16, f32)


def _hi(u):
    return pltpu.bitcast(u & jnp.uint32(0xFFFF0000), f32)


def _pk(e, o):
    return pltpu.pack_elementwise([e, o], packed_dtype=bf16)


def _a7(a11, a12, a21, a22):
    return [a11 + a22, a21 + a22, a11, a22, a11 + a12, a21 - a11, a12 - a22]


def _b7(b11, b12, b21, b22):
    return [b11 + b22, b11, b12 - b22, b21 - b11, b22, b11 + b12, b21 + b22]


def _c4(m):
    return m[0] + m[3] - m[4] + m[6], m[2] + m[4], m[1] + m[3], m[0] - m[1] + m[2] + m[5]


_C_OF = (((0, 1), (3, 1)), ((2, 1), (3, -1)), ((1, 1), (3, 1)), ((0, 1), (2, 1)), ((0, -1), (1, 1)), ((3, 1),), ((0, 1),))
_C_CNT = (4, 2, 2, 4)
_A_OF = {0: (0, 3, 1), 1: (2, 3, 1), 4: (0, 1, 1), 5: (2, 0, -1), 6: (1, 3, -1)}


def _combos_u(f7, blk):
    e = f7(*[_lo(x) for x in blk])
    o = f7(*[_hi(x) for x in blk])
    plain = {2: 0, 3: 3} if f7 is _a7 else {1: 0, 4: 3}
    return [blk[plain[n]] if n in plain else _pk(e[n], o[n]) for n in range(7)]


def _quad(c11, c12, c21, c22):
    return jnp.concatenate([jnp.concatenate([c11, c12], axis=1), jnp.concatenate([c21, c22], axis=1)], axis=0)


def _fold(c, op):
    return op(c.reshape(-1, 8, c.shape[1]), axis=0)


def _rsum(p):
    cols = []
    for c in range(0, p.shape[1], 128):
        acc = None
        for r in range(112, -16, -16):
            t = p[r:r + 8, c:c + 128] + p[r + 8:r + 16, c:c + 128]
            acc = t if acc is None else acc + t
        cols.append(acc)
    return jnp.concatenate(cols, axis=1) if len(cols) > 1 else cols[0]


def _tok(vals):
    parts = []
    for v in vals:
        for r in range(0, v.shape[0], 8):
            for c in range(0, v.shape[1], 128):
                parts.append(v[r:r + 8, c:c + 128])
    while len(parts) > 1:
        parts = [parts[i] | parts[i + 1] if i + 1 < len(parts) else parts[i] for i in range(0, len(parts), 2)]
    return (parts[0] >> 31) >> 1


def _gate(x, tok):
    if tok is None:
        return x
    top = x[:8, :128] | tok
    if x.shape[1] > 128:
        top = jnp.concatenate([top, x[:8, 128:]], axis=1)
    return jnp.concatenate([top, x[8:]], axis=0)


def _side_pieces():
    ps = [(k, g) for g in range(PRE) for k in ('HD', 'SC')]
    cur, cost = [], 0
    for a in range(NB):
        if a % 4 == 0 and a // 4 + PRE < 4:
            ps += [('HD', a // 4 + PRE), ('SC', a // 4 + PRE)]
        for half in range(2):
            if cur and cost + a + 1 > CVMAX:
                ps.append(('CV', tuple(cur)))
                cur, cost = [], 0
            cur.append((a, half))
            cost += a + 1
        if a % 4 == 3:
            ps += [('CV', tuple(cur)), ('ID', a // 4)]
            cur, cost = [], 0
    ps.insert(W7P, ('W7', 0, 7))
    ps.insert(W7P + W7D, ('W7', 7, 14))
    return ps


def _schedule():
    side = _side_pieces()
    out = []
    cnt = [0]

    def block(subs, att, with_side):
        for k, u in enumerate(subs):
            out.append(u)
            out.extend(att.get(k, []))
            if with_side:
                cnt[0] += 1
                if side and cnt[0] >= SIDE0 and (cnt[0] - SIDE0) % SIDEP == 0:
                    out.append(side.pop(0))

    def kv(p, half):
        return [('KV', p, t) for t in (range(KVH) if half == 0 else range(KVH, 49))]

    def op_(*idx):
        return [('OP', i, t) for i in idx for t in range(7)]

    def softmax_head(i, n):
        att = {max(n - EXB, 0): [('PACE',), ('EX', i, 0)]}
        if i > 0:
            att.setdefault(n - 1, []).extend([('PACE',), ('EX', i, 1)])
        return att

    ops_left = list(range(NT - 1))
    block(kv(0, 0) + kv(0, 1), {}, True)
    block(op_(NT - 1), {6: [('AT',), ('QK', 0, 0)]}, False)
    block(kv(1, 0), softmax_head(0, KVH), True)
    for i in range(NT - 1):
        for j in range(i + 1):
            out.append(('QK', i + 1, j))
            if j + 2 <= i:
                out.append(('EX', i, j + 2))
            out.append(('PV', i, j))
        out.append(('QK', i + 1, i + 1))
        if i < 5:
            subs = kv((i + 3) // 2, (i + 1) % 2)
            block(subs, softmax_head(i + 1, len(subs)), True)
        else:
            n = NOP6 if i == 5 else NOP
            block(op_(*ops_left[:n]), softmax_head(i + 1, 7 * n), False)
            del ops_left[:n]
    out.append(('PACE',))
    for j in range(NT):
        if j + 2 < NT:
            out.append(('EX', NT - 1, j + 2))
        out.append(('PV', NT - 1, j))
        if len(ops_left) > 2:
            block(op_(ops_left.pop(0)), {}, False)
        out.append(('PACE',))
    block(op_(*ops_left), {}, False)
    assert not side
    w7 = [k for k, o in enumerate(out) if o[0] == 'W7']
    assert out.index(('OP', NT - 1, 6)) < min(w7) and max(w7) < out.index(('OP', 0, 0))
    out.remove(('ID', 3))
    out.append(('ID', 3))
    return out


def _kernel(qT_hbm, kT_hbm, vT_hbm, sk_ref, ssmk_hbm, dd_ref, xT_hbm, ckv_hbm,
            wq_hbm, wk_hbm, wv_hbm, woT_hbm, out_hbm,
            qT, kT, vT, ssmk, xT, ckv, wq_raw, wk_raw, wv_raw, woT,
            aq_s, bx_s, w1_s, w2_s, cT_s, QT_s, c2_s, acc, aT_s, out_s, taps, ff_s, fi_s,
            S0_s, S1_s, X_s, W7_s, pace_s, m0_s, m1_s, l0_s, l1_s,
            sem, sem_k, sem_v, sem_o, *rest):
    K_s, V_s, O_s, Y_s = rest[:NT], rest[NT:2 * NT], rest[2 * NT:3 * NT], rest[3 * NT:]

    def cp(src, dst, s):
        return pltpu.make_async_copy(src, dst, s)

    def c_x(j):
        cols = pl.ds(pl.multiple_of(j * 2 * T, 2 * T), 2 * T)
        return cp(xT_hbm.at[:, cols], xT.at[pl.ds(0, M), cols], sem.at[j])

    QP = ((0, 128), (128, 96))

    def c_wq(p):
        cs_ = []
        for half in range(2):
            r = pl.ds((half * 224 + QP[p][0]) * H, QP[p][1] * H)
            for g in range(2):
                cs_.append(cp(wq_hbm.at[r, pl.ds(128 * g, 128)], wq_raw.at[g, r], sem.at[18 + 4 * p + 2 * half + g]))
        return cs_

    def c_w(w_hbm, raw, sm, j, half, g):
        r = pl.ds(pl.multiple_of((half * 4 + j) * 2048, 2048), 2048)
        q = 2 * half + g
        return cp(w_hbm.at[r, pl.ds(128 * g, 128)], raw.at[j % 2, q, pl.ds(0, 2048)], sm.at[(j % 2) * 4 + q])

    def c_wk(j):
        return [c_w(wk_hbm, wk_raw, sem_k, j, half, g) for half in range(2) for g in range(2)]

    def c_wv(j):
        return [c_w(wv_hbm, wv_raw, sem_v, j, half, g) for half in range(2) for g in range(2)]

    def c_ckv(j):
        r = pl.ds(pl.multiple_of(j * 2 * T, 2 * T), 2 * T)
        return cp(ckv_hbm.at[r], ckv.at[r], sem.at[9 + j])

    a_pairs = ((kT_hbm, kT), (vT_hbm, vT), (ssmk_hbm, ssmk), (qT_hbm, qT))
    c_early = [cp(woT_hbm.at[pl.ds(0, 1)], woT.at[pl.ds(0, 1)], sem.at[4])]
    c_early += [cp(src.at[pl.ds(0, CH)], dst.at[pl.ds(0, CH)], sem.at[5 + n]) for n, (src, dst) in enumerate(a_pairs)]
    c_late = [cp(woT_hbm.at[pl.ds(1, H - 1)], woT.at[pl.ds(1, H - 1)], sem.at[13])]
    c_late += [cp(src.at[pl.ds(CH, M - CH)], dst.at[pl.ds(CH, M - CH)], sem.at[14 + n])
               for n, (src, dst) in enumerate(a_pairs)]
    for c in [c_x(0)] + c_wq(0) + c_wq(1):
        c.start()
    for c in c_wk(0) + [c_x(1)]:
        c.start(priority=1)

    n_i = jax.lax.broadcasted_iota(jnp.int32, (P, P), 0)
    k_i = jax.lax.broadcasted_iota(jnp.int32, (P, P), 1)
    ang = (((2 * k_i + 1) * n_i) & 511).astype(f32) * (math.pi / 256.0)
    cs, sn = jnp.cos(ang), jnp.sin(ang)
    ff_s[:, 0:P] = cs.astype(bf16)
    ff_s[:, P:2 * P] = (-sn).astype(bf16)
    fi_s[0:P, :] = (cs.T * (1.0 / P)).astype(bf16)
    fi_s[P:2 * P, :] = (sn.T * (-1.0 / P)).astype(bf16)
    sk = sk_ref[...].astype(f32)
    for t in range(KS):
        taps[t] = jnp.broadcast_to(sk[t:t + 1, :], (128, M)).T
    taps[KS] = jnp.broadcast_to(dd_ref[...].astype(f32).reshape(1, M), (128, M)).T
    acc[...] = jnp.zeros(acc.shape, f32)
    aT_s[...] = jnp.zeros(aT_s.shape, bf16)
    O_s[NT - 1][...] = jnp.zeros(O_s[0].shape, bf16)
    W7_s[...] = jnp.zeros(W7_s.shape, u32)

    def prep_x(jj, t, r0):
        c0 = (2 * jj + t) * T
        cs_ = [c0, c0 + 128] if isinstance(jj, int) else [pl.multiple_of(c0, 128), pl.multiple_of(c0 + 128, 128)]
        blk = [_u(xT[r:r + 32, pl.ds(c, 128)]) for r in (r0, 224 + r0) for c in cs_]
        row = (2 * jj + t) * 112 + r0 // 2
        row = pl.ds(row if isinstance(jj, int) else pl.multiple_of(row, 16), 16)
        for n, x in enumerate(_combos_u(_b7, blk)):
            bx_s[row, n * 128:(n + 1) * 128] = x
        return []

    c_x(0).wait()
    for t in range(2):
        for r0 in range(0, 224, 32):
            prep_x(0, t, r0)
    vq = wq_raw.bitcast(u32)
    for p, (c0, nc) in enumerate(QP):
        for c in c_wq(p):
            c.wait()
        for hp in range(H // 2):
            ut = [vq[g, pl.ds((half * 224 + c0) * 8 + hp, nc, stride=8), :].T for g in range(2) for half in range(2)]
            for r in range(0, 128, 16):
                u = [x[r:r + 16] for x in ut]
                for par, f in enumerate((_lo, _hi)):
                    r0 = (2 * hp + par) * 64 + r // 2
                    for n, x in enumerate(_a7(*[f(x) for x in u])):
                        aq_s[r0:r0 + 8, n * 256 + c0:n * 256 + c0 + nc] = _u(x.astype(bf16))
    for c in c_wv(0) + [c_ckv(0)]:
        c.start(priority=1)

    qscale = (D ** -0.5) * math.log2(math.e)

    def q_body(j, carry):
        mq = {}
        zq = j >> 4
        bx = [[bx_s[pl.ds(pl.multiple_of((2 * j + t) * 112, 16), 112), n * 128:(n + 1) * 128] for n in range(7)]
              for t in range(2)]

        def qproj(u, tok):
            hh, t, n = u // 14, (u // 7) % 2, SORD[u % 7]
            w = _b(_gate(aq_s[hh * 64:hh * 64 + 64, n * 256:n * 256 + 224], tok))
            mq[n] = _nn(w, _b(bx[t][n]))
            if u % 7 == 6:
                for k, x in enumerate(_c4(mq)):
                    cols = pl.ds(pl.multiple_of((2 * j + t) * T + (k % 2) * 128, 128), 128)
                    r0 = hh * 128 + (k // 2) * 64
                    QT_s[r0:r0 + 64, cols] = _u((x * qscale).astype(bf16))
            return mq[n]

        wt = {}

        def prep_w(kv, hp, part):
            if part == 0:
                v = (wk_raw, wv_raw)[kv].bitcast(u32).at[j % 2]
                wt[kv, hp] = [v[q, pl.ds(hp, 128, stride=8), :].T for q in (0, 2, 1, 3)]
                return [x[120:] for x in wt[kv, hp]]
            for r in range(32 * (part - 1), 32 * part, 16):
                u = [x[r:r + 16] for x in wt[kv, hp]]
                for par, f in enumerate((_lo, _hi)):
                    r0 = (2 * hp + par) * 128 + kv * 64 + r // 2
                    for n, c in enumerate(_a7(*[f(x) for x in u])):
                        cols = pl.ds(pl.multiple_of(n * 512 + j * 128, 128), 128)
                        w1_s[r0:r0 + 8, cols] = _u(c.astype(bf16))
            return []

        def prep_ct(half, cq):
            res = []
            ct = 2 * cq + half
            for tb in range(4):
                x = _u(ckv[pl.ds(pl.multiple_of(j * 512 + tb * 128, 128), 128), ct * 128:(ct + 1) * 128].T)
                cT_s[pl.ds(pl.multiple_of(zq * 64 + ct * 64, 64), 64), tb * 128:(tb + 1) * 128] = x
                res.append(x[56:])
            return res

        def prep_c2(r):
            blk = [[cT_s[cq * 128 + r:cq * 128 + r + 8, tb * 128:(tb + 1) * 128] for tb in range(4)] for cq in range(4)]
            two = []
            for f in (_lo, _hi):
                x = [[f(v) for v in row] for row in blk]
                outer = [[_b7(x[ci][ti], x[ci][2 + ti], x[2 + ci][ti], x[2 + ci][2 + ti]) for ti in range(2)]
                         for ci in range(2)]
                two.append([_b7(outer[0][0][n], outer[0][1][n], outer[1][0][n], outer[1][1][n]) for n in range(7)])
            row = pl.ds(pl.multiple_of(j * 128 + r, 8), 8)
            for n in range(7):
                for m in range(7):
                    c2_s[row, (n * 7 + m) * 128:(n * 7 + m + 1) * 128] = _pk(two[0][n][m], two[1][n][m])
            return []

        fill = {}

        def spread(pieces, u0, u1):
            for n, p in enumerate(pieces):
                fill.setdefault(u0 + n * (u1 - u0) // len(pieces), []).append(p)

        spread([functools.partial(prep_w, 0, hp, part) for hp in range(8) for part in range(5)], QW1, QW2)
        spread([functools.partial(prep_w, 1, hp, part) for hp in range(8) for part in range(5)], QW2, QW3)
        spread([functools.partial(prep_ct, 0, cq) for cq in range(4)], QW2 + 2, QC1)
        spread([functools.partial(prep_ct, 1, cq) for cq in range(4)], QC1, QW3)
        spread([functools.partial(prep_c2, r) for r in range(0, 128, 8)], QW3, QW4)
        spread([functools.partial(prep_x, jnp.minimum(j + 1, 3), t, r0)
                for t in range(2) for r0 in range(0, 224, 32)], QW4, 221)
        toks = {}
        for u in range(224):
            if u == QW1:
                @pl.when(j < 3)
                def _():
                    for c in c_wk(j + 1):
                        c.start(priority=1)

                @pl.when(j == 3)
                def _():
                    for c in c_early + c_late:
                        c.start(priority=1)

                for c in c_wk(j):
                    c.wait()
            if u == QW2:
                @pl.when(j < 3)
                def _():
                    for c in c_wv(j + 1) + [c_ckv(j + 1)]:
                        c.start(priority=1)

                @pl.when(j < 2)
                def _():
                    c_x(j + 2).start(priority=1)

                @pl.when(j < 3)
                def _():
                    c_x(j + 1).wait()

                for c in c_wv(j) + [c_ckv(j)]:
                    c.wait()
            q = qproj(u, toks.pop(u, None))
            res = []
            ps = fill.get(u, [])
            for n, p in enumerate(ps):
                row = (n * 128 // len(ps)) // 16 * 16
                if p.func is prep_w and p.args[2] == 0:
                    (wk_raw, wv_raw)[p.args[0]].bitcast(u32)[zq, 0, 1024:1032, :] = _u(q[row:row + 8])
                elif p.func is prep_c2:
                    cT_s[pl.ds(pl.multiple_of(512 + zq * 8, 8), 8), 0:128] = _u(q[row:row + 8])
                elif p.func is prep_x:
                    xT[pl.ds(pl.multiple_of(M + zq * 16, 16), 16), 0:128] = q[row:row + 16].astype(bf16)
                elif p.func is prep_ct:
                    ckv[pl.ds(pl.multiple_of(S + zq * 16, 16), 16), 0:128] = q[row:row + 16].astype(bf16)
                res += p()
            if res:
                toks[u + QLAG] = _tok(res)
        return carry

    jax.lax.fori_loop(0, 4, q_body, 0)
    for c in c_early:
        c.wait()

    tri = n_i <= k_i
    sgn = jnp.where((jax.lax.broadcasted_iota(jnp.int32, (1, P), 1) & 1) == 0, 1.0, -1.0).astype(f32)
    c_outa = cp(out_s.at[:, pl.ds(0, 384)], out_hbm.at[:, pl.ds(0, 384)], sem_o.at[8])
    HR, HI, PR, PI, KV = range(5)

    def blk_at(c, half=None):
        r0 = (c % 8) * CH
        rs = slice(r0, r0 + CH) if half is None else slice(r0 + 16 * half, r0 + 16 * half + 16)
        return rs, slice((c // 8) * P, (c // 8 + 1) * P)

    def tile(ref, n):
        return ref[:, n * 128:(n + 1) * 128]

    def head_body(h, carry):
        @pl.when(h == 1)
        def _():
            for c in c_late:
                c.wait()

        @pl.when(h == H - 1)
        def _():
            c_outa.start()

        st = dict(co={}, cnt={}, fin=set(), M={}, P={}, Q7={}, mfin={}, o={})
        zs = h >> 10
        z64 = pl.ds(pl.multiple_of(zs * 64, 64), 64)
        m_s, l_s = (m0_s, m1_s), (l0_s, l1_s)
        hrows = pl.ds(pl.multiple_of(h * 128, 128), 128)
        rows = pl.ds(pl.multiple_of(jnp.minimum(h, NCH - 1) * CH, CH), CH)

        def rep(t, n):
            return jnp.concatenate([taps[t, rows, :]] * n, axis=1)

        toks = []

        def due():
            for t in toks:
                t[0] -= 1
            ready = [t[1] for t in toks if t[0] <= 0]
            toks[:] = [t for t in toks if t[0] > 0]
            return functools.reduce(lambda x, y: x | y, ready) if ready else None

        def gate_later(vals):
            toks.append([SLAG, _tok([v if v.dtype == u32 else _u(v) for v in vals])])

        def row_offset(i):
            if i not in st['mfin']:
                m = m_s[i % 2][0, 0]
                for t in range(1, i + 1):
                    m = jnp.maximum(m, m_s[i % 2][0, t])
                m = jnp.max(m, axis=0, keepdims=True)
                if i > 0:
                    lo_ = jnp.exp2(m_s[i % 2][0, 0] - m)
                    for t in range(1, i + 1):
                        lo_ = lo_ + jnp.exp2(m_s[i % 2][0, t] - m)
                    m = m + jnp.log2(jnp.sum(lo_, axis=0, keepdims=True))
                st['mfin'][i] = m
            return st['mfin'][i]

        for op in _schedule():
            kind = op[0]
            if kind == 'KV':
                _, p, t = op
                n, m = SK[t // 7], SV[t % 7]

                def wblk(q):
                    w = w1_s[hrows, n * 512 + (q % 2) * 256:n * 512 + (q % 2) * 256 + 256]
                    r = (q // 2) * 32
                    return jnp.concatenate([w[r:r + 32], w[64 + r:64 + r + 32]], axis=0)

                cols = slice((n * 7 + m) * 256, (n * 7 + m + 1) * 256)
                if m in (2, 3):
                    w = wblk(0 if m == 2 else 3)
                elif p > 0:
                    w = w2_s[:, cols]
                else:
                    i1, i2, sg = _A_OF[m]
                    x, y = wblk(i1), wblk(i2)
                    w = _pk(*[f(x) + f(y) if sg > 0 else f(x) - f(y) for f in (_lo, _hi)])
                    w2_s[z64, cols] = w
                c2 = c2_s[p * 128:(p + 1) * 128, (n * 7 + m) * 128:(n * 7 + m + 1) * 128]
                st['M'][m] = st['last'] = _nn(_b(_gate(w, due())), _b(c2))
                if t % 7 < 6:
                    continue
                mo = _quad(*_c4(st['M']))
                for o, sg in _C_OF[n]:
                    k = st['cnt'][o] = st['cnt'].get(o, 0) + 1
                    if k == 1:
                        st['co'][o] = mo if sg > 0 else -mo
                    else:
                        st['co'][o] = st['co'][o] + mo if sg > 0 else st['co'][o] - mo
                    if k == _C_CNT[o]:
                        st['cnt'][o] = 0
                        st['fin'].add(o)
                for tok in range(2):
                    if not {tok, 2 + tok} <= st['fin']:
                        continue
                    st['fin'] -= {tok, 2 + tok}
                    c = 2 * p + tok

                    def full(dh, kb, off):
                        x = st['co'][2 * dh + tok][:, kb * 128:(kb + 1) * 128]
                        return jnp.concatenate([x[off:off + 64], x[128 + off:128 + off + 64]], axis=0)

                    kb4 = (full(0, 0, 0).T, full(1, 0, 0).T, full(0, 1, 0).T, full(1, 1, 0).T)
                    vb4 = (full(0, 0, 64), full(0, 1, 64), full(1, 0, 64), full(1, 1, 64))
                    for ref, c4 in ((K_s[c], kb4), (V_s[c], vb4)):
                        blks = dict(zip((2, 7, 8, 3), c4))
                        if c < NT - 1:
                            blks.update({k: x for k, x in enumerate(_a7(*c4)) if k not in (2, 3)})
                        for k, x in blks.items():
                            ref[z64, k * 128:(k + 1) * 128] = _u(x.astype(bf16))
            elif kind == 'QK':
                _, i, j = op
                S_s = (S0_s, S1_s)[i % 2]
                if j < i:
                    if i not in st['Q7']:
                        qu = QT_s[hrows, i * T:(i + 1) * T]
                        st['Q7'][i] = _combos_u(_b7, [qu[:64, :128], qu[:64, 128:], qu[64:, :128], qu[64:, 128:]])
                    s = _quad(*_c4({n: _nn(_b(tile(K_s[j], n)), _b(st['Q7'][i][n])) for n in SQ}))
                    S_s[zs, j] = s
                    f = _fold(s, jnp.max)
                else:
                    q = _b(QT_s[hrows, i * T:(i + 1) * T])
                    sa = _nn(_b(jnp.concatenate([tile(K_s[j], 2), tile(K_s[j], 7)], axis=1)), q)
                    sa = jnp.concatenate([jnp.where(tri, sa[:, :128], NEG), sa[:, 128:]], axis=1)
                    sb = _nn(_b(jnp.concatenate([tile(K_s[j], 8), tile(K_s[j], 3)], axis=1)), q[:, 128:])
                    sb = jnp.where(tri, sb, NEG)
                    S_s[zs, j, 0:128, :] = sa
                    S_s[zs, j, 128:T, 128:T] = sb
                    fa = _fold(sa, jnp.max)
                    f = jnp.concatenate([fa[:, :128], jnp.maximum(fa[:, 128:], _fold(sb, jnp.max))], axis=1)
                m_s[i % 2][zs, j] = f
                pace_s[zs] = f
            elif kind == 'EX':
                _, i, j = op
                S_s = (S0_s, S1_s)[i % 2]
                m = row_offset(i)
                m = jnp.where(pace_s[0, 0:1, :] == jnp.inf, jnp.inf, m)
                if j < i:
                    parts, lj = [], None
                    for r in range(112, -16, -16):
                        pt = jnp.exp2(S_s[0, j, r:r + 16, :] - m)
                        pb = jnp.exp2(S_s[0, j, 128 + r:128 + r + 16, :] - m)
                        parts.insert(0, _b7(pt[:, :128], pt[:, 128:], pb[:, :128], pb[:, 128:]))
                        x = (pt[:8] + pt[8:]) + (pb[:8] + pb[8:])
                        lj = x if lj is None else lj + x
                    st['P'][i, j] = [jnp.concatenate([x[n] for x in parts], axis=0).astype(bf16) for n in range(7)]
                else:
                    pa = jnp.exp2(S_s[0, j, 0:128, :] - m)
                    pb = jnp.exp2(S_s[0, j, 128:T, 128:T] - m[:, 128:])
                    la = _rsum(pa)
                    lj = jnp.concatenate([la[:, :128], la[:, 128:] + _rsum(pb)], axis=1)
                    st['P'][i, j] = (pa.astype(bf16), pb.astype(bf16))
                l_s[i % 2][zs, j] = lj
            elif kind == 'PV':
                _, i, j = op
                p = st['P'].pop((i, j))
                if j < i:
                    for n in SP:
                        st['last'] = _nn(_b(tile(V_s[j], n)), p[n])
                        st['o'][i, n] = st['o'][i, n] + st['last'] if j > 0 else st['last']
                    continue
                oa = _nn(_b(jnp.concatenate([tile(V_s[j], 2), tile(V_s[j], 8)], axis=0)), p[0])
                ob = _nn(_b(jnp.concatenate([tile(V_s[j], 7), tile(V_s[j], 3)], axis=0)), p[1])
                o = st['last'] = jnp.concatenate([oa[:, :128], oa[:, 128:] + ob], axis=1)
                if i > 0:
                    o = o + _quad(*_c4({n: st['o'].pop((i, n)) for n in range(7)}))
                l = l_s[i % 2][0, 0]
                for t in range(1, i + 1):
                    l = l + l_s[i % 2][0, t]
                o = o * (1.0 / jnp.sum(l, axis=0, keepdims=True))
                for n, x in enumerate(_b7(o[:128, :128], o[:128, 128:], o[128:, :128], o[128:, 128:])):
                    O_s[i][zs, n] = x.astype(bf16)
            elif kind == 'PACE':
                pace_s[zs] = jnp.concatenate([st['last'][-8:, -128:]] * 2, axis=1)
            elif kind == 'OP':
                _, i, t = op
                n = SO[t]
                st['M'][n] = st['last'] = _nn(_b(_gate(W7_s[0, n], due())), O_s[i][0, n])
                if t == 6:
                    acc[:, T * i:T * (i + 1)] += _quad(*_c4(st['M']))
            elif kind == 'W7':
                res = []
                for r0 in range(16 * op[1], 16 * op[2], 16):
                    blk = [_u(woT[h, r:r + 16, c:c + 128]) for r in (r0, 224 + r0) for c in (0, 128)]
                    w7 = _combos_u(_a7, blk)
                    for n, x in enumerate(w7):
                        W7_s[zs, n, r0 // 2:r0 // 2 + 8] = x
                    res += w7
                gate_later(res)
            elif kind == 'AT':
                g = jnp.clip((h - 4) // 4, 0, 2)
                t0 = jnp.minimum(((h + 12) % 4) * 6, NB - 6)
                grow = pl.ds(pl.multiple_of(g * 128, 128), 128)
                gcol = pl.ds(pl.multiple_of(jnp.where(h == H - 1, 3, g) * 128, 128), 128)
                res = []
                for n in range(6):
                    tok = pl.ds(pl.multiple_of((t0 + n) * 128, 128), 128)
                    x = aT_s[grow, tok].T
                    out_s[tok, gcol] = x
                    res.append(_u(x)[56:])
                gate_later(res)
            elif kind == 'HD':
                g = op[1]
                hs = jnp.concatenate([ssmk[rows, c * P:(c + 1) * P] for c in range(4 * g, 4 * g + 4)], axis=0)
                hf = _nn(hs, ff_s[...])
                for n in range(4):
                    X_s[(zs, HR) + blk_at(4 * g + n)] = hf[n * CH:(n + 1) * CH, :P]
                    X_s[(zs, HI) + blk_at(4 * g + n)] = hf[n * CH:(n + 1) * CH, P:]
            elif kind == 'SC':
                g = op[1]
                if g == 0:
                    k = jnp.concatenate([jnp.zeros((CH, P), f32), kT[rows, 0:4 * P].astype(f32)], axis=1)
                else:
                    k = kT[rows, (4 * g - 1) * P:(4 * g + 4) * P].astype(f32)
                ks = k[:, P:] * rep(0, 4)
                for j in range(1, KS):
                    ks = ks + pltpu.roll(k, j, 1)[:, P:] * rep(j, 4)
                kv = ks * vT[rows, 4 * g * P:(4 * g + 4) * P].astype(f32)
                kvs = jnp.concatenate([kv[:, n * P:(n + 1) * P] for n in range(4)], axis=0)
                xf = _nn(kvs.astype(bf16), ff_s[...])
                for n in range(4):
                    c = 4 * g + n
                    xr, xi = xf[n * CH:(n + 1) * CH, :P], xf[n * CH:(n + 1) * CH, P:]
                    X_s[(zs, KV) + blk_at(c)] = kvs[n * CH:(n + 1) * CH]
                    pr = xr if c == 0 else xr - sgn * st['x'][1]
                    pi = xi if c == 0 else xi + sgn * st['x'][0]
                    X_s[(zs, PR) + blk_at(c)] = pr
                    X_s[(zs, PI) + blk_at(c)] = pi
                    st['x'] = (xr, xi)
            elif kind == 'CV':
                res = []
                for a, half in op[1]:
                    wr = wi = None
                    for j in range(a + 1):
                        hr, hi_ = X_s[(0, HR) + blk_at(j, half)], X_s[(0, HI) + blk_at(j, half)]
                        pr, pi = X_s[(0, PR) + blk_at(a - j, half)], X_s[(0, PI) + blk_at(a - j, half)]
                        tr, ti = hr * pr - hi_ * pi, hr * pi + hi_ * pr
                        wr, wi = (tr, ti) if wr is None else (wr + tr, wi + ti)
                    r0 = (a % 4) * CH + 16 * half
                    Y_s[a // 4][zs, r0:r0 + 16, :P] = wr
                    Y_s[a // 4][zs, r0:r0 + 16, P:] = wi
                    res += [wr, wi]
                gate_later(res)
            elif kind == 'ID':
                g = op[1]
                y = _nn(Y_s[g][0].astype(bf16), fi_s[...])
                for n in range(4):
                    c = 4 * g + n
                    cols = slice(c * P, (c + 1) * P)
                    ya = y[n * CH:(n + 1) * CH, :] + X_s[(0, KV) + blk_at(c)] * taps[KS, rows, :]
                    aT_s[rows, cols] = (qT[rows, cols].astype(f32) * ya).astype(bf16)
        return carry

    jax.lax.fori_loop(0, H, head_body, 0)

    acc[:, T * (NT - 1):] += _quad(*_c4({n: _nn(_b(W7_s[0, n]), O_s[NT - 1][0, n]) for n in SORD}))
    outs = [c_outa]
    for i in range(NT):
        cols = slice(T * i, T * (i + 1))
        blk = jnp.concatenate([aT_s[384:M, cols], acc[:, cols].astype(bf16)], axis=0)
        out_s[cols, 384:2 * M] = blk.T
        c = cp(out_s.at[pl.ds(T * i, T), pl.ds(384, 512)], out_hbm.at[pl.ds(T * i, T), pl.ds(384, 512)], sem_o.at[i])
        c.start()
        outs.append(c)
    for c in outs:
        c.wait()


@jax.jit
def pallas_concat_heads__ssm_conv_h3__compressed_kv_cla__prompt_kernel(
    A_q: jax.Array,
    A_k: jax.Array,
    A_v: jax.Array,
    A_shift_k: jax.Array,
    A_ssm_k: jax.Array,
    A_ssm_D: jax.Array,
    B_x: jax.Array,
    B_c_kv: jax.Array,
    B_w_q: jax.Array,
    B_w_uk: jax.Array,
    B_w_uv: jax.Array,
    B_w_o: jax.Array,
):
    hbm = pl.BlockSpec(memory_space=pl.ANY)
    vmem = pl.BlockSpec(memory_space=pltpu.VMEM)
    V = pltpu.VMEM
    out = pl.pallas_call(
        _kernel,
        out_shape=jax.ShapeDtypeStruct((S, 2 * M), bf16),
        in_specs=[hbm, hbm, hbm, vmem, hbm, vmem, hbm, hbm, hbm, hbm, hbm, hbm],
        out_specs=hbm,
        scratch_shapes=[
            V((M, S), bf16), V((M, S), bf16), V((M, S), bf16), V((M, S), bf16),
            V((M + 16, S), bf16), V((S + 16, DC), bf16),
            V((2, M * H, 128), bf16),
            V((2, 4, 128 * H + 16, 128), bf16), V((2, 4, 128 * H + 16, 128), bf16),
            V((H, M, D), bf16),
            V((H * 64, 7 * 256), u32), V((NT * 112, 7 * 128), u32),
            V((H * 128, 7 * 512), u32), V((64, 49 * 256), u32),
            V((512 + 8, 512), u32),
            V((H * D // 2, S), u32), V((4 * 128, 49 * 128), u32),
            V((M, S), f32), V((M, S), bf16), V((S, 2 * M), bf16),
            V((KS + 1, M, 128), f32), V((P, 2 * P), bf16), V((2 * P, P), bf16),
            V((1, NT, T, T), f32), V((1, NT, T, T), f32), V((1, 5, T, T), f32),
            V((1, 7, 112, 128), u32), V((1, 8, T), f32),
            V((1, NT, 8, T), f32), V((1, NT, 8, T), f32), V((1, NT, 8, T), f32), V((1, NT, 8, T), f32),
            pltpu.SemaphoreType.DMA((26,)), pltpu.SemaphoreType.DMA((8,)),
            pltpu.SemaphoreType.DMA((8,)), pltpu.SemaphoreType.DMA((9,)),
        ] + [V((64, 9 * 128), u32)] * (2 * NT) + [V((1, 7, 128, 128), bf16)] * NT
        + [V((1, 4 * CH, 2 * P), f32)] * 4,
        compiler_params=pltpu.CompilerParams(vmem_limit_bytes=126 * 1024 * 1024,
                                             shape_invariant_numerics=False),
    )(
        A_q[0].T, A_k[0].T, A_v[0].T, A_shift_k.T, A_ssm_k, A_ssm_D,
        B_x[0].T, B_c_kv[0],
        B_w_q.reshape(M * H, D), B_w_uk.reshape(DC * H, D), B_w_uv.reshape(DC * H, D),
        jnp.transpose(B_w_o, (0, 2, 1)),
    )
    return out[None]
```

```python
import functools
import math

import jax
import jax.numpy as jnp
import jax.experimental.pallas as pl
import jax.experimental.pallas.tpu as pltpu

bf16 = jnp.bfloat16
f32 = jnp.float32
u32 = jnp.uint32

S = 2048
M = 448
DC = 1024
H = 16
D = 256
KS = 4
P = 128
NB = S // P
CH = 32
NCH = M // CH
T = 256
NT = S // T
NEG = -1e30

SORD = tuple(int(c) for c in '6430125')
SK = tuple(int(c) for c in '0364125')
SV = tuple(int(c) for c in '0125364')
SQ = tuple(int(c) for c in '6043125')
SP = tuple(int(c) for c in '3640125')
SO = tuple(int(c) for c in '5210346')
QW1 = 70
QW2 = 126
QW3 = 188
QW4 = 211
QC1 = 150
QLAG = 12
CVMAX = 12
SIDE0 = 30
SIDEP = 4
SLAG = 5
PRE = 0
W7P = 16
W7D = 6
KVH = 35
EXB = 10
NOP6 = 2
LA = 3
NOP = 2


def _nn(a, b):
    return jnp.dot(a, b, preferred_element_type=f32)


def _b(u):
    return pltpu.bitcast(u, bf16)


def _u(x):
    return pltpu.bitcast(x, u32)


def _lo(u):
    return pltpu.bitcast(u << 16, f32)


def _hi(u):
    return pltpu.bitcast(u & jnp.uint32(0xFFFF0000), f32)


def _pk(e, o):
    return pltpu.pack_elementwise([e, o], packed_dtype=bf16)


def _a7(a11, a12, a21, a22):
    return [a11 + a22, a21 + a22, a11, a22, a11 + a12, a21 - a11, a12 - a22]


def _b7(b11, b12, b21, b22):
    return [b11 + b22, b11, b12 - b22, b21 - b11, b22, b11 + b12, b21 + b22]


def _c4(m):
    return m[0] + m[3] - m[4] + m[6], m[2] + m[4], m[1] + m[3], m[0] - m[1] + m[2] + m[5]


_C_OF = (((0, 1), (3, 1)), ((2, 1), (3, -1)), ((1, 1), (3, 1)), ((0, 1), (2, 1)), ((0, -1), (1, 1)), ((3, 1),), ((0, 1),))
_C_CNT = (4, 2, 2, 4)
_A_OF = {0: (0, 3, 1), 1: (2, 3, 1), 4: (0, 1, 1), 5: (2, 0, -1), 6: (1, 3, -1)}


def _combos_u(f7, blk):
    e = f7(*[_lo(x) for x in blk])
    o = f7(*[_hi(x) for x in blk])
    plain = {2: 0, 3: 3} if f7 is _a7 else {1: 0, 4: 3}
    return [blk[plain[n]] if n in plain else _pk(e[n], o[n]) for n in range(7)]


def _quad(c11, c12, c21, c22):
    return jnp.concatenate([jnp.concatenate([c11, c12], axis=1), jnp.concatenate([c21, c22], axis=1)], axis=0)


def _fold(c, op):
    return op(c.reshape(-1, 8, c.shape[1]), axis=0)


def _rsum(p):
    cols = []
    for c in range(0, p.shape[1], 128):
        acc = None
        for r in range(112, -16, -16):
            t = p[r:r + 8, c:c + 128] + p[r + 8:r + 16, c:c + 128]
            acc = t if acc is None else acc + t
        cols.append(acc)
    return jnp.concatenate(cols, axis=1) if len(cols) > 1 else cols[0]


def _tok(vals):
    parts = []
    for v in vals:
        for r in range(0, v.shape[0], 8):
            for c in range(0, v.shape[1], 128):
                parts.append(v[r:r + 8, c:c + 128])
    while len(parts) > 1:
        parts = [parts[i] | parts[i + 1] if i + 1 < len(parts) else parts[i] for i in range(0, len(parts), 2)]
    return (parts[0] >> 31) >> 1


def _gate(x, tok):
    if tok is None:
        return x
    top = x[:8, :128] | tok
    if x.shape[1] > 128:
        top = jnp.concatenate([top, x[:8, 128:]], axis=1)
    return jnp.concatenate([top, x[8:]], axis=0)


def _side_pieces():
    ps = [(k, g) for g in range(PRE) for k in ('HD', 'SC')]
    cur, cost = [], 0
    for a in range(NB):
        if a % 4 == 0 and a // 4 + PRE < 4:
            ps += [('HD', a // 4 + PRE), ('SC', a // 4 + PRE)]
        for half in range(2):
            if cur and cost + a + 1 > CVMAX:
                ps.append(('CV', tuple(cur)))
                cur, cost = [], 0
            cur.append((a, half))
            cost += a + 1
        if a % 4 == 3:
            ps += [('CV', tuple(cur)), ('ID', a // 4)]
            cur, cost = [], 0
    ps.insert(W7P, ('W7', 0, 7))
    ps.insert(W7P + W7D, ('W7', 7, 14))
    return ps


def _schedule():
    side = _side_pieces()
    out = []
    cnt = [0]

    def block(subs, att, with_side):
        for k, u in enumerate(subs):
            out.append(u)
            out.extend(att.get(k, []))
            if with_side:
                cnt[0] += 1
                if side and cnt[0] >= SIDE0 and (cnt[0] - SIDE0) % SIDEP == 0:
                    out.append(side.pop(0))

    def kv(p, half):
        return [('KV', p, t) for t in (range(KVH) if half == 0 else range(KVH, 49))]

    def op_(*idx):
        return [('OP', i, t) for i in idx for t in range(7)]

    def softmax_head(i, n):
        att = {max(n - EXB, 0): [('PACE',), ('EX', i, 0)]}
        for k in range(1, min(LA, i + 1)):
            att.setdefault(n - 1 - (LA - 1 - k) * 2, []).extend([('PACE',), ('EX', i, k)])
        return att

    ops_left = list(range(NT - 1))
    block(kv(0, 0) + kv(0, 1), {}, True)
    block(op_(NT - 1), {6: [('AT',), ('QK', 0, 0)]}, False)
    block(kv(1, 0), softmax_head(0, KVH), True)
    for i in range(NT - 1):
        for j in range(i + 1):
            out.append(('QK', i + 1, j))
            if j + LA <= i:
                out.append(('EX', i, j + LA))
            out.append(('PV', i, j))
        out.append(('QK', i + 1, i + 1))
        if i < 5:
            subs = kv((i + 3) // 2, (i + 1) % 2)
            block(subs, softmax_head(i + 1, len(subs)), True)
        else:
            n = NOP6 if i == 5 else NOP
            block(op_(*ops_left[:n]), softmax_head(i + 1, 7 * n), False)
            del ops_left[:n]
    out.append(('PACE',))
    for j in range(NT):
        if j + LA < NT:
            out.append(('EX', NT - 1, j + LA))
        out.append(('PV', NT - 1, j))
        if len(ops_left) > 2:
            block(op_(ops_left.pop(0)), {}, False)
        out.append(('PACE',))
    block(op_(*ops_left), {}, False)
    assert not side
    w7 = [k for k, o in enumerate(out) if o[0] == 'W7']
    assert out.index(('OP', NT - 1, 6)) < min(w7) and max(w7) < out.index(('OP', 0, 0))
    out.remove(('ID', 3))
    out.append(('ID', 3))
    return out


def _kernel(qT_hbm, kT_hbm, vT_hbm, sk_ref, ssmk_hbm, dd_ref, xT_hbm, ckv_hbm,
            wq_hbm, wk_hbm, wv_hbm, woT_hbm, out_hbm,
            qT, kT, vT, ssmk, xT, ckv, wq_raw, wk_raw, wv_raw, woT,
            aq_s, bx_s, w1_s, w2_s, cT_s, QT_s, c2_s, acc, aT_s, out_s, taps, ff_s, fi_s,
            S0_s, S1_s, X_s, W7_s, pace_s, m0_s, m1_s, l0_s, l1_s,
            sem, sem_k, sem_v, sem_o, *rest):
    K_s, V_s, O_s, Y_s = rest[:NT], rest[NT:2 * NT], rest[2 * NT:3 * NT], rest[3 * NT:]

    def cp(src, dst, s):
        return pltpu.make_async_copy(src, dst, s)

    def c_x(j):
        cols = pl.ds(pl.multiple_of(j * 2 * T, 2 * T), 2 * T)
        return cp(xT_hbm.at[:, cols], xT.at[pl.ds(0, M), cols], sem.at[j])

    QP = ((0, 128), (128, 96))

    def c_wq(p):
        cs_ = []
        for half in range(2):
            r = pl.ds((half * 224 + QP[p][0]) * H, QP[p][1] * H)
            for g in range(2):
                cs_.append(cp(wq_hbm.at[r, pl.ds(128 * g, 128)], wq_raw.at[g, r], sem.at[18 + 4 * p + 2 * half + g]))
        return cs_

    def c_w(w_hbm, raw, sm, j, half, g):
        r = pl.ds(pl.multiple_of((half * 4 + j) * 2048, 2048), 2048)
        q = 2 * half + g
        return cp(w_hbm.at[r, pl.ds(128 * g, 128)], raw.at[j % 2, q, pl.ds(0, 2048)], sm.at[(j % 2) * 4 + q])

    def c_wk(j):
        return [c_w(wk_hbm, wk_raw, sem_k, j, half, g) for half in range(2) for g in range(2)]

    def c_wv(j):
        return [c_w(wv_hbm, wv_raw, sem_v, j, half, g) for half in range(2) for g in range(2)]

    def c_ckv(j):
        r = pl.ds(pl.multiple_of(j * 2 * T, 2 * T), 2 * T)
        return cp(ckv_hbm.at[r], ckv.at[r], sem.at[9 + j])

    a_pairs = ((kT_hbm, kT), (vT_hbm, vT), (ssmk_hbm, ssmk), (qT_hbm, qT))
    c_early = [cp(woT_hbm.at[pl.ds(0, 1)], woT.at[pl.ds(0, 1)], sem.at[4])]
    c_early += [cp(src.at[pl.ds(0, CH)], dst.at[pl.ds(0, CH)], sem.at[5 + n]) for n, (src, dst) in enumerate(a_pairs)]
    c_late = [cp(woT_hbm.at[pl.ds(1, H - 1)], woT.at[pl.ds(1, H - 1)], sem.at[13])]
    c_late += [cp(src.at[pl.ds(CH, M - CH)], dst.at[pl.ds(CH, M - CH)], sem.at[14 + n])
               for n, (src, dst) in enumerate(a_pairs)]
    for c in [c_x(0)] + c_wq(0) + c_wq(1):
        c.start()
    for c in c_wk(0) + [c_x(1)]:
        c.start(priority=1)

    n_i = jax.lax.broadcasted_iota(jnp.int32, (P, P), 0)
    k_i = jax.lax.broadcasted_iota(jnp.int32, (P, P), 1)
    ang = (((2 * k_i + 1) * n_i) & 511).astype(f32) * (math.pi / 256.0)
    cs, sn = jnp.cos(ang), jnp.sin(ang)
    ff_s[:, 0:P] = cs.astype(bf16)
    ff_s[:, P:2 * P] = (-sn).astype(bf16)
    fi_s[0:P, :] = (cs.T * (1.0 / P)).astype(bf16)
    fi_s[P:2 * P, :] = (sn.T * (-1.0 / P)).astype(bf16)
    sk = sk_ref[...].astype(f32)
    for t in range(KS):
        taps[t] = jnp.broadcast_to(sk[t:t + 1, :], (128, M)).T
    taps[KS] = jnp.broadcast_to(dd_ref[...].astype(f32).reshape(1, M), (128, M)).T
    acc[...] = jnp.zeros(acc.shape, f32)
    aT_s[...] = jnp.zeros(aT_s.shape, bf16)
    O_s[NT - 1][...] = jnp.zeros(O_s[0].shape, bf16)
    W7_s[...] = jnp.zeros(W7_s.shape, u32)

    def prep_x(jj, t, r0):
        c0 = (2 * jj + t) * T
        cs_ = [c0, c0 + 128] if isinstance(jj, int) else [pl.multiple_of(c0, 128), pl.multiple_of(c0 + 128, 128)]
        blk = [_u(xT[r:r + 32, pl.ds(c, 128)]) for r in (r0, 224 + r0) for c in cs_]
        row = (2 * jj + t) * 112 + r0 // 2
        row = pl.ds(row if isinstance(jj, int) else pl.multiple_of(row, 16), 16)
        for n, x in enumerate(_combos_u(_b7, blk)):
            bx_s[row, n * 128:(n + 1) * 128] = x
        return []

    c_x(0).wait()
    for t in range(2):
        for r0 in range(0, 224, 32):
            prep_x(0, t, r0)
    vq = wq_raw.bitcast(u32)
    for p, (c0, nc) in enumerate(QP):
        for c in c_wq(p):
            c.wait()
        for hp in range(H // 2):
            ut = [vq[g, pl.ds((half * 224 + c0) * 8 + hp, nc, stride=8), :].T for g in range(2) for half in range(2)]
            for r in range(0, 128, 16):
                u = [x[r:r + 16] for x in ut]
                for par, f in enumerate((_lo, _hi)):
                    r0 = (2 * hp + par) * 64 + r // 2
                    for n, x in enumerate(_a7(*[f(x) for x in u])):
                        aq_s[r0:r0 + 8, n * 256 + c0:n * 256 + c0 + nc] = _u(x.astype(bf16))
    for c in c_wv(0) + [c_ckv(0)]:
        c.start(priority=1)

    qscale = (D ** -0.5) * math.log2(math.e)

    def q_body(j, carry):
        mq = {}
        zq = j >> 4
        bx = [[bx_s[pl.ds(pl.multiple_of((2 * j + t) * 112, 16), 112), n * 128:(n + 1) * 128] for n in range(7)]
              for t in range(2)]

        def qproj(u, tok):
            hh, t, n = u // 14, (u // 7) % 2, SORD[u % 7]
            w = _b(_gate(aq_s[hh * 64:hh * 64 + 64, n * 256:n * 256 + 224], tok))
            mq[n] = _nn(w, _b(bx[t][n]))
            if u % 7 == 6:
                for k, x in enumerate(_c4(mq)):
                    cols = pl.ds(pl.multiple_of((2 * j + t) * T + (k % 2) * 128, 128), 128)
                    r0 = hh * 128 + (k // 2) * 64
                    QT_s[r0:r0 + 64, cols] = _u((x * qscale).astype(bf16))
            return mq[n]

        wt = {}

        def prep_w(kv, hp, part):
            if part == 0:
                v = (wk_raw, wv_raw)[kv].bitcast(u32).at[j % 2]
                wt[kv, hp] = [v[q, pl.ds(hp, 128, stride=8), :].T for q in (0, 2, 1, 3)]
                return [x[120:] for x in wt[kv, hp]]
            for r in range(32 * (part - 1), 32 * part, 16):
                u = [x[r:r + 16] for x in wt[kv, hp]]
                for par, f in enumerate((_lo, _hi)):
                    r0 = (2 * hp + par) * 128 + kv * 64 + r // 2
                    for n, c in enumerate(_a7(*[f(x) for x in u])):
                        cols = pl.ds(pl.multiple_of(n * 512 + j * 128, 128), 128)
                        w1_s[r0:r0 + 8, cols] = _u(c.astype(bf16))
            return []

        def prep_ct(half, cq):
            res = []
            ct = 2 * cq + half
            for tb in range(4):
                x = _u(ckv[pl.ds(pl.multiple_of(j * 512 + tb * 128, 128), 128), ct * 128:(ct + 1) * 128].T)
                cT_s[pl.ds(pl.multiple_of(zq * 64 + ct * 64, 64), 64), tb * 128:(tb + 1) * 128] = x
                res.append(x[56:])
            return res

        def prep_c2(r):
            blk = [[cT_s[cq * 128 + r:cq * 128 + r + 8, tb * 128:(tb + 1) * 128] for tb in range(4)] for cq in range(4)]
            two = []
            for f in (_lo, _hi):
                x = [[f(v) for v in row] for row in blk]
                outer = [[_b7(x[ci][ti], x[ci][2 + ti], x[2 + ci][ti], x[2 + ci][2 + ti]) for ti in range(2)]
                         for ci in range(2)]
                two.append([_b7(outer[0][0][n], outer[0][1][n], outer[1][0][n], outer[1][1][n]) for n in range(7)])
            row = pl.ds(pl.multiple_of(j * 128 + r, 8), 8)
            for n in range(7):
                for m in range(7):
                    c2_s[row, (n * 7 + m) * 128:(n * 7 + m + 1) * 128] = _pk(two[0][n][m], two[1][n][m])
            return []

        fill = {}

        def spread(pieces, u0, u1):
            for n, p in enumerate(pieces):
                fill.setdefault(u0 + n * (u1 - u0) // len(pieces), []).append(p)

        spread([functools.partial(prep_w, 0, hp, part) for hp in range(8) for part in range(5)], QW1, QW2)
        spread([functools.partial(prep_w, 1, hp, part) for hp in range(8) for part in range(5)], QW2, QW3)
        spread([functools.partial(prep_ct, 0, cq) for cq in range(4)], QW2 + 2, QC1)
        spread([functools.partial(prep_ct, 1, cq) for cq in range(4)], QC1, QW3)
        spread([functools.partial(prep_c2, r) for r in range(0, 128, 8)], QW3, QW4)
        spread([functools.partial(prep_x, jnp.minimum(j + 1, 3), t, r0)
                for t in range(2) for r0 in range(0, 224, 32)], QW4, 221)
        toks = {}
        for u in range(224):
            if u == QW1:
                @pl.when(j < 3)
                def _():
                    for c in c_wk(j + 1):
                        c.start(priority=1)

                @pl.when(j == 3)
                def _():
                    for c in c_early + c_late:
                        c.start(priority=1)

                for c in c_wk(j):
                    c.wait()
            if u == QW2:
                @pl.when(j < 3)
                def _():
                    for c in c_wv(j + 1) + [c_ckv(j + 1)]:
                        c.start(priority=1)

                @pl.when(j < 2)
                def _():
                    c_x(j + 2).start(priority=1)

                @pl.when(j < 3)
                def _():
                    c_x(j + 1).wait()

                for c in c_wv(j) + [c_ckv(j)]:
                    c.wait()
            q = qproj(u, toks.pop(u, None))
            res = []
            ps = fill.get(u, [])
            for n, p in enumerate(ps):
                row = (n * 128 // len(ps)) // 16 * 16
                if p.func is prep_w and p.args[2] == 0:
                    (wk_raw, wv_raw)[p.args[0]].bitcast(u32)[zq, 0, 1024:1032, :] = _u(q[row:row + 8])
                elif p.func is prep_c2:
                    cT_s[pl.ds(pl.multiple_of(512 + zq * 8, 8), 8), 0:128] = _u(q[row:row + 8])
                elif p.func is prep_x:
                    xT[pl.ds(pl.multiple_of(M + zq * 16, 16), 16), 0:128] = q[row:row + 16].astype(bf16)
                elif p.func is prep_ct:
                    ckv[pl.ds(pl.multiple_of(S + zq * 16, 16), 16), 0:128] = q[row:row + 16].astype(bf16)
                res += p()
            if res:
                toks[u + QLAG] = _tok(res)
        return carry

    jax.lax.fori_loop(0, 4, q_body, 0)
    for c in c_early:
        c.wait()

    tri = n_i <= k_i
    sgn = jnp.where((jax.lax.broadcasted_iota(jnp.int32, (1, P), 1) & 1) == 0, 1.0, -1.0).astype(f32)
    c_outa = cp(out_s.at[:, pl.ds(0, 384)], out_hbm.at[:, pl.ds(0, 384)], sem_o.at[8])
    HR, HI, PR, PI, KV = range(5)

    def blk_at(c, half=None):
        r0 = (c % 8) * CH
        rs = slice(r0, r0 + CH) if half is None else slice(r0 + 16 * half, r0 + 16 * half + 16)
        return rs, slice((c // 8) * P, (c // 8 + 1) * P)

    def tile(ref, n):
        return ref[:, n * 128:(n + 1) * 128]

    def head_body(h, carry):
        @pl.when(h == 1)
        def _():
            for c in c_late:
                c.wait()

        @pl.when(h == H - 1)
        def _():
            c_outa.start()

        st = dict(co={}, cnt={}, fin=set(), M={}, P={}, Q7={}, mfin={}, o={})
        zs = h >> 10
        z64 = pl.ds(pl.multiple_of(zs * 64, 64), 64)
        m_s, l_s = (m0_s, m1_s), (l0_s, l1_s)
        hrows = pl.ds(pl.multiple_of(h * 128, 128), 128)
        rows = pl.ds(pl.multiple_of(jnp.minimum(h, NCH - 1) * CH, CH), CH)

        def rep(t, n):
            return jnp.concatenate([taps[t, rows, :]] * n, axis=1)

        toks = []

        def due():
            for t in toks:
                t[0] -= 1
            ready = [t[1] for t in toks if t[0] <= 0]
            toks[:] = [t for t in toks if t[0] > 0]
            return functools.reduce(lambda x, y: x | y, ready) if ready else None

        def gate_later(vals):
            toks.append([SLAG, _tok([v if v.dtype == u32 else _u(v) for v in vals])])

        def row_offset(i):
            if i not in st['mfin']:
                m = m_s[i % 2][0, 0]
                for t in range(1, i + 1):
                    m = jnp.maximum(m, m_s[i % 2][0, t])
                m = jnp.max(m, axis=0, keepdims=True)
                if i > 0:
                    lo_ = jnp.exp2(m_s[i % 2][0, 0] - m)
                    for t in range(1, i + 1):
                        lo_ = lo_ + jnp.exp2(m_s[i % 2][0, t] - m)
                    m = m + jnp.log2(jnp.sum(lo_, axis=0, keepdims=True))
                st['mfin'][i] = m
            return st['mfin'][i]

        for op in _schedule():
            kind = op[0]
            if kind == 'KV':
                _, p, t = op
                n, m = SK[t // 7], SV[t % 7]

                def wblk(q):
                    w = w1_s[hrows, n * 512 + (q % 2) * 256:n * 512 + (q % 2) * 256 + 256]
                    r = (q // 2) * 32
                    return jnp.concatenate([w[r:r + 32], w[64 + r:64 + r + 32]], axis=0)

                cols = slice((n * 7 + m) * 256, (n * 7 + m + 1) * 256)
                if m in (2, 3):
                    w = wblk(0 if m == 2 else 3)
                elif p > 0:
                    w = w2_s[:, cols]
                else:
                    i1, i2, sg = _A_OF[m]
                    x, y = wblk(i1), wblk(i2)
                    w = _pk(*[f(x) + f(y) if sg > 0 else f(x) - f(y) for f in (_lo, _hi)])
                    w2_s[z64, cols] = w
                c2 = c2_s[p * 128:(p + 1) * 128, (n * 7 + m) * 128:(n * 7 + m + 1) * 128]
                st['M'][m] = st['last'] = _nn(_b(_gate(w, due())), _b(c2))
                if t % 7 < 6:
                    continue
                mo = _quad(*_c4(st['M']))
                for o, sg in _C_OF[n]:
                    k = st['cnt'][o] = st['cnt'].get(o, 0) + 1
                    if k == 1:
                        st['co'][o] = mo if sg > 0 else -mo
                    else:
                        st['co'][o] = st['co'][o] + mo if sg > 0 else st['co'][o] - mo
                    if k == _C_CNT[o]:
                        st['cnt'][o] = 0
                        st['fin'].add(o)
                for tok in range(2):
                    if not {tok, 2 + tok} <= st['fin']:
                        continue
                    st['fin'] -= {tok, 2 + tok}
                    c = 2 * p + tok

                    def full(dh, kb, off):
                        x = st['co'][2 * dh + tok][:, kb * 128:(kb + 1) * 128]
                        return jnp.concatenate([x[off:off + 64], x[128 + off:128 + off + 64]], axis=0)

                    kb4 = (full(0, 0, 0).T, full(1, 0, 0).T, full(0, 1, 0).T, full(1, 1, 0).T)
                    vb4 = (full(0, 0, 64), full(0, 1, 64), full(1, 0, 64), full(1, 1, 64))
                    for ref, c4 in ((K_s[c], kb4), (V_s[c], vb4)):
                        blks = dict(zip((2, 7, 8, 3), c4))
                        if c < NT - 1:
                            blks.update({k: x for k, x in enumerate(_a7(*c4)) if k not in (2, 3)})
                        for k, x in blks.items():
                            ref[z64, k * 128:(k + 1) * 128] = _u(x.astype(bf16))
            elif kind == 'QK':
                _, i, j = op
                S_s = (S0_s, S1_s)[i % 2]
                if j < i:
                    if i not in st['Q7']:
                        qu = QT_s[hrows, i * T:(i + 1) * T]
                        st['Q7'][i] = _combos_u(_b7, [qu[:64, :128], qu[:64, 128:], qu[64:, :128], qu[64:, 128:]])
                    s = _quad(*_c4({n: _nn(_b(tile(K_s[j], n)), _b(st['Q7'][i][n])) for n in SQ}))
                    S_s[zs, j] = s
                    f = _fold(s, jnp.max)
                else:
                    q = _b(QT_s[hrows, i * T:(i + 1) * T])
                    sa = _nn(_b(jnp.concatenate([tile(K_s[j], 2), tile(K_s[j], 7)], axis=1)), q)
                    sa = jnp.concatenate([jnp.where(tri, sa[:, :128], NEG), sa[:, 128:]], axis=1)
                    sb = _nn(_b(jnp.concatenate([tile(K_s[j], 8), tile(K_s[j], 3)], axis=1)), q[:, 128:])
                    sb = jnp.where(tri, sb, NEG)
                    S_s[zs, j, 0:128, :] = sa
                    S_s[zs, j, 128:T, 128:T] = sb
                    fa = _fold(sa, jnp.max)
                    f = jnp.concatenate([fa[:, :128], jnp.maximum(fa[:, 128:], _fold(sb, jnp.max))], axis=1)
                m_s[i % 2][zs, j] = f
                pace_s[zs] = f
            elif kind == 'EX':
                _, i, j = op
                S_s = (S0_s, S1_s)[i % 2]
                m = row_offset(i)
                m = jnp.where(pace_s[0, 0:1, :] == jnp.inf, jnp.inf, m)
                if j < i:
                    parts, lj = [], None
                    for r in range(112, -16, -16):
                        pt = jnp.exp2(S_s[0, j, r:r + 16, :] - m)
                        pb = jnp.exp2(S_s[0, j, 128 + r:128 + r + 16, :] - m)
                        parts.insert(0, _b7(pt[:, :128], pt[:, 128:], pb[:, :128], pb[:, 128:]))
                        x = (pt[:8] + pt[8:]) + (pb[:8] + pb[8:])
                        lj = x if lj is None else lj + x
                    st['P'][i, j] = [jnp.concatenate([x[n] for x in parts], axis=0).astype(bf16) for n in range(7)]
                else:
                    pa = jnp.exp2(S_s[0, j, 0:128, :] - m)
                    pb = jnp.exp2(S_s[0, j, 128:T, 128:T] - m[:, 128:])
                    la = _rsum(pa)
                    lj = jnp.concatenate([la[:, :128], la[:, 128:] + _rsum(pb)], axis=1)
                    st['P'][i, j] = (pa.astype(bf16), pb.astype(bf16))
                l_s[i % 2][zs, j] = lj
            elif kind == 'PV':
                _, i, j = op
                p = st['P'].pop((i, j))
                if j < i:
                    for n in SP:
                        st['last'] = _nn(_b(tile(V_s[j], n)), p[n])
                        st['o'][i, n] = st['o'][i, n] + st['last'] if j > 0 else st['last']
                    continue
                oa = _nn(_b(jnp.concatenate([tile(V_s[j], 2), tile(V_s[j], 8)], axis=0)), p[0])
                ob = _nn(_b(jnp.concatenate([tile(V_s[j], 7), tile(V_s[j], 3)], axis=0)), p[1])
                o = st['last'] = jnp.concatenate([oa[:, :128], oa[:, 128:] + ob], axis=1)
                if i > 0:
                    o = o + _quad(*_c4({n: st['o'].pop((i, n)) for n in range(7)}))
                l = l_s[i % 2][0, 0]
                for t in range(1, i + 1):
                    l = l + l_s[i % 2][0, t]
                o = o * (1.0 / jnp.sum(l, axis=0, keepdims=True))
                for n, x in enumerate(_b7(o[:128, :128], o[:128, 128:], o[128:, :128], o[128:, 128:])):
                    O_s[i][zs, n] = x.astype(bf16)
            elif kind == 'PACE':
                pace_s[zs] = jnp.concatenate([st['last'][-8:, -128:]] * 2, axis=1)
            elif kind == 'OP':
                _, i, t = op
                n = SO[t]
                st['M'][n] = st['last'] = _nn(_b(_gate(W7_s[0, n], due())), O_s[i][0, n])
                if t == 6:
                    acc[:, T * i:T * (i + 1)] += _quad(*_c4(st['M']))
            elif kind == 'W7':
                res = []
                for r0 in range(16 * op[1], 16 * op[2], 16):
                    blk = [_u(woT[h, r:r + 16, c:c + 128]) for r in (r0, 224 + r0) for c in (0, 128)]
                    w7 = _combos_u(_a7, blk)
                    for n, x in enumerate(w7):
                        W7_s[zs, n, r0 // 2:r0 // 2 + 8] = x
                    res += w7
                gate_later(res)
            elif kind == 'AT':
                g = jnp.clip((h - 4) // 4, 0, 2)
                t0 = jnp.minimum(((h + 12) % 4) * 6, NB - 6)
                grow = pl.ds(pl.multiple_of(g * 128, 128), 128)
                gcol = pl.ds(pl.multiple_of(jnp.where(h == H - 1, 3, g) * 128, 128), 128)
                res = []
                for n in range(6):
                    tok = pl.ds(pl.multiple_of((t0 + n) * 128, 128), 128)
                    x = aT_s[grow, tok].T
                    out_s[tok, gcol] = x
                    res.append(_u(x)[56:])
                gate_later(res)
            elif kind == 'HD':
                g = op[1]
                hs = jnp.concatenate([ssmk[rows, c * P:(c + 1) * P] for c in range(4 * g, 4 * g + 4)], axis=0)
                hf = _nn(hs, ff_s[...])
                for n in range(4):
                    X_s[(zs, HR) + blk_at(4 * g + n)] = hf[n * CH:(n + 1) * CH, :P]
                    X_s[(zs, HI) + blk_at(4 * g + n)] = hf[n * CH:(n + 1) * CH, P:]
            elif kind == 'SC':
                g = op[1]
                if g == 0:
                    k = jnp.concatenate([jnp.zeros((CH, P), f32), kT[rows, 0:4 * P].astype(f32)], axis=1)
                else:
                    k = kT[rows, (4 * g - 1) * P:(4 * g + 4) * P].astype(f32)
                ks = k[:, P:] * rep(0, 4)
                for j in range(1, KS):
                    ks = ks + pltpu.roll(k, j, 1)[:, P:] * rep(j, 4)
                kv = ks * vT[rows, 4 * g * P:(4 * g + 4) * P].astype(f32)
                kvs = jnp.concatenate([kv[:, n * P:(n + 1) * P] for n in range(4)], axis=0)
                xf = _nn(kvs.astype(bf16), ff_s[...])
                for n in range(4):
                    c = 4 * g + n
                    xr, xi = xf[n * CH:(n + 1) * CH, :P], xf[n * CH:(n + 1) * CH, P:]
                    X_s[(zs, KV) + blk_at(c)] = kvs[n * CH:(n + 1) * CH]
                    pr = xr if c == 0 else xr - sgn * st['x'][1]
                    pi = xi if c == 0 else xi + sgn * st['x'][0]
                    X_s[(zs, PR) + blk_at(c)] = pr
                    X_s[(zs, PI) + blk_at(c)] = pi
                    st['x'] = (xr, xi)
            elif kind == 'CV':
                res = []
                for a, half in op[1]:
                    wr = wi = None
                    for j in range(a + 1):
                        hr, hi_ = X_s[(0, HR) + blk_at(j, half)], X_s[(0, HI) + blk_at(j, half)]
                        pr, pi = X_s[(0, PR) + blk_at(a - j, half)], X_s[(0, PI) + blk_at(a - j, half)]
                        tr, ti = hr * pr - hi_ * pi, hr * pi + hi_ * pr
                        wr, wi = (tr, ti) if wr is None else (wr + tr, wi + ti)
                    r0 = (a % 4) * CH + 16 * half
                    Y_s[a // 4][zs, r0:r0 + 16, :P] = wr
                    Y_s[a // 4][zs, r0:r0 + 16, P:] = wi
                    res += [wr, wi]
                gate_later(res)
            elif kind == 'ID':
                g = op[1]
                y = _nn(Y_s[g][0].astype(bf16), fi_s[...])
                for n in range(4):
                    c = 4 * g + n
                    cols = slice(c * P, (c + 1) * P)
                    ya = y[n * CH:(n + 1) * CH, :] + X_s[(0, KV) + blk_at(c)] * taps[KS, rows, :]
                    aT_s[rows, cols] = (qT[rows, cols].astype(f32) * ya).astype(bf16)
        return carry

    jax.lax.fori_loop(0, H, head_body, 0)

    acc[:, T * (NT - 1):] += _quad(*_c4({n: _nn(_b(W7_s[0, n]), O_s[NT - 1][0, n]) for n in SORD}))
    outs = [c_outa]
    for i in range(NT):
        cols = slice(T * i, T * (i + 1))
        blk = jnp.concatenate([aT_s[384:M, cols], acc[:, cols].astype(bf16)], axis=0)
        out_s[cols, 384:2 * M] = blk.T
        c = cp(out_s.at[pl.ds(T * i, T), pl.ds(384, 512)], out_hbm.at[pl.ds(T * i, T), pl.ds(384, 512)], sem_o.at[i])
        c.start()
        outs.append(c)
    for c in outs:
        c.wait()


@jax.jit
def pallas_concat_heads__ssm_conv_h3__compressed_kv_cla__prompt_kernel(
    A_q: jax.Array,
    A_k: jax.Array,
    A_v: jax.Array,
    A_shift_k: jax.Array,
    A_ssm_k: jax.Array,
    A_ssm_D: jax.Array,
    B_x: jax.Array,
    B_c_kv: jax.Array,
    B_w_q: jax.Array,
    B_w_uk: jax.Array,
    B_w_uv: jax.Array,
    B_w_o: jax.Array,
):
    hbm = pl.BlockSpec(memory_space=pl.ANY)
    vmem = pl.BlockSpec(memory_space=pltpu.VMEM)
    V = pltpu.VMEM
    out = pl.pallas_call(
        _kernel,
        out_shape=jax.ShapeDtypeStruct((S, 2 * M), bf16),
        in_specs=[hbm, hbm, hbm, vmem, hbm, vmem, hbm, hbm, hbm, hbm, hbm, hbm],
        out_specs=hbm,
        scratch_shapes=[
            V((M, S), bf16), V((M, S), bf16), V((M, S), bf16), V((M, S), bf16),
            V((M + 16, S), bf16), V((S + 16, DC), bf16),
            V((2, M * H, 128), bf16),
            V((2, 4, 128 * H + 16, 128), bf16), V((2, 4, 128 * H + 16, 128), bf16),
            V((H, M, D), bf16),
            V((H * 64, 7 * 256), u32), V((NT * 112, 7 * 128), u32),
            V((H * 128, 7 * 512), u32), V((64, 49 * 256), u32),
            V((512 + 8, 512), u32),
            V((H * D // 2, S), u32), V((4 * 128, 49 * 128), u32),
            V((M, S), f32), V((M, S), bf16), V((S, 2 * M), bf16),
            V((KS + 1, M, 128), f32), V((P, 2 * P), bf16), V((2 * P, P), bf16),
            V((1, NT, T, T), f32), V((1, NT, T, T), f32), V((1, 5, T, T), f32),
            V((1, 7, 112, 128), u32), V((1, 8, T), f32),
            V((1, NT, 8, T), f32), V((1, NT, 8, T), f32), V((1, NT, 8, T), f32), V((1, NT, 8, T), f32),
            pltpu.SemaphoreType.DMA((26,)), pltpu.SemaphoreType.DMA((8,)),
            pltpu.SemaphoreType.DMA((8,)), pltpu.SemaphoreType.DMA((9,)),
        ] + [V((64, 9 * 128), u32)] * (2 * NT) + [V((1, 7, 128, 128), bf16)] * NT
        + [V((1, 4 * CH, 2 * P), f32)] * 4,
        compiler_params=pltpu.CompilerParams(vmem_limit_bytes=126 * 1024 * 1024,
                                             shape_invariant_numerics=False),
    )(
        A_q[0].T, A_k[0].T, A_v[0].T, A_shift_k.T, A_ssm_k, A_ssm_D,
        B_x[0].T, B_c_kv[0],
        B_w_q.reshape(M * H, D), B_w_uk.reshape(DC * H, D), B_w_uv.reshape(DC * H, D),
        jnp.transpose(B_w_o, (0, 2, 1)),
    )
    return out[None]
```

```python
import functools
import math

import jax
import jax.numpy as jnp
import jax.experimental.pallas as pl
import jax.experimental.pallas.tpu as pltpu

bf16 = jnp.bfloat16
f32 = jnp.float32
u32 = jnp.uint32

S = 2048
M = 448
DC = 1024
H = 16
D = 256
KS = 4
P = 128
NB = S // P
CH = 32
NCH = M // CH
T = 256
NT = S // T
NEG = -1e30

SORD = tuple(int(c) for c in '6430125')
SK = tuple(int(c) for c in '0364125')
SV = tuple(int(c) for c in '0125364')
SQ = tuple(int(c) for c in '6043125')
SP = tuple(int(c) for c in '3640125')
SO = tuple(int(c) for c in '5210346')
QW1 = 70
QW2 = 126
QW3 = 188
QW4 = 211
QC1 = 150
QLAG = 12
CVMAX = 12
SIDE0 = 30
SIDEP = 4
SLAG = 5
PRE = 0
W7P = 16
W7D = 6
KVH = 35
EXB = 10
NOP6 = 2
LA = 3
NOP = 2


def _nn(a, b):
    return jnp.dot(a, b, preferred_element_type=f32)


def _b(u):
    return pltpu.bitcast(u, bf16)


def _u(x):
    return pltpu.bitcast(x, u32)


def _lo(u):
    return pltpu.bitcast(u << 16, f32)


def _hi(u):
    return pltpu.bitcast(u & jnp.uint32(0xFFFF0000), f32)


def _f(u):
    return _b(u).astype(f32)


def _a7(a11, a12, a21, a22):
    return [a11 + a22, a21 + a22, a11, a22, a11 + a12, a21 - a11, a12 - a22]


def _b7(b11, b12, b21, b22):
    return [b11 + b22, b11, b12 - b22, b21 - b11, b22, b11 + b12, b21 + b22]


def _c4(m):
    return m[0] + m[3] - m[4] + m[6], m[2] + m[4], m[1] + m[3], m[0] - m[1] + m[2] + m[5]


_C_OF = (((0, 1), (3, 1)), ((2, 1), (3, -1)), ((1, 1), (3, 1)), ((0, 1), (2, 1)), ((0, -1), (1, 1)), ((3, 1),), ((0, 1),))
_C_CNT = (4, 2, 2, 4)
_A_OF = {0: (0, 3, 1), 1: (2, 3, 1), 4: (0, 1, 1), 5: (2, 0, -1), 6: (1, 3, -1)}


def _combos(f7, blk):
    x = f7(*[_f(v) for v in blk])
    plain = {2: 0, 3: 3} if f7 is _a7 else {1: 0, 4: 3}
    return [_b(blk[plain[n]]) if n in plain else x[n].astype(bf16) for n in range(7)]


def _quad(c11, c12, c21, c22):
    return jnp.concatenate([jnp.concatenate([c11, c12], axis=1), jnp.concatenate([c21, c22], axis=1)], axis=0)


def _fold(c, op):
    return op(c.reshape(-1, 8, c.shape[1]), axis=0)


def _rsum(p):
    cols = []
    for c in range(0, p.shape[1], 128):
        acc = None
        for r in range(112, -16, -16):
            t = p[r:r + 8, c:c + 128] + p[r + 8:r + 16, c:c + 128]
            acc = t if acc is None else acc + t
        cols.append(acc)
    return jnp.concatenate(cols, axis=1) if len(cols) > 1 else cols[0]


def _tok(vals):
    parts = []
    for v in vals:
        for r in range(0, v.shape[0], 8):
            for c in range(0, v.shape[1], 128):
                parts.append(v[r:r + 8, c:c + 128])
    while len(parts) > 1:
        parts = [parts[i] | parts[i + 1] if i + 1 < len(parts) else parts[i] for i in range(0, len(parts), 2)]
    return (parts[0] >> 31) >> 1


def _gate(x, tok):
    if tok is None:
        return x
    top = x[:8, :128] | tok
    if x.shape[1] > 128:
        top = jnp.concatenate([top, x[:8, 128:]], axis=1)
    return jnp.concatenate([top, x[8:]], axis=0)


def _side_pieces():
    ps = [(k, g) for g in range(PRE) for k in ('HD', 'SC')]
    cur, cost = [], 0
    for a in range(NB):
        if a % 4 == 0 and a // 4 + PRE < 4:
            ps += [('HD', a // 4 + PRE), ('SC', a // 4 + PRE)]
        for half in range(2):
            if cur and cost + a + 1 > CVMAX:
                ps.append(('CV', tuple(cur)))
                cur, cost = [], 0
            cur.append((a, half))
            cost += a + 1
        if a % 4 == 3:
            ps += [('CV', tuple(cur)), ('ID', a // 4)]
            cur, cost = [], 0
    ps.insert(W7P, ('W7', 0, 7))
    ps.insert(W7P + W7D, ('W7', 7, 14))
    return ps


def _schedule():
    side = _side_pieces()
    out = []
    cnt = [0]

    def block(subs, att, with_side):
        for k, u in enumerate(subs):
            out.append(u)
            out.extend(att.get(k, []))
            if with_side:
                cnt[0] += 1
                if side and cnt[0] >= SIDE0 and (cnt[0] - SIDE0) % SIDEP == 0:
                    out.append(side.pop(0))

    def kv(p, half):
        return [('KV', p, t) for t in (range(KVH) if half == 0 else range(KVH, 49))]

    def op_(*idx):
        return [('OP', i, t) for i in idx for t in range(7)]

    def softmax_head(i, n):
        att = {max(n - EXB, 0): [('PACE',), ('EX', i, 0)]}
        for k in range(1, min(LA, i + 1)):
            att.setdefault(n - 1 - (LA - 1 - k) * 2, []).extend([('PACE',), ('EX', i, k)])
        return att

    ops_left = list(range(NT - 1))
    block(kv(0, 0) + kv(0, 1), {}, True)
    block(op_(NT - 1), {6: [('AT',), ('QK', 0, 0)]}, False)
    block(kv(1, 0), softmax_head(0, KVH), True)
    for i in range(NT - 1):
        for j in range(i + 1):
            out.append(('QK', i + 1, j))
            if j + LA <= i:
                out.append(('EX', i, j + LA))
            out.append(('PV', i, j))
        out.append(('QK', i + 1, i + 1))
        if i < 5:
            subs = kv((i + 3) // 2, (i + 1) % 2)
            block(subs, softmax_head(i + 1, len(subs)), True)
        else:
            n = NOP6 if i == 5 else NOP
            block(op_(*ops_left[:n]), softmax_head(i + 1, 7 * n), False)
            del ops_left[:n]
    out.append(('PACE',))
    for j in range(NT):
        if j + LA < NT:
            out.append(('EX', NT - 1, j + LA))
        out.append(('PV', NT - 1, j))
        if len(ops_left) > 2:
            block(op_(ops_left.pop(0)), {}, False)
        out.append(('PACE',))
    block(op_(*ops_left), {}, False)
    assert not side
    w7 = [k for k, o in enumerate(out) if o[0] == 'W7']
    assert out.index(('OP', NT - 1, 6)) < min(w7) and max(w7) < out.index(('OP', 0, 0))
    out.remove(('ID', 3))
    out.append(('ID', 3))
    return out


def _kernel(qT_hbm, kT_hbm, vT_hbm, sk_ref, ssmk_hbm, dd_ref, xT_hbm, ckv_hbm,
            wq_hbm, wk_hbm, wv_hbm, woT_hbm, out_hbm,
            qT, kT, vT, ssmk, xT, ckv, wq_raw, wk_raw, wv_raw, woT,
            aq_s, bx_s, w1_s, w2_s, cT_s, QT_s, c2_s, acc, aT_s, out_s, taps, ff_s, fi_s,
            S0_s, S1_s, X_s, W7_s, pace_s, m0_s, m1_s, l0_s, l1_s,
            sem, sem_k, sem_v, sem_o, *rest):
    K_s, V_s, O_s, Y_s = rest[:NT], rest[NT:2 * NT], rest[2 * NT:3 * NT], rest[3 * NT:]

    def cp(src, dst, s):
        return pltpu.make_async_copy(src, dst, s)

    def c_x(j):
        cols = pl.ds(pl.multiple_of(j * 2 * T, 2 * T), 2 * T)
        return cp(xT_hbm.at[:, cols], xT.at[pl.ds(0, M), cols], sem.at[j])

    QP = ((0, 128), (128, 96))

    def c_wq(p):
        cs_ = []
        for half in range(2):
            r = pl.ds((half * 224 + QP[p][0]) * H, QP[p][1] * H)
            for g in range(2):
                cs_.append(cp(wq_hbm.at[r, pl.ds(128 * g, 128)], wq_raw.at[g, r], sem.at[18 + 4 * p + 2 * half + g]))
        return cs_

    def c_w(w_hbm, raw, sm, j, half, g):
        r = pl.ds(pl.multiple_of((half * 4 + j) * 2048, 2048), 2048)
        q = 2 * half + g
        return cp(w_hbm.at[r, pl.ds(128 * g, 128)], raw.at[j % 2, q, pl.ds(0, 2048)], sm.at[(j % 2) * 4 + q])

    def c_wk(j):
        return [c_w(wk_hbm, wk_raw, sem_k, j, half, g) for half in range(2) for g in range(2)]

    def c_wv(j):
        return [c_w(wv_hbm, wv_raw, sem_v, j, half, g) for half in range(2) for g in range(2)]

    def c_ckv(j):
        r = pl.ds(pl.multiple_of(j * 2 * T, 2 * T), 2 * T)
        return cp(ckv_hbm.at[r], ckv.at[r], sem.at[9 + j])

    a_pairs = ((kT_hbm, kT), (vT_hbm, vT), (ssmk_hbm, ssmk), (qT_hbm, qT))
    c_early = [cp(woT_hbm.at[pl.ds(0, 1)], woT.at[pl.ds(0, 1)], sem.at[4])]
    c_early += [cp(src.at[pl.ds(0, CH)], dst.at[pl.ds(0, CH)], sem.at[5 + n]) for n, (src, dst) in enumerate(a_pairs)]
    c_late = [cp(woT_hbm.at[pl.ds(1, H - 1)], woT.at[pl.ds(1, H - 1)], sem.at[13])]
    c_late += [cp(src.at[pl.ds(CH, M - CH)], dst.at[pl.ds(CH, M - CH)], sem.at[14 + n])
               for n, (src, dst) in enumerate(a_pairs)]
    for c in [c_x(0)] + c_wq(0) + c_wq(1):
        c.start()
    for c in c_wk(0) + [c_x(1)]:
        c.start(priority=1)

    n_i = jax.lax.broadcasted_iota(jnp.int32, (P, P), 0)
    k_i = jax.lax.broadcasted_iota(jnp.int32, (P, P), 1)
    ang = (((2 * k_i + 1) * n_i) & 511).astype(f32) * (math.pi / 256.0)
    cs, sn = jnp.cos(ang), jnp.sin(ang)
    ff_s[:, 0:P] = cs.astype(bf16)
    ff_s[:, P:2 * P] = (-sn).astype(bf16)
    fi_s[0:P, :] = (cs.T * (1.0 / P)).astype(bf16)
    fi_s[P:2 * P, :] = (sn.T * (-1.0 / P)).astype(bf16)
    sk = sk_ref[...].astype(f32)
    for t in range(KS):
        taps[t] = jnp.broadcast_to(sk[t:t + 1, :], (128, M)).T
    taps[KS] = jnp.broadcast_to(dd_ref[...].astype(f32).reshape(1, M), (128, M)).T
    acc[...] = jnp.zeros(acc.shape, f32)
    aT_s[...] = jnp.zeros(aT_s.shape, bf16)
    O_s[NT - 1][...] = jnp.zeros(O_s[0].shape, bf16)
    W7_s[...] = jnp.zeros(W7_s.shape, u32)

    def prep_x(jj, t, r0):
        c0 = (2 * jj + t) * T
        cs_ = [c0, c0 + 128] if isinstance(jj, int) else [pl.multiple_of(c0, 128), pl.multiple_of(c0 + 128, 128)]
        blk = [_u(xT[r:r + 32, pl.ds(c, 128)]) for r in (r0, 224 + r0) for c in cs_]
        row = (2 * jj + t) * 112 + r0 // 2
        row = pl.ds(row if isinstance(jj, int) else pl.multiple_of(row, 16), 16)
        for n, x in enumerate(_combos(_b7, blk)):
            bx_s[row, n * 128:(n + 1) * 128] = _u(x)
        return []

    c_x(0).wait()
    for t in range(2):
        for r0 in range(0, 224, 32):
            prep_x(0, t, r0)
    vq = wq_raw.bitcast(u32)
    for p, (c0, nc) in enumerate(QP):
        for c in c_wq(p):
            c.wait()
        for hp in range(H // 2):
            ut = [vq[g, pl.ds((half * 224 + c0) * 8 + hp, nc, stride=8), :].T for g in range(2) for half in range(2)]
            for r in range(0, 128, 16):
                u = [x[r:r + 16] for x in ut]
                for par, f in enumerate((_lo, _hi)):
                    r0 = (2 * hp + par) * 64 + r // 2
                    for n, x in enumerate(_a7(*[f(x) for x in u])):
                        aq_s[r0:r0 + 8, n * 256 + c0:n * 256 + c0 + nc] = _u(x.astype(bf16))
    for c in c_wv(0) + [c_ckv(0)]:
        c.start(priority=1)

    qscale = (D ** -0.5) * math.log2(math.e)

    def q_body(j, carry):
        mq = {}
        zq = j >> 4
        bx = [[bx_s[pl.ds(pl.multiple_of((2 * j + t) * 112, 16), 112), n * 128:(n + 1) * 128] for n in range(7)]
              for t in range(2)]

        def qproj(u, tok):
            hh, t, n = u // 14, (u // 7) % 2, SORD[u % 7]
            w = _b(_gate(aq_s[hh * 64:hh * 64 + 64, n * 256:n * 256 + 224], tok))
            mq[n] = _nn(w, _b(bx[t][n]))
            if u % 7 == 6:
                for k, x in enumerate(_c4(mq)):
                    cols = pl.ds(pl.multiple_of((2 * j + t) * T + (k % 2) * 128, 128), 128)
                    r0 = hh * 128 + (k // 2) * 64
                    QT_s[r0:r0 + 64, cols] = _u((x * qscale).astype(bf16))
            return mq[n]

        wt = {}

        def prep_w(kv, hp, part):
            if part == 0:
                v = (wk_raw, wv_raw)[kv].bitcast(u32).at[j % 2]
                wt[kv, hp] = [v[q, pl.ds(hp, 128, stride=8), :].T for q in (0, 2, 1, 3)]
                return [x[120:] for x in wt[kv, hp]]
            for r in range(32 * (part - 1), 32 * part, 16):
                u = [x[r:r + 16] for x in wt[kv, hp]]
                for par, f in enumerate((_lo, _hi)):
                    r0 = (2 * hp + par) * 128 + kv * 64 + r // 2
                    for n, c in enumerate(_a7(*[f(x) for x in u])):
                        cols = pl.ds(pl.multiple_of(n * 512 + j * 128, 128), 128)
                        w1_s[r0:r0 + 8, cols] = _u(c.astype(bf16))
            return []

        def prep_ct(half, cq):
            res = []
            ct = 2 * cq + half
            for tb in range(4):
                x = _u(ckv[pl.ds(pl.multiple_of(j * 512 + tb * 128, 128), 128), ct * 128:(ct + 1) * 128].T)
                cT_s[pl.ds(pl.multiple_of(zq * 64 + ct * 64, 64), 64), tb * 128:(tb + 1) * 128] = x
                res.append(x[56:])
            return res

        def prep_c2(r):
            blk = [[cT_s[cq * 128 + r:cq * 128 + r + 8, tb * 128:(tb + 1) * 128] for tb in range(4)] for cq in range(4)]
            x = [[_f(v) for v in row] for row in blk]
            outer = [[_b7(x[ci][ti], x[ci][2 + ti], x[2 + ci][ti], x[2 + ci][2 + ti]) for ti in range(2)]
                     for ci in range(2)]
            two = [_b7(outer[0][0][n], outer[0][1][n], outer[1][0][n], outer[1][1][n]) for n in range(7)]
            row = pl.ds(pl.multiple_of(j * 128 + r, 8), 8)
            for n in range(7):
                for m in range(7):
                    c2_s[row, (n * 7 + m) * 128:(n * 7 + m + 1) * 128] = _u(two[n][m].astype(bf16))
            return []

        fill = {}

        def spread(pieces, u0, u1):
            for n, p in enumerate(pieces):
                fill.setdefault(u0 + n * (u1 - u0) // len(pieces), []).append(p)

        spread([functools.partial(prep_w, 0, hp, part) for hp in range(8) for part in range(5)], QW1, QW2)
        spread([functools.partial(prep_w, 1, hp, part) for hp in range(8) for part in range(5)], QW2, QW3)
        spread([functools.partial(prep_ct, 0, cq) for cq in range(4)], QW2 + 2, QC1)
        spread([functools.partial(prep_ct, 1, cq) for cq in range(4)], QC1, QW3)
        spread([functools.partial(prep_c2, r) for r in range(0, 128, 8)], QW3, QW4)
        spread([functools.partial(prep_x, jnp.minimum(j + 1, 3), t, r0)
                for t in range(2) for r0 in range(0, 224, 32)], QW4, 221)
        toks = {}
        for u in range(224):
            if u == QW1:
                @pl.when(j < 3)
                def _():
                    for c in c_wk(j + 1):
                        c.start(priority=1)

                @pl.when(j == 3)
                def _():
                    for c in c_early + c_late:
                        c.start(priority=1)

                for c in c_wk(j):
                    c.wait()
            if u == QW2:
                @pl.when(j < 3)
                def _():
                    for c in c_wv(j + 1) + [c_ckv(j + 1)]:
                        c.start(priority=1)

                @pl.when(j < 2)
                def _():
                    c_x(j + 2).start(priority=1)

                @pl.when(j < 3)
                def _():
                    c_x(j + 1).wait()

                for c in c_wv(j) + [c_ckv(j)]:
                    c.wait()
            q = qproj(u, toks.pop(u, None))
            res = []
            ps = fill.get(u, [])
            for n, p in enumerate(ps):
                row = (n * 128 // len(ps)) // 16 * 16
                if p.func is prep_w and p.args[2] == 0:
                    (wk_raw, wv_raw)[p.args[0]].bitcast(u32)[zq, 0, 1024:1032, :] = _u(q[row:row + 8])
                elif p.func is prep_c2:
                    cT_s[pl.ds(pl.multiple_of(512 + zq * 8, 8), 8), 0:128] = _u(q[row:row + 8])
                elif p.func is prep_x:
                    xT[pl.ds(pl.multiple_of(M + zq * 16, 16), 16), 0:128] = q[row:row + 16].astype(bf16)
                elif p.func is prep_ct:
                    ckv[pl.ds(pl.multiple_of(S + zq * 16, 16), 16), 0:128] = q[row:row + 16].astype(bf16)
                res += p()
            if res:
                toks[u + QLAG] = _tok(res)
        return carry

    jax.lax.fori_loop(0, 4, q_body, 0)
    for c in c_early:
        c.wait()

    tri = n_i <= k_i
    sgn = jnp.where((jax.lax.broadcasted_iota(jnp.int32, (1, P), 1) & 1) == 0, 1.0, -1.0).astype(f32)
    c_outa = cp(out_s.at[:, pl.ds(0, 384)], out_hbm.at[:, pl.ds(0, 384)], sem_o.at[8])
    HR, HI, PR, PI, KV = range(5)

    def blk_at(c, half=None):
        r0 = (c % 8) * CH
        rs = slice(r0, r0 + CH) if half is None else slice(r0 + 16 * half, r0 + 16 * half + 16)
        return rs, slice((c // 8) * P, (c // 8 + 1) * P)

    def tile(ref, n):
        return ref[:, n * 128:(n + 1) * 128]

    def head_body(h, carry):
        @pl.when(h == 1)
        def _():
            for c in c_late:
                c.wait()

        @pl.when(h == H - 1)
        def _():
            c_outa.start()

        st = dict(co={}, cnt={}, fin=set(), M={}, P={}, Q7={}, mfin={}, o={})
        zs = h >> 10
        z64 = pl.ds(pl.multiple_of(zs * 64, 64), 64)
        m_s, l_s = (m0_s, m1_s), (l0_s, l1_s)
        hrows = pl.ds(pl.multiple_of(h * 128, 128), 128)
        rows = pl.ds(pl.multiple_of(jnp.minimum(h, NCH - 1) * CH, CH), CH)

        def rep(t, n):
            return jnp.concatenate([taps[t, rows, :]] * n, axis=1)

        toks = []

        def due():
            for t in toks:
                t[0] -= 1
            ready = [t[1] for t in toks if t[0] <= 0]
            toks[:] = [t for t in toks if t[0] > 0]
            return functools.reduce(lambda x, y: x | y, ready) if ready else None

        def gate_later(vals):
            toks.append([SLAG, _tok([v if v.dtype == u32 else _u(v) for v in vals])])

        def row_offset(i):
            if i not in st['mfin']:
                m = m_s[i % 2][0, 0]
                for t in range(1, i + 1):
                    m = jnp.maximum(m, m_s[i % 2][0, t])
                m = jnp.max(m, axis=0, keepdims=True)
                if i > 0:
                    lo_ = jnp.exp2(m_s[i % 2][0, 0] - m)
                    for t in range(1, i + 1):
                        lo_ = lo_ + jnp.exp2(m_s[i % 2][0, t] - m)
                    m = m + jnp.log2(jnp.sum(lo_, axis=0, keepdims=True))
                st['mfin'][i] = m
            return st['mfin'][i]

        for op in _schedule():
            kind = op[0]
            if kind == 'KV':
                _, p, t = op
                n, m = SK[t // 7], SV[t % 7]

                def wblk(q):
                    w = w1_s[hrows, n * 512 + (q % 2) * 256:n * 512 + (q % 2) * 256 + 256]
                    r = (q // 2) * 32
                    return jnp.concatenate([w[r:r + 32], w[64 + r:64 + r + 32]], axis=0)

                cols = slice((n * 7 + m) * 256, (n * 7 + m + 1) * 256)
                if m in (2, 3):
                    w = wblk(0 if m == 2 else 3)
                elif p > 0:
                    w = w2_s[:, cols]
                else:
                    i1, i2, sg = _A_OF[m]
                    x, y = wblk(i1), wblk(i2)
                    w = (_f(x) + _f(y) if sg > 0 else _f(x) - _f(y)).astype(bf16)
                    w2_s[z64, cols] = _u(w)
                c2 = c2_s[p * 128:(p + 1) * 128, (n * 7 + m) * 128:(n * 7 + m + 1) * 128]
                st['M'][m] = st['last'] = _nn(w if w.dtype == bf16 else _b(_gate(w, due())), _b(c2))
                if t % 7 < 6:
                    continue
                mo = _quad(*_c4(st['M']))
                for o, sg in _C_OF[n]:
                    k = st['cnt'][o] = st['cnt'].get(o, 0) + 1
                    if k == 1:
                        st['co'][o] = mo if sg > 0 else -mo
                    else:
                        st['co'][o] = st['co'][o] + mo if sg > 0 else st['co'][o] - mo
                    if k == _C_CNT[o]:
                        st['cnt'][o] = 0
                        st['fin'].add(o)
                for tok in range(2):
                    if not {tok, 2 + tok} <= st['fin']:
                        continue
                    st['fin'] -= {tok, 2 + tok}
                    c = 2 * p + tok

                    def full(dh, kb, off):
                        x = st['co'][2 * dh + tok][:, kb * 128:(kb + 1) * 128]
                        return jnp.concatenate([x[off:off + 64], x[128 + off:128 + off + 64]], axis=0)

                    kb4 = (full(0, 0, 0).T, full(1, 0, 0).T, full(0, 1, 0).T, full(1, 1, 0).T)
                    vb4 = (full(0, 0, 64), full(0, 1, 64), full(1, 0, 64), full(1, 1, 64))
                    for ref, c4 in ((K_s[c], kb4), (V_s[c], vb4)):
                        blks = dict(zip((2, 7, 8, 3), c4))
                        if c < NT - 1:
                            blks.update({k: x for k, x in enumerate(_a7(*c4)) if k not in (2, 3)})
                        for k, x in blks.items():
                            ref[z64, k * 128:(k + 1) * 128] = _u(x.astype(bf16))
            elif kind == 'QK':
                _, i, j = op
                S_s = (S0_s, S1_s)[i % 2]
                if j < i:
                    if i not in st['Q7']:
                        qu = QT_s[hrows, i * T:(i + 1) * T]
                        st['Q7'][i] = _combos(_b7, [qu[:64, :128], qu[:64, 128:], qu[64:, :128], qu[64:, 128:]])
                    s = _quad(*_c4({n: _nn(_b(tile(K_s[j], n)), st['Q7'][i][n]) for n in SQ}))
                    S_s[zs, j] = s
                    f = _fold(s, jnp.max)
                else:
                    q = _b(QT_s[hrows, i * T:(i + 1) * T])
                    sa = _nn(_b(jnp.concatenate([tile(K_s[j], 2), tile(K_s[j], 7)], axis=1)), q)
                    sa = jnp.concatenate([jnp.where(tri, sa[:, :128], NEG), sa[:, 128:]], axis=1)
                    sb = _nn(_b(jnp.concatenate([tile(K_s[j], 8), tile(K_s[j], 3)], axis=1)), q[:, 128:])
                    sb = jnp.where(tri, sb, NEG)
                    S_s[zs, j, 0:128, :] = sa
                    S_s[zs, j, 128:T, 128:T] = sb
                    fa = _fold(sa, jnp.max)
                    f = jnp.concatenate([fa[:, :128], jnp.maximum(fa[:, 128:], _fold(sb, jnp.max))], axis=1)
                m_s[i % 2][zs, j] = f
                pace_s[zs] = f
            elif kind == 'EX':
                _, i, j = op
                S_s = (S0_s, S1_s)[i % 2]
                m = row_offset(i)
                m = jnp.where(pace_s[0, 0:1, :] == jnp.inf, jnp.inf, m)
                if j < i:
                    parts, lj = [], None
                    for r in range(112, -16, -16):
                        pt = jnp.exp2(S_s[0, j, r:r + 16, :] - m)
                        pb = jnp.exp2(S_s[0, j, 128 + r:128 + r + 16, :] - m)
                        parts.insert(0, _b7(pt[:, :128], pt[:, 128:], pb[:, :128], pb[:, 128:]))
                        x = (pt[:8] + pt[8:]) + (pb[:8] + pb[8:])
                        lj = x if lj is None else lj + x
                    st['P'][i, j] = [jnp.concatenate([x[n] for x in parts], axis=0).astype(bf16) for n in range(7)]
                else:
                    pa = jnp.exp2(S_s[0, j, 0:128, :] - m)
                    pb = jnp.exp2(S_s[0, j, 128:T, 128:T] - m[:, 128:])
                    la = _rsum(pa)
                    lj = jnp.concatenate([la[:, :128], la[:, 128:] + _rsum(pb)], axis=1)
                    st['P'][i, j] = (pa.astype(bf16), pb.astype(bf16))
                l_s[i % 2][zs, j] = lj
            elif kind == 'PV':
                _, i, j = op
                p = st['P'].pop((i, j))
                if j < i:
                    for n in SP:
                        st['last'] = _nn(_b(tile(V_s[j], n)), p[n])
                        st['o'][i, n] = st['o'][i, n] + st['last'] if j > 0 else st['last']
                    continue
                oa = _nn(_b(jnp.concatenate([tile(V_s[j], 2), tile(V_s[j], 8)], axis=0)), p[0])
                ob = _nn(_b(jnp.concatenate([tile(V_s[j], 7), tile(V_s[j], 3)], axis=0)), p[1])
                o = st['last'] = jnp.concatenate([oa[:, :128], oa[:, 128:] + ob], axis=1)
                if i > 0:
                    o = o + _quad(*_c4({n: st['o'].pop((i, n)) for n in range(7)}))
                l = l_s[i % 2][0, 0]
                for t in range(1, i + 1):
                    l = l + l_s[i % 2][0, t]
                o = o * (1.0 / jnp.sum(l, axis=0, keepdims=True))
                for n, x in enumerate(_b7(o[:128, :128], o[:128, 128:], o[128:, :128], o[128:, 128:])):
                    O_s[i][zs, n] = x.astype(bf16)
            elif kind == 'PACE':
                pace_s[zs] = jnp.concatenate([st['last'][-8:, -128:]] * 2, axis=1)
            elif kind == 'OP':
                _, i, t = op
                n = SO[t]
                st['M'][n] = st['last'] = _nn(_b(_gate(tile(W7_s, n), due())), O_s[i][0, n])
                if t == 6:
                    acc[:, T * i:T * (i + 1)] += _quad(*_c4(st['M']))
            elif kind == 'W7':
                res = []
                for r0 in range(16 * op[1], 16 * op[2], 16):
                    blk = [_u(woT[h, r:r + 16, c:c + 128]) for r in (r0, 224 + r0) for c in (0, 128)]
                    row = pl.ds(pl.multiple_of(zs * 8 + r0 // 2, 8), 8)
                    for n, x in enumerate(_combos(_a7, blk)):
                        W7_s[row, n * 128:(n + 1) * 128] = _u(x)
                    res += blk
                gate_later(res)
            elif kind == 'AT':
                g = jnp.clip((h - 4) // 4, 0, 2)
                t0 = jnp.minimum(((h + 12) % 4) * 6, NB - 6)
                grow = pl.ds(pl.multiple_of(g * 128, 128), 128)
                gcol = pl.ds(pl.multiple_of(jnp.where(h == H - 1, 3, g) * 128, 128), 128)
                res = []
                for n in range(6):
                    tok = pl.ds(pl.multiple_of((t0 + n) * 128, 128), 128)
                    x = aT_s[grow, tok].T
                    out_s[tok, gcol] = x
                    res.append(_u(x)[56:])
                gate_later(res)
            elif kind == 'HD':
                g = op[1]
                hs = jnp.concatenate([ssmk[rows, c * P:(c + 1) * P] for c in range(4 * g, 4 * g + 4)], axis=0)
                hf = _nn(hs, ff_s[...])
                for n in range(4):
                    X_s[(zs, HR) + blk_at(4 * g + n)] = hf[n * CH:(n + 1) * CH, :P]
                    X_s[(zs, HI) + blk_at(4 * g + n)] = hf[n * CH:(n + 1) * CH, P:]
            elif kind == 'SC':
                g = op[1]
                if g == 0:
                    k = jnp.concatenate([jnp.zeros((CH, P), f32), kT[rows, 0:4 * P].astype(f32)], axis=1)
                else:
                    k = kT[rows, (4 * g - 1) * P:(4 * g + 4) * P].astype(f32)
                ks = k[:, P:] * rep(0, 4)
                for j in range(1, KS):
                    ks = ks + pltpu.roll(k, j, 1)[:, P:] * rep(j, 4)
                kv = ks * vT[rows, 4 * g * P:(4 * g + 4) * P].astype(f32)
                kvs = jnp.concatenate([kv[:, n * P:(n + 1) * P] for n in range(4)], axis=0)
                xf = _nn(kvs.astype(bf16), ff_s[...])
                for n in range(4):
                    c = 4 * g + n
                    xr, xi = xf[n * CH:(n + 1) * CH, :P], xf[n * CH:(n + 1) * CH, P:]
                    X_s[(zs, KV) + blk_at(c)] = kvs[n * CH:(n + 1) * CH]
                    pr = xr if c == 0 else xr - sgn * st['x'][1]
                    pi = xi if c == 0 else xi + sgn * st['x'][0]
                    X_s[(zs, PR) + blk_at(c)] = pr
                    X_s[(zs, PI) + blk_at(c)] = pi
                    st['x'] = (xr, xi)
            elif kind == 'CV':
                res = []
                for a, half in op[1]:
                    wr = wi = None
                    for j in range(a + 1):
                        hr, hi_ = X_s[(0, HR) + blk_at(j, half)], X_s[(0, HI) + blk_at(j, half)]
                        pr, pi = X_s[(0, PR) + blk_at(a - j, half)], X_s[(0, PI) + blk_at(a - j, half)]
                        tr, ti = hr * pr - hi_ * pi, hr * pi + hi_ * pr
                        wr, wi = (tr, ti) if wr is None else (wr + tr, wi + ti)
                    r0 = (a % 4) * CH + 16 * half
                    Y_s[a // 4][zs, r0:r0 + 16, :P] = wr
                    Y_s[a // 4][zs, r0:r0 + 16, P:] = wi
                    res += [wr, wi]
                gate_later(res)
            elif kind == 'ID':
                g = op[1]
                y = _nn(Y_s[g][0].astype(bf16), fi_s[...])
                for n in range(4):
                    c = 4 * g + n
                    cols = slice(c * P, (c + 1) * P)
                    ya = y[n * CH:(n + 1) * CH, :] + X_s[(0, KV) + blk_at(c)] * taps[KS, rows, :]
                    aT_s[rows, cols] = (qT[rows, cols].astype(f32) * ya).astype(bf16)
        return carry

    jax.lax.fori_loop(0, H, head_body, 0)

    acc[:, T * (NT - 1):] += _quad(*_c4({n: _nn(_b(tile(W7_s, n)), O_s[NT - 1][0, n]) for n in SORD}))
    outs = [c_outa]
    for i in range(NT):
        cols = slice(T * i, T * (i + 1))
        blk = jnp.concatenate([aT_s[384:M, cols], acc[:, cols].astype(bf16)], axis=0)
        out_s[cols, 384:2 * M] = blk.T
        c = cp(out_s.at[pl.ds(T * i, T), pl.ds(384, 512)], out_hbm.at[pl.ds(T * i, T), pl.ds(384, 512)], sem_o.at[i])
        c.start()
        outs.append(c)
    for c in outs:
        c.wait()


@jax.jit
def pallas_concat_heads__ssm_conv_h3__compressed_kv_cla__prompt_kernel(
    A_q: jax.Array,
    A_k: jax.Array,
    A_v: jax.Array,
    A_shift_k: jax.Array,
    A_ssm_k: jax.Array,
    A_ssm_D: jax.Array,
    B_x: jax.Array,
    B_c_kv: jax.Array,
    B_w_q: jax.Array,
    B_w_uk: jax.Array,
    B_w_uv: jax.Array,
    B_w_o: jax.Array,
):
    hbm = pl.BlockSpec(memory_space=pl.ANY)
    vmem = pl.BlockSpec(memory_space=pltpu.VMEM)
    V = pltpu.VMEM
    out = pl.pallas_call(
        _kernel,
        out_shape=jax.ShapeDtypeStruct((S, 2 * M), bf16),
        in_specs=[hbm, hbm, hbm, vmem, hbm, vmem, hbm, hbm, hbm, hbm, hbm, hbm],
        out_specs=hbm,
        scratch_shapes=[
            V((M, S), bf16), V((M, S), bf16), V((M, S), bf16), V((M, S), bf16),
            V((M + 16, S), bf16), V((S + 16, DC), bf16),
            V((2, M * H, 128), bf16),
            V((2, 4, 128 * H + 16, 128), bf16), V((2, 4, 128 * H + 16, 128), bf16),
            V((H, M, D), bf16),
            V((H * 64, 7 * 256), u32), V((NT * 112, 7 * 128), u32),
            V((H * 128, 7 * 512), u32), V((64, 49 * 256), u32),
            V((512 + 8, 512), u32),
            V((H * D // 2, S), u32), V((4 * 128, 49 * 128), u32),
            V((M, S), f32), V((M, S), bf16), V((S, 2 * M), bf16),
            V((KS + 1, M, 128), f32), V((P, 2 * P), bf16), V((2 * P, P), bf16),
            V((1, NT, T, T), f32), V((1, NT, T, T), f32), V((1, 5, T, T), f32),
            V((112, 7 * 128), u32), V((1, 8, T), f32),
            V((1, NT, 8, T), f32), V((1, NT, 8, T), f32), V((1, NT, 8, T), f32), V((1, NT, 8, T), f32),
            pltpu.SemaphoreType.DMA((26,)), pltpu.SemaphoreType.DMA((8,)),
            pltpu.SemaphoreType.DMA((8,)), pltpu.SemaphoreType.DMA((9,)),
        ] + [V((64, 9 * 128), u32)] * (2 * NT) + [V((1, 7, 128, 128), bf16)] * NT
        + [V((1, 4 * CH, 2 * P), f32)] * 4,
        compiler_params=pltpu.CompilerParams(vmem_limit_bytes=126 * 1024 * 1024,
                                             shape_invariant_numerics=False),
    )(
        A_q[0].T, A_k[0].T, A_v[0].T, A_shift_k.T, A_ssm_k, A_ssm_D,
        B_x[0].T, B_c_kv[0],
        B_w_q.reshape(M * H, D), B_w_uk.reshape(DC * H, D), B_w_uv.reshape(DC * H, D),
        jnp.transpose(B_w_o, (0, 2, 1)),
    )
    return out[None]
```

```python
import functools
import math

import jax
import jax.numpy as jnp
import jax.experimental.pallas as pl
import jax.experimental.pallas.tpu as pltpu

bf16 = jnp.bfloat16
f32 = jnp.float32
u32 = jnp.uint32

S = 2048
M = 448
DC = 1024
H = 16
D = 256
KS = 4
P = 128
NB = S // P
CH = 32
NCH = M // CH
T = 256
NT = S // T
NEG = -1e30

SORD = tuple(int(c) for c in '6430125')
SK = tuple(int(c) for c in '0364125')
SV = tuple(int(c) for c in '0125364')
SQ = tuple(int(c) for c in '6043125')
SP = tuple(int(c) for c in '3640125')
SO = tuple(int(c) for c in '5210346')
QW1 = 70
QW2 = 126
QW3 = 192
QW4 = 208
QC1 = 150
QLAG = 12
CVMAX = 12
SIDE0 = 30
SIDEP = 4
SLAG = 5
PRE = 0
W7P = 16
W7D = 6
KVH = 35
EXB = 10
NOP6 = 2
LA = 3
C2N = 64
NOP = 2


def _nn(a, b):
    return jnp.dot(a, b, preferred_element_type=f32)


def _b(u):
    return pltpu.bitcast(u, bf16)


def _u(x):
    return pltpu.bitcast(x, u32)


def _lo(u):
    return pltpu.bitcast(u << 16, f32)


def _hi(u):
    return pltpu.bitcast(u & jnp.uint32(0xFFFF0000), f32)


def _f(u):
    return _b(u).astype(f32)


def _a7(a11, a12, a21, a22):
    return [a11 + a22, a21 + a22, a11, a22, a11 + a12, a21 - a11, a12 - a22]


def _b7(b11, b12, b21, b22):
    return [b11 + b22, b11, b12 - b22, b21 - b11, b22, b11 + b12, b21 + b22]


def _c4(m):
    return m[0] + m[3] - m[4] + m[6], m[2] + m[4], m[1] + m[3], m[0] - m[1] + m[2] + m[5]


_C_OF = (((0, 1), (3, 1)), ((2, 1), (3, -1)), ((1, 1), (3, 1)), ((0, 1), (2, 1)), ((0, -1), (1, 1)), ((3, 1),), ((0, 1),))
_C_CNT = (4, 2, 2, 4)
_A_OF = {0: (0, 3, 1), 1: (2, 3, 1), 4: (0, 1, 1), 5: (2, 0, -1), 6: (1, 3, -1)}


def _combos(f7, blk):
    x = f7(*[_f(v) for v in blk])
    plain = {2: 0, 3: 3} if f7 is _a7 else {1: 0, 4: 3}
    return [_b(blk[plain[n]]) if n in plain else x[n].astype(bf16) for n in range(7)]


def _quad(c11, c12, c21, c22):
    return jnp.concatenate([jnp.concatenate([c11, c12], axis=1), jnp.concatenate([c21, c22], axis=1)], axis=0)


def _fold(c, op):
    return op(c.reshape(-1, 8, c.shape[1]), axis=0)


def _rsum(p):
    cols = []
    for c in range(0, p.shape[1], 128):
        acc = None
        for r in range(112, -16, -16):
            t = p[r:r + 8, c:c + 128] + p[r + 8:r + 16, c:c + 128]
            acc = t if acc is None else acc + t
        cols.append(acc)
    return jnp.concatenate(cols, axis=1) if len(cols) > 1 else cols[0]


def _tok(vals):
    parts = []
    for v in vals:
        for r in range(0, v.shape[0], 8):
            for c in range(0, v.shape[1], 128):
                parts.append(v[r:r + 8, c:c + 128])
    while len(parts) > 1:
        parts = [parts[i] | parts[i + 1] if i + 1 < len(parts) else parts[i] for i in range(0, len(parts), 2)]
    return (parts[0] >> 31) >> 1


def _gate(x, tok):
    if tok is None:
        return x
    top = x[:8, :128] | tok
    if x.shape[1] > 128:
        top = jnp.concatenate([top, x[:8, 128:]], axis=1)
    return jnp.concatenate([top, x[8:]], axis=0)


def _side_pieces():
    ps = [(k, g) for g in range(PRE) for k in ('HD', 'SC')]
    cur, cost = [], 0
    for a in range(NB):
        if a % 4 == 0 and a // 4 + PRE < 4:
            ps += [('HD', a // 4 + PRE), ('SC', a // 4 + PRE)]
        for half in range(2):
            if cur and cost + a + 1 > CVMAX:
                ps.append(('CV', tuple(cur)))
                cur, cost = [], 0
            cur.append((a, half))
            cost += a + 1
        if a % 4 == 3:
            ps += [('CV', tuple(cur)), ('ID', a // 4)]
            cur, cost = [], 0
    ps.insert(W7P, ('W7', 0, 7))
    ps.insert(W7P + W7D, ('W7', 7, 14))
    return ps


def _schedule():
    side = _side_pieces()
    out = []
    cnt = [0]

    def block(subs, att, with_side):
        for k, u in enumerate(subs):
            out.append(u)
            out.extend(att.get(k, []))
            if with_side:
                cnt[0] += 1
                if side and cnt[0] >= SIDE0 and (cnt[0] - SIDE0) % SIDEP == 0:
                    out.append(side.pop(0))

    def kv(p, half):
        return [('KV', p, t) for t in (range(KVH) if half == 0 else range(KVH, 49))]

    def op_(*idx):
        return [('OP', i, t) for i in idx for t in range(7)]

    def softmax_head(i, n):
        att = {max(n - EXB, 0): [('PACE',), ('EX', i, 0)]}
        for k in range(1, min(LA, i + 1)):
            att.setdefault(n - 1 - (LA - 1 - k) * 2, []).extend([('PACE',), ('EX', i, k)])
        return att

    ops_left = list(range(NT - 1))
    block(kv(0, 0) + kv(0, 1), {}, True)
    block(op_(NT - 1), {6: [('AT',), ('QK', 0, 0)]}, False)
    block(kv(1, 0), softmax_head(0, KVH), True)
    for i in range(NT - 1):
        for j in range(i + 1):
            out.append(('QK', i + 1, j))
            if j + LA <= i:
                out.append(('EX', i, j + LA))
            out.append(('PV', i, j))
        out.append(('QK', i + 1, i + 1))
        if i < 5:
            subs = kv((i + 3) // 2, (i + 1) % 2)
            block(subs, softmax_head(i + 1, len(subs)), True)
        else:
            n = NOP6 if i == 5 else NOP
            block(op_(*ops_left[:n]), softmax_head(i + 1, 7 * n), False)
            del ops_left[:n]
    out.append(('PACE',))
    for j in range(NT):
        if j + LA < NT:
            out.append(('EX', NT - 1, j + LA))
        out.append(('PV', NT - 1, j))
        if len(ops_left) > 2:
            block(op_(ops_left.pop(0)), {}, False)
        out.append(('PACE',))
    block(op_(*ops_left), {}, False)
    assert not side
    w7 = [k for k, o in enumerate(out) if o[0] == 'W7']
    assert out.index(('OP', NT - 1, 6)) < min(w7) and max(w7) < out.index(('OP', 0, 0))
    out.remove(('ID', 3))
    out.append(('ID', 3))
    return out


def _kernel(qT_hbm, kT_hbm, vT_hbm, sk_ref, ssmk_hbm, dd_ref, xT_hbm, ckv_hbm,
            wq_hbm, wk_hbm, wv_hbm, woT_hbm, out_hbm,
            qT, kT, vT, ssmk, xT, ckv, wq_raw, wk_raw, wv_raw, woT,
            aq_s, bx_s, w1_s, w2_s, cT_s, QT_s, c2_s, acc, aT_s, out_s, taps, ff_s, fi_s,
            S0_s, S1_s, X_s, W7_s, pace_s, m0_s, m1_s, l0_s, l1_s,
            sem, sem_k, sem_v, sem_o, *rest):
    K_s, V_s, O_s, Y_s = rest[:NT], rest[NT:2 * NT], rest[2 * NT:3 * NT], rest[3 * NT:]

    def cp(src, dst, s):
        return pltpu.make_async_copy(src, dst, s)

    def c_x(j):
        cols = pl.ds(pl.multiple_of(j * 2 * T, 2 * T), 2 * T)
        return cp(xT_hbm.at[:, cols], xT.at[pl.ds(0, M), cols], sem.at[j])

    QP = ((0, 128), (128, 96))

    def c_wq(p):
        cs_ = []
        for half in range(2):
            r = pl.ds((half * 224 + QP[p][0]) * H, QP[p][1] * H)
            for g in range(2):
                cs_.append(cp(wq_hbm.at[r, pl.ds(128 * g, 128)], wq_raw.at[g, r], sem.at[18 + 4 * p + 2 * half + g]))
        return cs_

    def c_w(w_hbm, raw, sm, j, half, g):
        r = pl.ds(pl.multiple_of((half * 4 + j) * 2048, 2048), 2048)
        q = 2 * half + g
        return cp(w_hbm.at[r, pl.ds(128 * g, 128)], raw.at[j % 2, q, pl.ds(0, 2048)], sm.at[(j % 2) * 4 + q])

    def c_wk(j):
        return [c_w(wk_hbm, wk_raw, sem_k, j, half, g) for half in range(2) for g in range(2)]

    def c_wv(j):
        return [c_w(wv_hbm, wv_raw, sem_v, j, half, g) for half in range(2) for g in range(2)]

    def c_ckv(j):
        r = pl.ds(pl.multiple_of(j * 2 * T, 2 * T), 2 * T)
        return cp(ckv_hbm.at[r], ckv.at[r], sem.at[9 + j])

    a_pairs = ((kT_hbm, kT), (vT_hbm, vT), (ssmk_hbm, ssmk), (qT_hbm, qT))
    c_early = [cp(woT_hbm.at[pl.ds(0, 1)], woT.at[pl.ds(0, 1)], sem.at[4])]
    c_early += [cp(src.at[pl.ds(0, CH)], dst.at[pl.ds(0, CH)], sem.at[5 + n]) for n, (src, dst) in enumerate(a_pairs)]
    c_late = [cp(woT_hbm.at[pl.ds(1, H - 1)], woT.at[pl.ds(1, H - 1)], sem.at[13])]
    c_late += [cp(src.at[pl.ds(CH, M - CH)], dst.at[pl.ds(CH, M - CH)], sem.at[14 + n])
               for n, (src, dst) in enumerate(a_pairs)]
    for c in [c_x(0)] + c_wq(0) + c_wq(1):
        c.start()
    for c in c_wk(0) + [c_x(1)]:
        c.start(priority=1)

    n_i = jax.lax.broadcasted_iota(jnp.int32, (P, P), 0)
    k_i = jax.lax.broadcasted_iota(jnp.int32, (P, P), 1)
    ang = (((2 * k_i + 1) * n_i) & 511).astype(f32) * (math.pi / 256.0)
    cs, sn = jnp.cos(ang), jnp.sin(ang)
    ff_s[:, 0:P] = cs.astype(bf16)
    ff_s[:, P:2 * P] = (-sn).astype(bf16)
    fi_s[0:P, :] = (cs.T * (1.0 / P)).astype(bf16)
    fi_s[P:2 * P, :] = (sn.T * (-1.0 / P)).astype(bf16)
    sk = sk_ref[...].astype(f32)
    for t in range(KS):
        taps[t] = jnp.broadcast_to(sk[t:t + 1, :], (128, M)).T
    taps[KS] = jnp.broadcast_to(dd_ref[...].astype(f32).reshape(1, M), (128, M)).T
    acc[...] = jnp.zeros(acc.shape, f32)
    aT_s[...] = jnp.zeros(aT_s.shape, bf16)
    O_s[NT - 1][...] = jnp.zeros(O_s[0].shape, bf16)
    W7_s[...] = jnp.zeros(W7_s.shape, u32)
    cT_s[...] = jnp.zeros(cT_s.shape, u32)

    def prep_x(jj, t, r0):
        c0 = (2 * jj + t) * T
        cs_ = [c0, c0 + 128] if isinstance(jj, int) else [pl.multiple_of(c0, 128), pl.multiple_of(c0 + 128, 128)]
        blk = [_u(xT[r:r + 32, pl.ds(c, 128)]) for r in (r0, 224 + r0) for c in cs_]
        row = (2 * jj + t) * 112 + r0 // 2
        row = pl.ds(row if isinstance(jj, int) else pl.multiple_of(row, 16), 16)
        for n, x in enumerate(_combos(_b7, blk)):
            bx_s[row, n * 128:(n + 1) * 128] = _u(x)
        return []

    c_x(0).wait()
    for t in range(2):
        for r0 in range(0, 224, 32):
            prep_x(0, t, r0)
    vq = wq_raw.bitcast(u32)
    for p, (c0, nc) in enumerate(QP):
        for c in c_wq(p):
            c.wait()
        for hp in range(H // 2):
            ut = [vq[g, pl.ds((half * 224 + c0) * 8 + hp, nc, stride=8), :].T for g in range(2) for half in range(2)]
            for r in range(0, 128, 16):
                u = [x[r:r + 16] for x in ut]
                for par, f in enumerate((_lo, _hi)):
                    r0 = (2 * hp + par) * 64 + r // 2
                    for n, x in enumerate(_a7(*[f(x) for x in u])):
                        aq_s[r0:r0 + 8, n * 256 + c0:n * 256 + c0 + nc] = _u(x.astype(bf16))
    for c in c_wv(0) + [c_ckv(0)]:
        c.start(priority=1)

    qscale = (D ** -0.5) * math.log2(math.e)

    def prep_c2(jj, r):
        blk = [[cT_s[cq * 128 + r:cq * 128 + r + 8, tb * 128:(tb + 1) * 128] for tb in range(4)] for cq in range(4)]
        x = [[_f(v) for v in row] for row in blk]
        outer = [[_b7(x[ci][ti], x[ci][2 + ti], x[2 + ci][ti], x[2 + ci][2 + ti]) for ti in range(2)]
                 for ci in range(2)]
        two = [_b7(outer[0][0][n], outer[0][1][n], outer[1][0][n], outer[1][1][n]) for n in range(7)]
        row = pl.ds(jj * 128 + r if isinstance(jj, int) else pl.multiple_of(jj * 128 + r, 8), 8)
        for n in range(7):
            for m in range(7):
                c2_s[row, (n * 7 + m) * 128:(n * 7 + m + 1) * 128] = _u(two[n][m].astype(bf16))
        return []

    def q_body(j, carry):
        mq = {}
        qtj = QT_s.at[pl.ds(pl.multiple_of(j * 4096, 4096), 4096)]
        zq = j >> 4
        bx = [[bx_s[pl.ds(pl.multiple_of((2 * j + t) * 112, 16), 112), n * 128:(n + 1) * 128] for n in range(7)]
              for t in range(2)]

        def qproj(u, tok):
            hh, t, n = u // 14, (u // 7) % 2, SORD[u % 7]
            w = _b(_gate(aq_s[hh * 64:hh * 64 + 64, n * 256:n * 256 + 224], tok))
            mq[n] = _nn(w, _b(bx[t][n]))
            if u % 7 == 6:
                for k, x in enumerate(_c4(mq)):
                    r0 = t * 2048 + hh * 128 + (k // 2) * 64
                    qtj[r0:r0 + 64, (k % 2) * 128:(k % 2 + 1) * 128] = _u((x * qscale).astype(bf16))
            return mq[n]

        wt = {}
        w1j = w1_s.at[pl.ds(pl.multiple_of(j * 2048, 2048), 2048)]

        def prep_w(kv, hp, part):
            if part == 0:
                v = (wk_raw, wv_raw)[kv].bitcast(u32).at[j % 2]
                wt[kv, hp] = [v[q, pl.ds(hp, 128, stride=8), :].T for q in (0, 2, 1, 3)]
                return [x[120:] for x in wt[kv, hp]]
            for r in range(32 * (part - 1), 32 * part, 16):
                u = [x[r:r + 16] for x in wt[kv, hp]]
                for par, f in enumerate((_lo, _hi)):
                    r0 = (2 * hp + par) * 128 + kv * 64 + r // 2
                    for n, c in enumerate(_a7(*[f(x) for x in u])):
                        w1j[r0:r0 + 8, n * 128:(n + 1) * 128] = _u(c.astype(bf16))
            return []

        def prep_ct(half, cq):
            res = []
            ct = 2 * cq + half
            for tb in range(4):
                x = _u(ckv[pl.ds(pl.multiple_of(j * 512 + tb * 128, 128), 128), ct * 128:(ct + 1) * 128].T)
                cT_s[pl.ds(pl.multiple_of(zq * 64 + ct * 64, 64), 64), tb * 128:(tb + 1) * 128] = x
                res.append(x[56:])
            return res

        fill = {}

        def spread(pieces, u0, u1):
            for n, p in enumerate(pieces):
                fill.setdefault(u0 + n * (u1 - u0) // len(pieces), []).append(p)

        spread([functools.partial(prep_w, 0, hp, part) for hp in range(8) for part in range(5)], QW1, QW2)
        spread([functools.partial(prep_w, 1, hp, part) for hp in range(8) for part in range(5)], QW2, QW3)
        spread([functools.partial(prep_ct, 0, cq) for cq in range(4)], QW2 + 2, QC1)
        spread([functools.partial(prep_ct, 1, cq) for cq in range(4)], QC1, QW3)
        spread([functools.partial(prep_c2, jnp.maximum(j - 1, 0), r) for r in range(C2N, 128, 8)], 2, QW1 - 4)
        if C2N:
            spread([functools.partial(prep_c2, j, r) for r in range(0, C2N, 8)], QW3, QW4)
        spread([functools.partial(prep_x, jnp.minimum(j + 1, 3), t, r0)
                for t in range(2) for r0 in range(0, 224, 32)], QW4, 221)
        toks = {}
        for u in range(224):
            if u == QW1:
                @pl.when(j < 3)
                def _():
                    for c in c_wk(j + 1):
                        c.start(priority=1)

                @pl.when(j == 3)
                def _():
                    for c in c_early + c_late:
                        c.start(priority=1)

                for c in c_wk(j):
                    c.wait()
            if u == QW2:
                @pl.when(j < 3)
                def _():
                    for c in c_wv(j + 1) + [c_ckv(j + 1)]:
                        c.start(priority=1)

                @pl.when(j < 2)
                def _():
                    c_x(j + 2).start(priority=1)

                @pl.when(j < 3)
                def _():
                    c_x(j + 1).wait()

                for c in c_wv(j) + [c_ckv(j)]:
                    c.wait()
            q = qproj(u, toks.pop(u, None))
            res = []
            ps = fill.get(u, [])
            for n, p in enumerate(ps):
                row = (n * 128 // len(ps)) // 16 * 16
                if p.func is prep_w and p.args[2] == 0:
                    (wk_raw, wv_raw)[p.args[0]].bitcast(u32)[zq, 0, 1024:1032, :] = _u(q[row:row + 8])
                elif p.func is prep_c2:
                    cT_s[pl.ds(pl.multiple_of(512 + zq * 8, 8), 8), 0:128] = _u(q[row:row + 8])
                elif p.func is prep_x:
                    xT[pl.ds(pl.multiple_of(M + zq * 16, 16), 16), 0:128] = q[row:row + 16].astype(bf16)
                elif p.func is prep_ct:
                    ckv[pl.ds(pl.multiple_of(S + zq * 16, 16), 16), 0:128] = q[row:row + 16].astype(bf16)
                res += p()
            if res:
                toks[u + QLAG] = _tok(res)
        return carry

    jax.lax.fori_loop(0, 4, q_body, 0)
    for r in range(C2N, 128, 8):
        prep_c2(3, r)
    for c in c_early:
        c.wait()

    tri = n_i <= k_i
    sgn = jnp.where((jax.lax.broadcasted_iota(jnp.int32, (1, P), 1) & 1) == 0, 1.0, -1.0).astype(f32)
    c_outa = cp(out_s.at[:, pl.ds(0, 384)], out_hbm.at[:, pl.ds(0, 384)], sem_o.at[8])
    HR, HI, PR, PI, KV = range(5)

    def blk_at(c, half=None):
        r0 = (c % 8) * CH
        rs = slice(r0, r0 + CH) if half is None else slice(r0 + 16 * half, r0 + 16 * half + 16)
        return rs, slice((c // 8) * P, (c // 8 + 1) * P)

    def tile(ref, n):
        return ref[:, n * 128:(n + 1) * 128]

    def head_body(h, carry):
        @pl.when(h == 1)
        def _():
            for c in c_late:
                c.wait()

        @pl.when(h == H - 1)
        def _():
            c_outa.start()

        st = dict(co={}, cnt={}, fin=set(), M={}, P={}, Q7={}, mfin={}, o={})
        zs = h >> 10
        z64 = pl.ds(pl.multiple_of(zs * 64, 64), 64)
        m_s, l_s = (m0_s, m1_s), (l0_s, l1_s)
        w1h = w1_s.at[pl.ds(pl.multiple_of(h * 128, 128), 3 * 2048 + 128)]
        qth = QT_s.at[pl.ds(pl.multiple_of(h * 128, 128), 7 * 2048 + 128)]
        rows = pl.ds(pl.multiple_of(jnp.minimum(h, NCH - 1) * CH, CH), CH)

        def rep(t, n):
            return jnp.concatenate([taps[t, rows, :]] * n, axis=1)

        toks = []

        def due():
            for t in toks:
                t[0] -= 1
            ready = [t[1] for t in toks if t[0] <= 0]
            toks[:] = [t for t in toks if t[0] > 0]
            return functools.reduce(lambda x, y: x | y, ready) if ready else None

        def gate_later(vals):
            toks.append([SLAG, _tok([v if v.dtype == u32 else _u(v) for v in vals])])

        def row_offset(i):
            if i not in st['mfin']:
                m = m_s[i % 2][0, 0]
                for t in range(1, i + 1):
                    m = jnp.maximum(m, m_s[i % 2][0, t])
                m = jnp.max(m, axis=0, keepdims=True)
                if i > 0:
                    lo_ = jnp.exp2(m_s[i % 2][0, 0] - m)
                    for t in range(1, i + 1):
                        lo_ = lo_ + jnp.exp2(m_s[i % 2][0, t] - m)
                    m = m + jnp.log2(jnp.sum(lo_, axis=0, keepdims=True))
                st['mfin'][i] = m
            return st['mfin'][i]

        for op in _schedule():
            kind = op[0]
            if kind == 'KV':
                _, p, t = op
                n, m = SK[t // 7], SV[t % 7]

                def wblk(q):
                    w = jnp.concatenate([w1h[k * 2048:k * 2048 + 128, n * 128:(n + 1) * 128]
                                         for k in (2 * (q % 2), 2 * (q % 2) + 1)], axis=1)
                    r = (q // 2) * 32
                    return jnp.concatenate([w[r:r + 32], w[64 + r:64 + r + 32]], axis=0)

                cols = slice((n * 7 + m) * 256, (n * 7 + m + 1) * 256)
                if m in (2, 3):
                    w = wblk(0 if m == 2 else 3)
                elif p > 0:
                    w = w2_s[:, cols]
                else:
                    i1, i2, sg = _A_OF[m]
                    x, y = wblk(i1), wblk(i2)
                    w = (_f(x) + _f(y) if sg > 0 else _f(x) - _f(y)).astype(bf16)
                    w2_s[z64, cols] = _u(w)
                c2 = c2_s[p * 128:(p + 1) * 128, (n * 7 + m) * 128:(n * 7 + m + 1) * 128]
                st['M'][m] = st['last'] = _nn(w if w.dtype == bf16 else _b(_gate(w, due())), _b(c2))
                if t % 7 < 6:
                    continue
                mo = _quad(*_c4(st['M']))
                for o, sg in _C_OF[n]:
                    k = st['cnt'][o] = st['cnt'].get(o, 0) + 1
                    if k == 1:
                        st['co'][o] = mo if sg > 0 else -mo
                    else:
                        st['co'][o] = st['co'][o] + mo if sg > 0 else st['co'][o] - mo
                    if k == _C_CNT[o]:
                        st['cnt'][o] = 0
                        st['fin'].add(o)
                for tok in range(2):
                    if not {tok, 2 + tok} <= st['fin']:
                        continue
                    st['fin'] -= {tok, 2 + tok}
                    c = 2 * p + tok

                    def full(dh, kb, off):
                        x = st['co'][2 * dh + tok][:, kb * 128:(kb + 1) * 128]
                        return jnp.concatenate([x[off:off + 64], x[128 + off:128 + off + 64]], axis=0)

                    kb4 = (full(0, 0, 0).T, full(1, 0, 0).T, full(0, 1, 0).T, full(1, 1, 0).T)
                    vb4 = (full(0, 0, 64), full(0, 1, 64), full(1, 0, 64), full(1, 1, 64))
                    for ref, c4 in ((K_s[c], kb4), (V_s[c], vb4)):
                        blks = dict(zip((2, 7, 8, 3), c4))
                        if c < NT - 1:
                            blks.update({k: x for k, x in enumerate(_a7(*c4)) if k not in (2, 3)})
                        for k, x in blks.items():
                            ref[z64, k * 128:(k + 1) * 128] = _u(x.astype(bf16))
            elif kind == 'QK':
                _, i, j = op
                S_s = (S0_s, S1_s)[i % 2]
                if j < i:
                    if i not in st['Q7']:
                        qu = qth[i * 2048:i * 2048 + 128, :]
                        st['Q7'][i] = _combos(_b7, [qu[:64, :128], qu[:64, 128:], qu[64:, :128], qu[64:, 128:]])
                    s = _quad(*_c4({n: _nn(_b(tile(K_s[j], n)), st['Q7'][i][n]) for n in SQ}))
                    S_s[zs, j] = s
                    f = _fold(s, jnp.max)
                else:
                    q = _b(qth[i * 2048:i * 2048 + 128, :])
                    sa = _nn(_b(jnp.concatenate([tile(K_s[j], 2), tile(K_s[j], 7)], axis=1)), q)
                    sa = jnp.concatenate([jnp.where(tri, sa[:, :128], NEG), sa[:, 128:]], axis=1)
                    sb = _nn(_b(jnp.concatenate([tile(K_s[j], 8), tile(K_s[j], 3)], axis=1)), q[:, 128:])
                    sb = jnp.where(tri, sb, NEG)
                    S_s[zs, j, 0:128, :] = sa
                    S_s[zs, j, 128:T, 128:T] = sb
                    fa = _fold(sa, jnp.max)
                    f = jnp.concatenate([fa[:, :128], jnp.maximum(fa[:, 128:], _fold(sb, jnp.max))], axis=1)
                m_s[i % 2][zs, j] = f
                pace_s[zs] = f
            elif kind == 'EX':
                _, i, j = op
                S_s = (S0_s, S1_s)[i % 2]
                m = row_offset(i)
                m = jnp.where(pace_s[0, 0:1, :] == jnp.inf, jnp.inf, m)
                if j < i:
                    parts, lj = [], None
                    for r in range(112, -16, -16):
                        pt = jnp.exp2(S_s[0, j, r:r + 16, :] - m)
                        pb = jnp.exp2(S_s[0, j, 128 + r:128 + r + 16, :] - m)
                        parts.insert(0, _b7(pt[:, :128], pt[:, 128:], pb[:, :128], pb[:, 128:]))
                        x = (pt[:8] + pt[8:]) + (pb[:8] + pb[8:])
                        lj = x if lj is None else lj + x
                    st['P'][i, j] = [jnp.concatenate([x[n] for x in parts], axis=0).astype(bf16) for n in range(7)]
                else:
                    pa = jnp.exp2(S_s[0, j, 0:128, :] - m)
                    pb = jnp.exp2(S_s[0, j, 128:T, 128:T] - m[:, 128:])
                    la = _rsum(pa)
                    lj = jnp.concatenate([la[:, :128], la[:, 128:] + _rsum(pb)], axis=1)
                    st['P'][i, j] = (pa.astype(bf16), pb.astype(bf16))
                l_s[i % 2][zs, j] = lj
            elif kind == 'PV':
                _, i, j = op
                p = st['P'].pop((i, j))
                if j < i:
                    for n in SP:
                        st['last'] = _nn(_b(tile(V_s[j], n)), p[n])
                        st['o'][i, n] = st['o'][i, n] + st['last'] if j > 0 else st['last']
                    continue
                oa = _nn(_b(jnp.concatenate([tile(V_s[j], 2), tile(V_s[j], 8)], axis=0)), p[0])
                ob = _nn(_b(jnp.concatenate([tile(V_s[j], 7), tile(V_s[j], 3)], axis=0)), p[1])
                o = st['last'] = jnp.concatenate([oa[:, :128], oa[:, 128:] + ob], axis=1)
                if i > 0:
                    o = o + _quad(*_c4({n: st['o'].pop((i, n)) for n in range(7)}))
                l = l_s[i % 2][0, 0]
                for t in range(1, i + 1):
                    l = l + l_s[i % 2][0, t]
                o = o * (1.0 / jnp.sum(l, axis=0, keepdims=True))
                for n, x in enumerate(_b7(o[:128, :128], o[:128, 128:], o[128:, :128], o[128:, 128:])):
                    O_s[i][zs, n] = x.astype(bf16)
            elif kind == 'PACE':
                pace_s[zs] = jnp.concatenate([st['last'][-8:, -128:]] * 2, axis=1)
            elif kind == 'OP':
                _, i, t = op
                n = SO[t]
                st['M'][n] = st['last'] = _nn(_b(_gate(tile(W7_s, n), due())), O_s[i][0, n])
                if t == 6:
                    acc[:, T * i:T * (i + 1)] += _quad(*_c4(st['M']))
            elif kind == 'W7':
                res = []
                for r0 in range(16 * op[1], 16 * op[2], 16):
                    blk = [_u(woT[h, r:r + 16, c:c + 128]) for r in (r0, 224 + r0) for c in (0, 128)]
                    row = pl.ds(pl.multiple_of(zs * 8 + r0 // 2, 8), 8)
                    for n, x in enumerate(_combos(_a7, blk)):
                        W7_s[row, n * 128:(n + 1) * 128] = _u(x)
                    res += blk
                gate_later(res)
            elif kind == 'AT':
                g = jnp.clip((h - 4) // 4, 0, 2)
                t0 = jnp.minimum(((h + 12) % 4) * 6, NB - 6)
                grow = pl.ds(pl.multiple_of(g * 128, 128), 128)
                gcol = pl.ds(pl.multiple_of(jnp.where(h == H - 1, 3, g) * 128, 128), 128)
                res = []
                for n in range(6):
                    tok = pl.ds(pl.multiple_of((t0 + n) * 128, 128), 128)
                    x = aT_s[grow, tok].T
                    out_s[tok, gcol] = x
                    res.append(_u(x)[56:])
                gate_later(res)
            elif kind == 'HD':
                g = op[1]
                hs = jnp.concatenate([ssmk[rows, c * P:(c + 1) * P] for c in range(4 * g, 4 * g + 4)], axis=0)
                hf = _nn(hs, ff_s[...])
                for n in range(4):
                    X_s[(zs, HR) + blk_at(4 * g + n)] = hf[n * CH:(n + 1) * CH, :P]
                    X_s[(zs, HI) + blk_at(4 * g + n)] = hf[n * CH:(n + 1) * CH, P:]
            elif kind == 'SC':
                g = op[1]
                if g == 0:
                    k = jnp.concatenate([jnp.zeros((CH, P), f32), kT[rows, 0:4 * P].astype(f32)], axis=1)
                else:
                    k = kT[rows, (4 * g - 1) * P:(4 * g + 4) * P].astype(f32)
                ks = k[:, P:] * rep(0, 4)
                for j in range(1, KS):
                    ks = ks + pltpu.roll(k, j, 1)[:, P:] * rep(j, 4)
                kv = ks * vT[rows, 4 * g * P:(4 * g + 4) * P].astype(f32)
                kvs = jnp.concatenate([kv[:, n * P:(n + 1) * P] for n in range(4)], axis=0)
                xf = _nn(kvs.astype(bf16), ff_s[...])
                for n in range(4):
                    c = 4 * g + n
                    xr, xi = xf[n * CH:(n + 1) * CH, :P], xf[n * CH:(n + 1) * CH, P:]
                    X_s[(zs, KV) + blk_at(c)] = kvs[n * CH:(n + 1) * CH]
                    pr = xr if c == 0 else xr - sgn * st['x'][1]
                    pi = xi if c == 0 else xi + sgn * st['x'][0]
                    X_s[(zs, PR) + blk_at(c)] = pr
                    X_s[(zs, PI) + blk_at(c)] = pi
                    st['x'] = (xr, xi)
            elif kind == 'CV':
                res = []
                for a, half in op[1]:
                    wr = wi = None
                    for j in range(a + 1):
                        hr, hi_ = X_s[(0, HR) + blk_at(j, half)], X_s[(0, HI) + blk_at(j, half)]
                        pr, pi = X_s[(0, PR) + blk_at(a - j, half)], X_s[(0, PI) + blk_at(a - j, half)]
                        tr, ti = hr * pr - hi_ * pi, hr * pi + hi_ * pr
                        wr, wi = (tr, ti) if wr is None else (wr + tr, wi + ti)
                    r0 = (a % 4) * CH + 16 * half
                    Y_s[a // 4][zs, r0:r0 + 16, :P] = wr
                    Y_s[a // 4][zs, r0:r0 + 16, P:] = wi
                    res += [wr, wi]
                gate_later(res)
            elif kind == 'ID':
                g = op[1]
                y = _nn(Y_s[g][0].astype(bf16), fi_s[...])
                for n in range(4):
                    c = 4 * g + n
                    cols = slice(c * P, (c + 1) * P)
                    ya = y[n * CH:(n + 1) * CH, :] + X_s[(0, KV) + blk_at(c)] * taps[KS, rows, :]
                    aT_s[rows, cols] = (qT[rows, cols].astype(f32) * ya).astype(bf16)
        return carry

    jax.lax.fori_loop(0, H, head_body, 0)

    acc[:, T * (NT - 1):] += _quad(*_c4({n: _nn(_b(tile(W7_s, n)), O_s[NT - 1][0, n]) for n in SORD}))
    outs = [c_outa]
    for i in range(NT):
        cols = slice(T * i, T * (i + 1))
        blk = jnp.concatenate([aT_s[384:M, cols], acc[:, cols].astype(bf16)], axis=0)
        out_s[cols, 384:2 * M] = blk.T
        c = cp(out_s.at[pl.ds(T * i, T), pl.ds(384, 512)], out_hbm.at[pl.ds(T * i, T), pl.ds(384, 512)], sem_o.at[i])
        c.start()
        outs.append(c)
    for c in outs:
        c.wait()


@jax.jit
def pallas_concat_heads__ssm_conv_h3__compressed_kv_cla__prompt_kernel(
    A_q: jax.Array,
    A_k: jax.Array,
    A_v: jax.Array,
    A_shift_k: jax.Array,
    A_ssm_k: jax.Array,
    A_ssm_D: jax.Array,
    B_x: jax.Array,
    B_c_kv: jax.Array,
    B_w_q: jax.Array,
    B_w_uk: jax.Array,
    B_w_uv: jax.Array,
    B_w_o: jax.Array,
):
    hbm = pl.BlockSpec(memory_space=pl.ANY)
    vmem = pl.BlockSpec(memory_space=pltpu.VMEM)
    V = pltpu.VMEM
    out = pl.pallas_call(
        _kernel,
        out_shape=jax.ShapeDtypeStruct((S, 2 * M), bf16),
        in_specs=[hbm, hbm, hbm, vmem, hbm, vmem, hbm, hbm, hbm, hbm, hbm, hbm],
        out_specs=hbm,
        scratch_shapes=[
            V((M, S), bf16), V((M, S), bf16), V((M, S), bf16), V((M, S), bf16),
            V((M + 16, S), bf16), V((S + 16, DC), bf16),
            V((2, M * H, 128), bf16),
            V((2, 4, 128 * H + 16, 128), bf16), V((2, 4, 128 * H + 16, 128), bf16),
            V((H, M, D), bf16),
            V((H * 64, 7 * 256), u32), V((NT * 112, 7 * 128), u32),
            V((4 * H * 128, 7 * 128), u32), V((64, 49 * 256), u32),
            V((512 + 8, 512), u32),
            V((NT * H * 128, T), u32), V((4 * 128, 49 * 128), u32),
            V((M, S), f32), V((M, S), bf16), V((S, 2 * M), bf16),
            V((KS + 1, M, 128), f32), V((P, 2 * P), bf16), V((2 * P, P), bf16),
            V((1, NT, T, T), f32), V((1, NT, T, T), f32), V((1, 5, T, T), f32),
            V((112, 7 * 128), u32), V((1, 8, T), f32),
            V((1, NT, 8, T), f32), V((1, NT, 8, T), f32), V((1, NT, 8, T), f32), V((1, NT, 8, T), f32),
            pltpu.SemaphoreType.DMA((26,)), pltpu.SemaphoreType.DMA((8,)),
            pltpu.SemaphoreType.DMA((8,)), pltpu.SemaphoreType.DMA((9,)),
        ] + [V((64, 9 * 128), u32)] * (2 * NT) + [V((1, 7, 128, 128), bf16)] * NT
        + [V((1, 4 * CH, 2 * P), f32)] * 4,
        compiler_params=pltpu.CompilerParams(vmem_limit_bytes=126 * 1024 * 1024,
                                             shape_invariant_numerics=False),
    )(
        A_q[0].T, A_k[0].T, A_v[0].T, A_shift_k.T, A_ssm_k, A_ssm_D,
        B_x[0].T, B_c_kv[0],
        B_w_q.reshape(M * H, D), B_w_uk.reshape(DC * H, D), B_w_uv.reshape(DC * H, D),
        jnp.transpose(B_w_o, (0, 2, 1)),
    )
    return out[None]
```

```python
import functools
import math

import jax
import jax.numpy as jnp
import jax.experimental.pallas as pl
import jax.experimental.pallas.tpu as pltpu

bf16 = jnp.bfloat16
f32 = jnp.float32
u32 = jnp.uint32

S = 2048
M = 448
DC = 1024
H = 16
D = 256
KS = 4
P = 128
NB = S // P
CH = 32
NCH = M // CH
T = 256
NT = S // T
NEG = -1e30

SORD = tuple(int(c) for c in '6430125')
SK = tuple(int(c) for c in '0364125')
SV = tuple(int(c) for c in '0125364')
SQ = tuple(int(c) for c in '6043125')
SP = tuple(int(c) for c in '3640125')
SO = tuple(int(c) for c in '5210346')
QW1 = 70
QW2 = 126
QW3 = 192
QW4 = 208
QC1 = 150
QLAG = 12
CVMAX = 12
SIDE0 = 30
SIDEP = 4
SLAG = 5
PRE = 0
W7P = 16
W7D = 6
KVH = 35
EXB = 10
NOP6 = 2
LA = 3
C2N = 64
NOP = 2


def _nn(a, b):
    return jnp.dot(a, b, preferred_element_type=f32)


def _b(u):
    return pltpu.bitcast(u, bf16)


def _u(x):
    return pltpu.bitcast(x, u32)


def _lo(u):
    return pltpu.bitcast(u << 16, f32)


def _hi(u):
    return pltpu.bitcast(u & jnp.uint32(0xFFFF0000), f32)


def _f(u):
    return _b(u).astype(f32)


def _a7(a11, a12, a21, a22):
    return [a11 + a22, a21 + a22, a11, a22, a11 + a12, a21 - a11, a12 - a22]


def _b7(b11, b12, b21, b22):
    return [b11 + b22, b11, b12 - b22, b21 - b11, b22, b11 + b12, b21 + b22]


def _c4(m):
    return m[0] + m[3] - m[4] + m[6], m[2] + m[4], m[1] + m[3], m[0] - m[1] + m[2] + m[5]


_C_OF = (((0, 1), (3, 1)), ((2, 1), (3, -1)), ((1, 1), (3, 1)), ((0, 1), (2, 1)), ((0, -1), (1, 1)), ((3, 1),), ((0, 1),))
_C_CNT = (4, 2, 2, 4)
_A_OF = {0: (0, 3, 1), 1: (2, 3, 1), 4: (0, 1, 1), 5: (2, 0, -1), 6: (1, 3, -1)}


def _combos(f7, blk):
    x = f7(*[_f(v) for v in blk])
    plain = {2: 0, 3: 3} if f7 is _a7 else {1: 0, 4: 3}
    return [_b(blk[plain[n]]) if n in plain else x[n].astype(bf16) for n in range(7)]


def _quad(c11, c12, c21, c22):
    return jnp.concatenate([jnp.concatenate([c11, c12], axis=1), jnp.concatenate([c21, c22], axis=1)], axis=0)


def _fold(c, op):
    return op(c.reshape(-1, 8, c.shape[1]), axis=0)


def _rsum(p):
    cols = []
    for c in range(0, p.shape[1], 128):
        acc = None
        for r in range(112, -16, -16):
            t = p[r:r + 8, c:c + 128] + p[r + 8:r + 16, c:c + 128]
            acc = t if acc is None else acc + t
        cols.append(acc)
    return jnp.concatenate(cols, axis=1) if len(cols) > 1 else cols[0]


def _tok(vals):
    parts = []
    for v in vals:
        for r in range(0, v.shape[0], 8):
            for c in range(0, v.shape[1], 128):
                parts.append(v[r:r + 8, c:c + 128])
    while len(parts) > 1:
        parts = [parts[i] | parts[i + 1] if i + 1 < len(parts) else parts[i] for i in range(0, len(parts), 2)]
    return (parts[0] >> 31) >> 1


def _gate(x, tok):
    if tok is None:
        return x
    top = x[:8, :128] | tok
    if x.shape[1] > 128:
        top = jnp.concatenate([top, x[:8, 128:]], axis=1)
    return jnp.concatenate([top, x[8:]], axis=0)


def _side_pieces():
    ps = [(k, g) for g in range(PRE) for k in ('HD', 'SC')]
    cur, cost = [], 0
    for a in range(NB):
        if a % 4 == 0 and a // 4 + PRE < 4:
            ps += [('HD', a // 4 + PRE), ('SC', a // 4 + PRE)]
        for half in range(2):
            if cur and cost + a + 1 > CVMAX:
                ps.append(('CV', tuple(cur)))
                cur, cost = [], 0
            cur.append((a, half))
            cost += a + 1
        if a % 4 == 3:
            ps += [('CV', tuple(cur)), ('ID', a // 4)]
            cur, cost = [], 0
    ps.insert(W7P, ('W7', 0, 7))
    ps.insert(W7P + W7D, ('W7', 7, 14))
    return ps


def _schedule():
    side = _side_pieces()
    out = []
    cnt = [0]

    def block(subs, att, with_side):
        for k, u in enumerate(subs):
            out.append(u)
            out.extend(att.get(k, []))
            if with_side:
                cnt[0] += 1
                if side and cnt[0] >= SIDE0 and (cnt[0] - SIDE0) % SIDEP == 0:
                    out.append(side.pop(0))

    def kv(p, half):
        return [('KV', p, t) for t in (range(KVH) if half == 0 else range(KVH, 49))]

    def op_(*idx):
        return [('OP', i, t) for i in idx for t in range(7)]

    def softmax_head(i, n):
        att = {max(n - EXB, 0): [('PACE',), ('EX', i, 0)]}
        for k in range(1, min(LA, i + 1)):
            att.setdefault(n - 1 - (LA - 1 - k) * 2, []).extend([('PACE',), ('EX', i, k)])
        return att

    ops_left = list(range(NT - 1))
    block(kv(0, 0) + kv(0, 1), {}, True)
    block(op_(NT - 1), {6: [('AT',), ('QK', 0, 0)]}, False)
    block(kv(1, 0), softmax_head(0, KVH), True)
    for i in range(NT - 1):
        for j in range(i + 1):
            out.append(('QK', i + 1, j))
            if j + LA <= i:
                out.append(('EX', i, j + LA))
            out.append(('PV', i, j))
        out.append(('QK', i + 1, i + 1))
        if i < 5:
            subs = kv((i + 3) // 2, (i + 1) % 2)
            block(subs, softmax_head(i + 1, len(subs)), True)
        else:
            n = NOP6 if i == 5 else NOP
            block(op_(*ops_left[:n]), softmax_head(i + 1, 7 * n), False)
            del ops_left[:n]
    out.append(('PACE',))
    for j in range(NT):
        if j + LA < NT:
            out.append(('EX', NT - 1, j + LA))
        out.append(('PV', NT - 1, j))
        if len(ops_left) > 2:
            block(op_(ops_left.pop(0)), {}, False)
        out.append(('PACE',))
    block(op_(*ops_left), {}, False)
    assert not side
    w7 = [k for k, o in enumerate(out) if o[0] == 'W7']
    assert out.index(('OP', NT - 1, 6)) < min(w7) and max(w7) < out.index(('OP', 0, 0))
    out.remove(('ID', 3))
    out.append(('ID', 3))
    return out


def _kernel(qT_hbm, kT_hbm, vT_hbm, sk_ref, ssmk_hbm, dd_ref, xT_hbm, ckv_hbm,
            wq_hbm, wk_hbm, wv_hbm, woT_hbm, out_hbm,
            qT, kT, vT, ssmk, xT, ckv, wq_raw, wk_raw, wv_raw, woT,
            aq_s, bx_s, w1_s, w2_s, cT_s, QT_s, c2_s, acc, aT_s, out_s, taps, ff_s, fi_s,
            S0_s, S1_s, X_s, W7_s, pace_s, m0_s, m1_s, l0_s, l1_s,
            sem, sem_k, sem_v, sem_o, *rest):
    K_s, V_s, O_s, Y_s = rest[:NT], rest[NT:2 * NT], rest[2 * NT:3 * NT], rest[3 * NT:]

    def cp(src, dst, s):
        return pltpu.make_async_copy(src, dst, s)

    def c_x(j):
        cols = pl.ds(pl.multiple_of(j * 2 * T, 2 * T), 2 * T)
        return cp(xT_hbm.at[:, cols], xT.at[pl.ds(pl.multiple_of(j * M, 16), M)], sem.at[j])

    QP = ((0, 128), (128, 96))

    def c_wq(p):
        cs_ = []
        for half in range(2):
            r = pl.ds((half * 224 + QP[p][0]) * H, QP[p][1] * H)
            for g in range(2):
                cs_.append(cp(wq_hbm.at[r, pl.ds(128 * g, 128)], wq_raw.at[g, r], sem.at[18 + 4 * p + 2 * half + g]))
        return cs_

    def c_w(w_hbm, raw, sm, j, half, g):
        r = pl.ds(pl.multiple_of((half * 4 + j) * 2048, 2048), 2048)
        q = 2 * half + g
        return cp(w_hbm.at[r, pl.ds(128 * g, 128)], raw.at[j % 2, q, pl.ds(0, 2048)], sm.at[(j % 2) * 4 + q])

    def c_wk(j):
        return [c_w(wk_hbm, wk_raw, sem_k, j, half, g) for half in range(2) for g in range(2)]

    def c_wv(j):
        return [c_w(wv_hbm, wv_raw, sem_v, j, half, g) for half in range(2) for g in range(2)]

    def c_ckv(j):
        r = pl.ds(pl.multiple_of(j * 2 * T, 2 * T), 2 * T)
        return cp(ckv_hbm.at[r], ckv.at[r], sem.at[9 + j])

    a_pairs = ((kT_hbm, kT), (vT_hbm, vT), (ssmk_hbm, ssmk), (qT_hbm, qT))
    c_early = [cp(woT_hbm.at[pl.ds(0, 1)], woT.at[pl.ds(0, 1)], sem.at[4])]
    c_early += [cp(src.at[pl.ds(0, CH)], dst.at[pl.ds(0, CH)], sem.at[5 + n]) for n, (src, dst) in enumerate(a_pairs)]
    c_late = [cp(woT_hbm.at[pl.ds(1, H - 1)], woT.at[pl.ds(1, H - 1)], sem.at[13])]
    c_late += [cp(src.at[pl.ds(CH, M - CH)], dst.at[pl.ds(CH, M - CH)], sem.at[14 + n])
               for n, (src, dst) in enumerate(a_pairs)]
    for c in [c_x(0)] + c_wq(0) + c_wq(1):
        c.start()
    for c in c_wk(0) + [c_x(1)]:
        c.start(priority=1)

    n_i = jax.lax.broadcasted_iota(jnp.int32, (P, P), 0)
    k_i = jax.lax.broadcasted_iota(jnp.int32, (P, P), 1)
    ang = (((2 * k_i + 1) * n_i) & 511).astype(f32) * (math.pi / 256.0)
    cs, sn = jnp.cos(ang), jnp.sin(ang)
    ff_s[:, 0:P] = cs.astype(bf16)
    ff_s[:, P:2 * P] = (-sn).astype(bf16)
    fi_s[0:P, :] = (cs.T * (1.0 / P)).astype(bf16)
    fi_s[P:2 * P, :] = (sn.T * (-1.0 / P)).astype(bf16)
    sk = sk_ref[...].astype(f32)
    for t in range(KS):
        taps[t] = jnp.broadcast_to(sk[t:t + 1, :], (128, M)).T
    taps[KS] = jnp.broadcast_to(dd_ref[...].astype(f32).reshape(1, M), (128, M)).T
    acc[...] = jnp.zeros(acc.shape, f32)
    aT_s[...] = jnp.zeros(aT_s.shape, bf16)
    O_s[NT - 1][...] = jnp.zeros(O_s[0].shape, bf16)
    W7_s[...] = jnp.zeros(W7_s.shape, u32)
    cT_s[...] = jnp.zeros(cT_s.shape, u32)

    def prep_x(jj, t, r0):
        xj = xT.at[pl.ds(pl.multiple_of(jj * M, 16), M)]
        bj = bx_s.at[pl.ds(pl.multiple_of(jj * 224, 16), 224)]
        blk = [_u(xj[r:r + 32, c:c + 128]) for r in (r0, 224 + r0) for c in (t * T, t * T + 128)]
        row = t * 112 + r0 // 2
        for n, x in enumerate(_combos(_b7, blk)):
            bj[row:row + 16, n * 128:(n + 1) * 128] = _u(x)
        return []

    c_x(0).wait()
    for t in range(2):
        for r0 in range(0, 224, 32):
            prep_x(0, t, r0)
    vq = wq_raw.bitcast(u32)
    for p, (c0, nc) in enumerate(QP):
        for c in c_wq(p):
            c.wait()
        for hp in range(H // 2):
            ut = [vq[g, pl.ds((half * 224 + c0) * 8 + hp, nc, stride=8), :].T for g in range(2) for half in range(2)]
            for r in range(0, 128, 16):
                u = [x[r:r + 16] for x in ut]
                for par, f in enumerate((_lo, _hi)):
                    r0 = (2 * hp + par) * 64 + r // 2
                    for n, x in enumerate(_a7(*[f(x) for x in u])):
                        aq_s[r0:r0 + 8, n * 256 + c0:n * 256 + c0 + nc] = _u(x.astype(bf16))
    for c in c_wv(0) + [c_ckv(0)]:
        c.start(priority=1)

    qscale = (D ** -0.5) * math.log2(math.e)

    def prep_c2(jj, r):
        blk = [[cT_s[cq * 128 + r:cq * 128 + r + 8, tb * 128:(tb + 1) * 128] for tb in range(4)] for cq in range(4)]
        x = [[_f(v) for v in row] for row in blk]
        outer = [[_b7(x[ci][ti], x[ci][2 + ti], x[2 + ci][ti], x[2 + ci][2 + ti]) for ti in range(2)]
                 for ci in range(2)]
        two = [_b7(outer[0][0][n], outer[0][1][n], outer[1][0][n], outer[1][1][n]) for n in range(7)]
        cj = c2_s.at[pl.ds(pl.multiple_of(jj * 128, 128), 128)]
        for n in range(7):
            for m in range(7):
                cj[r:r + 8, (n * 7 + m) * 128:(n * 7 + m + 1) * 128] = _u(two[n][m].astype(bf16))
        return []

    def q_body(j, carry):
        mq = {}
        qtj = QT_s.at[pl.ds(pl.multiple_of(j * 4096, 4096), 4096)]
        zq = j >> 4
        bx = [[bx_s[pl.ds(pl.multiple_of((2 * j + t) * 112, 16), 112), n * 128:(n + 1) * 128] for n in range(7)]
              for t in range(2)]

        def qproj(u, tok):
            hh, t, n = u // 14, (u // 7) % 2, SORD[u % 7]
            w = _b(_gate(aq_s[hh * 64:hh * 64 + 64, n * 256:n * 256 + 224], tok))
            mq[n] = _nn(w, _b(bx[t][n]))
            if u % 7 == 6:
                for k, x in enumerate(_c4(mq)):
                    r0 = t * 2048 + hh * 128 + (k // 2) * 64
                    qtj[r0:r0 + 64, (k % 2) * 128:(k % 2 + 1) * 128] = _u((x * qscale).astype(bf16))
            return mq[n]

        wt = {}
        ckj = ckv.at[pl.ds(pl.multiple_of(j * 512, 512), 512)]
        w1j = w1_s.at[pl.ds(pl.multiple_of(j * 2048, 2048), 2048)]

        def prep_w(kv, hp, part):
            if part == 0:
                v = (wk_raw, wv_raw)[kv].bitcast(u32).at[j % 2]
                wt[kv, hp] = [v[q, pl.ds(hp, 128, stride=8), :].T for q in (0, 2, 1, 3)]
                return [x[120:] for x in wt[kv, hp]]
            for r in range(32 * (part - 1), 32 * part, 16):
                u = [x[r:r + 16] for x in wt[kv, hp]]
                for par, f in enumerate((_lo, _hi)):
                    r0 = (2 * hp + par) * 128 + kv * 64 + r // 2
                    for n, c in enumerate(_a7(*[f(x) for x in u])):
                        w1j[r0:r0 + 8, n * 128:(n + 1) * 128] = _u(c.astype(bf16))
            return []

        def prep_ct(half, cq):
            res = []
            ct = 2 * cq + half
            for tb in range(4):
                x = _u(ckj[tb * 128:(tb + 1) * 128, ct * 128:(ct + 1) * 128].T)
                cT_s[pl.ds(pl.multiple_of(zq * 64 + ct * 64, 64), 64), tb * 128:(tb + 1) * 128] = x
                res.append(x[56:])
            return res

        fill = {}

        def spread(pieces, u0, u1):
            for n, p in enumerate(pieces):
                fill.setdefault(u0 + n * (u1 - u0) // len(pieces), []).append(p)

        spread([functools.partial(prep_w, 0, hp, part) for hp in range(8) for part in range(5)], QW1, QW2)
        spread([functools.partial(prep_w, 1, hp, part) for hp in range(8) for part in range(5)], QW2, QW3)
        spread([functools.partial(prep_ct, 0, cq) for cq in range(4)], QW2 + 2, QC1)
        spread([functools.partial(prep_ct, 1, cq) for cq in range(4)], QC1, QW3)
        spread([functools.partial(prep_c2, jnp.maximum(j - 1, 0), r) for r in range(C2N, 128, 8)], 2, QW1 - 4)
        if C2N:
            spread([functools.partial(prep_c2, j, r) for r in range(0, C2N, 8)], QW3, QW4)
        spread([functools.partial(prep_x, jnp.minimum(j + 1, 3), t, r0)
                for t in range(2) for r0 in range(0, 224, 32)], QW4, 221)
        toks = {}
        for u in range(224):
            if u == QW1:
                @pl.when(j < 3)
                def _():
                    for c in c_wk(j + 1):
                        c.start(priority=1)

                @pl.when(j == 3)
                def _():
                    for c in c_early + c_late:
                        c.start(priority=1)

                for c in c_wk(j):
                    c.wait()
            if u == QW2:
                @pl.when(j < 3)
                def _():
                    for c in c_wv(j + 1) + [c_ckv(j + 1)]:
                        c.start(priority=1)

                @pl.when(j < 2)
                def _():
                    c_x(j + 2).start(priority=1)

                @pl.when(j < 3)
                def _():
                    c_x(j + 1).wait()

                for c in c_wv(j) + [c_ckv(j)]:
                    c.wait()
            q = qproj(u, toks.pop(u, None))
            res = []
            ps = fill.get(u, [])
            for n, p in enumerate(ps):
                row = (n * 128 // len(ps)) // 16 * 16
                if p.func is prep_w and p.args[2] == 0:
                    (wk_raw, wv_raw)[p.args[0]].bitcast(u32)[zq, 0, 1024:1032, :] = _u(q[row:row + 8])
                elif p.func is prep_c2:
                    cT_s[pl.ds(pl.multiple_of(512 + zq * 8, 8), 8), 0:128] = _u(q[row:row + 8])
                elif p.func is prep_x:
                    xT[pl.ds(pl.multiple_of(4 * M + zq * 16, 16), 16), 0:128] = q[row:row + 16].astype(bf16)
                elif p.func is prep_ct:
                    ckv[pl.ds(pl.multiple_of(S + zq * 16, 16), 16), 0:128] = q[row:row + 16].astype(bf16)
                res += p()
            if res:
                toks[u + QLAG] = _tok(res)
        return carry

    jax.lax.fori_loop(0, 4, q_body, 0)
    for r in range(C2N, 128, 8):
        prep_c2(3, r)
    for c in c_early:
        c.wait()

    tri = n_i <= k_i
    sgn = jnp.where((jax.lax.broadcasted_iota(jnp.int32, (1, P), 1) & 1) == 0, 1.0, -1.0).astype(f32)
    c_outa = cp(out_s.at[:, pl.ds(0, 384)], out_hbm.at[:, pl.ds(0, 384)], sem_o.at[8])
    HR, HI, PR, PI, KV = range(5)

    def blk_at(c, half=None):
        r0 = (c % 8) * CH
        rs = slice(r0, r0 + CH) if half is None else slice(r0 + 16 * half, r0 + 16 * half + 16)
        return rs, slice((c // 8) * P, (c // 8 + 1) * P)

    def tile(ref, n):
        return ref[:, n * 128:(n + 1) * 128]

    def head_body(h, carry):
        @pl.when(h == 1)
        def _():
            for c in c_late:
                c.wait()

        @pl.when(h == H - 1)
        def _():
            c_outa.start()

        st = dict(co={}, cnt={}, fin=set(), M={}, P={}, Q7={}, mfin={}, o={})
        zs = h >> 10
        z64 = pl.ds(pl.multiple_of(zs * 64, 64), 64)
        m_s, l_s = (m0_s, m1_s), (l0_s, l1_s)
        w1h = w1_s.at[pl.ds(pl.multiple_of(h * 128, 128), 3 * 2048 + 128)]
        qth = QT_s.at[pl.ds(pl.multiple_of(h * 128, 128), 7 * 2048 + 128)]
        rows = pl.ds(pl.multiple_of(jnp.minimum(h, NCH - 1) * CH, CH), CH)

        def rep(t, n):
            return jnp.concatenate([taps[t, rows, :]] * n, axis=1)

        toks = []

        def due():
            for t in toks:
                t[0] -= 1
            ready = [t[1] for t in toks if t[0] <= 0]
            toks[:] = [t for t in toks if t[0] > 0]
            return functools.reduce(lambda x, y: x | y, ready) if ready else None

        def gate_later(vals):
            toks.append([SLAG, _tok([v if v.dtype == u32 else _u(v) for v in vals])])

        def row_offset(i):
            if i not in st['mfin']:
                m = m_s[i % 2][0, 0]
                for t in range(1, i + 1):
                    m = jnp.maximum(m, m_s[i % 2][0, t])
                m = jnp.max(m, axis=0, keepdims=True)
                if i > 0:
                    lo_ = jnp.exp2(m_s[i % 2][0, 0] - m)
                    for t in range(1, i + 1):
                        lo_ = lo_ + jnp.exp2(m_s[i % 2][0, t] - m)
                    m = m + jnp.log2(jnp.sum(lo_, axis=0, keepdims=True))
                st['mfin'][i] = m
            return st['mfin'][i]

        for op in _schedule():
            kind = op[0]
            if kind == 'KV':
                _, p, t = op
                n, m = SK[t // 7], SV[t % 7]

                def wblk(q):
                    w = jnp.concatenate([w1h[k * 2048:k * 2048 + 128, n * 128:(n + 1) * 128]
                                         for k in (2 * (q % 2), 2 * (q % 2) + 1)], axis=1)
                    r = (q // 2) * 32
                    return jnp.concatenate([w[r:r + 32], w[64 + r:64 + r + 32]], axis=0)

                cols = slice((n * 7 + m) * 256, (n * 7 + m + 1) * 256)
                if m in (2, 3):
                    w = wblk(0 if m == 2 else 3)
                elif p > 0:
                    w = w2_s[:, cols]
                else:
                    i1, i2, sg = _A_OF[m]
                    x, y = wblk(i1), wblk(i2)
                    w = (_f(x) + _f(y) if sg > 0 else _f(x) - _f(y)).astype(bf16)
                    w2_s[z64, cols] = _u(w)
                c2 = c2_s[p * 128:(p + 1) * 128, (n * 7 + m) * 128:(n * 7 + m + 1) * 128]
                st['M'][m] = st['last'] = _nn(w if w.dtype == bf16 else _b(_gate(w, due())), _b(c2))
                if t % 7 < 6:
                    continue
                mo = _quad(*_c4(st['M']))
                for o, sg in _C_OF[n]:
                    k = st['cnt'][o] = st['cnt'].get(o, 0) + 1
                    if k == 1:
                        st['co'][o] = mo if sg > 0 else -mo
                    else:
                        st['co'][o] = st['co'][o] + mo if sg > 0 else st['co'][o] - mo
                    if k == _C_CNT[o]:
                        st['cnt'][o] = 0
                        st['fin'].add(o)
                for tok in range(2):
                    if not {tok, 2 + tok} <= st['fin']:
                        continue
                    st['fin'] -= {tok, 2 + tok}
                    c = 2 * p + tok

                    def full(dh, kb, off):
                        x = st['co'][2 * dh + tok][:, kb * 128:(kb + 1) * 128]
                        return jnp.concatenate([x[off:off + 64], x[128 + off:128 + off + 64]], axis=0)

                    kb4 = (full(0, 0, 0).T, full(1, 0, 0).T, full(0, 1, 0).T, full(1, 1, 0).T)
                    vb4 = (full(0, 0, 64), full(0, 1, 64), full(1, 0, 64), full(1, 1, 64))
                    for ref, c4 in ((K_s[c], kb4), (V_s[c], vb4)):
                        blks = dict(zip((2, 7, 8, 3), c4))
                        if c < NT - 1:
                            blks.update({k: x for k, x in enumerate(_a7(*c4)) if k not in (2, 3)})
                        for k, x in blks.items():
                            ref[z64, k * 128:(k + 1) * 128] = _u(x.astype(bf16))
            elif kind == 'QK':
                _, i, j = op
                S_s = (S0_s, S1_s)[i % 2]
                if j < i:
                    if i not in st['Q7']:
                        qu = qth[i * 2048:i * 2048 + 128, :]
                        st['Q7'][i] = _combos(_b7, [qu[:64, :128], qu[:64, 128:], qu[64:, :128], qu[64:, 128:]])
                    s = _quad(*_c4({n: _nn(_b(tile(K_s[j], n)), st['Q7'][i][n]) for n in SQ}))
                    S_s[zs, j] = s
                    f = _fold(s, jnp.max)
                else:
                    q = _b(qth[i * 2048:i * 2048 + 128, :])
                    sa = _nn(_b(jnp.concatenate([tile(K_s[j], 2), tile(K_s[j], 7)], axis=1)), q)
                    sa = jnp.concatenate([jnp.where(tri, sa[:, :128], NEG), sa[:, 128:]], axis=1)
                    sb = _nn(_b(jnp.concatenate([tile(K_s[j], 8), tile(K_s[j], 3)], axis=1)), q[:, 128:])
                    sb = jnp.where(tri, sb, NEG)
                    S_s[zs, j, 0:128, :] = sa
                    S_s[zs, j, 128:T, 128:T] = sb
                    fa = _fold(sa, jnp.max)
                    f = jnp.concatenate([fa[:, :128], jnp.maximum(fa[:, 128:], _fold(sb, jnp.max))], axis=1)
                m_s[i % 2][zs, j] = f
                pace_s[zs] = f
            elif kind == 'EX':
                _, i, j = op
                S_s = (S0_s, S1_s)[i % 2]
                m = row_offset(i)
                m = jnp.where(pace_s[0, 0:1, :] == jnp.inf, jnp.inf, m)
                if j < i:
                    parts, lj = [], None
                    for r in range(112, -16, -16):
                        pt = jnp.exp2(S_s[0, j, r:r + 16, :] - m)
                        pb = jnp.exp2(S_s[0, j, 128 + r:128 + r + 16, :] - m)
                        parts.insert(0, _b7(pt[:, :128], pt[:, 128:], pb[:, :128], pb[:, 128:]))
                        x = (pt[:8] + pt[8:]) + (pb[:8] + pb[8:])
                        lj = x if lj is None else lj + x
                    st['P'][i, j] = [jnp.concatenate([x[n] for x in parts], axis=0).astype(bf16) for n in range(7)]
                else:
                    pa = jnp.exp2(S_s[0, j, 0:128, :] - m)
                    pb = jnp.exp2(S_s[0, j, 128:T, 128:T] - m[:, 128:])
                    la = _rsum(pa)
                    lj = jnp.concatenate([la[:, :128], la[:, 128:] + _rsum(pb)], axis=1)
                    st['P'][i, j] = (pa.astype(bf16), pb.astype(bf16))
                l_s[i % 2][zs, j] = lj
            elif kind == 'PV':
                _, i, j = op
                p = st['P'].pop((i, j))
                if j < i:
                    for n in SP:
                        st['last'] = _nn(_b(tile(V_s[j], n)), p[n])
                        st['o'][i, n] = st['o'][i, n] + st['last'] if j > 0 else st['last']
                    continue
                oa = _nn(_b(jnp.concatenate([tile(V_s[j], 2), tile(V_s[j], 8)], axis=0)), p[0])
                ob = _nn(_b(jnp.concatenate([tile(V_s[j], 7), tile(V_s[j], 3)], axis=0)), p[1])
                o = st['last'] = jnp.concatenate([oa[:, :128], oa[:, 128:] + ob], axis=1)
                if i > 0:
                    o = o + _quad(*_c4({n: st['o'].pop((i, n)) for n in range(7)}))
                l = l_s[i % 2][0, 0]
                for t in range(1, i + 1):
                    l = l + l_s[i % 2][0, t]
                o = o * (1.0 / jnp.sum(l, axis=0, keepdims=True))
                for n, x in enumerate(_b7(o[:128, :128], o[:128, 128:], o[128:, :128], o[128:, 128:])):
                    O_s[i][zs, n] = x.astype(bf16)
            elif kind == 'PACE':
                pace_s[zs] = jnp.concatenate([st['last'][-8:, -128:]] * 2, axis=1)
            elif kind == 'OP':
                _, i, t = op
                n = SO[t]
                st['M'][n] = st['last'] = _nn(_b(_gate(tile(W7_s, n), due())), O_s[i][0, n])
                if t == 6:
                    acc[:, T * i:T * (i + 1)] += _quad(*_c4(st['M']))
            elif kind == 'W7':
                res = []
                for r0 in range(16 * op[1], 16 * op[2], 16):
                    blk = [_u(woT[h, r:r + 16, c:c + 128]) for r in (r0, 224 + r0) for c in (0, 128)]
                    row = pl.ds(pl.multiple_of(zs * 8 + r0 // 2, 8), 8)
                    for n, x in enumerate(_combos(_a7, blk)):
                        W7_s[row, n * 128:(n + 1) * 128] = _u(x)
                    res += blk
                gate_later(res)
            elif kind == 'AT':
                g = jnp.clip((h - 4) // 4, 0, 2)
                t0 = jnp.minimum(((h + 12) % 4) * 6, NB - 6)
                grow = pl.ds(pl.multiple_of(g * 128, 128), 128)
                gcol = pl.ds(pl.multiple_of(jnp.where(h == H - 1, 3, g) * 128, 128), 128)
                res = []
                for n in range(6):
                    tok = pl.ds(pl.multiple_of((t0 + n) * 128, 128), 128)
                    x = aT_s[grow, tok].T
                    out_s[tok, gcol] = x
                    res.append(_u(x)[56:])
                gate_later(res)
            elif kind == 'HD':
                g = op[1]
                hs = jnp.concatenate([ssmk[rows, c * P:(c + 1) * P] for c in range(4 * g, 4 * g + 4)], axis=0)
                hf = _nn(hs, ff_s[...])
                for n in range(4):
                    X_s[(zs, HR) + blk_at(4 * g + n)] = hf[n * CH:(n + 1) * CH, :P]
                    X_s[(zs, HI) + blk_at(4 * g + n)] = hf[n * CH:(n + 1) * CH, P:]
            elif kind == 'SC':
                g = op[1]
                if g == 0:
                    k = jnp.concatenate([jnp.zeros((CH, P), f32), kT[rows, 0:4 * P].astype(f32)], axis=1)
                else:
                    k = kT[rows, (4 * g - 1) * P:(4 * g + 4) * P].astype(f32)
                ks = k[:, P:] * rep(0, 4)
                for j in range(1, KS):
                    ks = ks + pltpu.roll(k, j, 1)[:, P:] * rep(j, 4)
                kv = ks * vT[rows, 4 * g * P:(4 * g + 4) * P].astype(f32)
                kvs = jnp.concatenate([kv[:, n * P:(n + 1) * P] for n in range(4)], axis=0)
                xf = _nn(kvs.astype(bf16), ff_s[...])
                for n in range(4):
                    c = 4 * g + n
                    xr, xi = xf[n * CH:(n + 1) * CH, :P], xf[n * CH:(n + 1) * CH, P:]
                    X_s[(zs, KV) + blk_at(c)] = kvs[n * CH:(n + 1) * CH]
                    pr = xr if c == 0 else xr - sgn * st['x'][1]
                    pi = xi if c == 0 else xi + sgn * st['x'][0]
                    X_s[(zs, PR) + blk_at(c)] = pr
                    X_s[(zs, PI) + blk_at(c)] = pi
                    st['x'] = (xr, xi)
            elif kind == 'CV':
                res = []
                for a, half in op[1]:
                    wr = wi = None
                    for j in range(a + 1):
                        hr, hi_ = X_s[(0, HR) + blk_at(j, half)], X_s[(0, HI) + blk_at(j, half)]
                        pr, pi = X_s[(0, PR) + blk_at(a - j, half)], X_s[(0, PI) + blk_at(a - j, half)]
                        tr, ti = hr * pr - hi_ * pi, hr * pi + hi_ * pr
                        wr, wi = (tr, ti) if wr is None else (wr + tr, wi + ti)
                    r0 = (a % 4) * CH + 16 * half
                    Y_s[a // 4][zs, r0:r0 + 16, :P] = wr
                    Y_s[a // 4][zs, r0:r0 + 16, P:] = wi
                    res += [wr, wi]
                gate_later(res)
            elif kind == 'ID':
                g = op[1]
                y = _nn(Y_s[g][0].astype(bf16), fi_s[...])
                for n in range(4):
                    c = 4 * g + n
                    cols = slice(c * P, (c + 1) * P)
                    ya = y[n * CH:(n + 1) * CH, :] + X_s[(0, KV) + blk_at(c)] * taps[KS, rows, :]
                    aT_s[rows, cols] = (qT[rows, cols].astype(f32) * ya).astype(bf16)
        return carry

    jax.lax.fori_loop(0, H, head_body, 0)

    acc[:, T * (NT - 1):] += _quad(*_c4({n: _nn(_b(tile(W7_s, n)), O_s[NT - 1][0, n]) for n in SORD}))
    outs = [c_outa]
    for i in range(NT):
        cols = slice(T * i, T * (i + 1))
        blk = jnp.concatenate([aT_s[384:M, cols], acc[:, cols].astype(bf16)], axis=0)
        out_s[cols, 384:2 * M] = blk.T
        c = cp(out_s.at[pl.ds(T * i, T), pl.ds(384, 512)], out_hbm.at[pl.ds(T * i, T), pl.ds(384, 512)], sem_o.at[i])
        c.start()
        outs.append(c)
    for c in outs:
        c.wait()


@jax.jit
def pallas_concat_heads__ssm_conv_h3__compressed_kv_cla__prompt_kernel(
    A_q: jax.Array,
    A_k: jax.Array,
    A_v: jax.Array,
    A_shift_k: jax.Array,
    A_ssm_k: jax.Array,
    A_ssm_D: jax.Array,
    B_x: jax.Array,
    B_c_kv: jax.Array,
    B_w_q: jax.Array,
    B_w_uk: jax.Array,
    B_w_uv: jax.Array,
    B_w_o: jax.Array,
):
    hbm = pl.BlockSpec(memory_space=pl.ANY)
    vmem = pl.BlockSpec(memory_space=pltpu.VMEM)
    V = pltpu.VMEM
    out = pl.pallas_call(
        _kernel,
        out_shape=jax.ShapeDtypeStruct((S, 2 * M), bf16),
        in_specs=[hbm, hbm, hbm, vmem, hbm, vmem, hbm, hbm, hbm, hbm, hbm, hbm],
        out_specs=hbm,
        scratch_shapes=[
            V((M, S), bf16), V((M, S), bf16), V((M, S), bf16), V((M, S), bf16),
            V((4 * M + 16, 2 * T), bf16), V((S + 16, DC), bf16),
            V((2, M * H, 128), bf16),
            V((2, 4, 128 * H + 16, 128), bf16), V((2, 4, 128 * H + 16, 128), bf16),
            V((H, M, D), bf16),
            V((H * 64, 7 * 256), u32), V((NT * 112, 7 * 128), u32),
            V((4 * H * 128, 7 * 128), u32), V((64, 49 * 256), u32),
            V((512 + 8, 512), u32),
            V((NT * H * 128, T), u32), V((4 * 128, 49 * 128), u32),
            V((M, S), f32), V((M, S), bf16), V((S, 2 * M), bf16),
            V((KS + 1, M, 128), f32), V((P, 2 * P), bf16), V((2 * P, P), bf16),
            V((1, NT, T, T), f32), V((1, NT, T, T), f32), V((1, 5, T, T), f32),
            V((112, 7 * 128), u32), V((1, 8, T), f32),
            V((1, NT, 8, T), f32), V((1, NT, 8, T), f32), V((1, NT, 8, T), f32), V((1, NT, 8, T), f32),
            pltpu.SemaphoreType.DMA((26,)), pltpu.SemaphoreType.DMA((8,)),
            pltpu.SemaphoreType.DMA((8,)), pltpu.SemaphoreType.DMA((9,)),
        ] + [V((64, 9 * 128), u32)] * (2 * NT) + [V((1, 7, 128, 128), bf16)] * NT
        + [V((1, 4 * CH, 2 * P), f32)] * 4,
        compiler_params=pltpu.CompilerParams(vmem_limit_bytes=126 * 1024 * 1024,
                                             shape_invariant_numerics=False),
    )(
        A_q[0].T, A_k[0].T, A_v[0].T, A_shift_k.T, A_ssm_k, A_ssm_D,
        B_x[0].T, B_c_kv[0],
        B_w_q.reshape(M * H, D), B_w_uk.reshape(DC * H, D), B_w_uv.reshape(DC * H, D),
        jnp.transpose(B_w_o, (0, 2, 1)),
    )
    return out[None]
```

```python
import functools
import math

import jax
import jax.numpy as jnp
import jax.experimental.pallas as pl
import jax.experimental.pallas.tpu as pltpu

bf16 = jnp.bfloat16
f32 = jnp.float32
u32 = jnp.uint32

S = 2048
M = 448
DC = 1024
H = 16
D = 256
KS = 4
P = 128
NB = S // P
CH = 32
NCH = M // CH
T = 256
NT = S // T
NEG = -1e30

SORD = tuple(int(c) for c in '6430125')
SK = tuple(int(c) for c in '0364125')
SV = tuple(int(c) for c in '0125364')
SQ = tuple(int(c) for c in '6043125')
SP = tuple(int(c) for c in '3640125')
SO = tuple(int(c) for c in '5210346')
QW1 = 70
QW2 = 140
QW3 = 202
QW4 = 210
QC1 = 165
QLAG = 12
CVMAX = 12
SIDE0 = 30
SIDEP = 4
SLAG = 5
PRE = 0
W7P = 16
W7D = 6
KVH = 35
EXB = 10
NOP6 = 2
LA = 3
C2N = 32
NOP = 2


def _nn(a, b):
    return jnp.dot(a, b, preferred_element_type=f32)


def _b(u):
    return pltpu.bitcast(u, bf16)


def _u(x):
    return pltpu.bitcast(x, u32)


def _lo(u):
    return pltpu.bitcast(u << 16, f32)


def _hi(u):
    return pltpu.bitcast(u & jnp.uint32(0xFFFF0000), f32)


def _f(u):
    return _b(u).astype(f32)


def _a7(a11, a12, a21, a22):
    return [a11 + a22, a21 + a22, a11, a22, a11 + a12, a21 - a11, a12 - a22]


def _b7(b11, b12, b21, b22):
    return [b11 + b22, b11, b12 - b22, b21 - b11, b22, b11 + b12, b21 + b22]


def _c4(m):
    return m[0] + m[3] - m[4] + m[6], m[2] + m[4], m[1] + m[3], m[0] - m[1] + m[2] + m[5]


_C_OF = (((0, 1), (3, 1)), ((2, 1), (3, -1)), ((1, 1), (3, 1)), ((0, 1), (2, 1)), ((0, -1), (1, 1)), ((3, 1),), ((0, 1),))
_C_CNT = (4, 2, 2, 4)
_A_OF = {0: (0, 3, 1), 1: (2, 3, 1), 4: (0, 1, 1), 5: (2, 0, -1), 6: (1, 3, -1)}


def _combos(f7, blk):
    x = f7(*[_f(v) for v in blk])
    plain = {2: 0, 3: 3} if f7 is _a7 else {1: 0, 4: 3}
    return [_b(blk[plain[n]]) if n in plain else x[n].astype(bf16) for n in range(7)]


def _quad(c11, c12, c21, c22):
    return jnp.concatenate([jnp.concatenate([c11, c12], axis=1), jnp.concatenate([c21, c22], axis=1)], axis=0)


def _fold(c, op):
    return op(c.reshape(-1, 8, c.shape[1]), axis=0)


def _rsum(p):
    cols = []
    for c in range(0, p.shape[1], 128):
        acc = None
        for r in range(112, -16, -16):
            t = p[r:r + 8, c:c + 128] + p[r + 8:r + 16, c:c + 128]
            acc = t if acc is None else acc + t
        cols.append(acc)
    return jnp.concatenate(cols, axis=1) if len(cols) > 1 else cols[0]


def _tok(vals):
    parts = []
    for v in vals:
        for r in range(0, v.shape[0], 8):
            for c in range(0, v.shape[1], 128):
                parts.append(v[r:r + 8, c:c + 128])
    while len(parts) > 1:
        parts = [parts[i] | parts[i + 1] if i + 1 < len(parts) else parts[i] for i in range(0, len(parts), 2)]
    return (parts[0] >> 31) >> 1


def _gate(x, tok):
    if tok is None:
        return x
    top = x[:8, :128] | tok
    if x.shape[1] > 128:
        top = jnp.concatenate([top, x[:8, 128:]], axis=1)
    return jnp.concatenate([top, x[8:]], axis=0)


def _side_pieces():
    ps = [(k, g) for g in range(PRE) for k in ('HD', 'SC')]
    cur, cost = [], 0
    for a in range(NB):
        if a % 4 == 0 and a // 4 + PRE < 4:
            ps += [('HD', a // 4 + PRE), ('SC', a // 4 + PRE)]
        for half in range(2):
            if cur and cost + a + 1 > CVMAX:
                ps.append(('CV', tuple(cur)))
                cur, cost = [], 0
            cur.append((a, half))
            cost += a + 1
        if a % 4 == 3:
            ps += [('CV', tuple(cur)), ('ID', a // 4)]
            cur, cost = [], 0
    ps.insert(W7P, ('W7', 0, 7))
    ps.insert(W7P + W7D, ('W7', 7, 14))
    return ps


def _schedule():
    side = _side_pieces()
    out = []
    cnt = [0]

    def block(subs, att, with_side):
        for k, u in enumerate(subs):
            out.append(u)
            out.extend(att.get(k, []))
            if with_side:
                cnt[0] += 1
                if side and cnt[0] >= SIDE0 and (cnt[0] - SIDE0) % SIDEP == 0:
                    out.append(side.pop(0))

    def kv(p, half):
        return [('KV', p, t) for t in (range(KVH) if half == 0 else range(KVH, 49))]

    def op_(*idx):
        return [('OP', i, t) for i in idx for t in range(7)]

    def softmax_head(i, n):
        att = {max(n - EXB, 0): [('PACE',), ('EX', i, 0)]}
        for k in range(1, min(LA, i + 1)):
            att.setdefault(n - 1 - (LA - 1 - k) * 2, []).extend([('PACE',), ('EX', i, k)])
        return att

    ops_left = list(range(NT - 1))
    block(kv(0, 0) + kv(0, 1), {}, True)
    block(op_(NT - 1), {6: [('AT',), ('QK', 0, 0)]}, False)
    block(kv(1, 0), softmax_head(0, KVH), True)
    for i in range(NT - 1):
        for j in range(i + 1):
            out.append(('QK', i + 1, j))
            if j + LA <= i:
                out.append(('EX', i, j + LA))
            out.append(('PV', i, j))
        out.append(('QK', i + 1, i + 1))
        if i < 5:
            subs = kv((i + 3) // 2, (i + 1) % 2)
            block(subs, softmax_head(i + 1, len(subs)), True)
        else:
            n = NOP6 if i == 5 else NOP
            block(op_(*ops_left[:n]), softmax_head(i + 1, 7 * n), False)
            del ops_left[:n]
    out.append(('PACE',))
    for j in range(NT):
        if j + LA < NT:
            out.append(('EX', NT - 1, j + LA))
        out.append(('PV', NT - 1, j))
        if len(ops_left) > 2:
            block(op_(ops_left.pop(0)), {}, False)
        out.append(('PACE',))
    block(op_(*ops_left), {}, False)
    assert not side
    w7 = [k for k, o in enumerate(out) if o[0] == 'W7']
    assert out.index(('OP', NT - 1, 6)) < min(w7) and max(w7) < out.index(('OP', 0, 0))
    out.remove(('ID', 3))
    out.append(('ID', 3))
    return out


def _kernel(qT_hbm, kT_hbm, vT_hbm, sk_hbm, ssmk_hbm, dd_hbm, xT_hbm, ckv_hbm,
            wq_hbm, wk_hbm, wv_hbm, woT_hbm, out_hbm,
            qT, kT, vT, ssmk, xT, ckv, wq_raw, wk_raw, wv_raw, woT,
            aq_s, bx_s, w1_s, w2_s, cT_s, QT_s, c2_s, acc, aT_s, out_s, taps, ff_s, fi_s,
            sk_ref, dd_ref, S0_s, S1_s, X_s, W7_s, pace_s, m0_s, m1_s, l0_s, l1_s,
            sem, sem_k, sem_v, sem_o, *rest):
    K_s, V_s, O_s, Y_s = rest[:NT], rest[NT:2 * NT], rest[2 * NT:3 * NT], rest[3 * NT:]

    def cp(src, dst, s):
        return pltpu.make_async_copy(src, dst, s)

    def c_x(j):
        cols = pl.ds(pl.multiple_of(j * 2 * T, 2 * T), 2 * T)
        return cp(xT_hbm.at[:, cols], xT.at[pl.ds(pl.multiple_of(j * M, 16), M)], sem.at[j])

    QP = ((0, 128), (128, 96))

    def c_wq(p):
        cs_ = []
        for half in range(2):
            r = pl.ds((half * 224 + QP[p][0]) * H, QP[p][1] * H)
            for g in range(2):
                cs_.append(cp(wq_hbm.at[r, pl.ds(128 * g, 128)], wq_raw.at[g, r], sem.at[18 + 4 * p + 2 * half + g]))
        return cs_

    def c_w(w_hbm, raw, sm, j, half, g):
        r = pl.ds(pl.multiple_of((half * 4 + j) * 2048, 2048), 2048)
        q = 2 * half + g
        return cp(w_hbm.at[r, pl.ds(128 * g, 128)], raw.at[j % 2, q, pl.ds(0, 2048)], sm.at[(j % 2) * 4 + q])

    def c_wk(j):
        return [c_w(wk_hbm, wk_raw, sem_k, j, half, g) for half in range(2) for g in range(2)]

    def c_wv(j):
        return [c_w(wv_hbm, wv_raw, sem_v, j, half, g) for half in range(2) for g in range(2)]

    def c_ckv(j):
        r = pl.ds(pl.multiple_of(j * 2 * T, 2 * T), 2 * T)
        return cp(ckv_hbm.at[r], ckv.at[r], sem.at[9 + j])

    a_pairs = ((kT_hbm, kT), (vT_hbm, vT), (ssmk_hbm, ssmk), (qT_hbm, qT))
    c_early = [cp(woT_hbm.at[pl.ds(0, 1)], woT.at[pl.ds(0, 1)], sem.at[4])]
    c_early += [cp(src.at[pl.ds(0, CH)], dst.at[pl.ds(0, CH)], sem.at[5 + n]) for n, (src, dst) in enumerate(a_pairs)]
    c_late = [cp(woT_hbm.at[pl.ds(1, H - 1)], woT.at[pl.ds(1, H - 1)], sem.at[13])]
    c_late += [cp(src.at[pl.ds(CH, M - CH)], dst.at[pl.ds(CH, M - CH)], sem.at[14 + n])
               for n, (src, dst) in enumerate(a_pairs)]
    c_small = [cp(sk_hbm, sk_ref, sem.at[26]), cp(dd_hbm, dd_ref, sem.at[27])]
    for c in c_small + c_wq(0) + c_wq(1) + [c_x(0)]:
        c.start()
    for c in c_wk(0) + [c_x(1)]:
        c.start(priority=1)

    n_i = jax.lax.broadcasted_iota(jnp.int32, (P, P), 0)
    k_i = jax.lax.broadcasted_iota(jnp.int32, (P, P), 1)
    ang = (((2 * k_i + 1) * n_i) & 511).astype(f32) * (math.pi / 256.0)
    cs, sn = jnp.cos(ang), jnp.sin(ang)
    ff_s[:, 0:P] = cs.astype(bf16)
    ff_s[:, P:2 * P] = (-sn).astype(bf16)
    fi_s[0:P, :] = (cs.T * (1.0 / P)).astype(bf16)
    fi_s[P:2 * P, :] = (sn.T * (-1.0 / P)).astype(bf16)
    acc[...] = jnp.zeros(acc.shape, f32)
    for c in c_small:
        c.wait()
    sk = sk_ref[...].astype(f32)
    for t in range(KS):
        taps[t] = jnp.broadcast_to(sk[t:t + 1, :], (128, M)).T
    taps[KS] = jnp.broadcast_to(dd_ref[...].astype(f32).reshape(1, M), (128, M)).T
    aT_s[...] = jnp.zeros(aT_s.shape, bf16)
    O_s[NT - 1][...] = jnp.zeros(O_s[0].shape, bf16)
    W7_s[...] = jnp.zeros(W7_s.shape, u32)
    cT_s[...] = jnp.zeros(cT_s.shape, u32)

    def prep_x(jj, t, r0):
        xj = xT.at[pl.ds(pl.multiple_of(jj * M, 16), M)]
        bj = bx_s.at[pl.ds(pl.multiple_of(jj * 224, 16), 224)]
        blk = [_u(xj[r:r + 32, c:c + 128]) for r in (r0, 224 + r0) for c in (t * T, t * T + 128)]
        row = t * 112 + r0 // 2
        for n, x in enumerate(_combos(_b7, blk)):
            bj[row:row + 16, n * 128:(n + 1) * 128] = _u(x)
        return []

    vq = wq_raw.bitcast(u32)
    for p, (c0, nc) in enumerate(QP):
        for c in c_wq(p):
            c.wait()
        for hp in range(H // 2):
            ut = [vq[g, pl.ds((half * 224 + c0) * 8 + hp, nc, stride=8), :].T for g in range(2) for half in range(2)]
            for r in range(0, 128, 16):
                u = [x[r:r + 16] for x in ut]
                for par, f in enumerate((_lo, _hi)):
                    r0 = (2 * hp + par) * 64 + r // 2
                    for n, x in enumerate(_a7(*[f(x) for x in u])):
                        aq_s[r0:r0 + 8, n * 256 + c0:n * 256 + c0 + nc] = _u(x.astype(bf16))
    for c in c_wv(0) + [c_ckv(0)]:
        c.start(priority=1)
    c_x(0).wait()
    for t in range(2):
        for r0 in range(0, 224, 32):
            prep_x(0, t, r0)

    qscale = (D ** -0.5) * math.log2(math.e)

    def prep_c2(jj, r):
        blk = [[cT_s[cq * 128 + r:cq * 128 + r + 8, tb * 128:(tb + 1) * 128] for tb in range(4)] for cq in range(4)]
        x = [[_f(v) for v in row] for row in blk]
        outer = [[_b7(x[ci][ti], x[ci][2 + ti], x[2 + ci][ti], x[2 + ci][2 + ti]) for ti in range(2)]
                 for ci in range(2)]
        two = [_b7(outer[0][0][n], outer[0][1][n], outer[1][0][n], outer[1][1][n]) for n in range(7)]
        cj = c2_s.at[pl.ds(pl.multiple_of(jj * 128, 128), 128)]
        for n in range(7):
            for m in range(7):
                cj[r:r + 8, (n * 7 + m) * 128:(n * 7 + m + 1) * 128] = _u(two[n][m].astype(bf16))
        return []

    def q_body(j, carry):
        mq = {}
        qtj = QT_s.at[pl.ds(pl.multiple_of(j * 4096, 4096), 4096)]
        zq = j >> 4
        bx = [[bx_s[pl.ds(pl.multiple_of((2 * j + t) * 112, 16), 112), n * 128:(n + 1) * 128] for n in range(7)]
              for t in range(2)]

        def qproj(u, tok):
            hh, t, n = u // 14, (u // 7) % 2, SORD[u % 7]
            w = _b(_gate(aq_s[hh * 64:hh * 64 + 64, n * 256:n * 256 + 224], tok))
            mq[n] = _nn(w, _b(bx[t][n]))
            if u % 7 == 6:
                for k, x in enumerate(_c4(mq)):
                    r0 = t * 2048 + hh * 128 + (k // 2) * 64
                    qtj[r0:r0 + 64, (k % 2) * 128:(k % 2 + 1) * 128] = _u((x * qscale).astype(bf16))
            return mq[n]

        wt = {}
        ckj = ckv.at[pl.ds(pl.multiple_of(j * 512, 512), 512)]
        w1j = w1_s.at[pl.ds(pl.multiple_of(j * 2048, 2048), 2048)]

        def prep_w(kv, hp, part):
            if part == 0:
                v = (wk_raw, wv_raw)[kv].bitcast(u32).at[j % 2]
                wt[kv, hp] = [v[q, pl.ds(hp, 128, stride=8), :].T for q in (0, 2, 1, 3)]
                return [x[120:] for x in wt[kv, hp]]
            for r in range(32 * (part - 1), 32 * part, 16):
                u = [x[r:r + 16] for x in wt[kv, hp]]
                for par, f in enumerate((_lo, _hi)):
                    r0 = (2 * hp + par) * 128 + kv * 64 + r // 2
                    for n, c in enumerate(_a7(*[f(x) for x in u])):
                        w1j[r0:r0 + 8, n * 128:(n + 1) * 128] = _u(c.astype(bf16))
            return []

        def prep_ct(half, cq):
            res = []
            ct = 2 * cq + half
            for tb in range(4):
                x = _u(ckj[tb * 128:(tb + 1) * 128, ct * 128:(ct + 1) * 128].T)
                cT_s[pl.ds(pl.multiple_of(zq * 64 + ct * 64, 64), 64), tb * 128:(tb + 1) * 128] = x
                res.append(x[56:])
            return res

        fill = {}

        def spread(pieces, u0, u1):
            for n, p in enumerate(pieces):
                fill.setdefault(u0 + n * (u1 - u0) // len(pieces), []).append(p)

        spread([functools.partial(prep_w, 0, hp, part) for hp in range(8) for part in range(5)], QW1, QW2)
        spread([functools.partial(prep_w, 1, hp, part) for hp in range(8) for part in range(5)], QW2, QW3)
        spread([functools.partial(prep_ct, 0, cq) for cq in range(4)], QW2 + 2, QC1)
        spread([functools.partial(prep_ct, 1, cq) for cq in range(4)], QC1, QW3)
        spread([functools.partial(prep_c2, jnp.maximum(j - 1, 0), r) for r in range(C2N, 128, 8)], 2, QW1 - 4)
        if C2N:
            spread([functools.partial(prep_c2, j, r) for r in range(0, C2N, 8)], QW3, QW4)
        spread([functools.partial(prep_x, jnp.minimum(j + 1, 3), t, r0)
                for t in range(2) for r0 in range(0, 224, 32)], QW4, 221)
        toks = {}
        for u in range(224):
            if u == QW1:
                @pl.when(j < 3)
                def _():
                    for c in c_wk(j + 1):
                        c.start(priority=1)

                @pl.when(j == 3)
                def _():
                    for c in c_early + c_late:
                        c.start(priority=1)

                for c in c_wk(j):
                    c.wait()
            if u == QW2:
                @pl.when(j < 3)
                def _():
                    for c in c_wv(j + 1) + [c_ckv(j + 1)]:
                        c.start(priority=1)

                @pl.when(j < 2)
                def _():
                    c_x(j + 2).start(priority=1)

                @pl.when(j < 3)
                def _():
                    c_x(j + 1).wait()

                for c in c_wv(j) + [c_ckv(j)]:
                    c.wait()
            q = qproj(u, toks.pop(u, None))
            res = []
            ps = fill.get(u, [])
            for n, p in enumerate(ps):
                row = (n * 128 // len(ps)) // 16 * 16
                if p.func is prep_w and p.args[2] == 0:
                    (wk_raw, wv_raw)[p.args[0]].bitcast(u32)[zq, 0, 1024:1032, :] = _u(q[row:row + 8])
                elif p.func is prep_c2:
                    cT_s[pl.ds(pl.multiple_of(512 + zq * 8, 8), 8), 0:128] = _u(q[row:row + 8])
                elif p.func is prep_x:
                    xT[pl.ds(pl.multiple_of(4 * M + zq * 16, 16), 16), 0:128] = q[row:row + 16].astype(bf16)
                elif p.func is prep_ct:
                    ckv[pl.ds(pl.multiple_of(S + zq * 16, 16), 16), 0:128] = q[row:row + 16].astype(bf16)
                res += p()
            if res:
                toks[u + QLAG] = _tok(res)
        return carry

    jax.lax.fori_loop(0, 4, q_body, 0)
    for r in range(C2N, 128, 8):
        prep_c2(3, r)
    for c in c_early:
        c.wait()

    tri = n_i <= k_i
    sgn = jnp.where((jax.lax.broadcasted_iota(jnp.int32, (1, P), 1) & 1) == 0, 1.0, -1.0).astype(f32)
    c_outa = cp(out_s.at[:, pl.ds(0, 384)], out_hbm.at[:, pl.ds(0, 384)], sem_o.at[8])
    HR, HI, PR, PI, KV = range(5)

    def blk_at(c, half=None):
        r0 = (c % 8) * CH
        rs = slice(r0, r0 + CH) if half is None else slice(r0 + 16 * half, r0 + 16 * half + 16)
        return rs, slice((c // 8) * P, (c // 8 + 1) * P)

    def tile(ref, n):
        return ref[:, n * 128:(n + 1) * 128]

    def head_body(h, carry):
        @pl.when(h == 1)
        def _():
            for c in c_late:
                c.wait()

        @pl.when(h == H - 1)
        def _():
            c_outa.start()

        st = dict(co={}, cnt={}, fin=set(), M={}, P={}, Q7={}, mfin={}, o={})
        zs = h >> 10
        z64 = pl.ds(pl.multiple_of(zs * 64, 64), 64)
        m_s, l_s = (m0_s, m1_s), (l0_s, l1_s)
        w1h = w1_s.at[pl.ds(pl.multiple_of(h * 128, 128), 3 * 2048 + 128)]
        qth = QT_s.at[pl.ds(pl.multiple_of(h * 128, 128), 7 * 2048 + 128)]
        rows = pl.ds(pl.multiple_of(jnp.minimum(h, NCH - 1) * CH, CH), CH)

        def rep(t, n):
            return jnp.concatenate([taps[t, rows, :]] * n, axis=1)

        toks = []

        def due():
            for t in toks:
                t[0] -= 1
            ready = [t[1] for t in toks if t[0] <= 0]
            toks[:] = [t for t in toks if t[0] > 0]
            return functools.reduce(lambda x, y: x | y, ready) if ready else None

        def gate_later(vals):
            toks.append([SLAG, _tok([v if v.dtype == u32 else _u(v) for v in vals])])

        def row_offset(i):
            if i not in st['mfin']:
                m = m_s[i % 2][0, 0]
                for t in range(1, i + 1):
                    m = jnp.maximum(m, m_s[i % 2][0, t])
                m = jnp.max(m, axis=0, keepdims=True)
                if i > 0:
                    lo_ = jnp.exp2(m_s[i % 2][0, 0] - m)
                    for t in range(1, i + 1):
                        lo_ = lo_ + jnp.exp2(m_s[i % 2][0, t] - m)
                    m = m + jnp.log2(jnp.sum(lo_, axis=0, keepdims=True))
                st['mfin'][i] = m
            return st['mfin'][i]

        for op in _schedule():
            kind = op[0]
            if kind == 'KV':
                _, p, t = op
                n, m = SK[t // 7], SV[t % 7]

                def wblk(q):
                    w = jnp.concatenate([w1h[k * 2048:k * 2048 + 128, n * 128:(n + 1) * 128]
                                         for k in (2 * (q % 2), 2 * (q % 2) + 1)], axis=1)
                    r = (q // 2) * 32
                    return jnp.concatenate([w[r:r + 32], w[64 + r:64 + r + 32]], axis=0)

                cols = slice((n * 7 + m) * 256, (n * 7 + m + 1) * 256)
                if m in (2, 3):
                    w = wblk(0 if m == 2 else 3)
                elif p > 0:
                    w = w2_s[:, cols]
                else:
                    i1, i2, sg = _A_OF[m]
                    x, y = wblk(i1), wblk(i2)
                    w = (_f(x) + _f(y) if sg > 0 else _f(x) - _f(y)).astype(bf16)
                    w2_s[z64, cols] = _u(w)
                c2 = c2_s[p * 128:(p + 1) * 128, (n * 7 + m) * 128:(n * 7 + m + 1) * 128]
                st['M'][m] = st['last'] = _nn(w if w.dtype == bf16 else _b(_gate(w, due())), _b(c2))
                if t % 7 < 6:
                    continue
                mo = _quad(*_c4(st['M']))
                for o, sg in _C_OF[n]:
                    k = st['cnt'][o] = st['cnt'].get(o, 0) + 1
                    if k == 1:
                        st['co'][o] = mo if sg > 0 else -mo
                    else:
                        st['co'][o] = st['co'][o] + mo if sg > 0 else st['co'][o] - mo
                    if k == _C_CNT[o]:
                        st['cnt'][o] = 0
                        st['fin'].add(o)
                for tok in range(2):
                    if not {tok, 2 + tok} <= st['fin']:
                        continue
                    st['fin'] -= {tok, 2 + tok}
                    c = 2 * p + tok

                    def full(dh, kb, off):
                        x = st['co'][2 * dh + tok][:, kb * 128:(kb + 1) * 128]
                        return jnp.concatenate([x[off:off + 64], x[128 + off:128 + off + 64]], axis=0)

                    kb4 = (full(0, 0, 0).T, full(1, 0, 0).T, full(0, 1, 0).T, full(1, 1, 0).T)
                    vb4 = (full(0, 0, 64), full(0, 1, 64), full(1, 0, 64), full(1, 1, 64))
                    for ref, c4 in ((K_s[c], kb4), (V_s[c], vb4)):
                        blks = dict(zip((2, 7, 8, 3), c4))
                        if c < NT - 1:
                            blks.update({k: x for k, x in enumerate(_a7(*c4)) if k not in (2, 3)})
                        for k, x in blks.items():
                            ref[z64, k * 128:(k + 1) * 128] = _u(x.astype(bf16))
            elif kind == 'QK':
                _, i, j = op
                S_s = (S0_s, S1_s)[i % 2]
                if j < i:
                    if i not in st['Q7']:
                        qu = qth[i * 2048:i * 2048 + 128, :]
                        st['Q7'][i] = _combos(_b7, [qu[:64, :128], qu[:64, 128:], qu[64:, :128], qu[64:, 128:]])
                    s = _quad(*_c4({n: _nn(_b(tile(K_s[j], n)), st['Q7'][i][n]) for n in SQ}))
                    S_s[zs, j] = s
                    f = _fold(s, jnp.max)
                else:
                    q = _b(qth[i * 2048:i * 2048 + 128, :])
                    sa = _nn(_b(jnp.concatenate([tile(K_s[j], 2), tile(K_s[j], 7)], axis=1)), q)
                    sa = jnp.concatenate([jnp.where(tri, sa[:, :128], NEG), sa[:, 128:]], axis=1)
                    sb = _nn(_b(jnp.concatenate([tile(K_s[j], 8), tile(K_s[j], 3)], axis=1)), q[:, 128:])
                    sb = jnp.where(tri, sb, NEG)
                    S_s[zs, j, 0:128, :] = sa
                    S_s[zs, j, 128:T, 128:T] = sb
                    fa = _fold(sa, jnp.max)
                    f = jnp.concatenate([fa[:, :128], jnp.maximum(fa[:, 128:], _fold(sb, jnp.max))], axis=1)
                m_s[i % 2][zs, j] = f
                pace_s[zs] = f
            elif kind == 'EX':
                _, i, j = op
                S_s = (S0_s, S1_s)[i % 2]
                m = row_offset(i)
                m = jnp.where(pace_s[0, 0:1, :] == jnp.inf, jnp.inf, m)
                if j < i:
                    parts, lj = [], None
                    for r in range(112, -16, -16):
                        pt = jnp.exp2(S_s[0, j, r:r + 16, :] - m)
                        pb = jnp.exp2(S_s[0, j, 128 + r:128 + r + 16, :] - m)
                        parts.insert(0, _b7(pt[:, :128], pt[:, 128:], pb[:, :128], pb[:, 128:]))
                        x = (pt[:8] + pt[8:]) + (pb[:8] + pb[8:])
                        lj = x if lj is None else lj + x
                    st['P'][i, j] = [jnp.concatenate([x[n] for x in parts], axis=0).astype(bf16) for n in range(7)]
                else:
                    pa = jnp.exp2(S_s[0, j, 0:128, :] - m)
                    pb = jnp.exp2(S_s[0, j, 128:T, 128:T] - m[:, 128:])
                    la = _rsum(pa)
                    lj = jnp.concatenate([la[:, :128], la[:, 128:] + _rsum(pb)], axis=1)
                    st['P'][i, j] = (pa.astype(bf16), pb.astype(bf16))
                l_s[i % 2][zs, j] = lj
            elif kind == 'PV':
                _, i, j = op
                p = st['P'].pop((i, j))
                if j < i:
                    for n in SP:
                        st['last'] = _nn(_b(tile(V_s[j], n)), p[n])
                        st['o'][i, n] = st['o'][i, n] + st['last'] if j > 0 else st['last']
                    continue
                oa = _nn(_b(jnp.concatenate([tile(V_s[j], 2), tile(V_s[j], 8)], axis=0)), p[0])
                ob = _nn(_b(jnp.concatenate([tile(V_s[j], 7), tile(V_s[j], 3)], axis=0)), p[1])
                o = st['last'] = jnp.concatenate([oa[:, :128], oa[:, 128:] + ob], axis=1)
                if i > 0:
                    o = o + _quad(*_c4({n: st['o'].pop((i, n)) for n in range(7)}))
                l = l_s[i % 2][0, 0]
                for t in range(1, i + 1):
                    l = l + l_s[i % 2][0, t]
                o = o * (1.0 / jnp.sum(l, axis=0, keepdims=True))
                for n, x in enumerate(_b7(o[:128, :128], o[:128, 128:], o[128:, :128], o[128:, 128:])):
                    O_s[i][zs, n] = x.astype(bf16)
            elif kind == 'PACE':
                pace_s[zs] = jnp.concatenate([st['last'][-8:, -128:]] * 2, axis=1)
            elif kind == 'OP':
                _, i, t = op
                n = SO[t]
                st['M'][n] = st['last'] = _nn(_b(_gate(tile(W7_s, n), due())), O_s[i][0, n])
                if t == 6:
                    acc[:, T * i:T * (i + 1)] += _quad(*_c4(st['M']))
            elif kind == 'W7':
                res = []
                for r0 in range(16 * op[1], 16 * op[2], 16):
                    blk = [_u(woT[h, r:r + 16, c:c + 128]) for r in (r0, 224 + r0) for c in (0, 128)]
                    row = pl.ds(pl.multiple_of(zs * 8 + r0 // 2, 8), 8)
                    for n, x in enumerate(_combos(_a7, blk)):
                        W7_s[row, n * 128:(n + 1) * 128] = _u(x)
                    res += blk
                gate_later(res)
            elif kind == 'AT':
                g = jnp.clip((h - 4) // 4, 0, 2)
                t0 = jnp.minimum(((h + 12) % 4) * 6, NB - 6)
                grow = pl.ds(pl.multiple_of(g * 128, 128), 128)
                gcol = pl.ds(pl.multiple_of(jnp.where(h == H - 1, 3, g) * 128, 128), 128)
                res = []
                for n in range(6):
                    tok = pl.ds(pl.multiple_of((t0 + n) * 128, 128), 128)
                    x = aT_s[grow, tok].T
                    out_s[tok, gcol] = x
                    res.append(_u(x)[56:])
                gate_later(res)
            elif kind == 'HD':
                g = op[1]
                hs = jnp.concatenate([ssmk[rows, c * P:(c + 1) * P] for c in range(4 * g, 4 * g + 4)], axis=0)
                hf = _nn(hs, ff_s[...])
                for n in range(4):
                    X_s[(zs, HR) + blk_at(4 * g + n)] = hf[n * CH:(n + 1) * CH, :P]
                    X_s[(zs, HI) + blk_at(4 * g + n)] = hf[n * CH:(n + 1) * CH, P:]
            elif kind == 'SC':
                g = op[1]
                if g == 0:
                    k = jnp.concatenate([jnp.zeros((CH, P), f32), kT[rows, 0:4 * P].astype(f32)], axis=1)
                else:
                    k = kT[rows, (4 * g - 1) * P:(4 * g + 4) * P].astype(f32)
                ks = k[:, P:] * rep(0, 4)
                for j in range(1, KS):
                    ks = ks + pltpu.roll(k, j, 1)[:, P:] * rep(j, 4)
                kv = ks * vT[rows, 4 * g * P:(4 * g + 4) * P].astype(f32)
                kvs = jnp.concatenate([kv[:, n * P:(n + 1) * P] for n in range(4)], axis=0)
                xf = _nn(kvs.astype(bf16), ff_s[...])
                for n in range(4):
                    c = 4 * g + n
                    xr, xi = xf[n * CH:(n + 1) * CH, :P], xf[n * CH:(n + 1) * CH, P:]
                    X_s[(zs, KV) + blk_at(c)] = kvs[n * CH:(n + 1) * CH]
                    pr = xr if c == 0 else xr - sgn * st['x'][1]
                    pi = xi if c == 0 else xi + sgn * st['x'][0]
                    X_s[(zs, PR) + blk_at(c)] = pr
                    X_s[(zs, PI) + blk_at(c)] = pi
                    st['x'] = (xr, xi)
            elif kind == 'CV':
                res = []
                for a, half in op[1]:
                    wr = wi = None
                    for j in range(a + 1):
                        hr, hi_ = X_s[(0, HR) + blk_at(j, half)], X_s[(0, HI) + blk_at(j, half)]
                        pr, pi = X_s[(0, PR) + blk_at(a - j, half)], X_s[(0, PI) + blk_at(a - j, half)]
                        tr, ti = hr * pr - hi_ * pi, hr * pi + hi_ * pr
                        wr, wi = (tr, ti) if wr is None else (wr + tr, wi + ti)
                    r0 = (a % 4) * CH + 16 * half
                    Y_s[a // 4][zs, r0:r0 + 16, :P] = wr
                    Y_s[a // 4][zs, r0:r0 + 16, P:] = wi
                    res += [wr, wi]
                gate_later(res)
            elif kind == 'ID':
                g = op[1]
                y = _nn(Y_s[g][0].astype(bf16), fi_s[...])
                for n in range(4):
                    c = 4 * g + n
                    cols = slice(c * P, (c + 1) * P)
                    ya = y[n * CH:(n + 1) * CH, :] + X_s[(0, KV) + blk_at(c)] * taps[KS, rows, :]
                    aT_s[rows, cols] = (qT[rows, cols].astype(f32) * ya).astype(bf16)
        return carry

    jax.lax.fori_loop(0, H, head_body, 0)

    acc[:, T * (NT - 1):] += _quad(*_c4({n: _nn(_b(tile(W7_s, n)), O_s[NT - 1][0, n]) for n in SORD}))
    outs = [c_outa]
    for i in range(NT):
        cols = slice(T * i, T * (i + 1))
        blk = jnp.concatenate([aT_s[384:M, cols], acc[:, cols].astype(bf16)], axis=0)
        out_s[cols, 384:2 * M] = blk.T
        c = cp(out_s.at[pl.ds(T * i, T), pl.ds(384, 512)], out_hbm.at[pl.ds(T * i, T), pl.ds(384, 512)], sem_o.at[i])
        c.start()
        outs.append(c)
    for c in outs:
        c.wait()


@jax.jit
def pallas_concat_heads__ssm_conv_h3__compressed_kv_cla__prompt_kernel(
    A_q: jax.Array,
    A_k: jax.Array,
    A_v: jax.Array,
    A_shift_k: jax.Array,
    A_ssm_k: jax.Array,
    A_ssm_D: jax.Array,
    B_x: jax.Array,
    B_c_kv: jax.Array,
    B_w_q: jax.Array,
    B_w_uk: jax.Array,
    B_w_uv: jax.Array,
    B_w_o: jax.Array,
):
    hbm = pl.BlockSpec(memory_space=pl.ANY)
    V = pltpu.VMEM
    out = pl.pallas_call(
        _kernel,
        out_shape=jax.ShapeDtypeStruct((S, 2 * M), bf16),
        in_specs=[hbm] * 12,
        out_specs=hbm,
        scratch_shapes=[
            V((M, S), bf16), V((M, S), bf16), V((M, S), bf16), V((M, S), bf16),
            V((4 * M + 16, 2 * T), bf16), V((S + 16, DC), bf16),
            V((2, M * H, 128), bf16),
            V((2, 4, 128 * H + 16, 128), bf16), V((2, 4, 128 * H + 16, 128), bf16),
            V((H, M, D), bf16),
            V((H * 64, 7 * 256), u32), V((NT * 112, 7 * 128), u32),
            V((4 * H * 128, 7 * 128), u32), V((64, 49 * 256), u32),
            V((512 + 8, 512), u32),
            V((NT * H * 128, T), u32), V((4 * 128, 49 * 128), u32),
            V((M, S), f32), V((M, S), bf16), V((S, 2 * M), bf16),
            V((KS + 1, M, 128), f32), V((P, 2 * P), bf16), V((2 * P, P), bf16),
            V((KS, M), bf16), V((M,), bf16),
            V((1, NT, T, T), f32), V((1, NT, T, T), f32), V((1, 5, T, T), f32),
            V((112, 7 * 128), u32), V((1, 8, T), f32),
            V((1, NT, 8, T), f32), V((1, NT, 8, T), f32), V((1, NT, 8, T), f32), V((1, NT, 8, T), f32),
            pltpu.SemaphoreType.DMA((28,)), pltpu.SemaphoreType.DMA((8,)),
            pltpu.SemaphoreType.DMA((8,)), pltpu.SemaphoreType.DMA((9,)),
        ] + [V((64, 9 * 128), u32)] * (2 * NT) + [V((1, 7, 128, 128), bf16)] * NT
        + [V((1, 4 * CH, 2 * P), f32)] * 4,
        compiler_params=pltpu.CompilerParams(vmem_limit_bytes=126 * 1024 * 1024,
                                             shape_invariant_numerics=False,
                                             disable_bounds_checks=True, disable_semaphore_checks=True),
    )(
        A_q[0].T, A_k[0].T, A_v[0].T, A_shift_k.T, A_ssm_k, A_ssm_D,
        B_x[0].T, B_c_kv[0],
        B_w_q.reshape(M * H, D), B_w_uk.reshape(DC * H, D), B_w_uv.reshape(DC * H, D),
        jnp.transpose(B_w_o, (0, 2, 1)),
    )
    return out[None]
```

```python
import functools
import math

import jax
import jax.numpy as jnp
import jax.experimental.pallas as pl
import jax.experimental.pallas.tpu as pltpu

bf16 = jnp.bfloat16
f32 = jnp.float32
u32 = jnp.uint32

S = 2048
M = 448
DC = 1024
H = 16
D = 256
KS = 4
P = 128
NB = S // P
CH = 32
NCH = M // CH
T = 256
NT = S // T
NEG = -1e30

SORD = tuple(int(c) for c in '6430125')
SK = tuple(int(c) for c in '0364125')
SV = tuple(int(c) for c in '0125364')
SQ = tuple(int(c) for c in '6043125')
SP = tuple(int(c) for c in '3640125')
SO = tuple(int(c) for c in '5210346')
QW1 = 56
QW2 = 140
QW3 = 208
QW4 = 222
QC1 = 165
QLAG = 12
CVMAX = 12
SIDE0 = 30
SIDEP = 4
SLAG = 5
PRE = 0
W7P = 16
W7D = 6
KVH = 35
EXB = 10
NOP6 = 2
LA = 3
C2N = 64
C2S = 16
NOP = 2


def _nn(a, b):
    return jnp.dot(a, b, preferred_element_type=f32)


def _b(u):
    return pltpu.bitcast(u, bf16)


def _u(x):
    return pltpu.bitcast(x, u32)


def _lo(u):
    return pltpu.bitcast(u << 16, f32)


def _hi(u):
    return pltpu.bitcast(u & jnp.uint32(0xFFFF0000), f32)


def _f(u):
    return _b(u).astype(f32)


def _a7(a11, a12, a21, a22):
    return [a11 + a22, a21 + a22, a11, a22, a11 + a12, a21 - a11, a12 - a22]


def _b7(b11, b12, b21, b22):
    return [b11 + b22, b11, b12 - b22, b21 - b11, b22, b11 + b12, b21 + b22]


def _c4(m):
    return m[0] + m[3] - m[4] + m[6], m[2] + m[4], m[1] + m[3], m[0] - m[1] + m[2] + m[5]


_C_OF = (((0, 1), (3, 1)), ((2, 1), (3, -1)), ((1, 1), (3, 1)), ((0, 1), (2, 1)), ((0, -1), (1, 1)), ((3, 1),), ((0, 1),))
_C_CNT = (4, 2, 2, 4)
_A_OF = {0: (0, 3, 1), 1: (2, 3, 1), 4: (0, 1, 1), 5: (2, 0, -1), 6: (1, 3, -1)}


def _combos(f7, blk):
    x = f7(*[_f(v) for v in blk])
    plain = {2: 0, 3: 3} if f7 is _a7 else {1: 0, 4: 3}
    return [_b(blk[plain[n]]) if n in plain else x[n].astype(bf16) for n in range(7)]


def _quad(c11, c12, c21, c22):
    return jnp.concatenate([jnp.concatenate([c11, c12], axis=1), jnp.concatenate([c21, c22], axis=1)], axis=0)


def _fold(c, op):
    return op(c.reshape(-1, 8, c.shape[1]), axis=0)


def _rsum(p):
    cols = []
    for c in range(0, p.shape[1], 128):
        acc = None
        for r in range(112, -16, -16):
            t = p[r:r + 8, c:c + 128] + p[r + 8:r + 16, c:c + 128]
            acc = t if acc is None else acc + t
        cols.append(acc)
    return jnp.concatenate(cols, axis=1) if len(cols) > 1 else cols[0]


def _tok(vals):
    parts = []
    for v in vals:
        for r in range(0, v.shape[0], 8):
            for c in range(0, v.shape[1], 128):
                parts.append(v[r:r + 8, c:c + 128])
    while len(parts) > 1:
        parts = [parts[i] | parts[i + 1] if i + 1 < len(parts) else parts[i] for i in range(0, len(parts), 2)]
    return (parts[0] >> 31) >> 1


def _gate(x, tok):
    if tok is None:
        return x
    top = x[:8, :128] | tok
    if x.shape[1] > 128:
        top = jnp.concatenate([top, x[:8, 128:]], axis=1)
    return jnp.concatenate([top, x[8:]], axis=0)


def _side_pieces():
    ps = [(k, g) for g in range(PRE) for k in ('HD', 'SC')]
    cur, cost = [], 0
    for a in range(NB):
        if a % 4 == 0 and a // 4 + PRE < 4:
            ps += [('HD', a // 4 + PRE), ('SC', a // 4 + PRE)]
        for half in range(2):
            if cur and cost + a + 1 > CVMAX:
                ps.append(('CV', tuple(cur)))
                cur, cost = [], 0
            cur.append((a, half))
            cost += a + 1
        if a % 4 == 3:
            ps += [('CV', tuple(cur)), ('ID', a // 4)]
            cur, cost = [], 0
    ps.insert(W7P, ('W7', 0, 7))
    ps.insert(W7P + W7D, ('W7', 7, 14))
    return ps


def _schedule():
    side = _side_pieces()
    out = []
    cnt = [0]

    def block(subs, att, with_side):
        for k, u in enumerate(subs):
            out.append(u)
            out.extend(att.get(k, []))
            if with_side:
                cnt[0] += 1
                if side and cnt[0] >= SIDE0 and (cnt[0] - SIDE0) % SIDEP == 0:
                    out.append(side.pop(0))

    def kv(p, half):
        return [('KV', p, t) for t in (range(KVH) if half == 0 else range(KVH, 49))]

    def op_(*idx):
        return [('OP', i, t) for i in idx for t in range(7)]

    def softmax_head(i, n):
        att = {max(n - EXB, 0): [('PACE',), ('EX', i, 0)]}
        for k in range(1, min(LA, i + 1)):
            att.setdefault(n - 1 - (LA - 1 - k) * 2, []).extend([('PACE',), ('EX', i, k)])
        return att

    ops_left = list(range(NT - 1))
    block(kv(0, 0) + kv(0, 1), {}, True)
    block(op_(NT - 1), {6: [('AT',), ('QK', 0, 0)]}, False)
    block(kv(1, 0), softmax_head(0, KVH), True)
    for i in range(NT - 1):
        for j in range(i + 1):
            out.append(('QK', i + 1, j))
            if j + LA <= i:
                out.append(('EX', i, j + LA))
            out.append(('PV', i, j))
        out.append(('QK', i + 1, i + 1))
        if i < 5:
            subs = kv((i + 3) // 2, (i + 1) % 2)
            block(subs, softmax_head(i + 1, len(subs)), True)
        else:
            n = NOP6 if i == 5 else NOP
            block(op_(*ops_left[:n]), softmax_head(i + 1, 7 * n), False)
            del ops_left[:n]
    out.append(('PACE',))
    for j in range(NT):
        if j + LA < NT:
            out.append(('EX', NT - 1, j + LA))
        out.append(('PV', NT - 1, j))
        if len(ops_left) > 2:
            block(op_(ops_left.pop(0)), {}, False)
        out.append(('PACE',))
    block(op_(*ops_left), {}, False)
    assert not side
    w7 = [k for k, o in enumerate(out) if o[0] == 'W7']
    assert out.index(('OP', NT - 1, 6)) < min(w7) and max(w7) < out.index(('OP', 0, 0))
    out.remove(('ID', 3))
    out.append(('ID', 3))
    return out


def _kernel(qT_hbm, kT_hbm, vT_hbm, sk_hbm, ssmk_hbm, dd_hbm, xT_hbm, ckv_hbm,
            wq_hbm, wk_hbm, wv_hbm, woT_hbm, out_hbm,
            qT, kT, vT, ssmk, xT, ckv, wq_raw, wk_raw, wv_raw, woT,
            aq_s, w1_s, w2_s, cT_s, QT_s, c2_s, acc, aT_s, out_s, taps, ff_s, fi_s,
            sk_ref, dd_ref, S0_s, S1_s, X_s, W7_s, pace_s, m0_s, m1_s, l0_s, l1_s,
            sem, sem_k, sem_v, sem_o, *rest):
    K_s, V_s, O_s, Y_s = rest[:NT], rest[NT:2 * NT], rest[2 * NT:3 * NT], rest[3 * NT:]

    def cp(src, dst, s):
        return pltpu.make_async_copy(src, dst, s)

    def c_x(j):
        cols = pl.ds(pl.multiple_of(j * 2 * T, 2 * T), 2 * T)
        return cp(xT_hbm.at[:, cols], xT.at[pl.ds(pl.multiple_of(j * M, 16), M)], sem.at[j])

    QP = ((0, 128), (128, 96))

    def c_wq(p):
        cs_ = []
        for half in range(2):
            r = pl.ds((half * 224 + QP[p][0]) * H, QP[p][1] * H)
            for g in range(2):
                cs_.append(cp(wq_hbm.at[r, pl.ds(128 * g, 128)], wq_raw.at[g, r], sem.at[18 + 4 * p + 2 * half + g]))
        return cs_

    def c_w(w_hbm, raw, sm, j, half, g):
        r = pl.ds(pl.multiple_of((half * 4 + j) * 2048, 2048), 2048)
        q = 2 * half + g
        return cp(w_hbm.at[r, pl.ds(128 * g, 128)], raw.at[j % 2, q, pl.ds(0, 2048)], sm.at[(j % 2) * 4 + q])

    def c_wk(j):
        return [c_w(wk_hbm, wk_raw, sem_k, j, half, g) for half in range(2) for g in range(2)]

    def c_wv(j):
        return [c_w(wv_hbm, wv_raw, sem_v, j, half, g) for half in range(2) for g in range(2)]

    def c_ckv(j):
        r = pl.ds(pl.multiple_of(j * 2 * T, 2 * T), 2 * T)
        return cp(ckv_hbm.at[r], ckv.at[r], sem.at[9 + j])

    a_pairs = ((kT_hbm, kT), (vT_hbm, vT), (ssmk_hbm, ssmk), (qT_hbm, qT))
    c_early = [cp(woT_hbm.at[pl.ds(0, 1)], woT.at[pl.ds(0, 1)], sem.at[4])]
    c_early += [cp(src.at[pl.ds(0, CH)], dst.at[pl.ds(0, CH)], sem.at[5 + n]) for n, (src, dst) in enumerate(a_pairs)]
    c_late = [cp(woT_hbm.at[pl.ds(1, H - 1)], woT.at[pl.ds(1, H - 1)], sem.at[13])]
    c_late += [cp(src.at[pl.ds(CH, M - CH)], dst.at[pl.ds(CH, M - CH)], sem.at[14 + n])
               for n, (src, dst) in enumerate(a_pairs)]
    c_small = [cp(sk_hbm, sk_ref, sem.at[26]), cp(dd_hbm, dd_ref, sem.at[27])]
    for c in c_small + c_wq(0) + c_wq(1) + [c_x(0)]:
        c.start()
    for c in c_wk(0):
        c.start(priority=1)

    n_i = jax.lax.broadcasted_iota(jnp.int32, (P, P), 0)
    k_i = jax.lax.broadcasted_iota(jnp.int32, (P, P), 1)
    ang = (((2 * k_i + 1) * n_i) & 511).astype(f32) * (math.pi / 256.0)
    cs, sn = jnp.cos(ang), jnp.sin(ang)
    ff_s[:, 0:P] = cs.astype(bf16)
    ff_s[:, P:2 * P] = (-sn).astype(bf16)
    fi_s[0:P, :] = (cs.T * (1.0 / P)).astype(bf16)
    fi_s[P:2 * P, :] = (sn.T * (-1.0 / P)).astype(bf16)
    acc[...] = jnp.zeros(acc.shape, f32)
    for c in c_small:
        c.wait()
    sk = sk_ref[...].astype(f32)
    for t in range(KS):
        taps[t] = jnp.broadcast_to(sk[t:t + 1, :], (128, M)).T
    taps[KS] = jnp.broadcast_to(dd_ref[...].astype(f32).reshape(1, M), (128, M)).T
    aT_s[...] = jnp.zeros(aT_s.shape, bf16)
    O_s[NT - 1][...] = jnp.zeros(O_s[0].shape, bf16)
    W7_s[...] = jnp.zeros(W7_s.shape, u32)
    cT_s[...] = jnp.zeros(cT_s.shape, u32)

    vq = wq_raw.bitcast(u32)
    for p, (c0, nc) in enumerate(QP):
        for c in c_wq(p):
            c.wait()
        for hp in range(H // 2):
            ut = [vq[g, pl.ds((half * 224 + c0) * 8 + hp, nc, stride=8), :].T for g in range(2) for half in range(2)]
            for r in range(0, 128, 16):
                u = [x[r:r + 16] for x in ut]
                for par, f in enumerate((_lo, _hi)):
                    r0 = (2 * hp + par) * 64 + r // 2
                    for n, x in enumerate(_a7(*[f(x) for x in u])):
                        aq_s[r0:r0 + 8, n * 256 + c0:n * 256 + c0 + nc] = _u(x.astype(bf16))
    for c in c_wv(0) + [c_ckv(0)]:
        c.start(priority=1)

    qscale = (D ** -0.5) * math.log2(math.e)

    def prep_c2(jj, r):
        blk = [[cT_s[cq * 128 + r:cq * 128 + r + 8, tb * 128:(tb + 1) * 128] for tb in range(4)] for cq in range(4)]
        x = [[_f(v) for v in row] for row in blk]
        outer = [[_b7(x[ci][ti], x[ci][2 + ti], x[2 + ci][ti], x[2 + ci][2 + ti]) for ti in range(2)]
                 for ci in range(2)]
        two = [_b7(outer[0][0][n], outer[0][1][n], outer[1][0][n], outer[1][1][n]) for n in range(7)]
        cj = c2_s.at[pl.ds(pl.multiple_of(jj * 128, 128), 128)]
        for n in range(7):
            for m in range(7):
                cj[r:r + 8, (n * 7 + m) * 128:(n * 7 + m + 1) * 128] = _u(two[n][m].astype(bf16))
        return []

    def q_body(j, carry):
        mq = {}
        qtj = QT_s.at[pl.ds(pl.multiple_of(j * 4096, 4096), 4096)]
        zq = j >> 4
        c_x(j).wait()
        xj = xT.at[pl.ds(pl.multiple_of(j * M, 16), M)]
        bx = [_combos(_b7, [_u(xj[r:r + 224, c:c + 128]) for r in (0, 224) for c in (t * T, t * T + 128)])
              for t in range(2)]

        def qproj(u, tok):
            hh, t, n = u // 14, (u // 7) % 2, SORD[u % 7]
            w = _b(_gate(aq_s[hh * 64:hh * 64 + 64, n * 256:n * 256 + 224], tok))
            mq[n] = _nn(w, bx[t][n])
            if u % 7 == 6:
                for k, x in enumerate(_c4(mq)):
                    r0 = t * 2048 + hh * 128 + (k // 2) * 64
                    qtj[r0:r0 + 64, (k % 2) * 128:(k % 2 + 1) * 128] = _u((x * qscale).astype(bf16))
            return mq[n]

        wt = {}
        ckj = ckv.at[pl.ds(pl.multiple_of(j * 512, 512), 512)]
        w1j = w1_s.at[pl.ds(pl.multiple_of(j * 2048, 2048), 2048)]

        def prep_w(kv, hp, part):
            if part == 0:
                v = (wk_raw, wv_raw)[kv].bitcast(u32).at[j % 2]
                wt[kv, hp] = [v[q, pl.ds(hp, 128, stride=8), :].T for q in (0, 2, 1, 3)]
                return [x[120:] for x in wt[kv, hp]]
            for r in range(32 * (part - 1), 32 * part, 16):
                u = [x[r:r + 16] for x in wt[kv, hp]]
                for par, f in enumerate((_lo, _hi)):
                    r0 = (2 * hp + par) * 128 + kv * 64 + r // 2
                    for n, c in enumerate(_a7(*[f(x) for x in u])):
                        w1j[r0:r0 + 8, n * 128:(n + 1) * 128] = _u(c.astype(bf16))
            return []

        def prep_ct(half, cq):
            res = []
            ct = 2 * cq + half
            for tb in range(4):
                x = _u(ckj[tb * 128:(tb + 1) * 128, ct * 128:(ct + 1) * 128].T)
                cT_s[pl.ds(pl.multiple_of(zq * 64 + ct * 64, 64), 64), tb * 128:(tb + 1) * 128] = x
                res.append(x[56:])
            return res

        fill = {}

        def spread(pieces, u0, u1):
            for n, p in enumerate(pieces):
                fill.setdefault(u0 + n * (u1 - u0) // len(pieces), []).append(p)

        spread([functools.partial(prep_w, 0, hp, part) for hp in range(8) for part in range(5)], QW1, QW2)
        spread([functools.partial(prep_w, 1, hp, part) for hp in range(8) for part in range(5)], QW2, QW3)
        spread([functools.partial(prep_ct, 0, cq) for cq in range(4)], QW2 + 2, QC1)
        spread([functools.partial(prep_ct, 1, cq) for cq in range(4)], QC1, QW3)
        spread([functools.partial(prep_c2, jnp.maximum(j - 1, 0), r) for r in range(C2N, 128, 8)], C2S, QW1 - 4)
        if C2N:
            spread([functools.partial(prep_c2, j, r) for r in range(0, C2N, 8)], QW3, QW4)
        toks = {}
        for u in range(224):
            if u == QW1:
                @pl.when(j < 3)
                def _():
                    for c in c_wk(j + 1):
                        c.start(priority=1)

                @pl.when(j == 3)
                def _():
                    for c in c_early + c_late:
                        c.start(priority=1)

                for c in c_wk(j):
                    c.wait()
            if u == QW2:
                @pl.when(j < 3)
                def _():
                    for c in [c_x(j + 1)] + c_wv(j + 1) + [c_ckv(j + 1)]:
                        c.start(priority=1)

                for c in c_wv(j) + [c_ckv(j)]:
                    c.wait()
            q = qproj(u, toks.pop(u, None))
            res = []
            ps = fill.get(u, [])
            for n, p in enumerate(ps):
                row = (n * 128 // len(ps)) // 16 * 16
                if p.func is prep_w and p.args[2] == 0:
                    (wk_raw, wv_raw)[p.args[0]].bitcast(u32)[zq, 0, 1024:1032, :] = _u(q[row:row + 8])
                elif p.func is prep_c2:
                    cT_s[pl.ds(pl.multiple_of(512 + zq * 8, 8), 8), 0:128] = _u(q[row:row + 8])
                elif p.func is prep_ct:
                    ckv[pl.ds(pl.multiple_of(S + zq * 16, 16), 16), 0:128] = q[row:row + 16].astype(bf16)
                res += p()
            if res:
                toks[u + QLAG] = _tok(res)
        return carry

    jax.lax.fori_loop(0, 4, q_body, 0)
    for r in range(C2N, 128, 8):
        prep_c2(3, r)
    for c in c_early:
        c.wait()

    tri = n_i <= k_i
    sgn = jnp.where((jax.lax.broadcasted_iota(jnp.int32, (1, P), 1) & 1) == 0, 1.0, -1.0).astype(f32)
    c_outa = cp(out_s.at[:, pl.ds(0, 384)], out_hbm.at[:, pl.ds(0, 384)], sem_o.at[8])
    HR, HI, PR, PI, KV = range(5)

    def blk_at(c, half=None):
        r0 = (c % 8) * CH
        rs = slice(r0, r0 + CH) if half is None else slice(r0 + 16 * half, r0 + 16 * half + 16)
        return rs, slice((c // 8) * P, (c // 8 + 1) * P)

    def tile(ref, n):
        return ref[:, n * 128:(n + 1) * 128]

    def head_body(h, carry):
        @pl.when(h == 1)
        def _():
            for c in c_late:
                c.wait()

        @pl.when(h == H - 1)
        def _():
            c_outa.start()

        st = dict(co={}, cnt={}, fin=set(), M={}, P={}, Q7={}, mfin={}, o={})
        zs = h >> 10
        z64 = pl.ds(pl.multiple_of(zs * 64, 64), 64)
        m_s, l_s = (m0_s, m1_s), (l0_s, l1_s)
        w1h = w1_s.at[pl.ds(pl.multiple_of(h * 128, 128), 3 * 2048 + 128)]
        qth = QT_s.at[pl.ds(pl.multiple_of(h * 128, 128), 7 * 2048 + 128)]
        rows = pl.ds(pl.multiple_of(jnp.minimum(h, NCH - 1) * CH, CH), CH)

        def rep(t, n):
            return jnp.concatenate([taps[t, rows, :]] * n, axis=1)

        toks = []

        def due():
            for t in toks:
                t[0] -= 1
            ready = [t[1] for t in toks if t[0] <= 0]
            toks[:] = [t for t in toks if t[0] > 0]
            return functools.reduce(lambda x, y: x | y, ready) if ready else None

        def gate_later(vals):
            toks.append([SLAG, _tok([v if v.dtype == u32 else _u(v) for v in vals])])

        def row_offset(i):
            if i not in st['mfin']:
                m = m_s[i % 2][0, 0]
                for t in range(1, i + 1):
                    m = jnp.maximum(m, m_s[i % 2][0, t])
                m = jnp.max(m, axis=0, keepdims=True)
                if i > 0:
                    lo_ = jnp.exp2(m_s[i % 2][0, 0] - m)
                    for t in range(1, i + 1):
                        lo_ = lo_ + jnp.exp2(m_s[i % 2][0, t] - m)
                    m = m + jnp.log2(jnp.sum(lo_, axis=0, keepdims=True))
                st['mfin'][i] = m
            return st['mfin'][i]

        for op in _schedule():
            kind = op[0]
            if kind == 'KV':
                _, p, t = op
                n, m = SK[t // 7], SV[t % 7]

                def wblk(q):
                    w = jnp.concatenate([w1h[k * 2048:k * 2048 + 128, n * 128:(n + 1) * 128]
                                         for k in (2 * (q % 2), 2 * (q % 2) + 1)], axis=1)
                    r = (q // 2) * 32
                    return jnp.concatenate([w[r:r + 32], w[64 + r:64 + r + 32]], axis=0)

                cols = slice((n * 7 + m) * 256, (n * 7 + m + 1) * 256)
                if m in (2, 3):
                    w = wblk(0 if m == 2 else 3)
                elif p > 0:
                    w = w2_s[:, cols]
                else:
                    i1, i2, sg = _A_OF[m]
                    x, y = wblk(i1), wblk(i2)
                    w = (_f(x) + _f(y) if sg > 0 else _f(x) - _f(y)).astype(bf16)
                    w2_s[z64, cols] = _u(w)
                c2 = c2_s[p * 128:(p + 1) * 128, (n * 7 + m) * 128:(n * 7 + m + 1) * 128]
                st['M'][m] = st['last'] = _nn(w if w.dtype == bf16 else _b(_gate(w, due())), _b(c2))
                if t % 7 < 6:
                    continue
                mo = _quad(*_c4(st['M']))
                for o, sg in _C_OF[n]:
                    k = st['cnt'][o] = st['cnt'].get(o, 0) + 1
                    if k == 1:
                        st['co'][o] = mo if sg > 0 else -mo
                    else:
                        st['co'][o] = st['co'][o] + mo if sg > 0 else st['co'][o] - mo
                    if k == _C_CNT[o]:
                        st['cnt'][o] = 0
                        st['fin'].add(o)
                for tok in range(2):
                    if not {tok, 2 + tok} <= st['fin']:
                        continue
                    st['fin'] -= {tok, 2 + tok}
                    c = 2 * p + tok

                    def full(dh, kb, off):
                        x = st['co'][2 * dh + tok][:, kb * 128:(kb + 1) * 128]
                        return jnp.concatenate([x[off:off + 64], x[128 + off:128 + off + 64]], axis=0)

                    kb4 = (full(0, 0, 0).T, full(1, 0, 0).T, full(0, 1, 0).T, full(1, 1, 0).T)
                    vb4 = (full(0, 0, 64), full(0, 1, 64), full(1, 0, 64), full(1, 1, 64))
                    for ref, c4 in ((K_s[c], kb4), (V_s[c], vb4)):
                        blks = dict(zip((2, 7, 8, 3), c4))
                        if c < NT - 1:
                            blks.update({k: x for k, x in enumerate(_a7(*c4)) if k not in (2, 3)})
                        for k, x in blks.items():
                            ref[z64, k * 128:(k + 1) * 128] = _u(x.astype(bf16))
            elif kind == 'QK':
                _, i, j = op
                S_s = (S0_s, S1_s)[i % 2]
                if j < i:
                    if i not in st['Q7']:
                        qu = qth[i * 2048:i * 2048 + 128, :]
                        st['Q7'][i] = _combos(_b7, [qu[:64, :128], qu[:64, 128:], qu[64:, :128], qu[64:, 128:]])
                    s = _quad(*_c4({n: _nn(_b(tile(K_s[j], n)), st['Q7'][i][n]) for n in SQ}))
                    S_s[zs, j] = s
                    f = _fold(s, jnp.max)
                else:
                    q = _b(qth[i * 2048:i * 2048 + 128, :])
                    sa = _nn(_b(jnp.concatenate([tile(K_s[j], 2), tile(K_s[j], 7)], axis=1)), q)
                    sa = jnp.concatenate([jnp.where(tri, sa[:, :128], NEG), sa[:, 128:]], axis=1)
                    sb = _nn(_b(jnp.concatenate([tile(K_s[j], 8), tile(K_s[j], 3)], axis=1)), q[:, 128:])
                    sb = jnp.where(tri, sb, NEG)
                    S_s[zs, j, 0:128, :] = sa
                    S_s[zs, j, 128:T, 128:T] = sb
                    fa = _fold(sa, jnp.max)
                    f = jnp.concatenate([fa[:, :128], jnp.maximum(fa[:, 128:], _fold(sb, jnp.max))], axis=1)
                m_s[i % 2][zs, j] = f
                pace_s[zs] = f
            elif kind == 'EX':
                _, i, j = op
                S_s = (S0_s, S1_s)[i % 2]
                m = row_offset(i)
                m = jnp.where(pace_s[0, 0:1, :] == jnp.inf, jnp.inf, m)
                if j < i:
                    parts, lj = [], None
                    for r in range(112, -16, -16):
                        pt = jnp.exp2(S_s[0, j, r:r + 16, :] - m)
                        pb = jnp.exp2(S_s[0, j, 128 + r:128 + r + 16, :] - m)
                        parts.insert(0, _b7(pt[:, :128], pt[:, 128:], pb[:, :128], pb[:, 128:]))
                        x = (pt[:8] + pt[8:]) + (pb[:8] + pb[8:])
                        lj = x if lj is None else lj + x
                    st['P'][i, j] = [jnp.concatenate([x[n] for x in parts], axis=0).astype(bf16) for n in range(7)]
                else:
                    pa = jnp.exp2(S_s[0, j, 0:128, :] - m)
                    pb = jnp.exp2(S_s[0, j, 128:T, 128:T] - m[:, 128:])
                    la = _rsum(pa)
                    lj = jnp.concatenate([la[:, :128], la[:, 128:] + _rsum(pb)], axis=1)
                    st['P'][i, j] = (pa.astype(bf16), pb.astype(bf16))
                l_s[i % 2][zs, j] = lj
            elif kind == 'PV':
                _, i, j = op
                p = st['P'].pop((i, j))
                if j < i:
                    for n in SP:
                        st['last'] = _nn(_b(tile(V_s[j], n)), p[n])
                        st['o'][i, n] = st['o'][i, n] + st['last'] if j > 0 else st['last']
                    continue
                oa = _nn(_b(jnp.concatenate([tile(V_s[j], 2), tile(V_s[j], 8)], axis=0)), p[0])
                ob = _nn(_b(jnp.concatenate([tile(V_s[j], 7), tile(V_s[j], 3)], axis=0)), p[1])
                o = st['last'] = jnp.concatenate([oa[:, :128], oa[:, 128:] + ob], axis=1)
                if i > 0:
                    o = o + _quad(*_c4({n: st['o'].pop((i, n)) for n in range(7)}))
                l = l_s[i % 2][0, 0]
                for t in range(1, i + 1):
                    l = l + l_s[i % 2][0, t]
                o = o * (1.0 / jnp.sum(l, axis=0, keepdims=True))
                for n, x in enumerate(_b7(o[:128, :128], o[:128, 128:], o[128:, :128], o[128:, 128:])):
                    O_s[i][zs, n] = x.astype(bf16)
            elif kind == 'PACE':
                pace_s[zs] = jnp.concatenate([st['last'][-8:, -128:]] * 2, axis=1)
            elif kind == 'OP':
                _, i, t = op
                n = SO[t]
                st['M'][n] = st['last'] = _nn(_b(_gate(tile(W7_s, n), due())), O_s[i][0, n])
                if t == 6:
                    acc[:, T * i:T * (i + 1)] += _quad(*_c4(st['M']))
            elif kind == 'W7':
                res = []
                for r0 in range(16 * op[1], 16 * op[2], 16):
                    blk = [_u(woT[h, r:r + 16, c:c + 128]) for r in (r0, 224 + r0) for c in (0, 128)]
                    row = pl.ds(pl.multiple_of(zs * 8 + r0 // 2, 8), 8)
                    for n, x in enumerate(_combos(_a7, blk)):
                        W7_s[row, n * 128:(n + 1) * 128] = _u(x)
                    res += blk
                gate_later(res)
            elif kind == 'AT':
                g = jnp.clip((h - 4) // 4, 0, 2)
                t0 = jnp.minimum(((h + 12) % 4) * 6, NB - 6)
                grow = pl.ds(pl.multiple_of(g * 128, 128), 128)
                gcol = pl.ds(pl.multiple_of(jnp.where(h == H - 1, 3, g) * 128, 128), 128)
                res = []
                for n in range(6):
                    tok = pl.ds(pl.multiple_of((t0 + n) * 128, 128), 128)
                    x = aT_s[grow, tok].T
                    out_s[tok, gcol] = x
                    res.append(_u(x)[56:])
                gate_later(res)
            elif kind == 'HD':
                g = op[1]
                hs = jnp.concatenate([ssmk[rows, c * P:(c + 1) * P] for c in range(4 * g, 4 * g + 4)], axis=0)
                hf = _nn(hs, ff_s[...])
                for n in range(4):
                    X_s[(zs, HR) + blk_at(4 * g + n)] = hf[n * CH:(n + 1) * CH, :P]
                    X_s[(zs, HI) + blk_at(4 * g + n)] = hf[n * CH:(n + 1) * CH, P:]
            elif kind == 'SC':
                g = op[1]
                if g == 0:
                    k = jnp.concatenate([jnp.zeros((CH, P), f32), kT[rows, 0:4 * P].astype(f32)], axis=1)
                else:
                    k = kT[rows, (4 * g - 1) * P:(4 * g + 4) * P].astype(f32)
                ks = k[:, P:] * rep(0, 4)
                for j in range(1, KS):
                    ks = ks + pltpu.roll(k, j, 1)[:, P:] * rep(j, 4)
                kv = ks * vT[rows, 4 * g * P:(4 * g + 4) * P].astype(f32)
                kvs = jnp.concatenate([kv[:, n * P:(n + 1) * P] for n in range(4)], axis=0)
                xf = _nn(kvs.astype(bf16), ff_s[...])
                for n in range(4):
                    c = 4 * g + n
                    xr, xi = xf[n * CH:(n + 1) * CH, :P], xf[n * CH:(n + 1) * CH, P:]
                    X_s[(zs, KV) + blk_at(c)] = kvs[n * CH:(n + 1) * CH]
                    pr = xr if c == 0 else xr - sgn * st['x'][1]
                    pi = xi if c == 0 else xi + sgn * st['x'][0]
                    X_s[(zs, PR) + blk_at(c)] = pr
                    X_s[(zs, PI) + blk_at(c)] = pi
                    st['x'] = (xr, xi)
            elif kind == 'CV':
                res = []
                for a, half in op[1]:
                    wr = wi = None
                    for j in range(a + 1):
                        hr, hi_ = X_s[(0, HR) + blk_at(j, half)], X_s[(0, HI) + blk_at(j, half)]
                        pr, pi = X_s[(0, PR) + blk_at(a - j, half)], X_s[(0, PI) + blk_at(a - j, half)]
                        tr, ti = hr * pr - hi_ * pi, hr * pi + hi_ * pr
                        wr, wi = (tr, ti) if wr is None else (wr + tr, wi + ti)
                    r0 = (a % 4) * CH + 16 * half
                    Y_s[a // 4][zs, r0:r0 + 16, :P] = wr
                    Y_s[a // 4][zs, r0:r0 + 16, P:] = wi
                    res += [wr, wi]
                gate_later(res)
            elif kind == 'ID':
                g = op[1]
                y = _nn(Y_s[g][0].astype(bf16), fi_s[...])
                for n in range(4):
                    c = 4 * g + n
                    cols = slice(c * P, (c + 1) * P)
                    ya = y[n * CH:(n + 1) * CH, :] + X_s[(0, KV) + blk_at(c)] * taps[KS, rows, :]
                    aT_s[rows, cols] = (qT[rows, cols].astype(f32) * ya).astype(bf16)
        return carry

    jax.lax.fori_loop(0, H, head_body, 0)

    acc[:, T * (NT - 1):] += _quad(*_c4({n: _nn(_b(tile(W7_s, n)), O_s[NT - 1][0, n]) for n in SORD}))
    outs = [c_outa]
    for i in range(NT):
        cols = slice(T * i, T * (i + 1))
        blk = jnp.concatenate([aT_s[384:M, cols], acc[:, cols].astype(bf16)], axis=0)
        out_s[cols, 384:2 * M] = blk.T
        c = cp(out_s.at[pl.ds(T * i, T), pl.ds(384, 512)], out_hbm.at[pl.ds(T * i, T), pl.ds(384, 512)], sem_o.at[i])
        c.start()
        outs.append(c)
    for c in outs:
        c.wait()


@jax.jit
def pallas_concat_heads__ssm_conv_h3__compressed_kv_cla__prompt_kernel(
    A_q: jax.Array,
    A_k: jax.Array,
    A_v: jax.Array,
    A_shift_k: jax.Array,
    A_ssm_k: jax.Array,
    A_ssm_D: jax.Array,
    B_x: jax.Array,
    B_c_kv: jax.Array,
    B_w_q: jax.Array,
    B_w_uk: jax.Array,
    B_w_uv: jax.Array,
    B_w_o: jax.Array,
):
    hbm = pl.BlockSpec(memory_space=pl.ANY)
    V = pltpu.VMEM
    out = pl.pallas_call(
        _kernel,
        out_shape=jax.ShapeDtypeStruct((S, 2 * M), bf16),
        in_specs=[hbm] * 12,
        out_specs=hbm,
        scratch_shapes=[
            V((M, S), bf16), V((M, S), bf16), V((M, S), bf16), V((M, S), bf16),
            V((4 * M, 2 * T), bf16), V((S + 16, DC), bf16),
            V((2, M * H, 128), bf16),
            V((2, 4, 128 * H + 16, 128), bf16), V((2, 4, 128 * H + 16, 128), bf16),
            V((H, M, D), bf16),
            V((H * 64, 7 * 256), u32),
            V((4 * H * 128, 7 * 128), u32), V((64, 49 * 256), u32),
            V((512 + 8, 512), u32),
            V((NT * H * 128, T), u32), V((4 * 128, 49 * 128), u32),
            V((M, S), f32), V((M, S), bf16), V((S, 2 * M), bf16),
            V((KS + 1, M, 128), f32), V((P, 2 * P), bf16), V((2 * P, P), bf16),
            V((KS, M), bf16), V((M,), bf16),
            V((1, NT, T, T), f32), V((1, NT, T, T), f32), V((1, 5, T, T), f32),
            V((112, 7 * 128), u32), V((1, 8, T), f32),
            V((1, NT, 8, T), f32), V((1, NT, 8, T), f32), V((1, NT, 8, T), f32), V((1, NT, 8, T), f32),
            pltpu.SemaphoreType.DMA((28,)), pltpu.SemaphoreType.DMA((8,)),
            pltpu.SemaphoreType.DMA((8,)), pltpu.SemaphoreType.DMA((9,)),
        ] + [V((64, 9 * 128), u32)] * (2 * NT) + [V((1, 7, 128, 128), bf16)] * NT
        + [V((1, 4 * CH, 2 * P), f32)] * 4,
        compiler_params=pltpu.CompilerParams(vmem_limit_bytes=126 * 1024 * 1024,
                                             shape_invariant_numerics=False,
                                             disable_bounds_checks=True, disable_semaphore_checks=True),
    )(
        A_q[0].T, A_k[0].T, A_v[0].T, A_shift_k.T, A_ssm_k, A_ssm_D,
        B_x[0].T, B_c_kv[0],
        B_w_q.reshape(M * H, D), B_w_uk.reshape(DC * H, D), B_w_uv.reshape(DC * H, D),
        jnp.transpose(B_w_o, (0, 2, 1)),
    )
    return out[None]
```

```python
import functools
import math

import jax
import jax.numpy as jnp
import jax.experimental.pallas as pl
import jax.experimental.pallas.tpu as pltpu

bf16 = jnp.bfloat16
f32 = jnp.float32
u32 = jnp.uint32

S = 2048
M = 448
DC = 1024
H = 16
D = 256
KS = 4
P = 128
NB = S // P
CH = 32
NCH = M // CH
T = 256
NT = S // T
NEG = -1e30

SORD = tuple(int(c) for c in '6430125')
SK = tuple(int(c) for c in '0364125')
SV = tuple(int(c) for c in '0125364')
SQ = tuple(int(c) for c in '6043125')
SP = tuple(int(c) for c in '3640125')
SO = tuple(int(c) for c in '5210346')
QW1 = 56
QW2 = 140
QW3 = 208
QW4 = 222
QC1 = 165
QLAG = 12
CVMAX = 12
SIDE0 = 30
SIDEP = 4
SLAG = 5
PRE = 0
W7P = 16
W7D = 6
KVH = 35
EXB = 10
NOP6 = 2
LA = 3
C2N = 64
C2S = 16
NOP = 2


def _nn(a, b):
    return jnp.dot(a, b, preferred_element_type=f32)


def _b(u):
    return pltpu.bitcast(u, bf16)


def _u(x):
    return pltpu.bitcast(x, u32)


def _lo(u):
    return pltpu.bitcast(u << 16, f32)


def _hi(u):
    return pltpu.bitcast(u & jnp.uint32(0xFFFF0000), f32)


def _f(u):
    return _b(u).astype(f32)


def _a7(a11, a12, a21, a22):
    return [a11 + a22, a21 + a22, a11, a22, a11 + a12, a21 - a11, a12 - a22]


def _b7(b11, b12, b21, b22):
    return [b11 + b22, b11, b12 - b22, b21 - b11, b22, b11 + b12, b21 + b22]


def _c4(m):
    return m[0] + m[3] - m[4] + m[6], m[2] + m[4], m[1] + m[3], m[0] - m[1] + m[2] + m[5]


_C_OF = (((0, 1), (3, 1)), ((2, 1), (3, -1)), ((1, 1), (3, 1)), ((0, 1), (2, 1)), ((0, -1), (1, 1)), ((3, 1),), ((0, 1),))
_C_CNT = (4, 2, 2, 4)
_A_OF = {0: (0, 3, 1), 1: (2, 3, 1), 4: (0, 1, 1), 5: (2, 0, -1), 6: (1, 3, -1)}


def _combos(f7, blk):
    x = f7(*[_f(v) for v in blk])
    plain = {2: 0, 3: 3} if f7 is _a7 else {1: 0, 4: 3}
    return [_b(blk[plain[n]]) if n in plain else x[n].astype(bf16) for n in range(7)]


def _quad(c11, c12, c21, c22):
    return jnp.concatenate([jnp.concatenate([c11, c12], axis=1), jnp.concatenate([c21, c22], axis=1)], axis=0)


def _fold(c, op):
    return op(c.reshape(-1, 8, c.shape[1]), axis=0)


def _rsum(p):
    cols = []
    for c in range(0, p.shape[1], 128):
        acc = None
        for r in range(112, -16, -16):
            t = p[r:r + 8, c:c + 128] + p[r + 8:r + 16, c:c + 128]
            acc = t if acc is None else acc + t
        cols.append(acc)
    return jnp.concatenate(cols, axis=1) if len(cols) > 1 else cols[0]


def _tok(vals):
    parts = []
    for v in vals:
        for r in range(0, v.shape[0], 8):
            for c in range(0, v.shape[1], 128):
                parts.append(v[r:r + 8, c:c + 128])
    while len(parts) > 1:
        parts = [parts[i] | parts[i + 1] if i + 1 < len(parts) else parts[i] for i in range(0, len(parts), 2)]
    return (parts[0] >> 31) >> 1


def _gate(x, tok):
    if tok is None:
        return x
    top = x[:8, :128] | tok
    if x.shape[1] > 128:
        top = jnp.concatenate([top, x[:8, 128:]], axis=1)
    return jnp.concatenate([top, x[8:]], axis=0)


def _side_pieces():
    ps = [(k, g) for g in range(PRE) for k in ('HD', 'SC')]
    cur, cost = [], 0
    for a in range(NB):
        if a % 4 == 0 and a // 4 + PRE < 4:
            ps += [('HD', a // 4 + PRE), ('SC', a // 4 + PRE)]
        for half in range(2):
            if cur and cost + a + 1 > CVMAX:
                ps.append(('CV', tuple(cur)))
                cur, cost = [], 0
            cur.append((a, half))
            cost += a + 1
        if a % 4 == 3:
            ps += [('CV', tuple(cur)), ('ID', a // 4)]
            cur, cost = [], 0
    ps.insert(W7P, ('W7', 0, 7))
    ps.insert(W7P + W7D, ('W7', 7, 14))
    return ps


def _schedule():
    side = _side_pieces()
    out = []
    cnt = [0]

    def block(subs, att, with_side):
        for k, u in enumerate(subs):
            out.append(u)
            out.extend(att.get(k, []))
            if with_side:
                cnt[0] += 1
                if side and cnt[0] >= SIDE0 and (cnt[0] - SIDE0) % SIDEP == 0:
                    out.append(side.pop(0))

    def kv(p, half):
        return [('KV', p, t) for t in (range(KVH) if half == 0 else range(KVH, 49))]

    def op_(*idx):
        return [('OP', i, t) for i in idx for t in range(7)]

    def softmax_head(i, n):
        att = {max(n - EXB, 0): [('PACE',), ('EX', i, 0)]}
        for k in range(1, min(LA, i + 1)):
            att.setdefault(n - 1 - (LA - 1 - k) * 2, []).extend([('PACE',), ('EX', i, k)])
        return att

    ops_left = list(range(NT - 1))
    block(kv(0, 0) + kv(0, 1), {}, True)
    block(op_(NT - 1), {6: [('AT',), ('QK', 0, 0)]}, False)
    block(kv(1, 0), softmax_head(0, KVH), True)
    for i in range(NT - 1):
        for j in range(i + 1):
            out.append(('QK', i + 1, j))
            if j + LA <= i:
                out.append(('EX', i, j + LA))
            out.append(('PV', i, j))
        out.append(('QK', i + 1, i + 1))
        if i < 5:
            subs = kv((i + 3) // 2, (i + 1) % 2)
            block(subs, softmax_head(i + 1, len(subs)), True)
        else:
            n = NOP6 if i == 5 else NOP
            block(op_(*ops_left[:n]), softmax_head(i + 1, 7 * n), False)
            del ops_left[:n]
    out.append(('PACE',))
    for j in range(NT):
        if j + LA < NT:
            out.append(('EX', NT - 1, j + LA))
        out.append(('PV', NT - 1, j))
        if len(ops_left) > 2:
            block(op_(ops_left.pop(0)), {}, False)
        out.append(('PACE',))
    block(op_(*ops_left), {}, False)
    assert not side
    w7 = [k for k, o in enumerate(out) if o[0] == 'W7']
    assert out.index(('OP', NT - 1, 6)) < min(w7) and max(w7) < out.index(('OP', 0, 0))
    out.remove(('ID', 3))
    out.append(('ID', 3))
    return out


def _kernel(qT_hbm, kT_hbm, vT_hbm, sk_hbm, ssmk_hbm, dd_hbm, xT_hbm, ckv_hbm,
            wq_hbm, wk_hbm, wv_hbm, woT_hbm, out_hbm,
            qT, kT, vT, ssmk, xT, ckv, wq_raw, wk_raw, wv_raw, woT,
            aq_s, w1_s, w2_s, cT_s, QT_s, c2_s, acc, aT_s, out_s, taps, ff_s, fi_s,
            sk_ref, dd_ref, S0_s, S1_s, X_s, W7_s, pace_s, m0_s, m1_s, l0_s, l1_s,
            sem, sem_k, sem_v, sem_o, *rest):
    K_s, V_s, O_s, Y_s = rest[:NT], rest[NT:2 * NT], rest[2 * NT:3 * NT], rest[3 * NT:]

    def cp(src, dst, s):
        return pltpu.make_async_copy(src, dst, s)

    def c_x(j):
        cols = pl.ds(pl.multiple_of(j * 2 * T, 2 * T), 2 * T)
        return cp(xT_hbm.at[:, cols], xT.at[pl.ds(pl.multiple_of(j * M, 16), M)], sem.at[j])

    QP = ((0, 128), (128, 96))

    def c_wq(k):
        r = pl.ds((k % 2) * 224 * H, 224 * H)
        return cp(wq_hbm.at[r, pl.ds(128 * (k // 2), 128)], wq_raw.at[k // 2, r], sem.at[18 + k])

    def c_w(w_hbm, raw, sm, j, half, g):
        r = pl.ds(pl.multiple_of((half * 4 + j) * 2048, 2048), 2048)
        q = 2 * half + g
        return cp(w_hbm.at[r, pl.ds(128 * g, 128)], raw.at[j % 2, q, pl.ds(0, 2048)], sm.at[(j % 2) * 4 + q])

    def c_wk(j):
        return [c_w(wk_hbm, wk_raw, sem_k, j, half, g) for half in range(2) for g in range(2)]

    def c_wv(j):
        return [c_w(wv_hbm, wv_raw, sem_v, j, half, g) for half in range(2) for g in range(2)]

    def c_ckv(j):
        r = pl.ds(pl.multiple_of(j * 2 * T, 2 * T), 2 * T)
        return cp(ckv_hbm.at[r], ckv.at[r], sem.at[9 + j])

    a_pairs = ((kT_hbm, kT), (vT_hbm, vT), (ssmk_hbm, ssmk), (qT_hbm, qT))
    c_early = [cp(woT_hbm.at[pl.ds(0, 1)], woT.at[pl.ds(0, 1)], sem.at[4])]
    c_early += [cp(src.at[pl.ds(0, CH)], dst.at[pl.ds(0, CH)], sem.at[5 + n]) for n, (src, dst) in enumerate(a_pairs)]
    c_late = [cp(woT_hbm.at[pl.ds(1, H - 1)], woT.at[pl.ds(1, H - 1)], sem.at[13])]
    c_late += [cp(src.at[pl.ds(CH, M - CH)], dst.at[pl.ds(CH, M - CH)], sem.at[14 + n])
               for n, (src, dst) in enumerate(a_pairs)]
    c_small = [cp(sk_hbm, sk_ref, sem.at[22]), cp(dd_hbm, dd_ref, sem.at[23])]
    for c in c_small + [c_wq(k) for k in (0, 3, 2, 1)] + [c_x(0)]:
        c.start()
    for c in c_wk(0):
        c.start(priority=1)

    n_i = jax.lax.broadcasted_iota(jnp.int32, (P, P), 0)
    k_i = jax.lax.broadcasted_iota(jnp.int32, (P, P), 1)
    ang = (((2 * k_i + 1) * n_i) & 511).astype(f32) * (math.pi / 256.0)
    cs, sn = jnp.cos(ang), jnp.sin(ang)
    ff_s[:, 0:P] = cs.astype(bf16)
    ff_s[:, P:2 * P] = (-sn).astype(bf16)
    fi_s[0:P, :] = (cs.T * (1.0 / P)).astype(bf16)
    fi_s[P:2 * P, :] = (sn.T * (-1.0 / P)).astype(bf16)
    acc[...] = jnp.zeros(acc.shape, f32)
    for c in c_small:
        c.wait()
    sk = sk_ref[...].astype(f32)
    for t in range(KS):
        taps[t] = jnp.broadcast_to(sk[t:t + 1, :], (128, M)).T
    taps[KS] = jnp.broadcast_to(dd_ref[...].astype(f32).reshape(1, M), (128, M)).T
    aT_s[...] = jnp.zeros(aT_s.shape, bf16)
    O_s[NT - 1][...] = jnp.zeros(O_s[0].shape, bf16)
    W7_s[...] = jnp.zeros(W7_s.shape, u32)
    cT_s[...] = jnp.zeros(cT_s.shape, u32)

    vq = wq_raw.bitcast(u32)
    ut = {}
    for k, ready in ((0, ()), (3, (0, 2, 3)), (2, (1, 5)), (1, (4, 6))):
        c_wq(k).wait()
        for hp in range(H // 2):
            for c0, nc in QP:
                ut[k, hp, c0] = vq[k // 2, pl.ds(((k % 2) * 224 + c0) * 8 + hp, nc, stride=8), :].T
                for r in range(0, 128, 16):
                    for par, f in enumerate((_lo, _hi)):
                        r0 = (2 * hp + par) * 64 + r // 2
                        for n in ready:
                            i1, i2, sg = _A_OF.get(n, (0 if n == 2 else 3, None, 0))
                            x = f(ut[i1, hp, c0][r:r + 16])
                            if i2 is not None:
                                y = f(ut[i2, hp, c0][r:r + 16])
                                x = x + y if sg > 0 else x - y
                            aq_s[r0:r0 + 8, n * 256 + c0:n * 256 + c0 + nc] = _u(x.astype(bf16))
    for c in c_wv(0) + [c_ckv(0)]:
        c.start(priority=1)

    qscale = (D ** -0.5) * math.log2(math.e)

    def prep_c2(jj, r):
        blk = [[cT_s[cq * 128 + r:cq * 128 + r + 8, tb * 128:(tb + 1) * 128] for tb in range(4)] for cq in range(4)]
        x = [[_f(v) for v in row] for row in blk]
        outer = [[_b7(x[ci][ti], x[ci][2 + ti], x[2 + ci][ti], x[2 + ci][2 + ti]) for ti in range(2)]
                 for ci in range(2)]
        two = [_b7(outer[0][0][n], outer[0][1][n], outer[1][0][n], outer[1][1][n]) for n in range(7)]
        cj = c2_s.at[pl.ds(pl.multiple_of(jj * 128, 128), 128)]
        for n in range(7):
            for m in range(7):
                cj[r:r + 8, (n * 7 + m) * 128:(n * 7 + m + 1) * 128] = _u(two[n][m].astype(bf16))
        return []

    def q_body(j, carry):
        mq = {}
        qtj = QT_s.at[pl.ds(pl.multiple_of(j * 4096, 4096), 4096)]
        zq = j >> 4
        c_x(j).wait()
        xj = xT.at[pl.ds(pl.multiple_of(j * M, 16), M)]
        bx = [_combos(_b7, [_u(xj[r:r + 224, c:c + 128]) for r in (0, 224) for c in (t * T, t * T + 128)])
              for t in range(2)]

        def qproj(u, tok):
            hh, t, n = u // 14, (u // 7) % 2, SORD[u % 7]
            w = _b(_gate(aq_s[hh * 64:hh * 64 + 64, n * 256:n * 256 + 224], tok))
            mq[n] = _nn(w, bx[t][n])
            if u % 7 == 6:
                for k, x in enumerate(_c4(mq)):
                    r0 = t * 2048 + hh * 128 + (k // 2) * 64
                    qtj[r0:r0 + 64, (k % 2) * 128:(k % 2 + 1) * 128] = _u((x * qscale).astype(bf16))
            return mq[n]

        wt = {}
        ckj = ckv.at[pl.ds(pl.multiple_of(j * 512, 512), 512)]
        w1j = w1_s.at[pl.ds(pl.multiple_of(j * 2048, 2048), 2048)]

        def prep_w(kv, hp, part):
            if part == 0:
                v = (wk_raw, wv_raw)[kv].bitcast(u32).at[j % 2]
                wt[kv, hp] = [v[q, pl.ds(hp, 128, stride=8), :].T for q in (0, 2, 1, 3)]
                return [x[120:] for x in wt[kv, hp]]
            for r in range(32 * (part - 1), 32 * part, 16):
                u = [x[r:r + 16] for x in wt[kv, hp]]
                for par, f in enumerate((_lo, _hi)):
                    r0 = (2 * hp + par) * 128 + kv * 64 + r // 2
                    for n, c in enumerate(_a7(*[f(x) for x in u])):
                        w1j[r0:r0 + 8, n * 128:(n + 1) * 128] = _u(c.astype(bf16))
            return []

        def prep_ct(half, cq):
            res = []
            ct = 2 * cq + half
            for tb in range(4):
                x = _u(ckj[tb * 128:(tb + 1) * 128, ct * 128:(ct + 1) * 128].T)
                cT_s[pl.ds(pl.multiple_of(zq * 64 + ct * 64, 64), 64), tb * 128:(tb + 1) * 128] = x
                res.append(x[56:])
            return res

        fill = {}

        def spread(pieces, u0, u1):
            for n, p in enumerate(pieces):
                fill.setdefault(u0 + n * (u1 - u0) // len(pieces), []).append(p)

        spread([functools.partial(prep_w, 0, hp, part) for hp in range(8) for part in range(5)], QW1, QW2)
        spread([functools.partial(prep_w, 1, hp, part) for hp in range(8) for part in range(5)], QW2, QW3)
        spread([functools.partial(prep_ct, 0, cq) for cq in range(4)], QW2 + 2, QC1)
        spread([functools.partial(prep_ct, 1, cq) for cq in range(4)], QC1, QW3)
        spread([functools.partial(prep_c2, jnp.maximum(j - 1, 0), r) for r in range(C2N, 128, 8)], C2S, QW1 - 4)
        if C2N:
            spread([functools.partial(prep_c2, j, r) for r in range(0, C2N, 8)], QW3, QW4)
        toks = {}
        for u in range(224):
            if u == QW1:
                @pl.when(j < 3)
                def _():
                    for c in c_wk(j + 1):
                        c.start(priority=1)

                @pl.when(j == 3)
                def _():
                    for c in c_early + c_late:
                        c.start(priority=1)

                for c in c_wk(j):
                    c.wait()
            if u == QW2:
                @pl.when(j < 3)
                def _():
                    for c in [c_x(j + 1)] + c_wv(j + 1) + [c_ckv(j + 1)]:
                        c.start(priority=1)

                for c in c_wv(j) + [c_ckv(j)]:
                    c.wait()
            q = qproj(u, toks.pop(u, None))
            res = []
            ps = fill.get(u, [])
            for n, p in enumerate(ps):
                row = (n * 128 // len(ps)) // 16 * 16
                if p.func is prep_w and p.args[2] == 0:
                    (wk_raw, wv_raw)[p.args[0]].bitcast(u32)[zq, 0, 1024:1032, :] = _u(q[row:row + 8])
                elif p.func is prep_c2:
                    cT_s[pl.ds(pl.multiple_of(512 + zq * 8, 8), 8), 0:128] = _u(q[row:row + 8])
                elif p.func is prep_ct:
                    ckv[pl.ds(pl.multiple_of(S + zq * 16, 16), 16), 0:128] = q[row:row + 16].astype(bf16)
                res += p()
            if res:
                toks[u + QLAG] = _tok(res)
        return carry

    jax.lax.fori_loop(0, 4, q_body, 0)
    for r in range(C2N, 128, 8):
        prep_c2(3, r)
    for c in c_early:
        c.wait()

    tri = n_i <= k_i
    sgn = jnp.where((jax.lax.broadcasted_iota(jnp.int32, (1, P), 1) & 1) == 0, 1.0, -1.0).astype(f32)
    c_outa = cp(out_s.at[:, pl.ds(0, 384)], out_hbm.at[:, pl.ds(0, 384)], sem_o.at[8])
    HR, HI, PR, PI, KV = range(5)

    def blk_at(c, half=None):
        r0 = (c % 8) * CH
        rs = slice(r0, r0 + CH) if half is None else slice(r0 + 16 * half, r0 + 16 * half + 16)
        return rs, slice((c // 8) * P, (c // 8 + 1) * P)

    def tile(ref, n):
        return ref[:, n * 128:(n + 1) * 128]

    def head_body(h, carry):
        @pl.when(h == 1)
        def _():
            for c in c_late:
                c.wait()

        @pl.when(h == H - 1)
        def _():
            c_outa.start()

        st = dict(co={}, cnt={}, fin=set(), M={}, P={}, Q7={}, mfin={}, o={})
        zs = h >> 10
        z64 = pl.ds(pl.multiple_of(zs * 64, 64), 64)
        m_s, l_s = (m0_s, m1_s), (l0_s, l1_s)
        w1h = w1_s.at[pl.ds(pl.multiple_of(h * 128, 128), 3 * 2048 + 128)]
        qth = QT_s.at[pl.ds(pl.multiple_of(h * 128, 128), 7 * 2048 + 128)]
        rows = pl.ds(pl.multiple_of(jnp.minimum(h, NCH - 1) * CH, CH), CH)

        def rep(t, n):
            return jnp.concatenate([taps[t, rows, :]] * n, axis=1)

        toks = []

        def due():
            for t in toks:
                t[0] -= 1
            ready = [t[1] for t in toks if t[0] <= 0]
            toks[:] = [t for t in toks if t[0] > 0]
            return functools.reduce(lambda x, y: x | y, ready) if ready else None

        def gate_later(vals):
            toks.append([SLAG, _tok([v if v.dtype == u32 else _u(v) for v in vals])])

        def row_offset(i):
            if i not in st['mfin']:
                m = m_s[i % 2][0, 0]
                for t in range(1, i + 1):
                    m = jnp.maximum(m, m_s[i % 2][0, t])
                m = jnp.max(m, axis=0, keepdims=True)
                if i > 0:
                    lo_ = jnp.exp2(m_s[i % 2][0, 0] - m)
                    for t in range(1, i + 1):
                        lo_ = lo_ + jnp.exp2(m_s[i % 2][0, t] - m)
                    m = m + jnp.log2(jnp.sum(lo_, axis=0, keepdims=True))
                st['mfin'][i] = m
            return st['mfin'][i]

        for op in _schedule():
            kind = op[0]
            if kind == 'KV':
                _, p, t = op
                n, m = SK[t // 7], SV[t % 7]

                def wblk(q):
                    w = jnp.concatenate([w1h[k * 2048:k * 2048 + 128, n * 128:(n + 1) * 128]
                                         for k in (2 * (q % 2), 2 * (q % 2) + 1)], axis=1)
                    r = (q // 2) * 32
                    return jnp.concatenate([w[r:r + 32], w[64 + r:64 + r + 32]], axis=0)

                cols = slice((n * 7 + m) * 256, (n * 7 + m + 1) * 256)
                if m in (2, 3):
                    w = wblk(0 if m == 2 else 3)
                elif p > 0:
                    w = w2_s[:, cols]
                else:
                    i1, i2, sg = _A_OF[m]
                    x, y = wblk(i1), wblk(i2)
                    w = (_f(x) + _f(y) if sg > 0 else _f(x) - _f(y)).astype(bf16)
                    w2_s[z64, cols] = _u(w)
                c2 = c2_s[p * 128:(p + 1) * 128, (n * 7 + m) * 128:(n * 7 + m + 1) * 128]
                st['M'][m] = st['last'] = _nn(w if w.dtype == bf16 else _b(_gate(w, due())), _b(c2))
                if t % 7 < 6:
                    continue
                mo = _quad(*_c4(st['M']))
                for o, sg in _C_OF[n]:
                    k = st['cnt'][o] = st['cnt'].get(o, 0) + 1
                    if k == 1:
                        st['co'][o] = mo if sg > 0 else -mo
                    else:
                        st['co'][o] = st['co'][o] + mo if sg > 0 else st['co'][o] - mo
                    if k == _C_CNT[o]:
                        st['cnt'][o] = 0
                        st['fin'].add(o)
                for tok in range(2):
                    if not {tok, 2 + tok} <= st['fin']:
                        continue
                    st['fin'] -= {tok, 2 + tok}
                    c = 2 * p + tok

                    def full(dh, kb, off):
                        x = st['co'][2 * dh + tok][:, kb * 128:(kb + 1) * 128]
                        return jnp.concatenate([x[off:off + 64], x[128 + off:128 + off + 64]], axis=0)

                    kb4 = (full(0, 0, 0).T, full(1, 0, 0).T, full(0, 1, 0).T, full(1, 1, 0).T)
                    vb4 = (full(0, 0, 64), full(0, 1, 64), full(1, 0, 64), full(1, 1, 64))
                    for ref, c4 in ((K_s[c], kb4), (V_s[c], vb4)):
                        blks = dict(zip((2, 7, 8, 3), c4))
                        if c < NT - 1:
                            blks.update({k: x for k, x in enumerate(_a7(*c4)) if k not in (2, 3)})
                        for k, x in blks.items():
                            ref[z64, k * 128:(k + 1) * 128] = _u(x.astype(bf16))
            elif kind == 'QK':
                _, i, j = op
                S_s = (S0_s, S1_s)[i % 2]
                if j < i:
                    if i not in st['Q7']:
                        qu = qth[i * 2048:i * 2048 + 128, :]
                        st['Q7'][i] = _combos(_b7, [qu[:64, :128], qu[:64, 128:], qu[64:, :128], qu[64:, 128:]])
                    s = _quad(*_c4({n: _nn(_b(tile(K_s[j], n)), st['Q7'][i][n]) for n in SQ}))
                    S_s[zs, j] = s
                    f = _fold(s, jnp.max)
                else:
                    q = _b(qth[i * 2048:i * 2048 + 128, :])
                    sa = _nn(_b(jnp.concatenate([tile(K_s[j], 2), tile(K_s[j], 7)], axis=1)), q)
                    sa = jnp.concatenate([jnp.where(tri, sa[:, :128], NEG), sa[:, 128:]], axis=1)
                    sb = _nn(_b(jnp.concatenate([tile(K_s[j], 8), tile(K_s[j], 3)], axis=1)), q[:, 128:])
                    sb = jnp.where(tri, sb, NEG)
                    S_s[zs, j, 0:128, :] = sa
                    S_s[zs, j, 128:T, 128:T] = sb
                    fa = _fold(sa, jnp.max)
                    f = jnp.concatenate([fa[:, :128], jnp.maximum(fa[:, 128:], _fold(sb, jnp.max))], axis=1)
                m_s[i % 2][zs, j] = f
                pace_s[zs] = f
            elif kind == 'EX':
                _, i, j = op
                S_s = (S0_s, S1_s)[i % 2]
                m = row_offset(i)
                m = jnp.where(pace_s[0, 0:1, :] == jnp.inf, jnp.inf, m)
                if j < i:
                    parts, lj = [], None
                    for r in range(112, -16, -16):
                        pt = jnp.exp2(S_s[0, j, r:r + 16, :] - m)
                        pb = jnp.exp2(S_s[0, j, 128 + r:128 + r + 16, :] - m)
                        parts.insert(0, _b7(pt[:, :128], pt[:, 128:], pb[:, :128], pb[:, 128:]))
                        x = (pt[:8] + pt[8:]) + (pb[:8] + pb[8:])
                        lj = x if lj is None else lj + x
                    st['P'][i, j] = [jnp.concatenate([x[n] for x in parts], axis=0).astype(bf16) for n in range(7)]
                else:
                    pa = jnp.exp2(S_s[0, j, 0:128, :] - m)
                    pb = jnp.exp2(S_s[0, j, 128:T, 128:T] - m[:, 128:])
                    la = _rsum(pa)
                    lj = jnp.concatenate([la[:, :128], la[:, 128:] + _rsum(pb)], axis=1)
                    st['P'][i, j] = (pa.astype(bf16), pb.astype(bf16))
                l_s[i % 2][zs, j] = lj
            elif kind == 'PV':
                _, i, j = op
                p = st['P'].pop((i, j))
                if j < i:
                    for n in SP:
                        st['last'] = _nn(_b(tile(V_s[j], n)), p[n])
                        st['o'][i, n] = st['o'][i, n] + st['last'] if j > 0 else st['last']
                    continue
                oa = _nn(_b(jnp.concatenate([tile(V_s[j], 2), tile(V_s[j], 8)], axis=0)), p[0])
                ob = _nn(_b(jnp.concatenate([tile(V_s[j], 7), tile(V_s[j], 3)], axis=0)), p[1])
                o = st['last'] = jnp.concatenate([oa[:, :128], oa[:, 128:] + ob], axis=1)
                if i > 0:
                    o = o + _quad(*_c4({n: st['o'].pop((i, n)) for n in range(7)}))
                l = l_s[i % 2][0, 0]
                for t in range(1, i + 1):
                    l = l + l_s[i % 2][0, t]
                o = o * (1.0 / jnp.sum(l, axis=0, keepdims=True))
                for n, x in enumerate(_b7(o[:128, :128], o[:128, 128:], o[128:, :128], o[128:, 128:])):
                    O_s[i][zs, n] = x.astype(bf16)
            elif kind == 'PACE':
                pace_s[zs] = jnp.concatenate([st['last'][-8:, -128:]] * 2, axis=1)
            elif kind == 'OP':
                _, i, t = op
                n = SO[t]
                st['M'][n] = st['last'] = _nn(_b(_gate(tile(W7_s, n), due())), O_s[i][0, n])
                if t == 6:
                    acc[:, T * i:T * (i + 1)] += _quad(*_c4(st['M']))
            elif kind == 'W7':
                res = []
                for r0 in range(16 * op[1], 16 * op[2], 16):
                    blk = [_u(woT[h, r:r + 16, c:c + 128]) for r in (r0, 224 + r0) for c in (0, 128)]
                    row = pl.ds(pl.multiple_of(zs * 8 + r0 // 2, 8), 8)
                    for n, x in enumerate(_combos(_a7, blk)):
                        W7_s[row, n * 128:(n + 1) * 128] = _u(x)
                    res += blk
                gate_later(res)
            elif kind == 'AT':
                g = jnp.clip((h - 4) // 4, 0, 2)
                t0 = jnp.minimum(((h + 12) % 4) * 6, NB - 6)
                grow = pl.ds(pl.multiple_of(g * 128, 128), 128)
                gcol = pl.ds(pl.multiple_of(jnp.where(h == H - 1, 3, g) * 128, 128), 128)
                res = []
                for n in range(6):
                    tok = pl.ds(pl.multiple_of((t0 + n) * 128, 128), 128)
                    x = aT_s[grow, tok].T
                    out_s[tok, gcol] = x
                    res.append(_u(x)[56:])
                gate_later(res)
            elif kind == 'HD':
                g = op[1]
                hs = jnp.concatenate([ssmk[rows, c * P:(c + 1) * P] for c in range(4 * g, 4 * g + 4)], axis=0)
                hf = _nn(hs, ff_s[...])
                for n in range(4):
                    X_s[(zs, HR) + blk_at(4 * g + n)] = hf[n * CH:(n + 1) * CH, :P]
                    X_s[(zs, HI) + blk_at(4 * g + n)] = hf[n * CH:(n + 1) * CH, P:]
            elif kind == 'SC':
                g = op[1]
                if g == 0:
                    k = jnp.concatenate([jnp.zeros((CH, P), f32), kT[rows, 0:4 * P].astype(f32)], axis=1)
                else:
                    k = kT[rows, (4 * g - 1) * P:(4 * g + 4) * P].astype(f32)
                ks = k[:, P:] * rep(0, 4)
                for j in range(1, KS):
                    ks = ks + pltpu.roll(k, j, 1)[:, P:] * rep(j, 4)
                kv = ks * vT[rows, 4 * g * P:(4 * g + 4) * P].astype(f32)
                kvs = jnp.concatenate([kv[:, n * P:(n + 1) * P] for n in range(4)], axis=0)
                xf = _nn(kvs.astype(bf16), ff_s[...])
                for n in range(4):
                    c = 4 * g + n
                    xr, xi = xf[n * CH:(n + 1) * CH, :P], xf[n * CH:(n + 1) * CH, P:]
                    X_s[(zs, KV) + blk_at(c)] = kvs[n * CH:(n + 1) * CH]
                    pr = xr if c == 0 else xr - sgn * st['x'][1]
                    pi = xi if c == 0 else xi + sgn * st['x'][0]
                    X_s[(zs, PR) + blk_at(c)] = pr
                    X_s[(zs, PI) + blk_at(c)] = pi
                    st['x'] = (xr, xi)
            elif kind == 'CV':
                res = []
                for a, half in op[1]:
                    wr = wi = None
                    for j in range(a + 1):
                        hr, hi_ = X_s[(0, HR) + blk_at(j, half)], X_s[(0, HI) + blk_at(j, half)]
                        pr, pi = X_s[(0, PR) + blk_at(a - j, half)], X_s[(0, PI) + blk_at(a - j, half)]
                        tr, ti = hr * pr - hi_ * pi, hr * pi + hi_ * pr
                        wr, wi = (tr, ti) if wr is None else (wr + tr, wi + ti)
                    r0 = (a % 4) * CH + 16 * half
                    Y_s[a // 4][zs, r0:r0 + 16, :P] = wr
                    Y_s[a // 4][zs, r0:r0 + 16, P:] = wi
                    res += [wr, wi]
                gate_later(res)
            elif kind == 'ID':
                g = op[1]
                y = _nn(Y_s[g][0].astype(bf16), fi_s[...])
                for n in range(4):
                    c = 4 * g + n
                    cols = slice(c * P, (c + 1) * P)
                    ya = y[n * CH:(n + 1) * CH, :] + X_s[(0, KV) + blk_at(c)] * taps[KS, rows, :]
                    aT_s[rows, cols] = (qT[rows, cols].astype(f32) * ya).astype(bf16)
        return carry

    jax.lax.fori_loop(0, H, head_body, 0)

    acc[:, T * (NT - 1):] += _quad(*_c4({n: _nn(_b(tile(W7_s, n)), O_s[NT - 1][0, n]) for n in SORD}))
    outs = [c_outa]
    for i in range(NT):
        cols = slice(T * i, T * (i + 1))
        blk = jnp.concatenate([aT_s[384:M, cols], acc[:, cols].astype(bf16)], axis=0)
        out_s[cols, 384:2 * M] = blk.T
        c = cp(out_s.at[pl.ds(T * i, T), pl.ds(384, 512)], out_hbm.at[pl.ds(T * i, T), pl.ds(384, 512)], sem_o.at[i])
        c.start()
        outs.append(c)
    for c in outs:
        c.wait()


@jax.jit
def pallas_concat_heads__ssm_conv_h3__compressed_kv_cla__prompt_kernel(
    A_q: jax.Array,
    A_k: jax.Array,
    A_v: jax.Array,
    A_shift_k: jax.Array,
    A_ssm_k: jax.Array,
    A_ssm_D: jax.Array,
    B_x: jax.Array,
    B_c_kv: jax.Array,
    B_w_q: jax.Array,
    B_w_uk: jax.Array,
    B_w_uv: jax.Array,
    B_w_o: jax.Array,
):
    hbm = pl.BlockSpec(memory_space=pl.ANY)
    V = pltpu.VMEM
    out = pl.pallas_call(
        _kernel,
        out_shape=jax.ShapeDtypeStruct((S, 2 * M), bf16),
        in_specs=[hbm] * 12,
        out_specs=hbm,
        scratch_shapes=[
            V((M, S), bf16), V((M, S), bf16), V((M, S), bf16), V((M, S), bf16),
            V((4 * M, 2 * T), bf16), V((S + 16, DC), bf16),
            V((2, M * H, 128), bf16),
            V((2, 4, 128 * H + 16, 128), bf16), V((2, 4, 128 * H + 16, 128), bf16),
            V((H, M, D), bf16),
            V((H * 64, 7 * 256), u32),
            V((4 * H * 128, 7 * 128), u32), V((64, 49 * 256), u32),
            V((512 + 8, 512), u32),
            V((NT * H * 128, T), u32), V((4 * 128, 49 * 128), u32),
            V((M, S), f32), V((M, S), bf16), V((S, 2 * M), bf16),
            V((KS + 1, M, 128), f32), V((P, 2 * P), bf16), V((2 * P, P), bf16),
            V((KS, M), bf16), V((M,), bf16),
            V((1, NT, T, T), f32), V((1, NT, T, T), f32), V((1, 5, T, T), f32),
            V((112, 7 * 128), u32), V((1, 8, T), f32),
            V((1, NT, 8, T), f32), V((1, NT, 8, T), f32), V((1, NT, 8, T), f32), V((1, NT, 8, T), f32),
            pltpu.SemaphoreType.DMA((24,)), pltpu.SemaphoreType.DMA((8,)),
            pltpu.SemaphoreType.DMA((8,)), pltpu.SemaphoreType.DMA((9,)),
        ] + [V((64, 9 * 128), u32)] * (2 * NT) + [V((1, 7, 128, 128), bf16)] * NT
        + [V((1, 4 * CH, 2 * P), f32)] * 4,
        compiler_params=pltpu.CompilerParams(vmem_limit_bytes=126 * 1024 * 1024,
                                             shape_invariant_numerics=False,
                                             disable_bounds_checks=True, disable_semaphore_checks=True),
    )(
        A_q[0].T, A_k[0].T, A_v[0].T, A_shift_k.T, A_ssm_k, A_ssm_D,
        B_x[0].T, B_c_kv[0],
        B_w_q.reshape(M * H, D), B_w_uk.reshape(DC * H, D), B_w_uv.reshape(DC * H, D),
        jnp.transpose(B_w_o, (0, 2, 1)),
    )
    return out[None]
```

```python
import functools
import math

import jax
import jax.numpy as jnp
import jax.experimental.pallas as pl
import jax.experimental.pallas.tpu as pltpu

bf16 = jnp.bfloat16
f32 = jnp.float32
u32 = jnp.uint32

S = 2048
M = 448
DC = 1024
H = 16
D = 256
KS = 4
P = 128
NB = S // P
CH = 32
NCH = M // CH
T = 256
NT = S // T
NEG = -1e30

SORD = tuple(int(c) for c in '6430125')
SK = tuple(int(c) for c in '0364152')
SV = tuple(int(c) for c in '0125364')
SQ = tuple(int(c) for c in '6043125')
SP = tuple(int(c) for c in '3640125')
SO = tuple(int(c) for c in '3640125')
QW1 = 56
QW2 = 140
QW3 = 208
QW4 = 222
QC1 = 165
QLAG = 12
CVMAX = 12
SIDE0 = 26
SIDEP = 4
SLAG = 5
PRE = 0
W7P = 16
W7D = 6
KVH = 42
EXB = 6
NOP6 = 2
LA = 3
C2N = 64
C2S = 16
KVO = -1
OPF = 0
QK0 = 3
ATP = 0
NOP = 2


def _nn(a, b):
    return jnp.dot(a, b, preferred_element_type=f32)


def _b(u):
    return pltpu.bitcast(u, bf16)


def _u(x):
    return pltpu.bitcast(x, u32)


def _lo(u):
    return pltpu.bitcast(u << 16, f32)


def _hi(u):
    return pltpu.bitcast(u & jnp.uint32(0xFFFF0000), f32)


def _f(u):
    return _b(u).astype(f32)


def _a7(a11, a12, a21, a22):
    return [a11 + a22, a21 + a22, a11, a22, a11 + a12, a21 - a11, a12 - a22]


def _b7(b11, b12, b21, b22):
    return [b11 + b22, b11, b12 - b22, b21 - b11, b22, b11 + b12, b21 + b22]


def _c4(m):
    return m[0] + m[3] - m[4] + m[6], m[2] + m[4], m[1] + m[3], m[0] - m[1] + m[2] + m[5]


_C_OF = (((0, 1), (3, 1)), ((2, 1), (3, -1)), ((1, 1), (3, 1)), ((0, 1), (2, 1)), ((0, -1), (1, 1)), ((3, 1),), ((0, 1),))
_C_CNT = (4, 2, 2, 4)
_A_OF = {0: (0, 3, 1), 1: (2, 3, 1), 4: (0, 1, 1), 5: (2, 0, -1), 6: (1, 3, -1)}


def _combos(f7, blk):
    x = f7(*[_f(v) for v in blk])
    plain = {2: 0, 3: 3} if f7 is _a7 else {1: 0, 4: 3}
    return [_b(blk[plain[n]]) if n in plain else x[n].astype(bf16) for n in range(7)]


def _quad(c11, c12, c21, c22):
    return jnp.concatenate([jnp.concatenate([c11, c12], axis=1), jnp.concatenate([c21, c22], axis=1)], axis=0)


def _fold(c, op):
    return op(c.reshape(-1, 8, c.shape[1]), axis=0)


def _rsum(p):
    cols = []
    for c in range(0, p.shape[1], 128):
        acc = None
        for r in range(112, -16, -16):
            t = p[r:r + 8, c:c + 128] + p[r + 8:r + 16, c:c + 128]
            acc = t if acc is None else acc + t
        cols.append(acc)
    return jnp.concatenate(cols, axis=1) if len(cols) > 1 else cols[0]


def _tok(vals):
    parts = []
    for v in vals:
        for r in range(0, v.shape[0], 8):
            for c in range(0, v.shape[1], 128):
                parts.append(v[r:r + 8, c:c + 128])
    while len(parts) > 1:
        parts = [parts[i] | parts[i + 1] if i + 1 < len(parts) else parts[i] for i in range(0, len(parts), 2)]
    return (parts[0] >> 31) >> 1


def _gate(x, tok):
    if tok is None:
        return x
    top = x[:8, :128] | tok
    if x.shape[1] > 128:
        top = jnp.concatenate([top, x[:8, 128:]], axis=1)
    return jnp.concatenate([top, x[8:]], axis=0)


def _side_pieces():
    ps = [(k, g) for g in range(PRE) for k in ('HD', 'SC')]
    cur, cost = [], 0
    for a in range(NB):
        if a % 4 == 0 and a // 4 + PRE < 4:
            ps += [('HD', a // 4 + PRE), ('SC', a // 4 + PRE)]
        for half in range(2):
            if cur and cost + a + 1 > CVMAX:
                ps.append(('CV', tuple(cur)))
                cur, cost = [], 0
            cur.append((a, half))
            cost += a + 1
        if a % 4 == 3:
            ps += [('CV', tuple(cur)), ('ID', a // 4)]
            cur, cost = [], 0
    ps.insert(ATP, ('AT',))
    ps.insert(W7P, ('W7', 0, 7))
    ps.insert(W7P + W7D, ('W7', 7, 14))
    return ps


def _schedule():
    side = _side_pieces()
    out = []
    cnt = [0]

    def block(subs, att, with_side):
        for k, u in enumerate(subs):
            out.append(u)
            out.extend(att.get(k, []))
            if with_side:
                cnt[0] += 1
                if side and cnt[0] >= SIDE0 and (cnt[0] - SIDE0) % SIDEP == 0:
                    out.append(side.pop(0))

    def kv(p, half):
        return [('KV', p, t) for t in (range(KVH) if half == 0 else range(KVH, 49))]

    def op_(*idx):
        return [('OP', i, t) for i in idx for t in range(7)]

    def softmax_head(i, n):
        att = {max(n - EXB, 0): [('PACE',), ('EX', i, 0)]}
        for k in range(1, min(LA, i + 1)):
            att.setdefault(n - 1 - (LA - 1 - k) * 2, []).extend([('PACE',), ('EX', i, k)])
        return att

    ops_left = list(range(NT - 1))
    if OPF:
        block(op_(NT - 1), {}, False)
    block(kv(0, 0) + kv(0, 1), {}, True)
    if not OPF:
        block(op_(NT - 1), {}, False)
    att = softmax_head(0, KVH)
    if QK0 < 0:
        out.append(('QK', 0, 0))
    else:
        att.setdefault(QK0, []).insert(0, ('QK', 0, 0))
    block(kv(1, 0), att, True)
    for i in range(NT - 1):
        for j in range(i + 1):
            out.append(('QK', i + 1, j))
            if j + LA <= i:
                out.append(('EX', i, j + LA))
            out.append(('PV', i, j))
        out.append(('QK', i + 1, i + 1))
        if i < 5:
            subs = kv((i + 3) // 2, (i + 1) % 2)
            block(subs, softmax_head(i + 1, len(subs)), True)
        else:
            n = NOP6 if i == 5 else NOP
            block(op_(*ops_left[:n]), softmax_head(i + 1, 7 * n), False)
            del ops_left[:n]
    out.append(('PACE',))
    for j in range(NT):
        if j + LA < NT:
            out.append(('EX', NT - 1, j + LA))
        out.append(('PV', NT - 1, j))
        if len(ops_left) > 2:
            block(op_(ops_left.pop(0)), {}, False)
        out.append(('PACE',))
    block(op_(*ops_left), {}, False)
    assert not side
    w7 = [k for k, o in enumerate(out) if o[0] == 'W7']
    assert out.index(('OP', NT - 1, 6)) < min(w7) and max(w7) < out.index(('OP', 0, 0))
    out.remove(('ID', 3))
    out.append(('ID', 3))
    return out


def _kernel(qT_hbm, kT_hbm, vT_hbm, sk_hbm, ssmk_hbm, dd_hbm, xT_hbm, ckv_hbm,
            wq_hbm, wk_hbm, wv_hbm, woT_hbm, out_hbm,
            qT, kT, vT, ssmk, xT, ckv, wq_raw, wk_raw, wv_raw, woT,
            aq_s, w1_s, w2_s, cT_s, QT_s, c2_s, acc, aT_s, out_s, taps, ff_s, fi_s,
            sk_ref, dd_ref, S0_s, S1_s, X_s, W7_s, pace_s, m0_s, m1_s, l0_s, l1_s,
            sem, sem_k, sem_v, sem_o, *rest):
    K_s, V_s, O_s, Y_s = rest[:NT], rest[NT:2 * NT], rest[2 * NT:3 * NT], rest[3 * NT:]

    def cp(src, dst, s):
        return pltpu.make_async_copy(src, dst, s)

    def c_x(j):
        cols = pl.ds(pl.multiple_of(j * 2 * T, 2 * T), 2 * T)
        return cp(xT_hbm.at[:, cols], xT.at[pl.ds(pl.multiple_of(j * M, 16), M)], sem.at[j])

    QP = ((0, 128), (128, 96))

    def c_wq(k):
        r = pl.ds((k % 2) * 224 * H, 224 * H)
        return cp(wq_hbm.at[r, pl.ds(128 * (k // 2), 128)], wq_raw.at[k // 2, r], sem.at[18 + k])

    def c_w(w_hbm, raw, sm, j, half, g):
        r = pl.ds(pl.multiple_of((half * 4 + j) * 2048, 2048), 2048)
        q = 2 * half + g
        return cp(w_hbm.at[r, pl.ds(128 * g, 128)], raw.at[j % 2, q, pl.ds(0, 2048)], sm.at[(j % 2) * 4 + q])

    def c_wk(j):
        return [c_w(wk_hbm, wk_raw, sem_k, j, half, g) for half in range(2) for g in range(2)]

    def c_wv(j):
        return [c_w(wv_hbm, wv_raw, sem_v, j, half, g) for half in range(2) for g in range(2)]

    def c_ckv(j):
        r = pl.ds(pl.multiple_of(j * 2 * T, 2 * T), 2 * T)
        return cp(ckv_hbm.at[r], ckv.at[r], sem.at[9 + j])

    a_pairs = ((kT_hbm, kT), (vT_hbm, vT), (ssmk_hbm, ssmk), (qT_hbm, qT))
    c_early = [cp(woT_hbm.at[pl.ds(0, 1)], woT.at[pl.ds(0, 1)], sem.at[4])]
    c_early += [cp(src.at[pl.ds(0, CH)], dst.at[pl.ds(0, CH)], sem.at[5 + n]) for n, (src, dst) in enumerate(a_pairs)]
    c_late = [cp(woT_hbm.at[pl.ds(1, H - 1)], woT.at[pl.ds(1, H - 1)], sem.at[13])]
    c_late += [cp(src.at[pl.ds(CH, M - CH)], dst.at[pl.ds(CH, M - CH)], sem.at[14 + n])
               for n, (src, dst) in enumerate(a_pairs)]
    c_small = [cp(sk_hbm, sk_ref, sem.at[22]), cp(dd_hbm, dd_ref, sem.at[23])]
    for c in c_small + [c_wq(k) for k in (0, 3, 2, 1)] + [c_x(0)]:
        c.start()
    for c in c_wk(0):
        c.start(priority=1)

    n_i = jax.lax.broadcasted_iota(jnp.int32, (P, P), 0)
    k_i = jax.lax.broadcasted_iota(jnp.int32, (P, P), 1)
    ang = (((2 * k_i + 1) * n_i) & 511).astype(f32) * (math.pi / 256.0)
    cs, sn = jnp.cos(ang), jnp.sin(ang)
    ff_s[:, 0:P] = cs.astype(bf16)
    ff_s[:, P:2 * P] = (-sn).astype(bf16)
    fi_s[0:P, :] = (cs.T * (1.0 / P)).astype(bf16)
    fi_s[P:2 * P, :] = (sn.T * (-1.0 / P)).astype(bf16)
    acc[...] = jnp.zeros(acc.shape, f32)
    for c in c_small:
        c.wait()
    sk = sk_ref[...].astype(f32)
    for t in range(KS):
        taps[t] = jnp.broadcast_to(sk[t:t + 1, :], (128, M)).T
    taps[KS] = jnp.broadcast_to(dd_ref[...].astype(f32).reshape(1, M), (128, M)).T
    aT_s[...] = jnp.zeros(aT_s.shape, bf16)
    O_s[NT - 1][...] = jnp.zeros(O_s[0].shape, bf16)
    W7_s[...] = jnp.zeros(W7_s.shape, u32)
    cT_s[...] = jnp.zeros(cT_s.shape, u32)

    vq = wq_raw.bitcast(u32)
    ut = {}
    for k, ready in ((0, ()), (3, (0, 2, 3)), (2, (1, 5)), (1, (4, 6))):
        c_wq(k).wait()
        for hp in range(H // 2):
            for c0, nc in QP:
                ut[k, hp, c0] = vq[k // 2, pl.ds(((k % 2) * 224 + c0) * 8 + hp, nc, stride=8), :].T
                for r in range(0, 128, 16):
                    for par, f in enumerate((_lo, _hi)):
                        r0 = (2 * hp + par) * 64 + r // 2
                        for n in ready:
                            i1, i2, sg = _A_OF.get(n, (0 if n == 2 else 3, None, 0))
                            x = f(ut[i1, hp, c0][r:r + 16])
                            if i2 is not None:
                                y = f(ut[i2, hp, c0][r:r + 16])
                                x = x + y if sg > 0 else x - y
                            aq_s[r0:r0 + 8, n * 256 + c0:n * 256 + c0 + nc] = _u(x.astype(bf16))
    for c in c_wv(0) + [c_ckv(0)]:
        c.start(priority=1)

    qscale = (D ** -0.5) * math.log2(math.e)

    def prep_c2(jj, r):
        blk = [[cT_s[cq * 128 + r:cq * 128 + r + 8, tb * 128:(tb + 1) * 128] for tb in range(4)] for cq in range(4)]
        x = [[_f(v) for v in row] for row in blk]
        outer = [[_b7(x[ci][ti], x[ci][2 + ti], x[2 + ci][ti], x[2 + ci][2 + ti]) for ti in range(2)]
                 for ci in range(2)]
        two = [_b7(outer[0][0][n], outer[0][1][n], outer[1][0][n], outer[1][1][n]) for n in range(7)]
        cj = c2_s.at[pl.ds(pl.multiple_of(jj * 128, 128), 128)]
        for n in range(7):
            for m in range(7):
                cj[r:r + 8, (n * 7 + m) * 128:(n * 7 + m + 1) * 128] = _u(two[n][m].astype(bf16))
        return []

    def q_body(j, carry):
        mq = {}
        qtj = QT_s.at[pl.ds(pl.multiple_of(j * 4096, 4096), 4096)]
        zq = j >> 4
        c_x(j).wait()
        xj = xT.at[pl.ds(pl.multiple_of(j * M, 16), M)]
        bx = [_combos(_b7, [_u(xj[r:r + 224, c:c + 128]) for r in (0, 224) for c in (t * T, t * T + 128)])
              for t in range(2)]

        def qproj(u, tok):
            hh, t, n = u // 14, (u // 7) % 2, SORD[u % 7]
            w = _b(_gate(aq_s[hh * 64:hh * 64 + 64, n * 256:n * 256 + 224], tok))
            mq[n] = _nn(w, bx[t][n])
            if u % 7 == 6:
                for k, x in enumerate(_c4(mq)):
                    r0 = t * 2048 + hh * 128 + (k // 2) * 64
                    qtj[r0:r0 + 64, (k % 2) * 128:(k % 2 + 1) * 128] = _u((x * qscale).astype(bf16))
            return mq[n]

        wt = {}
        ckj = ckv.at[pl.ds(pl.multiple_of(j * 512, 512), 512)]
        w1j = w1_s.at[pl.ds(pl.multiple_of(j * 2048, 2048), 2048)]

        def prep_w(kv, hp, part):
            if part == 0:
                v = (wk_raw, wv_raw)[kv].bitcast(u32).at[j % 2]
                wt[kv, hp] = [v[q, pl.ds(hp, 128, stride=8), :].T for q in (0, 2, 1, 3)]
                return [x[120:] for x in wt[kv, hp]]
            for r in range(32 * (part - 1), 32 * part, 16):
                u = [x[r:r + 16] for x in wt[kv, hp]]
                for par, f in enumerate((_lo, _hi)):
                    r0 = (2 * hp + par) * 128 + kv * 64 + r // 2
                    for n, c in enumerate(_a7(*[f(x) for x in u])):
                        w1j[r0:r0 + 8, n * 128:(n + 1) * 128] = _u(c.astype(bf16))
            return []

        def prep_ct(half, cq):
            res = []
            ct = 2 * cq + half
            for tb in range(4):
                x = _u(ckj[tb * 128:(tb + 1) * 128, ct * 128:(ct + 1) * 128].T)
                cT_s[pl.ds(pl.multiple_of(zq * 64 + ct * 64, 64), 64), tb * 128:(tb + 1) * 128] = x
                res.append(x[56:])
            return res

        fill = {}

        def spread(pieces, u0, u1):
            for n, p in enumerate(pieces):
                fill.setdefault(u0 + n * (u1 - u0) // len(pieces), []).append(p)

        spread([functools.partial(prep_w, 0, hp, part) for hp in range(8) for part in range(5)], QW1, QW2)
        spread([functools.partial(prep_w, 1, hp, part) for hp in range(8) for part in range(5)], QW2, QW3)
        spread([functools.partial(prep_ct, 0, cq) for cq in range(4)], QW2 + 2, QC1)
        spread([functools.partial(prep_ct, 1, cq) for cq in range(4)], QC1, QW3)
        spread([functools.partial(prep_c2, jnp.maximum(j - 1, 0), r) for r in range(C2N, 128, 8)], C2S, QW1 - 4)
        if C2N:
            spread([functools.partial(prep_c2, j, r) for r in range(0, C2N, 8)], QW3, QW4)
        toks = {}
        for u in range(224):
            if u == QW1:
                @pl.when(j < 3)
                def _():
                    for c in c_wk(j + 1):
                        c.start(priority=1)

                @pl.when(j == 3)
                def _():
                    for c in c_early + c_late:
                        c.start(priority=1)

                for c in c_wk(j):
                    c.wait()
            if u == QW2:
                @pl.when(j < 3)
                def _():
                    for c in [c_x(j + 1)] + c_wv(j + 1) + [c_ckv(j + 1)]:
                        c.start(priority=1)

                for c in c_wv(j) + [c_ckv(j)]:
                    c.wait()
            q = qproj(u, toks.pop(u, None))
            res = []
            ps = fill.get(u, [])
            for n, p in enumerate(ps):
                row = (n * 128 // len(ps)) // 16 * 16
                if p.func is prep_w and p.args[2] == 0:
                    (wk_raw, wv_raw)[p.args[0]].bitcast(u32)[zq, 0, 1024:1032, :] = _u(q[row:row + 8])
                elif p.func is prep_c2:
                    cT_s[pl.ds(pl.multiple_of(512 + zq * 8, 8), 8), 0:128] = _u(q[row:row + 8])
                elif p.func is prep_ct:
                    ckv[pl.ds(pl.multiple_of(S + zq * 16, 16), 16), 0:128] = q[row:row + 16].astype(bf16)
                res += p()
            if res:
                toks[u + QLAG] = _tok(res)
        return carry

    jax.lax.fori_loop(0, 4, q_body, 0)
    for r in range(C2N, 128, 8):
        prep_c2(3, r)
    for c in c_early:
        c.wait()

    tri = n_i <= k_i
    sgn = jnp.where((jax.lax.broadcasted_iota(jnp.int32, (1, P), 1) & 1) == 0, 1.0, -1.0).astype(f32)
    c_outa = cp(out_s.at[:, pl.ds(0, 384)], out_hbm.at[:, pl.ds(0, 384)], sem_o.at[8])
    HR, HI, PR, PI, KV = range(5)

    def blk_at(c, half=None):
        r0 = (c % 8) * CH
        rs = slice(r0, r0 + CH) if half is None else slice(r0 + 16 * half, r0 + 16 * half + 16)
        return rs, slice((c // 8) * P, (c // 8 + 1) * P)

    def tile(ref, n):
        return ref[:, n * 128:(n + 1) * 128]

    def head_body(h, carry):
        @pl.when(h == 1)
        def _():
            for c in c_late:
                c.wait()

        @pl.when(h == H - 1)
        def _():
            c_outa.start()

        st = dict(co={}, cnt={}, fin=set(), M={}, P={}, Q7={}, mfin={}, o={})
        zs = h >> 10
        z64 = pl.ds(pl.multiple_of(zs * 64, 64), 64)
        m_s, l_s = (m0_s, m1_s), (l0_s, l1_s)
        w1h = w1_s.at[pl.ds(pl.multiple_of(h * 128, 128), 3 * 2048 + 128)]
        qth = QT_s.at[pl.ds(pl.multiple_of(h * 128, 128), 7 * 2048 + 128)]
        rows = pl.ds(pl.multiple_of(jnp.minimum(h, NCH - 1) * CH, CH), CH)

        def rep(t, n):
            return jnp.concatenate([taps[t, rows, :]] * n, axis=1)

        toks = []

        def due():
            for t in toks:
                t[0] -= 1
            ready = [t[1] for t in toks if t[0] <= 0]
            toks[:] = [t for t in toks if t[0] > 0]
            return functools.reduce(lambda x, y: x | y, ready) if ready else None

        def gate_later(vals):
            toks.append([SLAG, _tok([v if v.dtype == u32 else _u(v) for v in vals])])

        def row_offset(i):
            if i not in st['mfin']:
                m = m_s[i % 2][0, 0]
                for t in range(1, i + 1):
                    m = jnp.maximum(m, m_s[i % 2][0, t])
                m = jnp.max(m, axis=0, keepdims=True)
                if i > 0:
                    lo_ = jnp.exp2(m_s[i % 2][0, 0] - m)
                    for t in range(1, i + 1):
                        lo_ = lo_ + jnp.exp2(m_s[i % 2][0, t] - m)
                    m = m + jnp.log2(jnp.sum(lo_, axis=0, keepdims=True))
                st['mfin'][i] = m
            return st['mfin'][i]

        for op in _schedule():
            kind = op[0]
            if kind == 'KV':
                _, p, t = op
                n, m = SK[t // 7], SV[t % 7]

                def wblk(q):
                    w = jnp.concatenate([w1h[k * 2048:k * 2048 + 128, n * 128:(n + 1) * 128]
                                         for k in (2 * (q % 2), 2 * (q % 2) + 1)], axis=1)
                    r = (q // 2) * 32
                    return jnp.concatenate([w[r:r + 32], w[64 + r:64 + r + 32]], axis=0)

                cols = slice((n * 7 + m) * 256, (n * 7 + m + 1) * 256)
                if m in (2, 3):
                    w = wblk(0 if m == 2 else 3)
                elif p > 0:
                    w = w2_s[:, cols]
                else:
                    i1, i2, sg = _A_OF[m]
                    x, y = wblk(i1), wblk(i2)
                    w = (_f(x) + _f(y) if sg > 0 else _f(x) - _f(y)).astype(bf16)
                    w2_s[z64, cols] = _u(w)
                c2 = c2_s[p * 128:(p + 1) * 128, (n * 7 + m) * 128:(n * 7 + m + 1) * 128]
                st['M'][m] = st['last'] = _nn(w if w.dtype == bf16 else _b(_gate(w, due())), _b(c2))
                if t % 7 < 6:
                    continue
                mo = _quad(*_c4(st['M']))
                for o, sg in _C_OF[n]:
                    k = st['cnt'][o] = st['cnt'].get(o, 0) + 1
                    if k == 1:
                        st['co'][o] = mo if sg > 0 else -mo
                    else:
                        st['co'][o] = st['co'][o] + mo if sg > 0 else st['co'][o] - mo
                    if k == _C_CNT[o]:
                        st['cnt'][o] = 0
                        st['fin'].add(o)
                for tok in range(2):
                    if not {tok, 2 + tok} <= st['fin']:
                        continue
                    st['fin'] -= {tok, 2 + tok}
                    c = 2 * p + tok

                    def full(dh, kb, off):
                        x = st['co'][2 * dh + tok][:, kb * 128:(kb + 1) * 128]
                        return jnp.concatenate([x[off:off + 64], x[128 + off:128 + off + 64]], axis=0)

                    kb4 = (full(0, 0, 0).T, full(1, 0, 0).T, full(0, 1, 0).T, full(1, 1, 0).T)
                    vb4 = (full(0, 0, 64), full(0, 1, 64), full(1, 0, 64), full(1, 1, 64))
                    for ref, c4 in ((K_s[c], kb4), (V_s[c], vb4))[::KVO]:
                        blks = dict(zip((2, 7, 8, 3), c4))
                        if c < NT - 1:
                            blks.update({k: x for k, x in enumerate(_a7(*c4)) if k not in (2, 3)})
                        for k, x in blks.items():
                            ref[z64, k * 128:(k + 1) * 128] = _u(x.astype(bf16))
            elif kind == 'QK':
                _, i, j = op
                S_s = (S0_s, S1_s)[i % 2]
                if j < i:
                    if i not in st['Q7']:
                        qu = qth[i * 2048:i * 2048 + 128, :]
                        st['Q7'][i] = _combos(_b7, [qu[:64, :128], qu[:64, 128:], qu[64:, :128], qu[64:, 128:]])
                    s = _quad(*_c4({n: _nn(_b(tile(K_s[j], n)), st['Q7'][i][n]) for n in SQ}))
                    S_s[zs, j] = s
                    f = _fold(s, jnp.max)
                else:
                    q = _b(qth[i * 2048:i * 2048 + 128, :])
                    sa = _nn(_b(jnp.concatenate([tile(K_s[j], 2), tile(K_s[j], 7)], axis=1)), q)
                    sa = jnp.concatenate([jnp.where(tri, sa[:, :128], NEG), sa[:, 128:]], axis=1)
                    sb = _nn(_b(jnp.concatenate([tile(K_s[j], 8), tile(K_s[j], 3)], axis=1)), q[:, 128:])
                    sb = jnp.where(tri, sb, NEG)
                    S_s[zs, j, 0:128, :] = sa
                    S_s[zs, j, 128:T, 128:T] = sb
                    fa = _fold(sa, jnp.max)
                    f = jnp.concatenate([fa[:, :128], jnp.maximum(fa[:, 128:], _fold(sb, jnp.max))], axis=1)
                m_s[i % 2][zs, j] = f
                pace_s[zs] = f
            elif kind == 'EX':
                _, i, j = op
                S_s = (S0_s, S1_s)[i % 2]
                m = row_offset(i)
                m = jnp.where(pace_s[0, 0:1, :] == jnp.inf, jnp.inf, m)
                if j < i:
                    parts, lj = [], None
                    for r in range(112, -16, -16):
                        pt = jnp.exp2(S_s[0, j, r:r + 16, :] - m)
                        pb = jnp.exp2(S_s[0, j, 128 + r:128 + r + 16, :] - m)
                        parts.insert(0, _b7(pt[:, :128], pt[:, 128:], pb[:, :128], pb[:, 128:]))
                        x = (pt[:8] + pt[8:]) + (pb[:8] + pb[8:])
                        lj = x if lj is None else lj + x
                    st['P'][i, j] = [jnp.concatenate([x[n] for x in parts], axis=0).astype(bf16) for n in range(7)]
                else:
                    pa = jnp.exp2(S_s[0, j, 0:128, :] - m)
                    pb = jnp.exp2(S_s[0, j, 128:T, 128:T] - m[:, 128:])
                    la = _rsum(pa)
                    lj = jnp.concatenate([la[:, :128], la[:, 128:] + _rsum(pb)], axis=1)
                    st['P'][i, j] = (pa.astype(bf16), pb.astype(bf16))
                l_s[i % 2][zs, j] = lj
            elif kind == 'PV':
                _, i, j = op
                p = st['P'].pop((i, j))
                if j < i:
                    for n in SP:
                        st['last'] = _nn(_b(tile(V_s[j], n)), p[n])
                        st['o'][i, n] = st['o'][i, n] + st['last'] if j > 0 else st['last']
                    continue
                oa = _nn(_b(jnp.concatenate([tile(V_s[j], 2), tile(V_s[j], 8)], axis=0)), p[0])
                ob = _nn(_b(jnp.concatenate([tile(V_s[j], 7), tile(V_s[j], 3)], axis=0)), p[1])
                o = st['last'] = jnp.concatenate([oa[:, :128], oa[:, 128:] + ob], axis=1)
                if i > 0:
                    o = o + _quad(*_c4({n: st['o'].pop((i, n)) for n in range(7)}))
                l = l_s[i % 2][0, 0]
                for t in range(1, i + 1):
                    l = l + l_s[i % 2][0, t]
                o = o * (1.0 / jnp.sum(l, axis=0, keepdims=True))
                for n, x in enumerate(_b7(o[:128, :128], o[:128, 128:], o[128:, :128], o[128:, 128:])):
                    O_s[i][zs, n] = x.astype(bf16)
            elif kind == 'PACE':
                pace_s[zs] = jnp.concatenate([st['last'][-8:, -128:]] * 2, axis=1)
            elif kind == 'OP':
                _, i, t = op
                n = SO[t]
                st['M'][n] = st['last'] = _nn(_b(_gate(tile(W7_s, n), due())), O_s[i][0, n])
                if t == 6:
                    acc[:, T * i:T * (i + 1)] += _quad(*_c4(st['M']))
            elif kind == 'W7':
                res = []
                for r0 in range(16 * op[1], 16 * op[2], 16):
                    blk = [_u(woT[h, r:r + 16, c:c + 128]) for r in (r0, 224 + r0) for c in (0, 128)]
                    row = pl.ds(pl.multiple_of(zs * 8 + r0 // 2, 8), 8)
                    for n, x in enumerate(_combos(_a7, blk)):
                        W7_s[row, n * 128:(n + 1) * 128] = _u(x)
                    res += blk
                gate_later(res)
            elif kind == 'AT':
                g = jnp.clip((h - 4) // 4, 0, 2)
                t0 = jnp.minimum(((h + 12) % 4) * 6, NB - 6)
                grow = pl.ds(pl.multiple_of(g * 128, 128), 128)
                gcol = pl.ds(pl.multiple_of(jnp.where(h == H - 1, 3, g) * 128, 128), 128)
                res = []
                for n in range(6):
                    tok = pl.ds(pl.multiple_of((t0 + n) * 128, 128), 128)
                    x = aT_s[grow, tok].T
                    out_s[tok, gcol] = x
                    res.append(_u(x)[56:])
                gate_later(res)
            elif kind == 'HD':
                g = op[1]
                hs = jnp.concatenate([ssmk[rows, c * P:(c + 1) * P] for c in range(4 * g, 4 * g + 4)], axis=0)
                hf = _nn(hs, ff_s[...])
                for n in range(4):
                    X_s[(zs, HR) + blk_at(4 * g + n)] = hf[n * CH:(n + 1) * CH, :P]
                    X_s[(zs, HI) + blk_at(4 * g + n)] = hf[n * CH:(n + 1) * CH, P:]
            elif kind == 'SC':
                g = op[1]
                if g == 0:
                    k = jnp.concatenate([jnp.zeros((CH, P), f32), kT[rows, 0:4 * P].astype(f32)], axis=1)
                else:
                    k = kT[rows, (4 * g - 1) * P:(4 * g + 4) * P].astype(f32)
                ks = k[:, P:] * rep(0, 4)
                for j in range(1, KS):
                    ks = ks + pltpu.roll(k, j, 1)[:, P:] * rep(j, 4)
                kv = ks * vT[rows, 4 * g * P:(4 * g + 4) * P].astype(f32)
                kvs = jnp.concatenate([kv[:, n * P:(n + 1) * P] for n in range(4)], axis=0)
                xf = _nn(kvs.astype(bf16), ff_s[...])
                for n in range(4):
                    c = 4 * g + n
                    xr, xi = xf[n * CH:(n + 1) * CH, :P], xf[n * CH:(n + 1) * CH, P:]
                    X_s[(zs, KV) + blk_at(c)] = kvs[n * CH:(n + 1) * CH]
                    pr = xr if c == 0 else xr - sgn * st['x'][1]
                    pi = xi if c == 0 else xi + sgn * st['x'][0]
                    X_s[(zs, PR) + blk_at(c)] = pr
                    X_s[(zs, PI) + blk_at(c)] = pi
                    st['x'] = (xr, xi)
            elif kind == 'CV':
                res = []
                for a, half in op[1]:
                    wr = wi = None
                    for j in range(a + 1):
                        hr, hi_ = X_s[(0, HR) + blk_at(j, half)], X_s[(0, HI) + blk_at(j, half)]
                        pr, pi = X_s[(0, PR) + blk_at(a - j, half)], X_s[(0, PI) + blk_at(a - j, half)]
                        tr, ti = hr * pr - hi_ * pi, hr * pi + hi_ * pr
                        wr, wi = (tr, ti) if wr is None else (wr + tr, wi + ti)
                    r0 = (a % 4) * CH + 16 * half
                    Y_s[a // 4][zs, r0:r0 + 16, :P] = wr
                    Y_s[a // 4][zs, r0:r0 + 16, P:] = wi
                    res += [wr, wi]
                gate_later(res)
            elif kind == 'ID':
                g = op[1]
                y = _nn(Y_s[g][0].astype(bf16), fi_s[...])
                for n in range(4):
                    c = 4 * g + n
                    cols = slice(c * P, (c + 1) * P)
                    ya = y[n * CH:(n + 1) * CH, :] + X_s[(0, KV) + blk_at(c)] * taps[KS, rows, :]
                    aT_s[rows, cols] = (qT[rows, cols].astype(f32) * ya).astype(bf16)
        return carry

    jax.lax.fori_loop(0, H, head_body, 0)

    acc[:, T * (NT - 1):] += _quad(*_c4({n: _nn(_b(tile(W7_s, n)), O_s[NT - 1][0, n]) for n in SORD}))
    outs = [c_outa]
    for i in range(NT):
        cols = slice(T * i, T * (i + 1))
        blk = jnp.concatenate([aT_s[384:M, cols], acc[:, cols].astype(bf16)], axis=0)
        out_s[cols, 384:2 * M] = blk.T
        c = cp(out_s.at[pl.ds(T * i, T), pl.ds(384, 512)], out_hbm.at[pl.ds(T * i, T), pl.ds(384, 512)], sem_o.at[i])
        c.start()
        outs.append(c)
    for c in outs:
        c.wait()


@jax.jit
def pallas_concat_heads__ssm_conv_h3__compressed_kv_cla__prompt_kernel(
    A_q: jax.Array,
    A_k: jax.Array,
    A_v: jax.Array,
    A_shift_k: jax.Array,
    A_ssm_k: jax.Array,
    A_ssm_D: jax.Array,
    B_x: jax.Array,
    B_c_kv: jax.Array,
    B_w_q: jax.Array,
    B_w_uk: jax.Array,
    B_w_uv: jax.Array,
    B_w_o: jax.Array,
):
    hbm = pl.BlockSpec(memory_space=pl.ANY)
    V = pltpu.VMEM
    out = pl.pallas_call(
        _kernel,
        out_shape=jax.ShapeDtypeStruct((S, 2 * M), bf16),
        in_specs=[hbm] * 12,
        out_specs=hbm,
        scratch_shapes=[
            V((M, S), bf16), V((M, S), bf16), V((M, S), bf16), V((M, S), bf16),
            V((4 * M, 2 * T), bf16), V((S + 16, DC), bf16),
            V((2, M * H, 128), bf16),
            V((2, 4, 128 * H + 16, 128), bf16), V((2, 4, 128 * H + 16, 128), bf16),
            V((H, M, D), bf16),
            V((H * 64, 7 * 256), u32),
            V((4 * H * 128, 7 * 128), u32), V((64, 49 * 256), u32),
            V((512 + 8, 512), u32),
            V((NT * H * 128, T), u32), V((4 * 128, 49 * 128), u32),
            V((M, S), f32), V((M, S), bf16), V((S, 2 * M), bf16),
            V((KS + 1, M, 128), f32), V((P, 2 * P), bf16), V((2 * P, P), bf16),
            V((KS, M), bf16), V((M,), bf16),
            V((1, NT, T, T), f32), V((1, NT, T, T), f32), V((1, 5, T, T), f32),
            V((112, 7 * 128), u32), V((1, 8, T), f32),
            V((1, NT, 8, T), f32), V((1, NT, 8, T), f32), V((1, NT, 8, T), f32), V((1, NT, 8, T), f32),
            pltpu.SemaphoreType.DMA((24,)), pltpu.SemaphoreType.DMA((8,)),
            pltpu.SemaphoreType.DMA((8,)), pltpu.SemaphoreType.DMA((9,)),
        ] + [V((64, 9 * 128), u32)] * (2 * NT) + [V((1, 7, 128, 128), bf16)] * NT
        + [V((1, 4 * CH, 2 * P), f32)] * 4,
        compiler_params=pltpu.CompilerParams(vmem_limit_bytes=126 * 1024 * 1024,
                                             shape_invariant_numerics=False,
                                             disable_bounds_checks=True, disable_semaphore_checks=True),
    )(
        A_q[0].T, A_k[0].T, A_v[0].T, A_shift_k.T, A_ssm_k, A_ssm_D,
        B_x[0].T, B_c_kv[0],
        B_w_q.reshape(M * H, D), B_w_uk.reshape(DC * H, D), B_w_uv.reshape(DC * H, D),
        jnp.transpose(B_w_o, (0, 2, 1)),
    )
    return out[None]
```

```python
import functools
import math

import jax
import jax.numpy as jnp
import jax.experimental.pallas as pl
import jax.experimental.pallas.tpu as pltpu

bf16 = jnp.bfloat16
f32 = jnp.float32
u32 = jnp.uint32

S = 2048
M = 448
DC = 1024
H = 16
D = 256
KS = 4
P = 128
NB = S // P
CH = 32
NCH = M // CH
T = 256
NT = S // T
NEG = -1e30

SORD = tuple(int(c) for c in '6430125')
SK = tuple(int(c) for c in '0364152')
SV = tuple(int(c) for c in '0125364')
SQ = tuple(int(c) for c in '6043125')
SP = tuple(int(c) for c in '3640125')
SO = tuple(int(c) for c in '3640125')
QW1 = 56
QW2 = 140
QW3 = 208
QW4 = 222
QC1 = 165
QLAG = 12
CVMAX = 12
SIDE0 = 26
SIDEP = 4
SLAG = 5
PRE = 0
W7P = 16
W7D = 6
KVH = 42
EXB = 6
NOP6 = 2
LA = 3
C2N = 64
C2S = 16
QK0 = 3
ATP = 0
NOP = 2


def _nn(a, b):
    return jnp.dot(a, b, preferred_element_type=f32)


def _b(u):
    return pltpu.bitcast(u, bf16)


def _u(x):
    return pltpu.bitcast(x, u32)


def _lo(u):
    return pltpu.bitcast(u << 16, f32)


def _hi(u):
    return pltpu.bitcast(u & jnp.uint32(0xFFFF0000), f32)


def _f(u):
    return _b(u).astype(f32)


def _a7(a11, a12, a21, a22):
    return [a11 + a22, a21 + a22, a11, a22, a11 + a12, a21 - a11, a12 - a22]


def _b7(b11, b12, b21, b22):
    return [b11 + b22, b11, b12 - b22, b21 - b11, b22, b11 + b12, b21 + b22]


def _c4(m):
    return m[0] + m[3] - m[4] + m[6], m[2] + m[4], m[1] + m[3], m[0] - m[1] + m[2] + m[5]


_C_OF = (((0, 1), (3, 1)), ((2, 1), (3, -1)), ((1, 1), (3, 1)), ((0, 1), (2, 1)), ((0, -1), (1, 1)), ((3, 1),), ((0, 1),))
_C_CNT = (4, 2, 2, 4)
_A_OF = {0: (0, 3, 1), 1: (2, 3, 1), 4: (0, 1, 1), 5: (2, 0, -1), 6: (1, 3, -1)}


def _combos(f7, blk):
    x = f7(*[_f(v) for v in blk])
    plain = {2: 0, 3: 3} if f7 is _a7 else {1: 0, 4: 3}
    return [_b(blk[plain[n]]) if n in plain else x[n].astype(bf16) for n in range(7)]


def _quad(c11, c12, c21, c22):
    return jnp.concatenate([jnp.concatenate([c11, c12], axis=1), jnp.concatenate([c21, c22], axis=1)], axis=0)


def _fold(c, op):
    return op(c.reshape(-1, 8, c.shape[1]), axis=0)


def _rsum(p):
    cols = []
    for c in range(0, p.shape[1], 128):
        acc = None
        for r in range(112, -16, -16):
            t = p[r:r + 8, c:c + 128] + p[r + 8:r + 16, c:c + 128]
            acc = t if acc is None else acc + t
        cols.append(acc)
    return jnp.concatenate(cols, axis=1) if len(cols) > 1 else cols[0]


def _tok(vals):
    parts = []
    for v in vals:
        for r in range(0, v.shape[0], 8):
            for c in range(0, v.shape[1], 128):
                parts.append(v[r:r + 8, c:c + 128])
    while len(parts) > 1:
        parts = [parts[i] | parts[i + 1] if i + 1 < len(parts) else parts[i] for i in range(0, len(parts), 2)]
    return (parts[0] >> 31) >> 1


def _gate(x, tok):
    if tok is None:
        return x
    top = x[:8, :128] | tok
    if x.shape[1] > 128:
        top = jnp.concatenate([top, x[:8, 128:]], axis=1)
    return jnp.concatenate([top, x[8:]], axis=0)


def _side_pieces():
    ps = [(k, g) for g in range(PRE) for k in ('HD', 'SC')]
    cur, cost = [], 0
    for a in range(NB):
        if a % 4 == 0 and a // 4 + PRE < 4:
            ps += [('HD', a // 4 + PRE), ('SC', a // 4 + PRE)]
        for half in range(2):
            if cur and cost + a + 1 > CVMAX:
                ps.append(('CV', tuple(cur)))
                cur, cost = [], 0
            cur.append((a, half))
            cost += a + 1
        if a % 4 == 3:
            ps += [('CV', tuple(cur)), ('ID', a // 4)]
            cur, cost = [], 0
    ps.insert(ATP, ('AT',))
    ps.insert(W7P, ('W7', 0, 7))
    ps.insert(W7P + W7D, ('W7', 7, 14))
    return ps


def _schedule():
    side = _side_pieces()
    out = []
    cnt = [0]

    def block(subs, att, with_side):
        for k, u in enumerate(subs):
            out.append(u)
            out.extend(att.get(k, []))
            if with_side:
                cnt[0] += 1
                if side and cnt[0] >= SIDE0 and (cnt[0] - SIDE0) % SIDEP == 0:
                    out.append(side.pop(0))

    def kv(p, half):
        return [('KV', p, t) for t in (range(KVH) if half == 0 else range(KVH, 49))]

    def op_(*idx):
        return [('OP', i, t) for i in idx for t in range(7)]

    def softmax_head(i, n):
        att = {max(n - EXB, 0): [('PACE',), ('EX', i, 0)]}
        for k in range(1, min(LA, i + 1)):
            att.setdefault(n - 1 - (LA - 1 - k) * 2, []).extend([('PACE',), ('EX', i, k)])
        return att

    ops_left = list(range(NT - 1))
    block(kv(0, 0) + kv(0, 1), {}, True)
    block(op_(NT - 1), {}, False)
    att = softmax_head(0, KVH)
    att.setdefault(QK0, []).insert(0, ('QK', 0, 0))
    block(kv(1, 0), att, True)
    for i in range(NT - 1):
        for j in range(i + 1):
            out.append(('QK', i + 1, j))
            if j + LA <= i:
                out.append(('EX', i, j + LA))
            out.append(('PV', i, j))
        out.append(('QK', i + 1, i + 1))
        if i < 5:
            subs = kv((i + 3) // 2, (i + 1) % 2)
            block(subs, softmax_head(i + 1, len(subs)), True)
        else:
            n = NOP6 if i == 5 else NOP
            block(op_(*ops_left[:n]), softmax_head(i + 1, 7 * n), False)
            del ops_left[:n]
    out.append(('PACE',))
    for j in range(NT):
        if j + LA < NT:
            out.append(('EX', NT - 1, j + LA))
        out.append(('PV', NT - 1, j))
        if len(ops_left) > 2:
            block(op_(ops_left.pop(0)), {}, False)
        out.append(('PACE',))
    block(op_(*ops_left), {}, False)
    assert not side
    w7 = [k for k, o in enumerate(out) if o[0] == 'W7']
    assert out.index(('OP', NT - 1, 6)) < min(w7) and max(w7) < out.index(('OP', 0, 0))
    out.remove(('ID', 3))
    out.append(('ID', 3))
    return out


def _kernel(qT_hbm, kT_hbm, vT_hbm, sk_hbm, ssmk_hbm, dd_hbm, xT_hbm, ckv_hbm,
            wq_hbm, wk_hbm, wv_hbm, woT_hbm, out_hbm,
            qT, kT, vT, ssmk, xT, ckv, wq_raw, wk_raw, wv_raw, woT,
            aq_s, w1_s, w2_s, cT_s, QT_s, c2_s, acc, aT_s, out_s, taps, ff_s, fi_s,
            sk_ref, dd_ref, S0_s, S1_s, X_s, W7_s, pace_s, m0_s, m1_s, l0_s, l1_s,
            sem, sem_k, sem_v, sem_o, *rest):
    K_s, V_s, O_s, Y_s = rest[:NT], rest[NT:2 * NT], rest[2 * NT:3 * NT], rest[3 * NT:]

    def cp(src, dst, s):
        return pltpu.make_async_copy(src, dst, s)

    def c_x(j):
        cols = pl.ds(pl.multiple_of(j * 2 * T, 2 * T), 2 * T)
        return cp(xT_hbm.at[:, cols], xT.at[pl.ds(pl.multiple_of(j * M, 16), M)], sem.at[j])

    QP = ((0, 128), (128, 96))

    def c_wq(k):
        r = pl.ds((k % 2) * 224 * H, 224 * H)
        return cp(wq_hbm.at[r, pl.ds(128 * (k // 2), 128)], wq_raw.at[k, pl.ds(0, 224 * H)], sem.at[18 + k])

    def c_w(w_hbm, raw, sm, j, half, g):
        r = pl.ds(pl.multiple_of((half * 4 + j) * 2048, 2048), 2048)
        q = 2 * half + g
        return cp(w_hbm.at[r, pl.ds(128 * g, 128)], raw.at[j % 2, q, pl.ds(0, 2048)], sm.at[(j % 2) * 4 + q])

    def c_wk(j):
        return [c_w(wk_hbm, wk_raw, sem_k, j, half, g) for half in range(2) for g in range(2)]

    def c_wv(j):
        return [c_w(wv_hbm, wv_raw, sem_v, j, half, g) for half in range(2) for g in range(2)]

    def c_ckv(j):
        r = pl.ds(pl.multiple_of(j * 2 * T, 2 * T), 2 * T)
        return cp(ckv_hbm.at[r], ckv.at[r], sem.at[9 + j])

    a_pairs = ((kT_hbm, kT), (vT_hbm, vT), (ssmk_hbm, ssmk), (qT_hbm, qT))
    c_early = [cp(woT_hbm.at[pl.ds(0, 1)], woT.at[pl.ds(0, 1)], sem.at[4])]
    c_early += [cp(src.at[pl.ds(0, CH)], dst.at[pl.ds(0, CH)], sem.at[5 + n]) for n, (src, dst) in enumerate(a_pairs)]
    c_late = [cp(woT_hbm.at[pl.ds(1, H - 1)], woT.at[pl.ds(1, H - 1)], sem.at[13])]
    c_late += [cp(src.at[pl.ds(CH, M - CH)], dst.at[pl.ds(CH, M - CH)], sem.at[14 + n])
               for n, (src, dst) in enumerate(a_pairs)]
    c_small = [cp(sk_hbm, sk_ref, sem.at[22]), cp(dd_hbm, dd_ref, sem.at[23])]
    for c in c_small + [c_wq(k) for k in (0, 3, 2, 1)] + [c_x(0)]:
        c.start()
    for c in c_wk(0):
        c.start(priority=1)

    n_i = jax.lax.broadcasted_iota(jnp.int32, (P, P), 0)
    k_i = jax.lax.broadcasted_iota(jnp.int32, (P, P), 1)
    ang = (((2 * k_i + 1) * n_i) & 511).astype(f32) * (math.pi / 256.0)
    cs, sn = jnp.cos(ang), jnp.sin(ang)
    ff_s[:, 0:P] = cs.astype(bf16)
    ff_s[:, P:2 * P] = (-sn).astype(bf16)
    fi_s[0:P, :] = (cs.T * (1.0 / P)).astype(bf16)
    fi_s[P:2 * P, :] = (sn.T * (-1.0 / P)).astype(bf16)
    acc[...] = jnp.zeros(acc.shape, f32)
    for c in c_small:
        c.wait()
    sk = sk_ref[...].astype(f32)
    for t in range(KS):
        taps[t] = jnp.broadcast_to(sk[t:t + 1, :], (128, M)).T
    taps[KS] = jnp.broadcast_to(dd_ref[...].astype(f32).reshape(1, M), (128, M)).T
    aT_s[...] = jnp.zeros(aT_s.shape, bf16)
    O_s[NT - 1][...] = jnp.zeros(O_s[0].shape, bf16)
    W7_s[...] = jnp.zeros(W7_s.shape, u32)
    cT_s[...] = jnp.zeros(cT_s.shape, u32)

    vq = wq_raw.bitcast(u32)
    ut = {}
    for k, ready in ((0, ()), (3, (0, 2, 3)), (2, (1, 5)), (1, (4, 6))):
        c_wq(k).wait()
        for hp in range(H // 2):
            for c0, nc in QP:
                ut[k, hp, c0] = vq[k, pl.ds(c0 * 8 + hp, nc, stride=8), :].T
                for r in range(0, 128, 16):
                    for par, f in enumerate((_lo, _hi)):
                        r0 = (2 * hp + par) * 64 + r // 2
                        for n in ready:
                            i1, i2, sg = _A_OF.get(n, (0 if n == 2 else 3, None, 0))
                            x = f(ut[i1, hp, c0][r:r + 16])
                            if i2 is not None:
                                y = f(ut[i2, hp, c0][r:r + 16])
                                x = x + y if sg > 0 else x - y
                            aq_s[r0:r0 + 8, n * 256 + c0:n * 256 + c0 + nc] = _u(x.astype(bf16))
    for c in c_wv(0) + [c_ckv(0)]:
        c.start(priority=1)

    qscale = (D ** -0.5) * math.log2(math.e)

    def prep_c2(jj, r):
        blk = [[cT_s[cq * 128 + r:cq * 128 + r + 8, tb * 128:(tb + 1) * 128] for tb in range(4)] for cq in range(4)]
        x = [[_f(v) for v in row] for row in blk]
        outer = [[_b7(x[ci][ti], x[ci][2 + ti], x[2 + ci][ti], x[2 + ci][2 + ti]) for ti in range(2)]
                 for ci in range(2)]
        two = [_b7(outer[0][0][n], outer[0][1][n], outer[1][0][n], outer[1][1][n]) for n in range(7)]
        cj = c2_s.at[pl.ds(pl.multiple_of(jj * 128, 128), 128)]
        for n in range(7):
            for m in range(7):
                cj[r:r + 8, (n * 7 + m) * 128:(n * 7 + m + 1) * 128] = _u(two[n][m].astype(bf16))
        return []

    def q_body(j, carry):
        mq = {}
        qtj = QT_s.at[pl.ds(pl.multiple_of(j * 4096, 4096), 4096)]
        zq = j >> 4
        c_x(j).wait()
        xj = xT.at[pl.ds(pl.multiple_of(j * M, 16), M)]
        bx = [_combos(_b7, [_u(xj[r:r + 224, c:c + 128]) for r in (0, 224) for c in (t * T, t * T + 128)])
              for t in range(2)]

        def qproj(u, tok):
            hh, t, n = u // 14, (u // 7) % 2, SORD[u % 7]
            w = _b(_gate(aq_s[hh * 64:hh * 64 + 64, n * 256:n * 256 + 224], tok))
            mq[n] = _nn(w, bx[t][n])
            if u % 7 == 6:
                for k, x in enumerate(_c4(mq)):
                    r0 = t * 2048 + hh * 128 + (k // 2) * 64
                    qtj[r0:r0 + 64, (k % 2) * 128:(k % 2 + 1) * 128] = _u((x * qscale).astype(bf16))
            return mq[n]

        wt = {}
        ckj = ckv.at[pl.ds(pl.multiple_of(j * 512, 512), 512)]
        w1j = w1_s.at[pl.ds(pl.multiple_of(j * 2048, 2048), 2048)]

        def prep_w(kv, hp, part):
            if part == 0:
                v = (wk_raw, wv_raw)[kv].bitcast(u32).at[j % 2]
                wt[kv, hp] = [v[q, pl.ds(hp, 128, stride=8), :].T for q in (0, 2, 1, 3)]
                return [x[120:] for x in wt[kv, hp]]
            for r in range(32 * (part - 1), 32 * part, 16):
                u = [x[r:r + 16] for x in wt[kv, hp]]
                for par, f in enumerate((_lo, _hi)):
                    r0 = (2 * hp + par) * 128 + kv * 64 + r // 2
                    for n, c in enumerate(_a7(*[f(x) for x in u])):
                        w1j[r0:r0 + 8, n * 128:(n + 1) * 128] = _u(c.astype(bf16))
            return []

        def prep_ct(half, cq):
            res = []
            ct = 2 * cq + half
            for tb in range(4):
                x = _u(ckj[tb * 128:(tb + 1) * 128, ct * 128:(ct + 1) * 128].T)
                cT_s[pl.ds(pl.multiple_of(zq * 64 + ct * 64, 64), 64), tb * 128:(tb + 1) * 128] = x
                res.append(x[56:])
            return res

        fill = {}

        def spread(pieces, u0, u1):
            for n, p in enumerate(pieces):
                fill.setdefault(u0 + n * (u1 - u0) // len(pieces), []).append(p)

        spread([functools.partial(prep_w, 0, hp, part) for hp in range(8) for part in range(5)], QW1, QW2)
        spread([functools.partial(prep_w, 1, hp, part) for hp in range(8) for part in range(5)], QW2, QW3)
        spread([functools.partial(prep_ct, 0, cq) for cq in range(4)], QW2 + 2, QC1)
        spread([functools.partial(prep_ct, 1, cq) for cq in range(4)], QC1, QW3)
        spread([functools.partial(prep_c2, jnp.maximum(j - 1, 0), r) for r in range(C2N, 128, 8)], C2S, QW1 - 4)
        if C2N:
            spread([functools.partial(prep_c2, j, r) for r in range(0, C2N, 8)], QW3, QW4)
        toks = {}
        for u in range(224):
            if u == QW1:
                @pl.when(j < 3)
                def _():
                    for c in c_wk(j + 1):
                        c.start(priority=1)

                @pl.when(j == 3)
                def _():
                    for c in c_early + c_late:
                        c.start(priority=1)

                for c in c_wk(j):
                    c.wait()
            if u == QW2:
                @pl.when(j < 3)
                def _():
                    for c in [c_x(j + 1)] + c_wv(j + 1) + [c_ckv(j + 1)]:
                        c.start(priority=1)

                for c in c_wv(j) + [c_ckv(j)]:
                    c.wait()
            q = qproj(u, toks.pop(u, None))
            res = []
            ps = fill.get(u, [])
            for n, p in enumerate(ps):
                row = (n * 128 // len(ps)) // 16 * 16
                if p.func is prep_w and p.args[2] == 0:
                    (wk_raw, wv_raw)[p.args[0]].bitcast(u32)[zq, 0, 1024:1032, :] = _u(q[row:row + 8])
                elif p.func is prep_c2:
                    cT_s[pl.ds(pl.multiple_of(512 + zq * 8, 8), 8), 0:128] = _u(q[row:row + 8])
                elif p.func is prep_ct:
                    ckv[pl.ds(pl.multiple_of(S + zq * 16, 16), 16), 0:128] = q[row:row + 16].astype(bf16)
                res += p()
            if res:
                toks[u + QLAG] = _tok(res)
        return carry

    jax.lax.fori_loop(0, 4, q_body, 0)
    for r in range(C2N, 128, 8):
        prep_c2(3, r)
    for c in c_early:
        c.wait()

    tri = n_i <= k_i
    sgn = jnp.where((jax.lax.broadcasted_iota(jnp.int32, (1, P), 1) & 1) == 0, 1.0, -1.0).astype(f32)
    c_outa = cp(out_s.at[:, pl.ds(0, 384)], out_hbm.at[:, pl.ds(0, 384)], sem_o.at[8])
    HR, HI, PR, PI, KV = range(5)

    def blk_at(c, half=None):
        r0 = (c % 8) * CH
        rs = slice(r0, r0 + CH) if half is None else slice(r0 + 16 * half, r0 + 16 * half + 16)
        return rs, slice((c // 8) * P, (c // 8 + 1) * P)

    def tile(ref, n):
        return ref[:, n * 128:(n + 1) * 128]

    def head_body(h, carry):
        @pl.when(h == 1)
        def _():
            for c in c_late:
                c.wait()

        @pl.when(h == H - 1)
        def _():
            c_outa.start()

        st = dict(co={}, cnt={}, fin=set(), M={}, P={}, Q7={}, mfin={}, o={})
        zs = h >> 10
        z64 = pl.ds(pl.multiple_of(zs * 64, 64), 64)
        m_s, l_s = (m0_s, m1_s), (l0_s, l1_s)
        w1h = w1_s.at[pl.ds(pl.multiple_of(h * 128, 128), 3 * 2048 + 128)]
        qth = QT_s.at[pl.ds(pl.multiple_of(h * 128, 128), 7 * 2048 + 128)]
        rows = pl.ds(pl.multiple_of(jnp.minimum(h, NCH - 1) * CH, CH), CH)

        def rep(t, n):
            return jnp.concatenate([taps[t, rows, :]] * n, axis=1)

        toks = []

        def due():
            for t in toks:
                t[0] -= 1
            ready = [t[1] for t in toks if t[0] <= 0]
            toks[:] = [t for t in toks if t[0] > 0]
            return functools.reduce(lambda x, y: x | y, ready) if ready else None

        def gate_later(vals):
            toks.append([SLAG, _tok([v if v.dtype == u32 else _u(v) for v in vals])])

        def row_offset(i):
            if i not in st['mfin']:
                m = m_s[i % 2][0, 0]
                for t in range(1, i + 1):
                    m = jnp.maximum(m, m_s[i % 2][0, t])
                m = jnp.max(m, axis=0, keepdims=True)
                if i > 0:
                    lo_ = jnp.exp2(m_s[i % 2][0, 0] - m)
                    for t in range(1, i + 1):
                        lo_ = lo_ + jnp.exp2(m_s[i % 2][0, t] - m)
                    m = m + jnp.log2(jnp.sum(lo_, axis=0, keepdims=True))
                st['mfin'][i] = m
            return st['mfin'][i]

        for op in _schedule():
            kind = op[0]
            if kind == 'KV':
                _, p, t = op
                n, m = SK[t // 7], SV[t % 7]

                def wblk(q):
                    w = jnp.concatenate([w1h[k * 2048:k * 2048 + 128, n * 128:(n + 1) * 128]
                                         for k in (2 * (q % 2), 2 * (q % 2) + 1)], axis=1)
                    r = (q // 2) * 32
                    return jnp.concatenate([w[r:r + 32], w[64 + r:64 + r + 32]], axis=0)

                cols = slice((n * 7 + m) * 256, (n * 7 + m + 1) * 256)
                if m in (2, 3):
                    w = wblk(0 if m == 2 else 3)
                elif p > 0:
                    w = w2_s[:, cols]
                else:
                    i1, i2, sg = _A_OF[m]
                    x, y = wblk(i1), wblk(i2)
                    w = (_f(x) + _f(y) if sg > 0 else _f(x) - _f(y)).astype(bf16)
                    w2_s[z64, cols] = _u(w)
                c2 = c2_s[p * 128:(p + 1) * 128, (n * 7 + m) * 128:(n * 7 + m + 1) * 128]
                st['M'][m] = st['last'] = _nn(w if w.dtype == bf16 else _b(_gate(w, due())), _b(c2))
                if t % 7 < 6:
                    continue
                mo = _quad(*_c4(st['M']))
                for o, sg in _C_OF[n]:
                    k = st['cnt'][o] = st['cnt'].get(o, 0) + 1
                    if k == 1:
                        st['co'][o] = mo if sg > 0 else -mo
                    else:
                        st['co'][o] = st['co'][o] + mo if sg > 0 else st['co'][o] - mo
                    if k == _C_CNT[o]:
                        st['cnt'][o] = 0
                        st['fin'].add(o)
                for tok in range(2):
                    if not {tok, 2 + tok} <= st['fin']:
                        continue
                    st['fin'] -= {tok, 2 + tok}
                    c = 2 * p + tok

                    def full(dh, kb, off):
                        x = st['co'][2 * dh + tok][:, kb * 128:(kb + 1) * 128]
                        return jnp.concatenate([x[off:off + 64], x[128 + off:128 + off + 64]], axis=0)

                    kb4 = (full(0, 0, 0).T, full(1, 0, 0).T, full(0, 1, 0).T, full(1, 1, 0).T)
                    vb4 = (full(0, 0, 64), full(0, 1, 64), full(1, 0, 64), full(1, 1, 64))
                    for ref, c4 in ((V_s[c], vb4), (K_s[c], kb4)):
                        blks = dict(zip((2, 7, 8, 3), c4))
                        if c < NT - 1:
                            blks.update({k: x for k, x in enumerate(_a7(*c4)) if k not in (2, 3)})
                        for k, x in blks.items():
                            ref[z64, k * 128:(k + 1) * 128] = _u(x.astype(bf16))
            elif kind == 'QK':
                _, i, j = op
                S_s = (S0_s, S1_s)[i % 2]
                if j < i:
                    if i not in st['Q7']:
                        qu = qth[i * 2048:i * 2048 + 128, :]
                        st['Q7'][i] = _combos(_b7, [qu[:64, :128], qu[:64, 128:], qu[64:, :128], qu[64:, 128:]])
                    s = _quad(*_c4({n: _nn(_b(tile(K_s[j], n)), st['Q7'][i][n]) for n in SQ}))
                    S_s[zs, j] = s
                    f = _fold(s, jnp.max)
                else:
                    q = _b(qth[i * 2048:i * 2048 + 128, :])
                    sa = _nn(_b(jnp.concatenate([tile(K_s[j], 2), tile(K_s[j], 7)], axis=1)), q)
                    sa = jnp.concatenate([jnp.where(tri, sa[:, :128], NEG), sa[:, 128:]], axis=1)
                    sb = _nn(_b(jnp.concatenate([tile(K_s[j], 8), tile(K_s[j], 3)], axis=1)), q[:, 128:])
                    sb = jnp.where(tri, sb, NEG)
                    S_s[zs, j, 0:128, :] = sa
                    S_s[zs, j, 128:T, 128:T] = sb
                    fa = _fold(sa, jnp.max)
                    f = jnp.concatenate([fa[:, :128], jnp.maximum(fa[:, 128:], _fold(sb, jnp.max))], axis=1)
                m_s[i % 2][zs, j] = f
                pace_s[zs] = f
            elif kind == 'EX':
                _, i, j = op
                S_s = (S0_s, S1_s)[i % 2]
                m = row_offset(i)
                m = jnp.where(pace_s[0, 0:1, :] == jnp.inf, jnp.inf, m)
                if j < i:
                    parts, lj = [], None
                    for r in range(112, -16, -16):
                        pt = jnp.exp2(S_s[0, j, r:r + 16, :] - m)
                        pb = jnp.exp2(S_s[0, j, 128 + r:128 + r + 16, :] - m)
                        parts.insert(0, _b7(pt[:, :128], pt[:, 128:], pb[:, :128], pb[:, 128:]))
                        x = (pt[:8] + pt[8:]) + (pb[:8] + pb[8:])
                        lj = x if lj is None else lj + x
                    st['P'][i, j] = [jnp.concatenate([x[n] for x in parts], axis=0).astype(bf16) for n in range(7)]
                else:
                    pa = jnp.exp2(S_s[0, j, 0:128, :] - m)
                    pb = jnp.exp2(S_s[0, j, 128:T, 128:T] - m[:, 128:])
                    la = _rsum(pa)
                    lj = jnp.concatenate([la[:, :128], la[:, 128:] + _rsum(pb)], axis=1)
                    st['P'][i, j] = (pa.astype(bf16), pb.astype(bf16))
                l_s[i % 2][zs, j] = lj
            elif kind == 'PV':
                _, i, j = op
                p = st['P'].pop((i, j))
                if j < i:
                    for n in SP:
                        st['last'] = _nn(_b(tile(V_s[j], n)), p[n])
                        st['o'][i, n] = st['o'][i, n] + st['last'] if j > 0 else st['last']
                    continue
                oa = _nn(_b(jnp.concatenate([tile(V_s[j], 2), tile(V_s[j], 8)], axis=0)), p[0])
                ob = _nn(_b(jnp.concatenate([tile(V_s[j], 7), tile(V_s[j], 3)], axis=0)), p[1])
                o = st['last'] = jnp.concatenate([oa[:, :128], oa[:, 128:] + ob], axis=1)
                if i > 0:
                    o = o + _quad(*_c4({n: st['o'].pop((i, n)) for n in range(7)}))
                l = l_s[i % 2][0, 0]
                for t in range(1, i + 1):
                    l = l + l_s[i % 2][0, t]
                o = o * (1.0 / jnp.sum(l, axis=0, keepdims=True))
                for n, x in enumerate(_b7(o[:128, :128], o[:128, 128:], o[128:, :128], o[128:, 128:])):
                    O_s[i][zs, n] = x.astype(bf16)
            elif kind == 'PACE':
                pace_s[zs] = jnp.concatenate([st['last'][-8:, -128:]] * 2, axis=1)
            elif kind == 'OP':
                _, i, t = op
                n = SO[t]
                st['M'][n] = st['last'] = _nn(_b(_gate(tile(W7_s, n), due())), O_s[i][0, n])
                if t == 6:
                    acc[:, T * i:T * (i + 1)] += _quad(*_c4(st['M']))
            elif kind == 'W7':
                res = []
                for r0 in range(16 * op[1], 16 * op[2], 16):
                    blk = [_u(woT[h, r:r + 16, c:c + 128]) for r in (r0, 224 + r0) for c in (0, 128)]
                    row = pl.ds(pl.multiple_of(zs * 8 + r0 // 2, 8), 8)
                    for n, x in enumerate(_combos(_a7, blk)):
                        W7_s[row, n * 128:(n + 1) * 128] = _u(x)
                    res += blk
                gate_later(res)
            elif kind == 'AT':
                g = jnp.clip((h - 4) // 4, 0, 2)
                t0 = jnp.minimum(((h + 12) % 4) * 6, NB - 6)
                grow = pl.ds(pl.multiple_of(g * 128, 128), 128)
                gcol = pl.ds(pl.multiple_of(jnp.where(h == H - 1, 3, g) * 128, 128), 128)
                res = []
                for n in range(6):
                    tok = pl.ds(pl.multiple_of((t0 + n) * 128, 128), 128)
                    x = aT_s[grow, tok].T
                    out_s[tok, gcol] = x
                    res.append(_u(x)[56:])
                gate_later(res)
            elif kind == 'HD':
                g = op[1]
                hs = jnp.concatenate([ssmk[rows, c * P:(c + 1) * P] for c in range(4 * g, 4 * g + 4)], axis=0)
                hf = _nn(hs, ff_s[...])
                for n in range(4):
                    X_s[(zs, HR) + blk_at(4 * g + n)] = hf[n * CH:(n + 1) * CH, :P]
                    X_s[(zs, HI) + blk_at(4 * g + n)] = hf[n * CH:(n + 1) * CH, P:]
            elif kind == 'SC':
                g = op[1]
                if g == 0:
                    k = jnp.concatenate([jnp.zeros((CH, P), f32), kT[rows, 0:4 * P].astype(f32)], axis=1)
                else:
                    k = kT[rows, (4 * g - 1) * P:(4 * g + 4) * P].astype(f32)
                ks = k[:, P:] * rep(0, 4)
                for j in range(1, KS):
                    ks = ks + pltpu.roll(k, j, 1)[:, P:] * rep(j, 4)
                kv = ks * vT[rows, 4 * g * P:(4 * g + 4) * P].astype(f32)
                kvs = jnp.concatenate([kv[:, n * P:(n + 1) * P] for n in range(4)], axis=0)
                xf = _nn(kvs.astype(bf16), ff_s[...])
                for n in range(4):
                    c = 4 * g + n
                    xr, xi = xf[n * CH:(n + 1) * CH, :P], xf[n * CH:(n + 1) * CH, P:]
                    X_s[(zs, KV) + blk_at(c)] = kvs[n * CH:(n + 1) * CH]
                    pr = xr if c == 0 else xr - sgn * st['x'][1]
                    pi = xi if c == 0 else xi + sgn * st['x'][0]
                    X_s[(zs, PR) + blk_at(c)] = pr
                    X_s[(zs, PI) + blk_at(c)] = pi
                    st['x'] = (xr, xi)
            elif kind == 'CV':
                res = []
                for a, half in op[1]:
                    wr = wi = None
                    for j in range(a + 1):
                        hr, hi_ = X_s[(0, HR) + blk_at(j, half)], X_s[(0, HI) + blk_at(j, half)]
                        pr, pi = X_s[(0, PR) + blk_at(a - j, half)], X_s[(0, PI) + blk_at(a - j, half)]
                        tr, ti = hr * pr - hi_ * pi, hr * pi + hi_ * pr
                        wr, wi = (tr, ti) if wr is None else (wr + tr, wi + ti)
                    r0 = (a % 4) * CH + 16 * half
                    Y_s[a // 4][zs, r0:r0 + 16, :P] = wr
                    Y_s[a // 4][zs, r0:r0 + 16, P:] = wi
                    res += [wr, wi]
                gate_later(res)
            elif kind == 'ID':
                g = op[1]
                y = _nn(Y_s[g][0].astype(bf16), fi_s[...])
                for n in range(4):
                    c = 4 * g + n
                    cols = slice(c * P, (c + 1) * P)
                    ya = y[n * CH:(n + 1) * CH, :] + X_s[(0, KV) + blk_at(c)] * taps[KS, rows, :]
                    aT_s[rows, cols] = (qT[rows, cols].astype(f32) * ya).astype(bf16)
        return carry

    jax.lax.fori_loop(0, H, head_body, 0)

    acc[:, T * (NT - 1):] += _quad(*_c4({n: _nn(_b(tile(W7_s, n)), O_s[NT - 1][0, n]) for n in SORD}))
    outs = [c_outa]
    for i in range(NT):
        cols = slice(T * i, T * (i + 1))
        blk = jnp.concatenate([aT_s[384:M, cols], acc[:, cols].astype(bf16)], axis=0)
        out_s[cols, 384:2 * M] = blk.T
        c = cp(out_s.at[pl.ds(T * i, T), pl.ds(384, 512)], out_hbm.at[pl.ds(T * i, T), pl.ds(384, 512)], sem_o.at[i])
        c.start()
        outs.append(c)
    for c in outs:
        c.wait()


@jax.jit
def pallas_concat_heads__ssm_conv_h3__compressed_kv_cla__prompt_kernel(
    A_q: jax.Array,
    A_k: jax.Array,
    A_v: jax.Array,
    A_shift_k: jax.Array,
    A_ssm_k: jax.Array,
    A_ssm_D: jax.Array,
    B_x: jax.Array,
    B_c_kv: jax.Array,
    B_w_q: jax.Array,
    B_w_uk: jax.Array,
    B_w_uv: jax.Array,
    B_w_o: jax.Array,
):
    hbm = pl.BlockSpec(memory_space=pl.ANY)
    V = pltpu.VMEM
    out = pl.pallas_call(
        _kernel,
        out_shape=jax.ShapeDtypeStruct((S, 2 * M), bf16),
        in_specs=[hbm] * 12,
        out_specs=hbm,
        scratch_shapes=[
            V((M, S), bf16), V((M, S), bf16), V((M, S), bf16), V((M, S), bf16),
            V((4 * M, 2 * T), bf16), V((S + 16, DC), bf16),
            V((4, 224 * H + 16, 128), bf16),
            V((2, 4, 128 * H + 16, 128), bf16), V((2, 4, 128 * H + 16, 128), bf16),
            V((H, M, D), bf16),
            V((H * 64, 7 * 256), u32),
            V((4 * H * 128, 7 * 128), u32), V((64, 49 * 256), u32),
            V((512 + 8, 512), u32),
            V((NT * H * 128, T), u32), V((4 * 128, 49 * 128), u32),
            V((M, S), f32), V((M, S), bf16), V((S, 2 * M), bf16),
            V((KS + 1, M, 128), f32), V((P, 2 * P), bf16), V((2 * P, P), bf16),
            V((KS, M), bf16), V((M,), bf16),
            V((1, NT, T, T), f32), V((1, NT, T, T), f32), V((1, 5, T, T), f32),
            V((112, 7 * 128), u32), V((1, 8, T), f32),
            V((1, NT, 8, T), f32), V((1, NT, 8, T), f32), V((1, NT, 8, T), f32), V((1, NT, 8, T), f32),
            pltpu.SemaphoreType.DMA((24,)), pltpu.SemaphoreType.DMA((8,)),
            pltpu.SemaphoreType.DMA((8,)), pltpu.SemaphoreType.DMA((9,)),
        ] + [V((64, 9 * 128), u32)] * (2 * NT) + [V((1, 7, 128, 128), bf16)] * NT
        + [V((1, 4 * CH, 2 * P), f32)] * 4,
        compiler_params=pltpu.CompilerParams(vmem_limit_bytes=126 * 1024 * 1024,
                                             shape_invariant_numerics=False,
                                             disable_bounds_checks=True, disable_semaphore_checks=True),
    )(
        A_q[0].T, A_k[0].T, A_v[0].T, A_shift_k.T, A_ssm_k, A_ssm_D,
        B_x[0].T, B_c_kv[0],
        B_w_q.reshape(M * H, D), B_w_uk.reshape(DC * H, D), B_w_uv.reshape(DC * H, D),
        jnp.transpose(B_w_o, (0, 2, 1)),
    )
    return out[None]
```
